```python
import jax
import jax.numpy as jnp

def _softmax(x, axis=-1):
    return jax.nn.softmax(x, axis=axis)

def _gelu(x):
    return jax.nn.gelu(x, approximate=True)

def _silu(x):
    return jax.nn.silu(x)

def _sigmoid(x):
    return jax.nn.sigmoid(x)

def _layernorm(x, axis=-1, eps=1e-05):
    m = jnp.mean(x, axis=axis, keepdims=True)
    v = jnp.var(x, axis=axis, keepdims=True)
    return (x - m) / jnp.sqrt(v + eps)

def _scatter_add(tgt, idx, src, axis=0):
    return tgt.at[idx].add(src)

def _segment_sum(src, seg, n):
    return jax.ops.segment_sum(src, seg, n)

class _Rng:

    def __init__(self, key):
        self._k = key

    def _next(self):
        self._k, sub = jax.random.split(self._k)
        return sub

    def normal(self, shape):
        return jax.random.normal(self._next(), shape, dtype=jnp.bfloat16)

    def randint(self, lo, hi, shape):
        return jax.random.randint(self._next(), shape, lo, hi, dtype=jnp.int32)

    def uniform(self, shape, lo=0.0, hi=1.0):
        return jax.random.uniform(self._next(), shape, jnp.bfloat16, lo, hi)

    def permutation(self, n):
        return jax.random.permutation(self._next(), n)
kernel_name = 'gated_mix__memory_aug_recurrent_mem_tr__spectral_gfnet__prompt'

def setup_inputs():
    _rng = _Rng(jax.random.key(int.from_bytes(__import__("os").urandom(4), "little")))
    _w = lambda a: (lambda t: t.astype(jnp.bfloat16) if jnp.issubdtype(t.dtype, jnp.floating) else t)(jnp.asarray(a))

    def _A_setup():
        B, S, Dm = (1, 2048, 1024)
        H, Dh = (32, 128)
        M, seg = (8, 32)
        seg = min(seg, S)
        S = S // seg * seg
        return {'x': _w((lambda *s: _rng.normal(s) * 0.05)(B, S, Dm)), 'mem0': _w((lambda *s: _rng.normal(s) * 0.05)(B, M, Dm)), 'Wq': _w((lambda *s: _rng.normal(s) * 0.05)(Dm, H, Dh) * Dm ** (-0.5)), 'Wk': _w((lambda *s: _rng.normal(s) * 0.05)(Dm, H, Dh) * Dm ** (-0.5)), 'Wv': _w((lambda *s: _rng.normal(s) * 0.05)(Dm, H, Dh) * Dm ** (-0.5)), 'Wo': _w((lambda *s: _rng.normal(s) * 0.05)(H, Dh, Dm) * (H * Dh) ** (-0.5)), 'seg_len': seg}
    _A_in = _A_setup()

    def _B_setup():
        B, S, D = (1, 2048, 1024)
        Df = D // 2 + 1
        return {'x': _w((lambda *s: _rng.normal(s) * 0.05)(B, S, D)), 'w_r': _w((lambda *s: _rng.normal(s) * 0.05)(S, Df) * 0.02), 'w_i': _w((lambda *s: _rng.normal(s) * 0.05)(S, Df) * 0.02)}
    _B_in = _B_setup()
    return {'A_x': _A_in['x'], 'A_mem0': _A_in['mem0'], 'A_Wq': _A_in['Wq'], 'A_Wk': _A_in['Wk'], 'A_Wv': _A_in['Wv'], 'A_Wo': _A_in['Wo'], 'A_seg_len': _A_in['seg_len'], 'B_x': _B_in['x'], 'B_w_r': _B_in['w_r'], 'B_w_i': _B_in['w_i'], 'gate_w': _w((lambda *s: _rng.normal(s) * 0.05)(1024))}

def reference(A_x, A_mem0, A_Wq, A_Wk, A_Wv, A_Wo, A_seg_len, B_x, B_w_r, B_w_i, gate_w):

    def _A_ref(x, mem0, Wq, Wk, Wv, Wo, seg_len):
        B, S, Dm = x.shape
        H, Dh = (Wq.shape[1], Wq.shape[2])
        M = mem0.shape[1]
        scale = Dh ** (-0.5)
        n_seg = S // seg_len
        L = M + seg_len
        idx = jnp.arange(L)
        mask = (idx[:, None] < M) | (idx[:, None] >= idx[None, :])
        mem = mem0
        outs = []
        for s in range(n_seg):
            xs = x[:, s * seg_len:(s + 1) * seg_len, :].copy()
            h = jnp.concatenate([mem, xs], axis=1)
            q = jnp.einsum('btd,dhe->bhte', h, Wq)
            k = jnp.einsum('btd,dhe->bhte', h, Wk)
            v = jnp.einsum('btd,dhe->bhte', h, Wv)
            scores = jnp.einsum('bhqe,bhke->bhqk', q, k) * scale
            scores = jnp.where(mask[None, None], scores, -1000000000.0)
            p = _softmax(scores, axis=-1)
            o = jnp.einsum('bhqk,bhke->bhqe', p, v)
            o = jnp.einsum('bhte,hed->btd', o, Wo)
            mem = o[:, :M, :].copy()
            outs.append(o[:, M:, :])
        return jnp.concatenate(outs, axis=1)

    def _B_ref(x, w_r, w_i):
        B, S, D = x.shape
        X = (lambda x, axes=(-2, -1): jnp.fft.rfft2(x.astype(jnp.float32), axes=axes))(x, axes=(-2, -1))
        W = w_r + 1j * w_i
        X = X * W
        y = (lambda x, s, axes=(-2, -1): jnp.fft.irfft2(x, s=s, axes=axes).astype(jnp.bfloat16))(X, (S, D), axes=(-2, -1))
        return y
    x = A_x
    g = _sigmoid((x * gate_w).sum(-1, keepdims=True))
    a = _A_ref(x, A_mem0, A_Wq, A_Wk, A_Wv, A_Wo, A_seg_len)
    b = _B_ref(x, B_w_r, B_w_i)
    return g * a + (1 - g) * b
```

```python
import numpy as np
import ml_dtypes
import jax
import jax.numpy as jnp
from jax import lax
import jax.experimental.pallas as pl
import jax.experimental.pallas.tpu as pltpu

f32, bf16, u32 = jnp.float32, jnp.bfloat16, jnp.uint32
S, D, H, DH, M_MEM, SEG = 2048, 1024, 32, 128, 8, 32
NSEG = S // SEG
RS = float(1 / np.sqrt(2))
NT = (((1,), (1,)), ((), ()))
HI = 0xFFFF0000


def _np_tables():
    bf = ml_dtypes.bfloat16
    dp = np.arange(128)
    j = np.arange(64)

    def cs(f):
        ang = 2 * np.pi * ((f[:, None] * dp[None, :]) % 1024) / 1024
        return np.cos(ang), np.sin(ang)

    G = np.zeros((5, 256, 256))
    for t in range(3):
        r = t + 1
        C, Sn = cs(r + 8 * j)
        C2, S2 = cs(8 - r + 8 * j)
        G[t, 0:64, 0:128] = C
        G[t, 0:64, 128:] = Sn
        G[t, 64:128, 0:128] = C2
        G[t, 64:128, 128:] = -S2
        G[t, 128:192, 0:128] = -Sn
        G[t, 128:192, 128:] = C
        G[t, 192:256, 0:128] = -S2
        G[t, 192:256, 128:] = -C2
    C0, S0 = cs(8 * j)
    C4, S4 = cs(4 + 8 * j)
    G[3, 0:64, 0:128] = C0
    G[3, 128:192, 0:128] = -S0
    G[3, 64:128, 128:] = C4
    G[3, 192:256, 128:] = -S4
    G[4] = G[3]
    G[4, 0, 0:128] = 0.5
    G[4, 128, 0:128] = 0.5 * (-1.0) ** dp
    HH = np.zeros((16, 256, 128))
    for a in range(16):
        ang = 2 * np.pi * (((a + 16 * dp)[:, None] * dp[None, :]) % 2048) / 2048
        HH[a, :128] = np.cos(ang)
        HH[a, 128:] = np.sin(ang)
    misc = np.zeros((3, 128, 128))
    misc[0, 128 - dp[1:], dp[1:]] = 1
    misc[1, 0, 0] = 1
    misc[2, 0, :] = (-1.0) ** dp
    for blk in range(4):
        for k1 in range(16):
            misc[2, 64 + 16 * blk + k1, 16 * blk + 15 - k1] = 1
            misc[2, 64 + 16 * blk + k1, 64 + 16 * blk + (16 - k1) % 16] = 1
    return G.astype(bf), HH.astype(bf), misc.astype(bf)


_TAB_G, _TAB_H, _TAB_MISC = _np_tables()


def _bc(x, dt):
    return lax.bitcast_convert_type(x, dt)


def _w2b(w):
    return pltpu.bitcast(w, bf16)


def _fft16(xs, inverse):
    sg = 1.0 if inverse else -1.0

    def dft4(a, b, c, d):
        t0 = (a[0] + c[0], a[1] + c[1])
        t1 = (a[0] - c[0], a[1] - c[1])
        t2 = (b[0] + d[0], b[1] + d[1])
        t3 = (b[0] - d[0], b[1] - d[1])
        o0 = (t0[0] + t2[0], t0[1] + t2[1])
        o2 = (t0[0] - t2[0], t0[1] - t2[1])
        m = (t1[0] + t3[1], t1[1] - t3[0])
        p = (t1[0] - t3[1], t1[1] + t3[0])
        return [o0, p, o2, m] if inverse else [o0, m, o2, p]

    t = [dft4(xs[a0], xs[4 + a0], xs[8 + a0], xs[12 + a0]) for a0 in range(4)]

    def tw(v, e):
        e = e % 16
        if e == 0:
            return v
        if e == 4:
            return (-v[1], v[0]) if inverse else (v[1], -v[0])
        if e == 2:
            if inverse:
                return ((v[0] - v[1]) * RS, (v[0] + v[1]) * RS)
            return ((v[0] + v[1]) * RS, (v[1] - v[0]) * RS)
        if e == 6:
            if inverse:
                return ((-v[0] - v[1]) * RS, (v[0] - v[1]) * RS)
            return ((v[1] - v[0]) * RS, (-v[0] - v[1]) * RS)
        c = float(np.cos(2 * np.pi * e / 16))
        s = float(sg * np.sin(2 * np.pi * e / 16))
        return (v[0] * c - v[1] * s, v[0] * s + v[1] * c)

    out = [None] * 16
    for k in range(4):
        u = [tw(t[a0][k], a0 * k) for a0 in range(4)]
        r = dft4(*u)
        for m in range(4):
            out[k + 4 * m] = r[m]
    return out


def _b_phase(xb_hbm, wr_hbm, wi_hbm, g_hbm, h_hbm, misc_hbm, bs, sems, start_rest):
    def scoped(xs, wr, wi, wrn, win, G, HH, misc, Y, Zr, Zi, WS, PQ):
        xb32 = xb_hbm.bitcast(u32)
        xcp = [pltpu.make_async_copy(xb32.at[:, m, :], xs.at[m], sems.at[m]) for m in range(8)]
        cg = pltpu.make_async_copy(g_hbm, G, sems.at[8])
        ch = pltpu.make_async_copy(h_hbm, HH, sems.at[9])
        cm = pltpu.make_async_copy(misc_hbm, misc, sems.at[10])
        wcp = []
        for k in range(16):
            wcp.append(pltpu.make_async_copy(wr_hbm.at[pl.ds(0, 512), pl.ds(128 * k, 128)], wr.at[k], sems.at[11]))
            wcp.append(pltpu.make_async_copy(wi_hbm.at[pl.ds(0, 512), pl.ds(128 * k, 128)], wi.at[k], sems.at[12]))
        wcp.append(pltpu.make_async_copy(wr_hbm.at[pl.ds(512, 1), :], wrn, sems.at[11]))
        wcp.append(pltpu.make_async_copy(wi_hbm.at[pl.ds(512, 1), :], win, sems.at[12]))
        cg.start()
        cm.start()
        xcp[0].start()
        ch.start()
        for c in xcp[1:]:
            c.start()
        for c in wcp:
            c.start()
        start_rest()
        cg.wait()
        cm.wait()
        ch.wait()

        def getM(a):
            hc = HH[a, 0:128, :]
            hs = HH[a, 128:256, :]
            return jnp.concatenate(
                [jnp.concatenate([hc, -hs], axis=1), jnp.concatenate([hs, hc], axis=1)], axis=0)

        def phF(m, _):
            pltpu.make_async_copy(xb32.at[:, 0, :], xs.at[m], sems.at[m]).wait()
            for ch_ in range(8):
                w = xs[m, 16 * ch_:16 * ch_ + 16, :]
                for half, xv in enumerate((_bc(w << 16, f32), _bc(w & jnp.uint32(HI), f32))):
                    xc = [xv[:, 128 * c:128 * (c + 1)] for c in range(8)]
                    a0, a1 = xc[0] + xc[4], xc[0] - xc[4]
                    b0, b1 = xc[2] + xc[6], xc[2] - xc[6]
                    c0, c1 = xc[1] + xc[5], xc[1] - xc[5]
                    d0, d1 = xc[3] + xc[7], xc[3] - xc[7]
                    p, q = a0 + b0, c0 + d0
                    y0, y4 = p + q, p - q
                    y2r, y2i = a0 - b0, d0 - c0
                    cm_, cp_ = RS * (c1 - d1), RS * (c1 + d1)
                    y1r, y1i = a1 + cm_, -b1 - cp_
                    y3r, y3i = a1 - cm_, b1 - cp_
                    for t, (yr, yi) in enumerate([(y1r, y1i), (y2r, y2i), (y3r, y3i), (y0, y4)]):
                        Y[half, t, 16 * ch_:16 * ch_ + 16, :] = jnp.concatenate([yr, yi], axis=1).astype(bf16)
            for half in range(2):
                a = 2 * m + half
                Mx = getM(a)
                for t in range(4):
                    o = lax.dot_general(G[t], Y[half, t], NT, preferred_element_type=f32)
                    z = jnp.concatenate([o[:128], o[128:]], axis=1).astype(bf16)
                    X = jnp.dot(z, Mx, preferred_element_type=f32)
                    Zr[a, 128 * t:128 * t + 128, :] = X[:, 0:128]
                    Zi[a, 128 * t:128 * t + 128, :] = X[:, 128:256]
                ony = lax.dot_general(misc[2, 0:16, :], Y[half, 3, :, 0:128], NT, preferred_element_type=f32)
                Xn = jnp.dot(ony.astype(bf16), Mx[0:128, :], preferred_element_type=f32)
                Zr[a, 512:528, :] = Xn[:, 0:128]
                Zi[a, 512:528, :] = Xn[:, 128:256]
            return 0

        lax.fori_loop(0, 8, phF, 0)

        for c in wcp:
            c.wait()
        wr32 = wr.bitcast(u32)
        wi32 = wi.bitcast(u32)
        hi = jnp.uint32(HI)
        dcr = jnp.concatenate([_bc(wr32[k, 0:1, :] << 16, f32) for k in range(16)], axis=0)
        dci = jnp.concatenate([_bc(wi32[k, 0:1, :] << 16, f32) for k in range(16)], axis=0)
        nyr = jnp.concatenate([wrn[:, 128 * k:128 * (k + 1)].astype(f32) for k in range(16)], axis=0)
        nyi = jnp.concatenate([win[:, 128 * k:128 * (k + 1)].astype(f32) for k in range(16)], axis=0)
        st = jnp.concatenate([dcr, dci, nyr, nyi], axis=0)
        stb = st.astype(bf16)
        r1 = jnp.dot(stb, misc[0], preferred_element_type=f32)
        r2 = jnp.dot(stb, misc[1], preferred_element_type=f32)
        rr = jnp.concatenate([r1, r2], axis=0).astype(bf16)
        rp = jnp.dot(misc[2, 64:128, :], rr, preferred_element_type=f32)
        rid = lax.broadcasted_iota(jnp.int32, (64, 128), 0)
        sgn = jnp.where((rid & 16) == 0, 0.5, -0.5)
        WS[...] = 0.5 * st + sgn * rp

        POS = {1: 0, 7: 64, 2: 128, 6: 192, 3: 256, 5: 320, 0: 384, 4: 448}
        row8 = lax.broadcasted_iota(jnp.int32, (8, 128), 0)

        def mid(r, g, special):
            r0 = POS[r] + 8 * g
            if not special:
                r0 = pl.multiple_of(r0, 8)
            xs_ = [(Zr[a, pl.ds(r0, 8), :], Zi[a, pl.ds(r0, 8), :]) for a in range(16)]
            o = _fft16(xs_, False)
            if special:
                xn = [(Zr[a, 512:520, :], Zi[a, 512:520, :]) for a in range(16)]
                on = _fft16(xn, False)
                wsr, wsi = wr32, wi32
            else:
                g32 = pl.multiple_of(32 * g, 32)
                wsr = wr32.at[:, pl.ds(g32, 32), :]
                wsi = wi32.at[:, pl.ds(g32, 32), :]
            ys = []
            for k in range(16):
                a_ = wsr[k, pl.ds(r // 2, 8, stride=4), :]
                b_ = wsi[k, pl.ds(r // 2, 8, stride=4), :]
                if r % 2 == 0:
                    wre, wim = _bc(a_ << 16, f32), _bc(b_ << 16, f32)
                else:
                    wre, wim = _bc(a_ & hi, f32), _bc(b_ & hi, f32)
                if special:
                    wre = jnp.where(row8 == 0, jnp.broadcast_to(WS[k:k + 1, :], (8, 128)), wre)
                    wim = jnp.where(row8 == 0, jnp.broadcast_to(WS[16 + k:17 + k, :], (8, 128)), wim)
                xr, xi = o[k]
                yr = xr * wre - xi * wim
                yi = xr * wim + xi * wre
                if special:
                    nr = jnp.broadcast_to(WS[32 + k:33 + k, :], (8, 128))
                    ni = jnp.broadcast_to(WS[48 + k:49 + k, :], (8, 128))
                    zr_, zi_ = on[k]
                    yr = yr - (zr_ * ni + zi_ * nr)
                    yi = yi + (zr_ * nr - zi_ * ni)
                ys.append((yr, yi))
            u = _fft16(ys, True)
            for a in range(16):
                Zr[a, pl.ds(r0, 8), :] = u[a][0]
                Zi[a, pl.ds(r0, 8), :] = u[a][1]

        mid(0, 0, True)

        def phM(g, _):
            for r in range(1, 8):
                mid(r, g, False)

            @pl.when(g > 0)
            def _():
                mid(0, g, False)

            return 0

        lax.fori_loop(0, 8, phM, 0)

        def phI(m, _):
            for half in range(2):
                a = 2 * m + half
                Mx = getM(a)
                for t in range(4):
                    yy = jnp.concatenate(
                        [Zr[a, 128 * t:128 * t + 128, :], Zi[a, 128 * t:128 * t + 128, :]], axis=1).astype(bf16)
                    o = lax.dot_general(Mx, yy, NT, preferred_element_type=f32)
                    vv = jnp.concatenate([o[:128], o[128:]], axis=1).astype(bf16)
                    PQ[half, t] = jnp.dot(vv, G[t if t < 3 else 4], preferred_element_type=f32)
            for ch_ in range(8):
                rs = slice(16 * ch_, 16 * ch_ + 16)
                res = []
                for half in range(2):
                    P1, Q1 = PQ[half, 0, rs, 0:128], PQ[half, 0, rs, 128:256]
                    P2, Q2 = PQ[half, 1, rs, 0:128], PQ[half, 1, rs, 128:256]
                    P3, Q3 = PQ[half, 2, rs, 0:128], PQ[half, 2, rs, 128:256]
                    h0, h4 = PQ[half, 3, rs, 0:128], PQ[half, 3, rs, 128:256]
                    e, o_ = h0 + h4, h0 - h4
                    A, B = P1 + P3, Q1 - Q3
                    u, v = P1 - P3, Q1 + Q3
                    T1_, T2_ = RS * (u - v), RS * (-u - v)
                    e1, e2 = e + P2, e - P2
                    o1, o2 = o_ - Q2, o_ + Q2
                    cols = jnp.concatenate(
                        [e1 + A, o1 + T1_, e2 - B, o2 + T2_, e1 - A, o1 - T1_, e2 + B, o2 - T2_], axis=1)
                    res.append(_bc(cols.astype(bf16).astype(f32), u32))
                bs[m, rs, :] = (res[0] >> 16) | res[1]
            return 0

        lax.fori_loop(0, 8, phI, 0)

    pl.run_scoped(
        scoped,
        pltpu.VMEM((8, 128, D), u32), pltpu.VMEM((16, 512, 128), bf16), pltpu.VMEM((16, 512, 128), bf16),
        pltpu.VMEM((1, S), bf16), pltpu.VMEM((1, S), bf16),
        pltpu.VMEM((5, 256, 256), bf16), pltpu.VMEM((16, 256, 128), bf16), pltpu.VMEM((3, 128, 128), bf16),
        pltpu.VMEM((2, 4, 128, 256), bf16), pltpu.VMEM((16, 528, 128), f32), pltpu.VMEM((16, 528, 128), f32),
        pltpu.VMEM((64, 128), f32), pltpu.VMEM((2, 4, 128, 256), f32))


def _kernel(x_hbm, x3_hbm, mem0_hbm, wq_hbm, wk_hbm, wv_hbm, wo_hbm, xb_hbm, wr_hbm, wi_hbm, gw_hbm,
            g_hbm, h_hbm, misc_hbm, out_hbm,
            xv, xpre, mem0v, gwv, raw, wo, bs, bnat, gbuf, outb, bsems, wsems, msems, osem):
    x32 = x_hbm.bitcast(u32)
    cp_x = pltpu.make_async_copy(x32, xv, msems.at[0])
    cp_xpre = pltpu.make_async_copy(x3_hbm.bitcast(u32).at[:, pl.ds(12, 4), :], xpre, msems.at[1])
    cp_mem = pltpu.make_async_copy(mem0_hbm, mem0v, msems.at[2])
    cp_gw = pltpu.make_async_copy(gw_hbm, gwv, msems.at[3])
    wsrc = [w.bitcast(u32) for w in (wq_hbm, wk_hbm, wv_hbm)]
    wo32 = wo_hbm.bitcast(u32)
    cp_w = [[pltpu.make_async_copy(wsrc[i].at[:, p, :], raw.at[p, i], wsems.at[p]) for i in range(3)]
            for p in range(16)]
    cp_wo = [pltpu.make_async_copy(wo32.at[:, :, pl.ds(128 * j, 128)], wo.at[j], msems.at[4]) for j in range(8)]

    def start_rest():
        cp_gw.start()
        cp_mem.start()
        cp_xpre.start()
        for p in range(16):
            for c in cp_w[p]:
                c.start()
        cp_x.start()
        for c in cp_wo:
            c.start()

    _b_phase(xb_hbm, wr_hbm, wi_hbm, g_hbm, h_hbm, misc_hbm, bs, bsems, start_rest)

    bn32 = bnat.bitcast(u32)
    cp_b = [pltpu.make_async_copy(bs.at[m], bn32.at[:, m, :], msems.at[5]) for m in range(8)]
    for c in cp_b:
        c.start()

    def a_phase(w3, pre, oc, acc, lhs):
        cp_xpre.wait()

        def prebulk(p, _):
            for i in range(3):
                pltpu.make_async_copy(wsrc[i].at[:, 0, :], raw.at[p, i], wsems.at[p]).wait()
            for i in range(3):
                e = raw[p, i, pl.ds(0, 512, stride=2), :]
                o = raw[p, i, pl.ds(1, 512, stride=2), :]
                w3[p, 0, i] = (e & jnp.uint32(0xFFFF)) | (o << 16)
                w3[p, 1, i] = (e >> 16) | (o & jnp.uint32(HI))
            for r in range(2):
                for i in range(3):
                    for c in range(2):
                        xl = _w2b(xpre[pl.ds(32 * c, 32)].reshape(128, D))
                        pre[p, r, i, 256 * c:256 * c + 256, :] = jnp.dot(
                            xl, _w2b(w3[p, r, i]), preferred_element_type=f32)
            return 0

        lax.fori_loop(0, 16, prebulk, 0)

        cp_x.wait()
        cp_gw.wait()
        gwb = jnp.broadcast_to(gwv[...].astype(f32), (128, D)).astype(bf16)

        def gate(i, _):
            r0 = pl.multiple_of(i * 128, 128)
            lg = lax.dot_general(_w2b(xv[pl.ds(r0, 128), :]), gwb, NT, preferred_element_type=f32)
            gbuf[pl.ds(pl.multiple_of(i * 256, 256), 256), :] = jax.nn.sigmoid(lg)
            return 0

        lax.fori_loop(0, 8, gate, 0)
        cp_mem.wait()
        for c in cp_wo:
            c.wait()
        for c in cp_b:
            c.wait()
        oc[...] = jnp.zeros(oc.shape, f32)

        row = lax.broadcasted_iota(jnp.int32, (48, 128), 0)
        col = lax.broadcasted_iota(jnp.int32, (48, 128), 1)
        mask = ((col < 40) & (row >= 32)) | ((row < 32) & ((col <= row) | ((col >= 32) & (col < 40))))
        scale = DH ** -0.5
        bscale = 2.0 ** -20

        def wo_t(j, h):
            return _w2b(wo[j, h])

        def mix(a, b, g):
            return g * a + (1.0 - g) * (b.astype(f32) * bscale)

        def fill_piece(grp, gr, gw_, par, j, half, accs):
            hs = range(16 * half, 16 * half + 16)
            l = jnp.concatenate(
                [jnp.concatenate([oc[par, q, h] for q in range(4)], axis=0) for h in hs], axis=1).astype(bf16)
            w = _w2b(wo[j, 16 * half:16 * half + 16].reshape(16 * 64, 128))
            c = jnp.dot(l, w, preferred_element_type=f32)
            if half == 0:
                return c
            c = c + accs
            for q in range(4):
                sg = 4 * gr + q
                b = bnat[2 * sg + 1, 8:16, pl.ds(pl.multiple_of(128 * j, 128), 128)]
                g = gbuf[pl.ds(pl.multiple_of(32 * sg + 24, 8), 8), :]
                outb[pl.ds(pl.multiple_of(128 * gw_ + 32 * q + 24, 8), 8),
                     pl.ds(pl.multiple_of(128 * j, 128), 128)] = mix(c[8 * q:8 * q + 8], b, g).astype(bf16)
            return None

        def out_copy(gi):
            return pltpu.make_async_copy(
                outb.at[pl.ds(pl.multiple_of(128 * gi, 128), 128), :],
                out_hbm.at[pl.ds(pl.multiple_of(128 * gi, 128), 128), :], osem)

        def step(s, mem):
            @pl.when((s % 4 == 0) & (s >= 8))
            def _():
                out_copy(s // 4 - 2).start()

            r0 = pl.multiple_of(s * 16, 16)
            xs0 = _w2b(xv[pl.ds(r0, 8), :])
            xs1 = _w2b(xv[pl.ds(r0 + 8, 8), :])
            l1 = jnp.concatenate([xs1[0:8].astype(f32), mem], axis=0).astype(bf16)
            lhs[0:8, :] = pltpu.bitcast(xs0, u32)
            lhs[8:16, :] = pltpu.bitcast(l1, u32)
            grp = s // 4 - 1
            gr = jnp.maximum(grp, 0)
            gw_ = jnp.where(grp < 0, 16, grp)
            par = (s // 4 + 1) % 2
            cur = (s // 4) % 2
            q4 = s % 4
            st = {}
            z8 = jnp.zeros((8, 128), f32)
            s8 = pl.multiple_of(s * 8, 8)

            def proj(h, i):
                r = jnp.dot(_w2b(lhs[...]), _w2b(w3[h // 2, h % 2, i]), preferred_element_type=f32)
                p_ = pre[h // 2, h % 2, i, pl.ds(s8, 8), :]
                st[("qkv", h, i)] = jnp.concatenate([r[0:24], p_, r[24:32], z8], axis=0).astype(bf16)

            def qk(h):
                q = st.pop(("qkv", h, 0))
                k = st.pop(("qkv", h, 1))
                sc = lax.dot_general(q, k, NT, preferred_element_type=f32) * scale
                sc = jnp.concatenate([sc, jnp.zeros((48, 80), f32)], axis=1)
                sc = jnp.where(mask, sc, -1e9)
                m = jnp.max(sc, axis=1, keepdims=True)
                e = jnp.exp(sc - m)
                p = e * (1.0 / jnp.sum(e, axis=1, keepdims=True))
                st[("p", h)] = p[:, :48].astype(bf16)

            def pv(h):
                o = jnp.dot(st.pop(("p", h)), st.pop(("qkv", h, 2)), preferred_element_type=f32)
                st[("o", h)] = jnp.concatenate([o[0:24], o[32:40]], axis=0).astype(bf16)
                oc[cur, q4, h] = o[24:32]

            def oproj(h):
                w = jnp.concatenate([wo_t(j, h) for j in range(8)], axis=1)
                c = jnp.dot(st.pop(("o", h)), w, preferred_element_type=f32)
                if h == 0:
                    acc[...] = c
                else:
                    acc[...] += c

            ok = lambda h: 0 <= h < H
            for t in range(H + 4):
                if ok(t):
                    proj(t, 0)
                    proj(t, 1)
                if ok(t - 1):
                    qk(t - 1)
                if ok(t):
                    proj(t, 2)
                else:
                    jj, half = (t - H) // 2, (t - H) % 2
                    st["fill"] = fill_piece(grp, gr, gw_, par, 2 * q4 + jj, half, st.get("fill"))
                if ok(t - 3):
                    pv(t - 3)
                if ok(t - 4):
                    oproj(t - 4)
            a = acc[...]
            rs = pl.multiple_of(32 * s, 32)
            b0 = bnat[2 * s, :, :]
            b1 = bnat[2 * s + 1, 0:8, :]
            g0 = gbuf[pl.ds(rs, 16), :]
            g1 = gbuf[pl.ds(rs + 16, 8), :]
            outb[pl.ds(rs, 16), :] = mix(a[0:16], b0, jnp.tile(g0, (1, 8))).astype(bf16)
            outb[pl.ds(rs + 16, 8), :] = mix(a[16:24], b1, jnp.tile(g1, (1, 8))).astype(bf16)
            return a[24:32]

        lax.fori_loop(0, NSEG, step, mem0v[...].astype(f32))

        for j in range(8):
            c = fill_piece(15, 15, 15, 1, j, 0, None)
            fill_piece(15, 15, 15, 1, j, 1, c)
        out_copy(14).start()
        out_copy(15).start()
        for gi in range(16):
            out_copy(gi).wait()

    pl.run_scoped(
        a_phase,
        pltpu.VMEM((16, 2, 3, 512, 128), u32), pltpu.VMEM((16, 2, 3, 512, 128), f32),
        pltpu.VMEM((2, 4, H, 8, 128), f32), pltpu.VMEM((32, D), f32), pltpu.VMEM((16, D), u32))


@jax.jit
def pallas_gated_mix__memory_aug_recurrent_mem_tr__spectral_gfnet__prompt_kernel(
    A_x, A_mem0, A_Wq, A_Wk, A_Wv, A_Wo, A_seg_len, B_x, B_w_r, B_w_i, gate_w,
):
    del A_seg_len
    del B_x
    HB = pl.BlockSpec(memory_space=pltpu.HBM)
    out = pl.pallas_call(
        _kernel,
        out_shape=jax.ShapeDtypeStruct((S, D), bf16),
        in_specs=[HB] * 14,
        out_specs=HB,
        scratch_shapes=[
            pltpu.VMEM((S // 2, D), u32),
            pltpu.VMEM((NSEG, 4, D), u32),
            pltpu.VMEM((M_MEM, D), bf16),
            pltpu.VMEM((1, D), bf16),
            pltpu.VMEM((16, 3, D, DH), u32),
            pltpu.VMEM((8, H, DH // 2, 128), u32),
            pltpu.VMEM((8, 128, D), u32),
            pltpu.VMEM((128, 16, D), bf16),
            pltpu.VMEM((S, 128), f32),
            pltpu.VMEM((S + 128, D), bf16),
            pltpu.SemaphoreType.DMA((13,)),
            pltpu.SemaphoreType.DMA((16,)),
            pltpu.SemaphoreType.DMA((6,)),
            pltpu.SemaphoreType.DMA(()),
        ],
        compiler_params=pltpu.CompilerParams(vmem_limit_bytes=124 * 2 ** 20),
    )(
        A_x.reshape(S, D), A_x.reshape(NSEG, SEG, D), A_mem0.reshape(M_MEM, D), A_Wq, A_Wk, A_Wv, A_Wo,
        A_x.reshape(128, 16, D), B_w_r.T, B_w_i.T, gate_w.reshape(1, D), _TAB_G, _TAB_H, _TAB_MISC,
    )
    return out.reshape(1, S, D)
```

```python
import numpy as np
import ml_dtypes
import jax
import jax.numpy as jnp
from jax import lax
import jax.experimental.pallas as pl
import jax.experimental.pallas.tpu as pltpu

f32, bf16, u32 = jnp.float32, jnp.bfloat16, jnp.uint32
S, D, H, DH, M_MEM, SEG = 2048, 1024, 32, 128, 8, 32
NSEG = S // SEG
RS = float(1 / np.sqrt(2))
NT = (((1,), (1,)), ((), ()))
HI = 0xFFFF0000


def _np_tables():
    bf = ml_dtypes.bfloat16
    dp = np.arange(128)
    j = np.arange(64)

    def cs(f):
        ang = 2 * np.pi * ((f[:, None] * dp[None, :]) % 1024) / 1024
        return np.cos(ang), np.sin(ang)

    G = np.zeros((5, 256, 256))
    for t in range(3):
        r = t + 1
        C, Sn = cs(r + 8 * j)
        C2, S2 = cs(8 - r + 8 * j)
        G[t, 0:64, 0:128] = C
        G[t, 0:64, 128:] = Sn
        G[t, 64:128, 0:128] = C2
        G[t, 64:128, 128:] = -S2
        G[t, 128:192, 0:128] = -Sn
        G[t, 128:192, 128:] = C
        G[t, 192:256, 0:128] = -S2
        G[t, 192:256, 128:] = -C2
    C0, S0 = cs(8 * j)
    C4, S4 = cs(4 + 8 * j)
    G[3, 0:64, 0:128] = C0
    G[3, 128:192, 0:128] = -S0
    G[3, 64:128, 128:] = C4
    G[3, 192:256, 128:] = -S4
    G[4] = G[3]
    G[4, 0, 0:128] = 0.5
    G[4, 128, 0:128] = 0.5 * (-1.0) ** dp
    HH = np.zeros((16, 256, 128))
    for a in range(16):
        ang = 2 * np.pi * (((a + 16 * dp)[:, None] * dp[None, :]) % 2048) / 2048
        HH[a, :128] = np.cos(ang)
        HH[a, 128:] = np.sin(ang)
    misc = np.zeros((3, 128, 128))
    misc[0, 128 - dp[1:], dp[1:]] = 1
    misc[1, 0, 0] = 1
    misc[2, 0, :] = (-1.0) ** dp
    for blk in range(4):
        for k1 in range(16):
            misc[2, 64 + 16 * blk + k1, 16 * blk + 15 - k1] = 1
            misc[2, 64 + 16 * blk + k1, 64 + 16 * blk + (16 - k1) % 16] = 1
    return G.astype(bf), HH.astype(bf), misc.astype(bf)


_TAB_G, _TAB_H, _TAB_MISC = _np_tables()


def _bc(x, dt):
    return lax.bitcast_convert_type(x, dt)


def _w2b(w):
    return pltpu.bitcast(w, bf16)


def _fft16(xs, inverse):
    sg = 1.0 if inverse else -1.0

    def dft4(a, b, c, d):
        t0 = (a[0] + c[0], a[1] + c[1])
        t1 = (a[0] - c[0], a[1] - c[1])
        t2 = (b[0] + d[0], b[1] + d[1])
        t3 = (b[0] - d[0], b[1] - d[1])
        o0 = (t0[0] + t2[0], t0[1] + t2[1])
        o2 = (t0[0] - t2[0], t0[1] - t2[1])
        m = (t1[0] + t3[1], t1[1] - t3[0])
        p = (t1[0] - t3[1], t1[1] + t3[0])
        return [o0, p, o2, m] if inverse else [o0, m, o2, p]

    t = [dft4(xs[a0], xs[4 + a0], xs[8 + a0], xs[12 + a0]) for a0 in range(4)]

    def tw(v, e):
        e = e % 16
        if e == 0:
            return v
        if e == 4:
            return (-v[1], v[0]) if inverse else (v[1], -v[0])
        if e == 2:
            if inverse:
                return ((v[0] - v[1]) * RS, (v[0] + v[1]) * RS)
            return ((v[0] + v[1]) * RS, (v[1] - v[0]) * RS)
        if e == 6:
            if inverse:
                return ((-v[0] - v[1]) * RS, (v[0] - v[1]) * RS)
            return ((v[1] - v[0]) * RS, (-v[0] - v[1]) * RS)
        c = float(np.cos(2 * np.pi * e / 16))
        s = float(sg * np.sin(2 * np.pi * e / 16))
        return (v[0] * c - v[1] * s, v[0] * s + v[1] * c)

    out = [None] * 16
    for k in range(4):
        u = [tw(t[a0][k], a0 * k) for a0 in range(4)]
        r = dft4(*u)
        for m in range(4):
            out[k + 4 * m] = r[m]
    return out


def _b_phase(xb_hbm, wr_hbm, wi_hbm, g_hbm, h_hbm, misc_hbm, bs, sems, start_m, start_i):
    def scoped(xs, wr, wi, wrn, win, G, HH, misc, Y, Zr, Zi, WS, PQ):
        xb32 = xb_hbm.bitcast(u32)
        xcp = [pltpu.make_async_copy(xb32.at[:, m, :], xs.at[m], sems.at[m]) for m in range(2)]
        cg = pltpu.make_async_copy(g_hbm, G, sems.at[8])
        ch = pltpu.make_async_copy(h_hbm, HH, sems.at[9])
        cm = pltpu.make_async_copy(misc_hbm, misc, sems.at[10])
        def wblk(k):
            off = 128 * k if isinstance(k, int) else pl.multiple_of(128 * k, 128)
            return (pltpu.make_async_copy(wr_hbm.at[pl.ds(0, 512), pl.ds(off, 128)], wr.at[k], sems.at[11]),
                    pltpu.make_async_copy(wi_hbm.at[pl.ds(0, 512), pl.ds(off, 128)], wi.at[k], sems.at[12]))

        wny = (pltpu.make_async_copy(wr_hbm.at[pl.ds(512, 1), :], wrn, sems.at[11]),
               pltpu.make_async_copy(wi_hbm.at[pl.ds(512, 1), :], win, sems.at[12]))
        cg.start()
        xcp[0].start()
        ch.start()
        cm.start()
        xcp[1].start()
        for c in wny:
            c.start()
        cg.wait()
        cm.wait()
        ch.wait()

        def getM(a):
            hc = HH[a, 0:128, :]
            hs = HH[a, 128:256, :]
            return jnp.concatenate(
                [jnp.concatenate([hc, -hs], axis=1), jnp.concatenate([hs, hc], axis=1)], axis=0)

        def phF(m, _):
            @pl.when(m < 6)
            def _():
                pltpu.make_async_copy(xb32.at[:, m + 2, :], xs.at[m + 2], sems.at[m + 2]).start()

            for k in (2 * m, 2 * m + 1):
                for c in wblk(k):
                    c.start()
            pltpu.make_async_copy(xb32.at[:, 0, :], xs.at[m], sems.at[m]).wait()
            for ch_ in range(8):
                w = xs[m, 16 * ch_:16 * ch_ + 16, :]
                for half, xv in enumerate((_bc(w << 16, f32), _bc(w & jnp.uint32(HI), f32))):
                    xc = [xv[:, 128 * c:128 * (c + 1)] for c in range(8)]
                    a0, a1 = xc[0] + xc[4], xc[0] - xc[4]
                    b0, b1 = xc[2] + xc[6], xc[2] - xc[6]
                    c0, c1 = xc[1] + xc[5], xc[1] - xc[5]
                    d0, d1 = xc[3] + xc[7], xc[3] - xc[7]
                    p, q = a0 + b0, c0 + d0
                    y0, y4 = p + q, p - q
                    y2r, y2i = a0 - b0, d0 - c0
                    cm_, cp_ = RS * (c1 - d1), RS * (c1 + d1)
                    y1r, y1i = a1 + cm_, -b1 - cp_
                    y3r, y3i = a1 - cm_, b1 - cp_
                    for t, (yr, yi) in enumerate([(y1r, y1i), (y2r, y2i), (y3r, y3i), (y0, y4)]):
                        Y[half, t, 16 * ch_:16 * ch_ + 16, :] = jnp.concatenate([yr, yi], axis=1).astype(bf16)
            for half in range(2):
                a = 2 * m + half
                Mx = getM(a)
                for t in range(4):
                    o = lax.dot_general(G[t], Y[half, t], NT, preferred_element_type=f32)
                    z = jnp.concatenate([o[:128], o[128:]], axis=1).astype(bf16)
                    X = jnp.dot(z, Mx, preferred_element_type=f32)
                    Zr[a, 128 * t:128 * t + 128, :] = X[:, 0:128]
                    Zi[a, 128 * t:128 * t + 128, :] = X[:, 128:256]
                ony = lax.dot_general(misc[2, 0:16, :], Y[half, 3, :, 0:128], NT, preferred_element_type=f32)
                Xn = jnp.dot(ony.astype(bf16), Mx[0:128, :], preferred_element_type=f32)
                Zr[a, 512:528, :] = Xn[:, 0:128]
                Zi[a, 512:528, :] = Xn[:, 128:256]
            return 0

        lax.fori_loop(0, 8, phF, 0)

        for k in range(16):
            for c in wblk(k):
                c.wait()
        for c in wny:
            c.wait()
        wr32 = wr.bitcast(u32)
        wi32 = wi.bitcast(u32)
        hi = jnp.uint32(HI)
        dcr = jnp.concatenate([_bc(wr32[k, 0:1, :] << 16, f32) for k in range(16)], axis=0)
        dci = jnp.concatenate([_bc(wi32[k, 0:1, :] << 16, f32) for k in range(16)], axis=0)
        nyr = jnp.concatenate([wrn[:, 128 * k:128 * (k + 1)].astype(f32) for k in range(16)], axis=0)
        nyi = jnp.concatenate([win[:, 128 * k:128 * (k + 1)].astype(f32) for k in range(16)], axis=0)
        st = jnp.concatenate([dcr, dci, nyr, nyi], axis=0)
        stb = st.astype(bf16)
        r1 = jnp.dot(stb, misc[0], preferred_element_type=f32)
        r2 = jnp.dot(stb, misc[1], preferred_element_type=f32)
        rr = jnp.concatenate([r1, r2], axis=0).astype(bf16)
        rp = jnp.dot(misc[2, 64:128, :], rr, preferred_element_type=f32)
        rid = lax.broadcasted_iota(jnp.int32, (64, 128), 0)
        sgn = jnp.where((rid & 16) == 0, 0.5, -0.5)
        WS[...] = 0.5 * st + sgn * rp

        POS = {1: 0, 7: 64, 2: 128, 6: 192, 3: 256, 5: 320, 0: 384, 4: 448}
        row8 = lax.broadcasted_iota(jnp.int32, (8, 128), 0)

        def mid(r, g, special):
            r0 = POS[r] + 8 * g
            if not special:
                r0 = pl.multiple_of(r0, 8)
            xs_ = [(Zr[a, pl.ds(r0, 8), :], Zi[a, pl.ds(r0, 8), :]) for a in range(16)]
            o = _fft16(xs_, False)
            if special:
                xn = [(Zr[a, 512:520, :], Zi[a, 512:520, :]) for a in range(16)]
                on = _fft16(xn, False)
                wsr, wsi = wr32, wi32
            else:
                g32 = pl.multiple_of(32 * g, 32)
                wsr = wr32.at[:, pl.ds(g32, 32), :]
                wsi = wi32.at[:, pl.ds(g32, 32), :]
            ys = []
            for k in range(16):
                a_ = wsr[k, pl.ds(r // 2, 8, stride=4), :]
                b_ = wsi[k, pl.ds(r // 2, 8, stride=4), :]
                if r % 2 == 0:
                    wre, wim = _bc(a_ << 16, f32), _bc(b_ << 16, f32)
                else:
                    wre, wim = _bc(a_ & hi, f32), _bc(b_ & hi, f32)
                if special:
                    wre = jnp.where(row8 == 0, jnp.broadcast_to(WS[k:k + 1, :], (8, 128)), wre)
                    wim = jnp.where(row8 == 0, jnp.broadcast_to(WS[16 + k:17 + k, :], (8, 128)), wim)
                xr, xi = o[k]
                yr = xr * wre - xi * wim
                yi = xr * wim + xi * wre
                if special:
                    nr = jnp.broadcast_to(WS[32 + k:33 + k, :], (8, 128))
                    ni = jnp.broadcast_to(WS[48 + k:49 + k, :], (8, 128))
                    zr_, zi_ = on[k]
                    yr = yr - (zr_ * ni + zi_ * nr)
                    yi = yi + (zr_ * nr - zi_ * ni)
                ys.append((yr, yi))
            u = _fft16(ys, True)
            for a in range(16):
                Zr[a, pl.ds(r0, 8), :] = u[a][0]
                Zi[a, pl.ds(r0, 8), :] = u[a][1]

        mid(0, 0, True)

        def phM(g, _):
            start_m(g)
            for r in range(1, 8):
                mid(r, g, False)

            @pl.when(g > 0)
            def _():
                mid(0, g, False)

            return 0

        lax.fori_loop(0, 8, phM, 0)

        def phI(m, _):
            start_i(m)
            for half in range(2):
                a = 2 * m + half
                Mx = getM(a)
                for t in range(4):
                    yy = jnp.concatenate(
                        [Zr[a, 128 * t:128 * t + 128, :], Zi[a, 128 * t:128 * t + 128, :]], axis=1).astype(bf16)
                    o = lax.dot_general(Mx, yy, NT, preferred_element_type=f32)
                    vv = jnp.concatenate([o[:128], o[128:]], axis=1).astype(bf16)
                    PQ[half, t] = jnp.dot(vv, G[t if t < 3 else 4], preferred_element_type=f32)
            for ch_ in range(8):
                rs = slice(16 * ch_, 16 * ch_ + 16)
                res = []
                for half in range(2):
                    P1, Q1 = PQ[half, 0, rs, 0:128], PQ[half, 0, rs, 128:256]
                    P2, Q2 = PQ[half, 1, rs, 0:128], PQ[half, 1, rs, 128:256]
                    P3, Q3 = PQ[half, 2, rs, 0:128], PQ[half, 2, rs, 128:256]
                    h0, h4 = PQ[half, 3, rs, 0:128], PQ[half, 3, rs, 128:256]
                    e, o_ = h0 + h4, h0 - h4
                    A, B = P1 + P3, Q1 - Q3
                    u, v = P1 - P3, Q1 + Q3
                    T1_, T2_ = RS * (u - v), RS * (-u - v)
                    e1, e2 = e + P2, e - P2
                    o1, o2 = o_ - Q2, o_ + Q2
                    cols = jnp.concatenate(
                        [e1 + A, o1 + T1_, e2 - B, o2 + T2_, e1 - A, o1 - T1_, e2 + B, o2 - T2_], axis=1)
                    res.append(_bc(cols.astype(bf16).astype(f32), u32))
                bs[m, rs, :] = (res[0] >> 16) | res[1]
            return 0

        lax.fori_loop(0, 8, phI, 0)

    pl.run_scoped(
        scoped,
        pltpu.VMEM((8, 128, D), u32), pltpu.VMEM((16, 512, 128), bf16), pltpu.VMEM((16, 512, 128), bf16),
        pltpu.VMEM((1, S), bf16), pltpu.VMEM((1, S), bf16),
        pltpu.VMEM((5, 256, 256), bf16), pltpu.VMEM((16, 256, 128), bf16), pltpu.VMEM((3, 128, 128), bf16),
        pltpu.VMEM((2, 4, 128, 256), bf16), pltpu.VMEM((16, 528, 128), f32), pltpu.VMEM((16, 528, 128), f32),
        pltpu.VMEM((64, 128), f32), pltpu.VMEM((2, 4, 128, 256), f32))


def _kernel(x_hbm, mem0_hbm, wq_hbm, wk_hbm, wv_hbm, wo_hbm, xb_hbm, wr_hbm, wi_hbm, gw_hbm,
            g_hbm, h_hbm, misc_hbm, out_hbm,
            xv, xpre, mem0v, gwv, raw, wo, bs, bnat, gbuf, outb, bsems, wsems, msems, osem):
    cp_x = pltpu.make_async_copy(x_hbm.bitcast(u32), xv, msems.at[0])
    cp_mem = pltpu.make_async_copy(mem0_hbm, mem0v, msems.at[2])
    cp_gw = pltpu.make_async_copy(gw_hbm, gwv, msems.at[3])
    wsrc = [w.bitcast(u32) for w in (wq_hbm, wk_hbm, wv_hbm)]
    wo32 = wo_hbm.bitcast(u32)

    def cp_w(p):
        return [pltpu.make_async_copy(wsrc[i].at[:, p, :], raw.at[p, i], wsems.at[p]) for i in range(3)]

    def cp_wo(j):
        off = 128 * j if isinstance(j, int) else pl.multiple_of(128 * j, 128)
        return pltpu.make_async_copy(wo32.at[:, :, pl.ds(off, 128)], wo.at[j], msems.at[4])

    def start_m(g):
        @pl.when(g == 0)
        def _():
            cp_gw.start()
            cp_mem.start()
            cp_x.start()

        for c in cp_w(g):
            c.start()

    def start_i(m):
        for c in cp_w(m + 8):
            c.start()

    _b_phase(xb_hbm, wr_hbm, wi_hbm, g_hbm, h_hbm, misc_hbm, bs, bsems, start_m, start_i)
    bn32 = bnat.bitcast(u32)

    def a_phase(w3, pre, oc, acc, lhs):
        cp_x.wait()
        cp_gw.wait()
        gwf = gwv[...].astype(f32)
        for i in range(32):
            xpre[8 * i:8 * i + 8, :] = jnp.concatenate(
                [xv[32 * i + 12:32 * i + 16, :], xv[32 * i + 28:32 * i + 32, :]], axis=0)

        def prebulk(p, _):
            @pl.when(p < 8)
            def _():
                cp_wo(p).start()

            for i in range(3):
                pltpu.make_async_copy(wsrc[i].at[:, 0, :], raw.at[p, i], wsems.at[p]).wait()
            for i in range(3):
                e = raw[p, i, pl.ds(0, 512, stride=2), :]
                o = raw[p, i, pl.ds(1, 512, stride=2), :]
                w3[p, 0, i] = (e & jnp.uint32(0xFFFF)) | (o << 16)
                w3[p, 1, i] = (e >> 16) | (o & jnp.uint32(HI))
            for r in range(2):
                for i in range(3):
                    for c in range(2):
                        xl = _w2b(xpre[128 * c:128 * c + 128, :])
                        pre[p, r, i, 256 * c:256 * c + 256, :] = jnp.dot(
                            xl, _w2b(w3[p, r, i]), preferred_element_type=f32)
            for c in range(8):
                xw = xv[pl.ds(pl.multiple_of(64 * p + 8 * c, 8), 8), :]
                xx = _w2b(xw).astype(f32) * gwf
                part = xx[:, 0:128]
                for jj in range(1, 8):
                    part = part + xx[:, 128 * jj:128 * jj + 128]
                lg = jnp.sum(part, axis=1, keepdims=True)
                gbuf[pl.ds(pl.multiple_of(128 * p + 16 * c, 16), 16), :] = jnp.broadcast_to(
                    jax.nn.sigmoid(lg), (16, 128))
            for jj in range(8):
                dst = bn32.at[jj, pl.ds(pl.multiple_of(64 * p, 64), 64), :]
                for m in range(8):
                    dst[pl.ds(m, 8, stride=8), :] = bs[m, pl.ds(pl.multiple_of(8 * p, 8), 8), 128 * jj:128 * jj + 128]
            return 0

        lax.fori_loop(0, 16, prebulk, 0)
        cp_mem.wait()
        for j in range(8):
            cp_wo(j).wait()
        oc[...] = jnp.zeros(oc.shape, f32)

        row = lax.broadcasted_iota(jnp.int32, (48, 128), 0)
        col = lax.broadcasted_iota(jnp.int32, (48, 128), 1)
        mask = ((col < 40) & (row >= 32)) | ((row < 32) & ((col <= row) | ((col >= 32) & (col < 40))))
        scale = DH ** -0.5
        bscale = 2.0 ** -20

        def wo_t(j, h):
            return _w2b(wo[j, h])

        def mix(a, b, g):
            return g * a + (1.0 - g) * (b.astype(f32) * bscale)

        def fill_piece(grp, gr, gw_, par, j, half, accs):
            hs = range(16 * half, 16 * half + 16)
            l = jnp.concatenate(
                [jnp.concatenate([oc[par, q, h] for q in range(4)], axis=0) for h in hs], axis=1).astype(bf16)
            w = _w2b(wo[j, 16 * half:16 * half + 16].reshape(16 * 64, 128))
            c = jnp.dot(l, w, preferred_element_type=f32)
            if half == 0:
                return c
            c = c + accs
            for q in range(4):
                sg = 4 * gr + q
                b = bnat[j, pl.ds(pl.multiple_of(32 * sg + 24, 8), 8), :]
                g = gbuf[pl.ds(pl.multiple_of(32 * sg + 24, 8), 8), :]
                outb[pl.ds(pl.multiple_of(128 * gw_ + 32 * q + 24, 8), 8),
                     pl.ds(pl.multiple_of(128 * j, 128), 128)] = mix(c[8 * q:8 * q + 8], b, g).astype(bf16)
            return None

        def out_copy(gi):
            return pltpu.make_async_copy(
                outb.at[pl.ds(pl.multiple_of(128 * gi, 128), 128), :],
                out_hbm.at[pl.ds(pl.multiple_of(128 * gi, 128), 128), :], osem)

        def step(s, mem):
            @pl.when((s % 4 == 0) & (s >= 8))
            def _():
                out_copy(s // 4 - 2).start()

            r0 = pl.multiple_of(s * 16, 16)
            xs0 = _w2b(xv[pl.ds(r0, 8), :])
            xs1 = _w2b(xv[pl.ds(r0 + 8, 8), :])
            l1 = jnp.concatenate([xs1[0:8].astype(f32), mem], axis=0).astype(bf16)
            lhs[0:8, :] = pltpu.bitcast(xs0, u32)
            lhs[8:16, :] = pltpu.bitcast(l1, u32)
            grp = s // 4 - 1
            gr = jnp.maximum(grp, 0)
            gw_ = jnp.where(grp < 0, 16, grp)
            par = (s // 4 + 1) % 2
            cur = (s // 4) % 2
            q4 = s % 4
            st = {}
            z8 = jnp.zeros((8, 128), f32)
            s8 = pl.multiple_of(s * 8, 8)

            def proj(h, i):
                r = jnp.dot(_w2b(lhs[...]), _w2b(w3[h // 2, h % 2, i]), preferred_element_type=f32)
                p_ = pre[h // 2, h % 2, i, pl.ds(s8, 8), :]
                st[("qkv", h, i)] = jnp.concatenate([r[0:24], p_, r[24:32], z8], axis=0).astype(bf16)

            def qk(h):
                q = st.pop(("qkv", h, 0))
                k = st.pop(("qkv", h, 1))
                sc = lax.dot_general(q, k, NT, preferred_element_type=f32) * scale
                sc = jnp.concatenate([sc, jnp.zeros((48, 80), f32)], axis=1)
                sc = jnp.where(mask, sc, -1e9)
                m = jnp.max(sc, axis=1, keepdims=True)
                e = jnp.exp(sc - m)
                p = e * (1.0 / jnp.sum(e, axis=1, keepdims=True))
                st[("p", h)] = p[:, :48].astype(bf16)

            def pv(h):
                o = jnp.dot(st.pop(("p", h)), st.pop(("qkv", h, 2)), preferred_element_type=f32)
                st[("o", h)] = jnp.concatenate([o[0:24], o[32:40]], axis=0).astype(bf16)
                oc[cur, q4, h] = o[24:32]

            def oproj(h):
                w = jnp.concatenate([wo_t(j, h) for j in range(8)], axis=1)
                c = jnp.dot(st.pop(("o", h)), w, preferred_element_type=f32)
                if h == 0:
                    acc[...] = c
                else:
                    acc[...] += c

            ok = lambda h: 0 <= h < H
            for t in range(H + 4):
                if ok(t):
                    proj(t, 0)
                    proj(t, 1)
                if ok(t - 1):
                    qk(t - 1)
                if ok(t):
                    proj(t, 2)
                else:
                    jj, half = (t - H) // 2, (t - H) % 2
                    st["fill"] = fill_piece(grp, gr, gw_, par, 2 * q4 + jj, half, st.get("fill"))
                if ok(t - 3):
                    pv(t - 3)
                if ok(t - 4):
                    oproj(t - 4)
            a = acc[...]
            rs = pl.multiple_of(32 * s, 32)
            b0 = jnp.concatenate([bnat[j, pl.ds(rs, 16), :] for j in range(8)], axis=1)
            b1 = jnp.concatenate([bnat[j, pl.ds(rs + 16, 8), :] for j in range(8)], axis=1)
            g0 = gbuf[pl.ds(rs, 16), :]
            g1 = gbuf[pl.ds(rs + 16, 8), :]
            outb[pl.ds(rs, 16), :] = mix(a[0:16], b0, jnp.tile(g0, (1, 8))).astype(bf16)
            outb[pl.ds(rs + 16, 8), :] = mix(a[16:24], b1, jnp.tile(g1, (1, 8))).astype(bf16)
            return a[24:32]

        lax.fori_loop(0, NSEG, step, mem0v[...].astype(f32))

        for j in range(8):
            c = fill_piece(15, 15, 15, 1, j, 0, None)
            fill_piece(15, 15, 15, 1, j, 1, c)
        out_copy(14).start()
        out_copy(15).start()
        for gi in range(16):
            out_copy(gi).wait()

    pl.run_scoped(
        a_phase,
        pltpu.VMEM((16, 2, 3, 512, 128), u32), pltpu.VMEM((16, 2, 3, 512, 128), f32),
        pltpu.VMEM((2, 4, H, 8, 128), f32), pltpu.VMEM((32, D), f32), pltpu.VMEM((16, D), u32))


@jax.jit
def pallas_gated_mix__memory_aug_recurrent_mem_tr__spectral_gfnet__prompt_kernel(
    A_x, A_mem0, A_Wq, A_Wk, A_Wv, A_Wo, A_seg_len, B_x, B_w_r, B_w_i, gate_w,
):
    del A_seg_len
    del B_x
    HB = pl.BlockSpec(memory_space=pltpu.HBM)
    out = pl.pallas_call(
        _kernel,
        out_shape=jax.ShapeDtypeStruct((S, D), bf16),
        in_specs=[HB] * 13,
        out_specs=HB,
        scratch_shapes=[
            pltpu.VMEM((S // 2, D), u32),
            pltpu.VMEM((NSEG * 4, D), u32),
            pltpu.VMEM((M_MEM, D), bf16),
            pltpu.VMEM((1, D), bf16),
            pltpu.VMEM((16, 3, D, DH), u32),
            pltpu.VMEM((8, H, DH // 2, 128), u32),
            pltpu.VMEM((8, 128, D), u32),
            pltpu.VMEM((8, S, 128), bf16),
            pltpu.VMEM((S, 128), f32),
            pltpu.VMEM((S + 128, D), bf16),
            pltpu.SemaphoreType.DMA((13,)),
            pltpu.SemaphoreType.DMA((16,)),
            pltpu.SemaphoreType.DMA((6,)),
            pltpu.SemaphoreType.DMA(()),
        ],
        compiler_params=pltpu.CompilerParams(vmem_limit_bytes=124 * 2 ** 20),
    )(
        A_x.reshape(S, D), A_mem0.reshape(M_MEM, D), A_Wq, A_Wk, A_Wv, A_Wo,
        A_x.reshape(128, 16, D), B_w_r.T, B_w_i.T, gate_w.reshape(1, D), _TAB_G, _TAB_H, _TAB_MISC,
    )
    return out.reshape(1, S, D)
```

```python
import numpy as np
import ml_dtypes
import jax
import jax.numpy as jnp
from jax import lax
import jax.experimental.pallas as pl
import jax.experimental.pallas.tpu as pltpu

f32, bf16, u32 = jnp.float32, jnp.bfloat16, jnp.uint32
S, D, H, DH, M_MEM, SEG = 2048, 1024, 32, 128, 8, 32
NSEG = S // SEG
RS = float(1 / np.sqrt(2))
NT = (((1,), (1,)), ((), ()))
HI = 0xFFFF0000


def _np_tables():
    bf = ml_dtypes.bfloat16
    dp = np.arange(128)
    j = np.arange(64)

    def cs(f):
        ang = 2 * np.pi * ((f[:, None] * dp[None, :]) % 1024) / 1024
        return np.cos(ang), np.sin(ang)

    G = np.zeros((5, 256, 256))
    for t in range(3):
        r = t + 1
        C, Sn = cs(r + 8 * j)
        C2, S2 = cs(8 - r + 8 * j)
        G[t, 0:64, 0:128] = C
        G[t, 0:64, 128:] = Sn
        G[t, 64:128, 0:128] = C2
        G[t, 64:128, 128:] = -S2
        G[t, 128:192, 0:128] = -Sn
        G[t, 128:192, 128:] = C
        G[t, 192:256, 0:128] = -S2
        G[t, 192:256, 128:] = -C2
    C0, S0 = cs(8 * j)
    C4, S4 = cs(4 + 8 * j)
    G[3, 0:64, 0:128] = C0
    G[3, 128:192, 0:128] = -S0
    G[3, 64:128, 128:] = C4
    G[3, 192:256, 128:] = -S4
    G[4] = G[3]
    G[4, 0, 0:128] = 0.5
    G[4, 128, 0:128] = 0.5 * (-1.0) ** dp
    HH = np.zeros((16, 256, 128))
    for a in range(16):
        ang = 2 * np.pi * (((a + 16 * dp)[:, None] * dp[None, :]) % 2048) / 2048
        HH[a, :128] = np.cos(ang)
        HH[a, 128:] = np.sin(ang)
    misc = np.zeros((3, 128, 128))
    misc[0, 128 - dp[1:], dp[1:]] = 1
    misc[1, 0, 0] = 1
    misc[2, 0, :] = (-1.0) ** dp
    for blk in range(4):
        for k1 in range(16):
            misc[2, 64 + 16 * blk + k1, 16 * blk + 15 - k1] = 1
            misc[2, 64 + 16 * blk + k1, 64 + 16 * blk + (16 - k1) % 16] = 1
    return G.astype(bf), HH.astype(bf), misc.astype(bf)


_TAB_G, _TAB_H, _TAB_MISC = _np_tables()


def _bc(x, dt):
    return lax.bitcast_convert_type(x, dt)


def _w2b(w):
    return pltpu.bitcast(w, bf16)


def _fft16(xs, inverse):
    sg = 1.0 if inverse else -1.0

    def dft4(a, b, c, d):
        t0 = (a[0] + c[0], a[1] + c[1])
        t1 = (a[0] - c[0], a[1] - c[1])
        t2 = (b[0] + d[0], b[1] + d[1])
        t3 = (b[0] - d[0], b[1] - d[1])
        o0 = (t0[0] + t2[0], t0[1] + t2[1])
        o2 = (t0[0] - t2[0], t0[1] - t2[1])
        m = (t1[0] + t3[1], t1[1] - t3[0])
        p = (t1[0] - t3[1], t1[1] + t3[0])
        return [o0, p, o2, m] if inverse else [o0, m, o2, p]

    t = [dft4(xs[a0], xs[4 + a0], xs[8 + a0], xs[12 + a0]) for a0 in range(4)]

    def tw(v, e):
        e = e % 16
        if e == 0:
            return v
        if e == 4:
            return (-v[1], v[0]) if inverse else (v[1], -v[0])
        if e == 2:
            if inverse:
                return ((v[0] - v[1]) * RS, (v[0] + v[1]) * RS)
            return ((v[0] + v[1]) * RS, (v[1] - v[0]) * RS)
        if e == 6:
            if inverse:
                return ((-v[0] - v[1]) * RS, (v[0] - v[1]) * RS)
            return ((v[1] - v[0]) * RS, (-v[0] - v[1]) * RS)
        c = float(np.cos(2 * np.pi * e / 16))
        s = float(sg * np.sin(2 * np.pi * e / 16))
        return (v[0] * c - v[1] * s, v[0] * s + v[1] * c)

    out = [None] * 16
    for k in range(4):
        u = [tw(t[a0][k], a0 * k) for a0 in range(4)]
        r = dft4(*u)
        for m in range(4):
            out[k + 4 * m] = r[m]
    return out


def _b_phase(xb_hbm, wr_hbm, wi_hbm, g_hbm, h_hbm, misc_hbm, bs, sems, start_m, start_i):
    def scoped(xs, wr, wi, wrn, win, G, HH, misc, Y, Zr, Zi, WS, PQ):
        xb32 = xb_hbm.bitcast(u32)
        xcp = [pltpu.make_async_copy(xb32.at[:, m, :], xs.at[m], sems.at[m]) for m in range(2)]
        cg = pltpu.make_async_copy(g_hbm, G, sems.at[8])
        ch = pltpu.make_async_copy(h_hbm, HH, sems.at[9])
        cm = pltpu.make_async_copy(misc_hbm, misc, sems.at[10])
        def wblk(k):
            off = 128 * k if isinstance(k, int) else pl.multiple_of(128 * k, 128)
            return (pltpu.make_async_copy(wr_hbm.at[pl.ds(0, 512), pl.ds(off, 128)], wr.at[k], sems.at[11]),
                    pltpu.make_async_copy(wi_hbm.at[pl.ds(0, 512), pl.ds(off, 128)], wi.at[k], sems.at[12]))

        wny = (pltpu.make_async_copy(wr_hbm.at[pl.ds(512, 1), :], wrn, sems.at[11]),
               pltpu.make_async_copy(wi_hbm.at[pl.ds(512, 1), :], win, sems.at[12]))
        cg.start()
        xcp[0].start()
        ch.start()
        cm.start()
        xcp[1].start()
        for c in wny:
            c.start()
        cg.wait()
        cm.wait()
        ch.wait()

        def getM(a):
            hc = HH[a, 0:128, :]
            hs = HH[a, 128:256, :]
            return jnp.concatenate(
                [jnp.concatenate([hc, -hs], axis=1), jnp.concatenate([hs, hc], axis=1)], axis=0)

        def phF(m, _):
            @pl.when(m < 6)
            def _():
                pltpu.make_async_copy(xb32.at[:, m + 2, :], xs.at[m + 2], sems.at[m + 2]).start()

            for k in (2 * m, 2 * m + 1):
                for c in wblk(k):
                    c.start()
            pltpu.make_async_copy(xb32.at[:, 0, :], xs.at[m], sems.at[m]).wait()
            for ch_ in range(8):
                w = xs[m, 16 * ch_:16 * ch_ + 16, :]
                for half, xv in enumerate((_bc(w << 16, f32), _bc(w & jnp.uint32(HI), f32))):
                    xc = [xv[:, 128 * c:128 * (c + 1)] for c in range(8)]
                    a0, a1 = xc[0] + xc[4], xc[0] - xc[4]
                    b0, b1 = xc[2] + xc[6], xc[2] - xc[6]
                    c0, c1 = xc[1] + xc[5], xc[1] - xc[5]
                    d0, d1 = xc[3] + xc[7], xc[3] - xc[7]
                    p, q = a0 + b0, c0 + d0
                    y0, y4 = p + q, p - q
                    y2r, y2i = a0 - b0, d0 - c0
                    cm_, cp_ = RS * (c1 - d1), RS * (c1 + d1)
                    y1r, y1i = a1 + cm_, -b1 - cp_
                    y3r, y3i = a1 - cm_, b1 - cp_
                    for t, (yr, yi) in enumerate([(y1r, y1i), (y2r, y2i), (y3r, y3i), (y0, y4)]):
                        Y[half, t, 16 * ch_:16 * ch_ + 16, :] = jnp.concatenate([yr, yi], axis=1).astype(bf16)
            for half in range(2):
                a = 2 * m + half
                Mx = getM(a)
                for t in range(4):
                    o = lax.dot_general(G[t], Y[half, t], NT, preferred_element_type=f32)
                    z = jnp.concatenate([o[:128], o[128:]], axis=1).astype(bf16)
                    X = jnp.dot(z, Mx, preferred_element_type=f32)
                    Zr[a, 128 * t:128 * t + 128, :] = X[:, 0:128]
                    Zi[a, 128 * t:128 * t + 128, :] = X[:, 128:256]
                ony = lax.dot_general(misc[2, 0:16, :], Y[half, 3, :, 0:128], NT, preferred_element_type=f32)
                Xn = jnp.dot(ony.astype(bf16), Mx[0:128, :], preferred_element_type=f32)
                Zr[a, 512:528, :] = Xn[:, 0:128]
                Zi[a, 512:528, :] = Xn[:, 128:256]
            return 0

        lax.fori_loop(0, 8, phF, 0)

        for k in range(16):
            for c in wblk(k):
                c.wait()
        for c in wny:
            c.wait()
        wr32 = wr.bitcast(u32)
        wi32 = wi.bitcast(u32)
        hi = jnp.uint32(HI)
        dcr = jnp.concatenate([_bc(wr32[k, 0:1, :] << 16, f32) for k in range(16)], axis=0)
        dci = jnp.concatenate([_bc(wi32[k, 0:1, :] << 16, f32) for k in range(16)], axis=0)
        nyr = jnp.concatenate([wrn[:, 128 * k:128 * (k + 1)].astype(f32) for k in range(16)], axis=0)
        nyi = jnp.concatenate([win[:, 128 * k:128 * (k + 1)].astype(f32) for k in range(16)], axis=0)
        st = jnp.concatenate([dcr, dci, nyr, nyi], axis=0)
        stb = st.astype(bf16)
        r1 = jnp.dot(stb, misc[0], preferred_element_type=f32)
        r2 = jnp.dot(stb, misc[1], preferred_element_type=f32)
        rr = jnp.concatenate([r1, r2], axis=0).astype(bf16)
        rp = jnp.dot(misc[2, 64:128, :], rr, preferred_element_type=f32)
        rid = lax.broadcasted_iota(jnp.int32, (64, 128), 0)
        sgn = jnp.where((rid & 16) == 0, 0.5, -0.5)
        WS[...] = 0.5 * st + sgn * rp

        POS = {1: 0, 7: 64, 2: 128, 6: 192, 3: 256, 5: 320, 0: 384, 4: 448}
        row8 = lax.broadcasted_iota(jnp.int32, (8, 128), 0)

        def mid(r, g, special):
            r0 = POS[r] + 8 * g
            if not special:
                r0 = pl.multiple_of(r0, 8)
            xs_ = [(Zr[a, pl.ds(r0, 8), :], Zi[a, pl.ds(r0, 8), :]) for a in range(16)]
            o = _fft16(xs_, False)
            if special:
                xn = [(Zr[a, 512:520, :], Zi[a, 512:520, :]) for a in range(16)]
                on = _fft16(xn, False)
                wsr, wsi = wr32, wi32
            else:
                g32 = pl.multiple_of(32 * g, 32)
                wsr = wr32.at[:, pl.ds(g32, 32), :]
                wsi = wi32.at[:, pl.ds(g32, 32), :]
            ys = []
            for k in range(16):
                a_ = wsr[k, pl.ds(r // 2, 8, stride=4), :]
                b_ = wsi[k, pl.ds(r // 2, 8, stride=4), :]
                if r % 2 == 0:
                    wre, wim = _bc(a_ << 16, f32), _bc(b_ << 16, f32)
                else:
                    wre, wim = _bc(a_ & hi, f32), _bc(b_ & hi, f32)
                if special:
                    wre = jnp.where(row8 == 0, jnp.broadcast_to(WS[k:k + 1, :], (8, 128)), wre)
                    wim = jnp.where(row8 == 0, jnp.broadcast_to(WS[16 + k:17 + k, :], (8, 128)), wim)
                xr, xi = o[k]
                yr = xr * wre - xi * wim
                yi = xr * wim + xi * wre
                if special:
                    nr = jnp.broadcast_to(WS[32 + k:33 + k, :], (8, 128))
                    ni = jnp.broadcast_to(WS[48 + k:49 + k, :], (8, 128))
                    zr_, zi_ = on[k]
                    yr = yr - (zr_ * ni + zi_ * nr)
                    yi = yi + (zr_ * nr - zi_ * ni)
                ys.append((yr, yi))
            u = _fft16(ys, True)
            for a in range(16):
                Zr[a, pl.ds(r0, 8), :] = u[a][0]
                Zi[a, pl.ds(r0, 8), :] = u[a][1]

        mid(0, 0, True)

        def phM(g, _):
            start_m(g)
            for r in range(1, 8):
                mid(r, g, False)

            @pl.when(g > 0)
            def _():
                mid(0, g, False)

            return 0

        lax.fori_loop(0, 8, phM, 0)

        def phI(m, _):
            start_i(m)
            for half in range(2):
                a = 2 * m + half
                Mx = getM(a)
                for t in range(4):
                    yy = jnp.concatenate(
                        [Zr[a, 128 * t:128 * t + 128, :], Zi[a, 128 * t:128 * t + 128, :]], axis=1).astype(bf16)
                    o = lax.dot_general(Mx, yy, NT, preferred_element_type=f32)
                    vv = jnp.concatenate([o[:128], o[128:]], axis=1).astype(bf16)
                    PQ[half, t] = jnp.dot(vv, G[t if t < 3 else 4], preferred_element_type=f32)
            for ch_ in range(8):
                rs = slice(16 * ch_, 16 * ch_ + 16)
                res = []
                for half in range(2):
                    P1, Q1 = PQ[half, 0, rs, 0:128], PQ[half, 0, rs, 128:256]
                    P2, Q2 = PQ[half, 1, rs, 0:128], PQ[half, 1, rs, 128:256]
                    P3, Q3 = PQ[half, 2, rs, 0:128], PQ[half, 2, rs, 128:256]
                    h0, h4 = PQ[half, 3, rs, 0:128], PQ[half, 3, rs, 128:256]
                    e, o_ = h0 + h4, h0 - h4
                    A, B = P1 + P3, Q1 - Q3
                    u, v = P1 - P3, Q1 + Q3
                    T1_, T2_ = RS * (u - v), RS * (-u - v)
                    e1, e2 = e + P2, e - P2
                    o1, o2 = o_ - Q2, o_ + Q2
                    cols = jnp.concatenate(
                        [e1 + A, o1 + T1_, e2 - B, o2 + T2_, e1 - A, o1 - T1_, e2 + B, o2 - T2_], axis=1)
                    res.append(_bc(cols.astype(bf16).astype(f32), u32))
                bs[m, rs, :] = (res[0] >> 16) | res[1]
            return 0

        lax.fori_loop(0, 8, phI, 0)

    pl.run_scoped(
        scoped,
        pltpu.VMEM((8, 128, D), u32), pltpu.VMEM((16, 512, 128), bf16), pltpu.VMEM((16, 512, 128), bf16),
        pltpu.VMEM((1, S), bf16), pltpu.VMEM((1, S), bf16),
        pltpu.VMEM((5, 256, 256), bf16), pltpu.VMEM((16, 256, 128), bf16), pltpu.VMEM((3, 128, 128), bf16),
        pltpu.VMEM((2, 4, 128, 256), bf16), pltpu.VMEM((16, 528, 128), f32), pltpu.VMEM((16, 528, 128), f32),
        pltpu.VMEM((64, 128), f32), pltpu.VMEM((2, 4, 128, 256), f32))


def _kernel(x_hbm, mem0_hbm, wq_hbm, wk_hbm, wv_hbm, wo_hbm, xb_hbm, wr_hbm, wi_hbm, gw_hbm,
            g_hbm, h_hbm, misc_hbm, out_hbm,
            xv, xpre, mem0v, gwv, raw, wo, bs, bnat, gbuf, outb, bsems, wsems, msems, osem):
    cp_x = pltpu.make_async_copy(x_hbm.bitcast(u32), xv, msems.at[0])
    cp_mem = pltpu.make_async_copy(mem0_hbm, mem0v, msems.at[2])
    cp_gw = pltpu.make_async_copy(gw_hbm, gwv, msems.at[3])
    wsrc = [w.bitcast(u32) for w in (wq_hbm, wk_hbm, wv_hbm)]
    wo32 = wo_hbm.bitcast(u32)

    def cp_w(p):
        return [pltpu.make_async_copy(wsrc[i].at[:, p, :], raw.at[p, i], wsems.at[p]) for i in range(3)]

    def cp_wo(j):
        off = 128 * j if isinstance(j, int) else pl.multiple_of(128 * j, 128)
        return pltpu.make_async_copy(wo32.at[:, :, pl.ds(off, 128)], wo.at[j], msems.at[4])

    def start_m(g):
        @pl.when(g == 0)
        def _():
            cp_gw.start()
            cp_mem.start()
            cp_x.start()

        for c in cp_w(g):
            c.start()

    def start_i(m):
        for c in cp_w(m + 8):
            c.start()

    _b_phase(xb_hbm, wr_hbm, wi_hbm, g_hbm, h_hbm, misc_hbm, bs, bsems, start_m, start_i)
    bn32 = bnat.bitcast(u32)

    def a_phase(w3, pre, oc, ocr, acc, lhs):
        cp_x.wait()
        cp_gw.wait()
        gwf = gwv[...].astype(f32)
        for i in range(32):
            xpre[8 * i:8 * i + 8, :] = jnp.concatenate(
                [xv[32 * i + 12:32 * i + 16, :], xv[32 * i + 28:32 * i + 32, :]], axis=0)

        def prebulk(p, _):
            @pl.when(p < 8)
            def _():
                cp_wo(p).start()

            for i in range(3):
                pltpu.make_async_copy(wsrc[i].at[:, 0, :], raw.at[p, i], wsems.at[p]).wait()
            for i in range(3):
                e = raw[p, i, pl.ds(0, 512, stride=2), :]
                o = raw[p, i, pl.ds(1, 512, stride=2), :]
                w3[p, 0, i] = (e & jnp.uint32(0xFFFF)) | (o << 16)
                w3[p, 1, i] = (e >> 16) | (o & jnp.uint32(HI))
            for r in range(2):
                for i in range(3):
                    for c in range(2):
                        xl = _w2b(xpre[128 * c:128 * c + 128, :])
                        pre[p, r, i, 256 * c:256 * c + 256, :] = jnp.dot(
                            xl, _w2b(w3[p, r, i]), preferred_element_type=f32)
            for c in range(8):
                xw = xv[pl.ds(pl.multiple_of(64 * p + 8 * c, 8), 8), :]
                xx = _w2b(xw).astype(f32) * gwf
                part = xx[:, 0:128]
                for jj in range(1, 8):
                    part = part + xx[:, 128 * jj:128 * jj + 128]
                lg = jnp.sum(part, axis=1, keepdims=True)
                gbuf[pl.ds(pl.multiple_of(128 * p + 16 * c, 16), 16), :] = jnp.broadcast_to(
                    jax.nn.sigmoid(lg), (16, 128))
            for jj in range(8):
                dst = bn32.at[jj, pl.ds(pl.multiple_of(64 * p, 64), 64), :]
                for m in range(8):
                    dst[pl.ds(m, 8, stride=8), :] = bs[m, pl.ds(pl.multiple_of(8 * p, 8), 8), 128 * jj:128 * jj + 128]
            return 0

        lax.fori_loop(0, 16, prebulk, 0)
        cp_mem.wait()
        for j in range(8):
            cp_wo(j).wait()
        oc[...] = jnp.zeros(oc.shape, bf16)
        oc32 = oc.bitcast(u32)

        row = lax.broadcasted_iota(jnp.int32, (48, 128), 0)
        col = lax.broadcasted_iota(jnp.int32, (48, 128), 1)
        mask = ((col < 40) & (row >= 32)) | ((row < 32) & ((col <= row) | ((col >= 32) & (col < 40))))
        scale = DH ** -0.5
        bscale = 2.0 ** -20

        def wo_t(j, h):
            return _w2b(wo[j, h])

        def mix(a, b, g):
            return g * a + (1.0 - g) * (b.astype(f32) * bscale)

        def fill_piece(gr, gw_, src, j, half, accs):
            hs = range(16 * half, 16 * half + 16)
            l = jnp.concatenate([_w2b(src[h]) for h in hs], axis=1)
            w = _w2b(wo[j, 16 * half:16 * half + 16].reshape(16 * 64, 128))
            c = jnp.dot(l, w, preferred_element_type=f32)
            if half == 0:
                return c
            c = c + accs
            for q in range(4):
                sg = 4 * gr + q
                b = bnat[j, pl.ds(pl.multiple_of(32 * sg + 24, 8), 8), :]
                g = gbuf[pl.ds(pl.multiple_of(32 * sg + 24, 8), 8), :]
                outb[pl.ds(pl.multiple_of(128 * gw_ + 32 * q + 24, 8), 8),
                     pl.ds(pl.multiple_of(128 * j, 128), 128)] = mix(c[8 * q:8 * q + 8], b, g).astype(bf16)
            return None

        def out_copy(gi):
            return pltpu.make_async_copy(
                outb.at[pl.ds(pl.multiple_of(128 * gi, 128), 128), :],
                out_hbm.at[pl.ds(pl.multiple_of(128 * gi, 128), 128), :], osem)

        def step(s, mem):
            @pl.when((s % 4 == 0) & (s >= 8))
            def _():
                out_copy(s // 4 - 2).start()

            @pl.when(s % 4 == 0)
            def _():
                ocr[...] = oc32[...]

            r0 = pl.multiple_of(s * 16, 16)
            xs0 = _w2b(xv[pl.ds(r0, 8), :])
            xs1 = _w2b(xv[pl.ds(r0 + 8, 8), :])
            l1 = jnp.concatenate([xs1[0:8].astype(f32), mem], axis=0).astype(bf16)
            lhs[0:8, :] = pltpu.bitcast(xs0, u32)
            lhs[8:16, :] = pltpu.bitcast(l1, u32)
            grp = s // 4 - 1
            gr = jnp.maximum(grp, 0)
            gw_ = jnp.where(grp < 0, 16, grp)
            q4 = s % 4
            st = {}
            z8 = jnp.zeros((8, 128), f32)
            s8 = pl.multiple_of(s * 8, 8)

            def proj(h, i):
                r = jnp.dot(_w2b(lhs[...]), _w2b(w3[h // 2, h % 2, i]), preferred_element_type=f32)
                p_ = pre[h // 2, h % 2, i, pl.ds(s8, 8), :]
                st[("qkv", h, i)] = jnp.concatenate([r[0:24], p_, r[24:32], z8], axis=0).astype(bf16)

            def qk(h):
                q = st.pop(("qkv", h, 0))
                k = st.pop(("qkv", h, 1))
                sc = lax.dot_general(q, k, NT, preferred_element_type=f32) * scale
                sc = jnp.concatenate([sc, jnp.zeros((48, 80), f32)], axis=1)
                sc = jnp.where(mask, sc, -1e9)
                m = jnp.max(sc, axis=1, keepdims=True)
                e = jnp.exp(sc - m)
                p = e * (1.0 / jnp.sum(e, axis=1, keepdims=True))
                st[("p", h)] = p[:, :48].astype(bf16)

            def pv(h):
                o = jnp.dot(st.pop(("p", h)), st.pop(("qkv", h, 2)), preferred_element_type=f32)
                st[("o", h)] = jnp.concatenate([o[0:24], o[32:40]], axis=0).astype(bf16)
                oc[h, pl.ds(pl.multiple_of(8 * q4, 8), 8), :] = o[24:32].astype(bf16)

            def oproj(h):
                w = jnp.concatenate([wo_t(j, h) for j in range(8)], axis=1)
                c = jnp.dot(st.pop(("o", h)), w, preferred_element_type=f32)
                if h == 0:
                    acc[...] = c
                else:
                    acc[...] += c

            ok = lambda h: 0 <= h < H
            for t in range(H + 4):
                if ok(t):
                    proj(t, 0)
                    proj(t, 1)
                if ok(t - 1):
                    qk(t - 1)
                if ok(t):
                    proj(t, 2)
                else:
                    jj, half = (t - H) // 2, (t - H) % 2
                    st["fill"] = fill_piece(gr, gw_, ocr, 2 * q4 + jj, half, st.get("fill"))
                if ok(t - 3):
                    pv(t - 3)
                if ok(t - 4):
                    oproj(t - 4)
            a = acc[...]
            rs = pl.multiple_of(32 * s, 32)
            b0 = jnp.concatenate([bnat[j, pl.ds(rs, 16), :] for j in range(8)], axis=1)
            b1 = jnp.concatenate([bnat[j, pl.ds(rs + 16, 8), :] for j in range(8)], axis=1)
            g0 = gbuf[pl.ds(rs, 16), :]
            g1 = gbuf[pl.ds(rs + 16, 8), :]
            outb[pl.ds(rs, 16), :] = mix(a[0:16], b0, jnp.tile(g0, (1, 8))).astype(bf16)
            outb[pl.ds(rs + 16, 8), :] = mix(a[16:24], b1, jnp.tile(g1, (1, 8))).astype(bf16)
            return a[24:32]

        lax.fori_loop(0, NSEG, step, mem0v[...].astype(f32))

        for j in range(8):
            c = fill_piece(15, 15, oc32, j, 0, None)
            fill_piece(15, 15, oc32, j, 1, c)
        out_copy(14).start()
        out_copy(15).start()
        for gi in range(16):
            out_copy(gi).wait()

    pl.run_scoped(
        a_phase,
        pltpu.VMEM((16, 2, 3, 512, 128), u32), pltpu.VMEM((16, 2, 3, 512, 128), f32),
        pltpu.VMEM((H, 32, 128), bf16), pltpu.VMEM((H, 16, 128), u32), pltpu.VMEM((32, D), f32), pltpu.VMEM((16, D), u32))


@jax.jit
def pallas_gated_mix__memory_aug_recurrent_mem_tr__spectral_gfnet__prompt_kernel(
    A_x, A_mem0, A_Wq, A_Wk, A_Wv, A_Wo, A_seg_len, B_x, B_w_r, B_w_i, gate_w,
):
    del A_seg_len
    del B_x
    HB = pl.BlockSpec(memory_space=pltpu.HBM)
    out = pl.pallas_call(
        _kernel,
        out_shape=jax.ShapeDtypeStruct((S, D), bf16),
        in_specs=[HB] * 13,
        out_specs=HB,
        scratch_shapes=[
            pltpu.VMEM((S // 2, D), u32),
            pltpu.VMEM((NSEG * 4, D), u32),
            pltpu.VMEM((M_MEM, D), bf16),
            pltpu.VMEM((1, D), bf16),
            pltpu.VMEM((16, 3, D, DH), u32),
            pltpu.VMEM((8, H, DH // 2, 128), u32),
            pltpu.VMEM((8, 128, D), u32),
            pltpu.VMEM((8, S, 128), bf16),
            pltpu.VMEM((S, 128), f32),
            pltpu.VMEM((S + 128, D), bf16),
            pltpu.SemaphoreType.DMA((13,)),
            pltpu.SemaphoreType.DMA((16,)),
            pltpu.SemaphoreType.DMA((6,)),
            pltpu.SemaphoreType.DMA(()),
        ],
        compiler_params=pltpu.CompilerParams(vmem_limit_bytes=124 * 2 ** 20),
    )(
        A_x.reshape(S, D), A_mem0.reshape(M_MEM, D), A_Wq, A_Wk, A_Wv, A_Wo,
        A_x.reshape(128, 16, D), B_w_r.T, B_w_i.T, gate_w.reshape(1, D), _TAB_G, _TAB_H, _TAB_MISC,
    )
    return out.reshape(1, S, D)
```

```python
import numpy as np
import ml_dtypes
import jax
import jax.numpy as jnp
from jax import lax
import jax.experimental.pallas as pl
import jax.experimental.pallas.tpu as pltpu

f32, bf16, u32 = jnp.float32, jnp.bfloat16, jnp.uint32
S, D, H, DH, M_MEM, SEG = 2048, 1024, 32, 128, 8, 32
NSEG = S // SEG
RS = float(1 / np.sqrt(2))
NT = (((1,), (1,)), ((), ()))
NN = (((1,), (0,)), ((), ()))
HI = 0xFFFF0000


def _np_tables():
    bf = ml_dtypes.bfloat16
    dp = np.arange(128)
    j = np.arange(64)

    def cs(f):
        ang = 2 * np.pi * ((f[:, None] * dp[None, :]) % 1024) / 1024
        return np.cos(ang), np.sin(ang)

    G = np.zeros((5, 256, 256))
    for t in range(3):
        r = t + 1
        C, Sn = cs(r + 8 * j)
        C2, S2 = cs(8 - r + 8 * j)
        G[t, 0:64, 0:128] = C
        G[t, 0:64, 128:] = Sn
        G[t, 64:128, 0:128] = C2
        G[t, 64:128, 128:] = -S2
        G[t, 128:192, 0:128] = -Sn
        G[t, 128:192, 128:] = C
        G[t, 192:256, 0:128] = -S2
        G[t, 192:256, 128:] = -C2
    C0, S0 = cs(8 * j)
    C4, S4 = cs(4 + 8 * j)
    G[3, 0:64, 0:128] = C0
    G[3, 128:192, 0:128] = -S0
    G[3, 64:128, 128:] = C4
    G[3, 192:256, 128:] = -S4
    G[4] = G[3]
    G[4, 0, 0:128] = 0.5
    G[4, 128, 0:128] = 0.5 * (-1.0) ** dp
    HH = np.zeros((16, 256, 128))
    for a in range(16):
        ang = 2 * np.pi * (((a + 16 * dp)[:, None] * dp[None, :]) % 2048) / 2048
        HH[a, :128] = np.cos(ang)
        HH[a, 128:] = np.sin(ang)
    misc = np.zeros((3, 128, 128))
    misc[0, 128 - dp[1:], dp[1:]] = 1
    misc[1, 0, 0] = 1
    misc[2, 0, :] = (-1.0) ** dp
    for blk in range(4):
        for k1 in range(16):
            misc[2, 64 + 16 * blk + k1, 16 * blk + 15 - k1] = 1
            misc[2, 64 + 16 * blk + k1, 64 + 16 * blk + (16 - k1) % 16] = 1
    return G.astype(bf), HH.astype(bf), misc.astype(bf)


_TAB_G, _TAB_H, _TAB_MISC = _np_tables()


def _bc(x, dt):
    return lax.bitcast_convert_type(x, dt)


def _w2b(w):
    return pltpu.bitcast(w, bf16)


def _fft16(xs, inverse):
    sg = 1.0 if inverse else -1.0

    def dft4(a, b, c, d):
        t0 = (a[0] + c[0], a[1] + c[1])
        t1 = (a[0] - c[0], a[1] - c[1])
        t2 = (b[0] + d[0], b[1] + d[1])
        t3 = (b[0] - d[0], b[1] - d[1])
        o0 = (t0[0] + t2[0], t0[1] + t2[1])
        o2 = (t0[0] - t2[0], t0[1] - t2[1])
        m = (t1[0] + t3[1], t1[1] - t3[0])
        p = (t1[0] - t3[1], t1[1] + t3[0])
        return [o0, p, o2, m] if inverse else [o0, m, o2, p]

    t = [dft4(xs[a0], xs[4 + a0], xs[8 + a0], xs[12 + a0]) for a0 in range(4)]

    def tw(v, e):
        e = e % 16
        if e == 0:
            return v
        if e == 4:
            return (-v[1], v[0]) if inverse else (v[1], -v[0])
        if e == 2:
            if inverse:
                return ((v[0] - v[1]) * RS, (v[0] + v[1]) * RS)
            return ((v[0] + v[1]) * RS, (v[1] - v[0]) * RS)
        if e == 6:
            if inverse:
                return ((-v[0] - v[1]) * RS, (v[0] - v[1]) * RS)
            return ((v[1] - v[0]) * RS, (-v[0] - v[1]) * RS)
        c = float(np.cos(2 * np.pi * e / 16))
        s = float(sg * np.sin(2 * np.pi * e / 16))
        return (v[0] * c - v[1] * s, v[0] * s + v[1] * c)

    out = [None] * 16
    for k in range(4):
        u = [tw(t[a0][k], a0 * k) for a0 in range(4)]
        r = dft4(*u)
        for m in range(4):
            out[k + 4 * m] = r[m]
    return out


def _b_phase(xb_hbm, wr_hbm, wi_hbm, g_hbm, h_hbm, misc_hbm, bs, sems, start_m, start_i):
    def scoped(xs, wr, wi, wrn, win, G, HH, misc, Y, Zr, Zi, WS, PQ):
        xb32 = xb_hbm.bitcast(u32)
        xcp = [pltpu.make_async_copy(xb32.at[:, m, :], xs.at[m], sems.at[m]) for m in range(2)]
        cg = pltpu.make_async_copy(g_hbm, G, sems.at[8])
        ch = pltpu.make_async_copy(h_hbm, HH, sems.at[9])
        cm = pltpu.make_async_copy(misc_hbm, misc, sems.at[10])
        def wblk(k):
            off = 128 * k if isinstance(k, int) else pl.multiple_of(128 * k, 128)
            return (pltpu.make_async_copy(wr_hbm.at[pl.ds(0, 512), pl.ds(off, 128)], wr.at[k], sems.at[11]),
                    pltpu.make_async_copy(wi_hbm.at[pl.ds(0, 512), pl.ds(off, 128)], wi.at[k], sems.at[12]))

        wny = (pltpu.make_async_copy(wr_hbm.at[pl.ds(512, 1), :], wrn, sems.at[11]),
               pltpu.make_async_copy(wi_hbm.at[pl.ds(512, 1), :], win, sems.at[12]))
        cg.start()
        xcp[0].start()
        ch.start()
        cm.start()
        xcp[1].start()
        for c in wny:
            c.start()
        cg.wait()
        cm.wait()
        ch.wait()

        def getM(a):
            hc = HH[a, 0:128, :]
            hs = HH[a, 128:256, :]
            return jnp.concatenate(
                [jnp.concatenate([hc, -hs], axis=1), jnp.concatenate([hs, hc], axis=1)], axis=0)

        def phF(m, _):
            @pl.when(m < 6)
            def _():
                pltpu.make_async_copy(xb32.at[:, m + 2, :], xs.at[m + 2], sems.at[m + 2]).start()

            for k in (2 * m, 2 * m + 1):
                for c in wblk(k):
                    c.start()
            pltpu.make_async_copy(xb32.at[:, 0, :], xs.at[m], sems.at[m]).wait()
            for ch_ in range(8):
                w = xs[m, 16 * ch_:16 * ch_ + 16, :]
                for half, xv in enumerate((_bc(w << 16, f32), _bc(w & jnp.uint32(HI), f32))):
                    xc = [xv[:, 128 * c:128 * (c + 1)] for c in range(8)]
                    a0, a1 = xc[0] + xc[4], xc[0] - xc[4]
                    b0, b1 = xc[2] + xc[6], xc[2] - xc[6]
                    c0, c1 = xc[1] + xc[5], xc[1] - xc[5]
                    d0, d1 = xc[3] + xc[7], xc[3] - xc[7]
                    p, q = a0 + b0, c0 + d0
                    y0, y4 = p + q, p - q
                    y2r, y2i = a0 - b0, d0 - c0
                    cm_, cp_ = RS * (c1 - d1), RS * (c1 + d1)
                    y1r, y1i = a1 + cm_, -b1 - cp_
                    y3r, y3i = a1 - cm_, b1 - cp_
                    for t, (yr, yi) in enumerate([(y1r, y1i), (y2r, y2i), (y3r, y3i), (y0, y4)]):
                        Y[half, t, 16 * ch_:16 * ch_ + 16, :] = jnp.concatenate([yr, yi], axis=1).astype(bf16)
            for half in range(2):
                a = 2 * m + half
                Mx = getM(a)
                for t in range(4):
                    o = lax.dot_general(G[t], Y[half, t], NT, preferred_element_type=f32)
                    z = jnp.concatenate([o[:128], o[128:]], axis=1).astype(bf16)
                    X = jnp.dot(z, Mx, preferred_element_type=f32)
                    Zr[a, 128 * t:128 * t + 128, :] = X[:, 0:128]
                    Zi[a, 128 * t:128 * t + 128, :] = X[:, 128:256]
                ony = lax.dot_general(misc[2, 0:16, :], Y[half, 3, :, 0:128], NT, preferred_element_type=f32)
                Xn = jnp.dot(ony.astype(bf16), Mx[0:128, :], preferred_element_type=f32)
                Zr[a, 512:528, :] = Xn[:, 0:128]
                Zi[a, 512:528, :] = Xn[:, 128:256]
            return 0

        lax.fori_loop(0, 8, phF, 0)

        for k in range(16):
            for c in wblk(k):
                c.wait()
        for c in wny:
            c.wait()
        wr32 = wr.bitcast(u32)
        wi32 = wi.bitcast(u32)
        hi = jnp.uint32(HI)
        dcr = jnp.concatenate([_bc(wr32[k, 0:1, :] << 16, f32) for k in range(16)], axis=0)
        dci = jnp.concatenate([_bc(wi32[k, 0:1, :] << 16, f32) for k in range(16)], axis=0)
        nyr = jnp.concatenate([wrn[:, 128 * k:128 * (k + 1)].astype(f32) for k in range(16)], axis=0)
        nyi = jnp.concatenate([win[:, 128 * k:128 * (k + 1)].astype(f32) for k in range(16)], axis=0)
        st = jnp.concatenate([dcr, dci, nyr, nyi], axis=0)
        stb = st.astype(bf16)
        r1 = jnp.dot(stb, misc[0], preferred_element_type=f32)
        r2 = jnp.dot(stb, misc[1], preferred_element_type=f32)
        rr = jnp.concatenate([r1, r2], axis=0).astype(bf16)
        rp = jnp.dot(misc[2, 64:128, :], rr, preferred_element_type=f32)
        rid = lax.broadcasted_iota(jnp.int32, (64, 128), 0)
        sgn = jnp.where((rid & 16) == 0, 0.5, -0.5)
        WS[...] = 0.5 * st + sgn * rp

        POS = {1: 0, 7: 64, 2: 128, 6: 192, 3: 256, 5: 320, 0: 384, 4: 448}
        row8 = lax.broadcasted_iota(jnp.int32, (8, 128), 0)

        def mid(r, g, special):
            r0 = POS[r] + 8 * g
            if not special:
                r0 = pl.multiple_of(r0, 8)
            xs_ = [(Zr[a, pl.ds(r0, 8), :], Zi[a, pl.ds(r0, 8), :]) for a in range(16)]
            o = _fft16(xs_, False)
            if special:
                xn = [(Zr[a, 512:520, :], Zi[a, 512:520, :]) for a in range(16)]
                on = _fft16(xn, False)
                wsr, wsi = wr32, wi32
            else:
                g32 = pl.multiple_of(32 * g, 32)
                wsr = wr32.at[:, pl.ds(g32, 32), :]
                wsi = wi32.at[:, pl.ds(g32, 32), :]
            ys = []
            for k in range(16):
                a_ = wsr[k, pl.ds(r // 2, 8, stride=4), :]
                b_ = wsi[k, pl.ds(r // 2, 8, stride=4), :]
                if r % 2 == 0:
                    wre, wim = _bc(a_ << 16, f32), _bc(b_ << 16, f32)
                else:
                    wre, wim = _bc(a_ & hi, f32), _bc(b_ & hi, f32)
                if special:
                    wre = jnp.where(row8 == 0, jnp.broadcast_to(WS[k:k + 1, :], (8, 128)), wre)
                    wim = jnp.where(row8 == 0, jnp.broadcast_to(WS[16 + k:17 + k, :], (8, 128)), wim)
                xr, xi = o[k]
                yr = xr * wre - xi * wim
                yi = xr * wim + xi * wre
                if special:
                    nr = jnp.broadcast_to(WS[32 + k:33 + k, :], (8, 128))
                    ni = jnp.broadcast_to(WS[48 + k:49 + k, :], (8, 128))
                    zr_, zi_ = on[k]
                    yr = yr - (zr_ * ni + zi_ * nr)
                    yi = yi + (zr_ * nr - zi_ * ni)
                ys.append((yr, yi))
            u = _fft16(ys, True)
            for a in range(16):
                Zr[a, pl.ds(r0, 8), :] = u[a][0]
                Zi[a, pl.ds(r0, 8), :] = u[a][1]

        mid(0, 0, True)

        def phM(g, _):
            start_m(g)
            for r in range(1, 8):
                mid(r, g, False)

            @pl.when(g > 0)
            def _():
                mid(0, g, False)

            return 0

        lax.fori_loop(0, 8, phM, 0)

        def phI(m, _):
            start_i(m)
            for half in range(2):
                a = 2 * m + half
                Mx = getM(a)
                for t in range(4):
                    yy = jnp.concatenate(
                        [Zr[a, 128 * t:128 * t + 128, :], Zi[a, 128 * t:128 * t + 128, :]], axis=1).astype(bf16)
                    o = lax.dot_general(Mx, yy, NT, preferred_element_type=f32)
                    vv = jnp.concatenate([o[:128], o[128:]], axis=1).astype(bf16)
                    PQ[half, t] = jnp.dot(vv, G[t if t < 3 else 4], preferred_element_type=f32)
            for ch_ in range(8):
                rs = slice(16 * ch_, 16 * ch_ + 16)
                res = []
                for half in range(2):
                    P1, Q1 = PQ[half, 0, rs, 0:128], PQ[half, 0, rs, 128:256]
                    P2, Q2 = PQ[half, 1, rs, 0:128], PQ[half, 1, rs, 128:256]
                    P3, Q3 = PQ[half, 2, rs, 0:128], PQ[half, 2, rs, 128:256]
                    h0, h4 = PQ[half, 3, rs, 0:128], PQ[half, 3, rs, 128:256]
                    e, o_ = h0 + h4, h0 - h4
                    A, B = P1 + P3, Q1 - Q3
                    u, v = P1 - P3, Q1 + Q3
                    T1_, T2_ = RS * (u - v), RS * (-u - v)
                    e1, e2 = e + P2, e - P2
                    o1, o2 = o_ - Q2, o_ + Q2
                    cols = jnp.concatenate(
                        [e1 + A, o1 + T1_, e2 - B, o2 + T2_, e1 - A, o1 - T1_, e2 + B, o2 - T2_], axis=1)
                    res.append(_bc(cols.astype(bf16).astype(f32), u32))
                bs[m, rs, :] = (res[0] >> 16) | res[1]
            return 0

        lax.fori_loop(0, 8, phI, 0)

    pl.run_scoped(
        scoped,
        pltpu.VMEM((8, 128, D), u32), pltpu.VMEM((16, 512, 128), bf16), pltpu.VMEM((16, 512, 128), bf16),
        pltpu.VMEM((1, S), bf16), pltpu.VMEM((1, S), bf16),
        pltpu.VMEM((5, 256, 256), bf16), pltpu.VMEM((16, 256, 128), bf16), pltpu.VMEM((3, 128, 128), bf16),
        pltpu.VMEM((2, 4, 128, 256), bf16), pltpu.VMEM((16, 528, 128), f32), pltpu.VMEM((16, 528, 128), f32),
        pltpu.VMEM((64, 128), f32), pltpu.VMEM((2, 4, 128, 256), f32))


def _kernel(x_hbm, mem0_hbm, wq_hbm, wk_hbm, wv_hbm, wo_hbm, xb_hbm, wr_hbm, wi_hbm, gw_hbm,
            g_hbm, h_hbm, misc_hbm, out_hbm,
            xv, xpre, mem0v, gwv, raw, wo, bs, bnat, gbuf, outb, bsems, wsems, msems, osem):
    cp_x = pltpu.make_async_copy(x_hbm.bitcast(u32), xv, msems.at[0])
    cp_mem = pltpu.make_async_copy(mem0_hbm, mem0v, msems.at[2])
    cp_gw = pltpu.make_async_copy(gw_hbm, gwv, msems.at[3])
    wsrc = [w.bitcast(u32) for w in (wq_hbm, wk_hbm, wv_hbm)]
    wo32 = wo_hbm.bitcast(u32)

    def cp_w(p):
        return [pltpu.make_async_copy(wsrc[i].at[:, p, :], raw.at[p, i], wsems.at[p]) for i in range(3)]

    def cp_wo(j):
        off = 128 * j if isinstance(j, int) else pl.multiple_of(128 * j, 128)
        return pltpu.make_async_copy(wo32.at[:, :, pl.ds(off, 128)], wo.at[j], msems.at[4])

    def start_m(g):
        @pl.when(g == 0)
        def _():
            cp_gw.start()
            cp_mem.start()
            cp_x.start()

        for c in cp_w(g):
            c.start()

    def start_i(m):
        for c in cp_w(m + 8):
            c.start()

    _b_phase(xb_hbm, wr_hbm, wi_hbm, g_hbm, h_hbm, misc_hbm, bs, bsems, start_m, start_i)
    bn32 = bnat.bitcast(u32)

    def a_phase(w3, pre, oc, ocr, acc, lhs):
        cp_x.wait()
        cp_gw.wait()
        gwf = gwv[...].astype(f32)
        for i in range(32):
            xpre[8 * i:8 * i + 8, :] = jnp.concatenate(
                [xv[32 * i + 12:32 * i + 16, :], xv[32 * i + 28:32 * i + 32, :]], axis=0)

        def prebulk(p, _):
            @pl.when(p < 8)
            def _():
                cp_wo(p).start()

            for i in range(3):
                pltpu.make_async_copy(wsrc[i].at[:, 0, :], raw.at[p, i], wsems.at[p]).wait()
            for i in range(3):
                e = raw[p, i, pl.ds(0, 512, stride=2), :]
                o = raw[p, i, pl.ds(1, 512, stride=2), :]
                w3[p, 0, i] = (e & jnp.uint32(0xFFFF)) | (o << 16)
                w3[p, 1, i] = (e >> 16) | (o & jnp.uint32(HI))
            for r in range(2):
                for i in range(3):
                    for c in range(2):
                        xl = _w2b(xpre[128 * c:128 * c + 128, :])
                        pre[p, r, i, 256 * c:256 * c + 256, :] = jnp.dot(
                            xl, _w2b(w3[p, r, i]), preferred_element_type=f32)
            for c in range(8):
                xw = xv[pl.ds(pl.multiple_of(64 * p + 8 * c, 8), 8), :]
                xx = _w2b(xw).astype(f32) * gwf
                part = xx[:, 0:128]
                for jj in range(1, 8):
                    part = part + xx[:, 128 * jj:128 * jj + 128]
                lg = jnp.sum(part, axis=1, keepdims=True)
                gbuf[pl.ds(pl.multiple_of(128 * p + 16 * c, 16), 16), :] = jnp.broadcast_to(
                    jax.nn.sigmoid(lg), (16, 128))
            for jj in range(8):
                dst = bn32.at[jj, pl.ds(pl.multiple_of(64 * p, 64), 64), :]
                for m in range(8):
                    dst[pl.ds(m, 8, stride=8), :] = bs[m, pl.ds(pl.multiple_of(8 * p, 8), 8), 128 * jj:128 * jj + 128]
            return 0

        lax.fori_loop(0, 16, prebulk, 0)
        cp_mem.wait()
        for j in range(8):
            cp_wo(j).wait()
        oc[...] = jnp.zeros(oc.shape, bf16)
        oc32 = oc.bitcast(u32)

        row = lax.broadcasted_iota(jnp.int32, (40, 128), 0)
        col = lax.broadcasted_iota(jnp.int32, (40, 128), 1)
        mask = ((col < 40) & (row >= 32)) | ((row < 32) & ((col <= row) | ((col >= 32) & (col < 40))))
        scale = DH ** -0.5
        bscale = 2.0 ** -20

        def wo_t(j, h):
            return _w2b(wo[j, h])

        def mix(a, b, g):
            return g * a + (1.0 - g) * (b.astype(f32) * bscale)

        def fill_piece(gr, gw_, src, j, half, accs):
            hs = range(16 * half, 16 * half + 16)
            l = jnp.concatenate([_w2b(src[h]) for h in hs], axis=1)
            w = _w2b(wo[j, 16 * half:16 * half + 16].reshape(16 * 64, 128))
            c = jnp.dot(l, w, preferred_element_type=f32)
            if half == 0:
                return c
            c = c + accs
            for q in range(4):
                sg = 4 * gr + q
                b = bnat[j, pl.ds(pl.multiple_of(32 * sg + 24, 8), 8), :]
                g = gbuf[pl.ds(pl.multiple_of(32 * sg + 24, 8), 8), :]
                outb[pl.ds(pl.multiple_of(128 * gw_ + 32 * q + 24, 8), 8),
                     pl.ds(pl.multiple_of(128 * j, 128), 128)] = mix(c[8 * q:8 * q + 8], b, g).astype(bf16)
            return None

        def out_copy(gi):
            return pltpu.make_async_copy(
                outb.at[pl.ds(pl.multiple_of(128 * gi, 128), 128), :],
                out_hbm.at[pl.ds(pl.multiple_of(128 * gi, 128), 128), :], osem)

        def step(s, mem):
            @pl.when((s % 4 == 0) & (s >= 8))
            def _():
                out_copy(s // 4 - 2).start()

            @pl.when(s % 4 == 0)
            def _():
                ocr[...] = oc32[...]

            r0 = pl.multiple_of(s * 16, 16)
            xs0 = _w2b(xv[pl.ds(r0, 8), :])
            xs1 = _w2b(xv[pl.ds(r0 + 8, 8), :])
            l1 = jnp.concatenate([xs1[0:8].astype(f32), mem], axis=0).astype(bf16)
            lhs[0:8, :] = pltpu.bitcast(xs0, u32)
            lhs[8:16, :] = pltpu.bitcast(l1, u32)
            grp = s // 4 - 1
            gr = jnp.maximum(grp, 0)
            gw_ = jnp.where(grp < 0, 16, grp)
            q4 = s % 4
            st = {}
            z8 = jnp.zeros((8, 128), f32)
            s8 = pl.multiple_of(s * 8, 8)

            def proj(h, i):
                r = jnp.dot(_w2b(lhs[...]), _w2b(w3[h // 2, h % 2, i]), preferred_element_type=f32)
                p_ = pre[h // 2, h % 2, i, pl.ds(s8, 8), :]
                if i == 0:
                    st[("qkv", h, i)] = jnp.concatenate([r[0:24], p_, r[24:32]], axis=0)
                else:
                    st[("qkv", h, i)] = jnp.concatenate([r[0:24], p_, r[24:32], z8], axis=0).astype(bf16)

            def qk(h):
                q = st.pop(("qkv", h, 0))
                k = st.pop(("qkv", h, 1))
                sc = lax.dot_general(q, k, NT, preferred_element_type=f32) * scale
                sc = jnp.concatenate([sc, jnp.zeros((40, 80), f32)], axis=1)
                sc = jnp.where(mask, sc, -1e9)
                m = jnp.max(sc, axis=1, keepdims=True)
                e = jnp.exp(sc - m)
                p = e * (1.0 / jnp.sum(e, axis=1, keepdims=True))
                st[("p", h)] = p[:, :48]

            def pv(h):
                o = lax.dot_general(st.pop(("p", h)), st.pop(("qkv", h, 2)), NN, preferred_element_type=f32)
                st[("o", h)] = jnp.concatenate([o[0:24], o[32:40]], axis=0).astype(bf16)
                oc[h, pl.ds(pl.multiple_of(8 * q4, 8), 8), :] = o[24:32].astype(bf16)

            def oproj(h):
                w = jnp.concatenate([wo_t(j, h) for j in range(8)], axis=1)
                c = jnp.dot(st.pop(("o", h)), w, preferred_element_type=f32)
                if h == 0:
                    acc[...] = c
                else:
                    acc[...] += c

            ok = lambda h: 0 <= h < H
            for t in range(H + 4):
                if ok(t):
                    proj(t, 0)
                    proj(t, 1)
                if ok(t - 1):
                    qk(t - 1)
                if ok(t):
                    proj(t, 2)
                else:
                    jj, half = (t - H) // 2, (t - H) % 2
                    st["fill"] = fill_piece(gr, gw_, ocr, 2 * q4 + jj, half, st.get("fill"))
                if ok(t - 3):
                    pv(t - 3)
                if ok(t - 4):
                    oproj(t - 4)
            a = acc[...]
            rs = pl.multiple_of(32 * s, 32)
            b0 = jnp.concatenate([bnat[j, pl.ds(rs, 16), :] for j in range(8)], axis=1)
            b1 = jnp.concatenate([bnat[j, pl.ds(rs + 16, 8), :] for j in range(8)], axis=1)
            g0 = gbuf[pl.ds(rs, 16), :]
            g1 = gbuf[pl.ds(rs + 16, 8), :]
            outb[pl.ds(rs, 16), :] = mix(a[0:16], b0, jnp.tile(g0, (1, 8))).astype(bf16)
            outb[pl.ds(rs + 16, 8), :] = mix(a[16:24], b1, jnp.tile(g1, (1, 8))).astype(bf16)
            return a[24:32]

        lax.fori_loop(0, NSEG, step, mem0v[...].astype(f32))

        for j in range(8):
            c = fill_piece(15, 15, oc32, j, 0, None)
            fill_piece(15, 15, oc32, j, 1, c)
        out_copy(14).start()
        out_copy(15).start()
        for gi in range(16):
            out_copy(gi).wait()

    pl.run_scoped(
        a_phase,
        pltpu.VMEM((16, 2, 3, 512, 128), u32), pltpu.VMEM((16, 2, 3, 512, 128), f32),
        pltpu.VMEM((H, 32, 128), bf16), pltpu.VMEM((H, 16, 128), u32), pltpu.VMEM((32, D), f32), pltpu.VMEM((16, D), u32))


@jax.jit
def pallas_gated_mix__memory_aug_recurrent_mem_tr__spectral_gfnet__prompt_kernel(
    A_x, A_mem0, A_Wq, A_Wk, A_Wv, A_Wo, A_seg_len, B_x, B_w_r, B_w_i, gate_w,
):
    del A_seg_len
    del B_x
    HB = pl.BlockSpec(memory_space=pltpu.HBM)
    out = pl.pallas_call(
        _kernel,
        out_shape=jax.ShapeDtypeStruct((S, D), bf16),
        in_specs=[HB] * 13,
        out_specs=HB,
        scratch_shapes=[
            pltpu.VMEM((S // 2, D), u32),
            pltpu.VMEM((NSEG * 4, D), u32),
            pltpu.VMEM((M_MEM, D), bf16),
            pltpu.VMEM((1, D), bf16),
            pltpu.VMEM((16, 3, D, DH), u32),
            pltpu.VMEM((8, H, DH // 2, 128), u32),
            pltpu.VMEM((8, 128, D), u32),
            pltpu.VMEM((8, S, 128), bf16),
            pltpu.VMEM((S, 128), f32),
            pltpu.VMEM((S + 128, D), bf16),
            pltpu.SemaphoreType.DMA((13,)),
            pltpu.SemaphoreType.DMA((16,)),
            pltpu.SemaphoreType.DMA((6,)),
            pltpu.SemaphoreType.DMA(()),
        ],
        compiler_params=pltpu.CompilerParams(vmem_limit_bytes=124 * 2 ** 20),
    )(
        A_x.reshape(S, D), A_mem0.reshape(M_MEM, D), A_Wq, A_Wk, A_Wv, A_Wo,
        A_x.reshape(128, 16, D), B_w_r.T, B_w_i.T, gate_w.reshape(1, D), _TAB_G, _TAB_H, _TAB_MISC,
    )
    return out.reshape(1, S, D)
```

```python
import numpy as np
import ml_dtypes
import jax
import jax.numpy as jnp
from jax import lax
import jax.experimental.pallas as pl
import jax.experimental.pallas.tpu as pltpu

f32, bf16, u32 = jnp.float32, jnp.bfloat16, jnp.uint32
S, D, H, DH, M_MEM, SEG = 2048, 1024, 32, 128, 8, 32
NSEG = S // SEG
RS = float(1 / np.sqrt(2))
NT = (((1,), (1,)), ((), ()))
NN = (((1,), (0,)), ((), ()))
HI = 0xFFFF0000


def _np_tables():
    bf = ml_dtypes.bfloat16
    dp = np.arange(128)
    j = np.arange(64)

    def cs(f):
        ang = 2 * np.pi * ((f[:, None] * dp[None, :]) % 1024) / 1024
        return np.cos(ang), np.sin(ang)

    G = np.zeros((5, 256, 256))
    for t in range(3):
        r = t + 1
        C, Sn = cs(r + 8 * j)
        C2, S2 = cs(8 - r + 8 * j)
        G[t, 0:64, 0:128] = C
        G[t, 0:64, 128:] = Sn
        G[t, 64:128, 0:128] = C2
        G[t, 64:128, 128:] = -S2
        G[t, 128:192, 0:128] = -Sn
        G[t, 128:192, 128:] = C
        G[t, 192:256, 0:128] = -S2
        G[t, 192:256, 128:] = -C2
    C0, S0 = cs(8 * j)
    C4, S4 = cs(4 + 8 * j)
    G[3, 0:64, 0:128] = C0
    G[3, 128:192, 0:128] = -S0
    G[3, 64:128, 128:] = C4
    G[3, 192:256, 128:] = -S4
    G[4] = G[3]
    G[4, 0, 0:128] = 0.5
    G[4, 128, 0:128] = 0.5 * (-1.0) ** dp
    HH = np.zeros((16, 256, 128))
    for a in range(16):
        ang = 2 * np.pi * (((a + 16 * dp)[:, None] * dp[None, :]) % 2048) / 2048
        HH[a, :128] = np.cos(ang)
        HH[a, 128:] = np.sin(ang)
    misc = np.zeros((3, 128, 128))
    misc[0, 128 - dp[1:], dp[1:]] = 1
    misc[1, 0, 0] = 1
    misc[2, 0, :] = (-1.0) ** dp
    for blk in range(4):
        for k1 in range(16):
            misc[2, 64 + 16 * blk + k1, 16 * blk + 15 - k1] = 1
            misc[2, 64 + 16 * blk + k1, 64 + 16 * blk + (16 - k1) % 16] = 1
    return G.astype(bf), HH.astype(bf), misc.astype(bf)


_TAB_G, _TAB_H, _TAB_MISC = _np_tables()


def _bc(x, dt):
    return lax.bitcast_convert_type(x, dt)


def _w2b(w):
    return pltpu.bitcast(w, bf16)


def _fft16(xs, inverse):
    sg = 1.0 if inverse else -1.0

    def dft4(a, b, c, d):
        t0 = (a[0] + c[0], a[1] + c[1])
        t1 = (a[0] - c[0], a[1] - c[1])
        t2 = (b[0] + d[0], b[1] + d[1])
        t3 = (b[0] - d[0], b[1] - d[1])
        o0 = (t0[0] + t2[0], t0[1] + t2[1])
        o2 = (t0[0] - t2[0], t0[1] - t2[1])
        m = (t1[0] + t3[1], t1[1] - t3[0])
        p = (t1[0] - t3[1], t1[1] + t3[0])
        return [o0, p, o2, m] if inverse else [o0, m, o2, p]

    t = [dft4(xs[a0], xs[4 + a0], xs[8 + a0], xs[12 + a0]) for a0 in range(4)]

    def tw(v, e):
        e = e % 16
        if e == 0:
            return v
        if e == 4:
            return (-v[1], v[0]) if inverse else (v[1], -v[0])
        if e == 2:
            if inverse:
                return ((v[0] - v[1]) * RS, (v[0] + v[1]) * RS)
            return ((v[0] + v[1]) * RS, (v[1] - v[0]) * RS)
        if e == 6:
            if inverse:
                return ((-v[0] - v[1]) * RS, (v[0] - v[1]) * RS)
            return ((v[1] - v[0]) * RS, (-v[0] - v[1]) * RS)
        c = float(np.cos(2 * np.pi * e / 16))
        s = float(sg * np.sin(2 * np.pi * e / 16))
        return (v[0] * c - v[1] * s, v[0] * s + v[1] * c)

    out = [None] * 16
    for k in range(4):
        u = [tw(t[a0][k], a0 * k) for a0 in range(4)]
        r = dft4(*u)
        for m in range(4):
            out[k + 4 * m] = r[m]
    return out


def _b_phase(xb_hbm, wr_hbm, wi_hbm, g_hbm, h_hbm, misc_hbm, bs, sems, start_m, start_i):
    def scoped(xs, wr, wi, wrn, win, G, HH, misc, Y, Zr, Zi, WS, PQ):
        xb32 = xb_hbm.bitcast(u32)
        xcp = [pltpu.make_async_copy(xb32.at[:, m, :], xs.at[m], sems.at[m]) for m in range(2)]
        cg = pltpu.make_async_copy(g_hbm, G, sems.at[8])
        ch = pltpu.make_async_copy(h_hbm, HH, sems.at[9])
        cm = pltpu.make_async_copy(misc_hbm, misc, sems.at[10])
        def wblk(k):
            off = 128 * k if isinstance(k, int) else pl.multiple_of(128 * k, 128)
            return (pltpu.make_async_copy(wr_hbm.at[pl.ds(0, 512), pl.ds(off, 128)], wr.at[k], sems.at[11]),
                    pltpu.make_async_copy(wi_hbm.at[pl.ds(0, 512), pl.ds(off, 128)], wi.at[k], sems.at[12]))

        wny = (pltpu.make_async_copy(wr_hbm.at[pl.ds(512, 1), :], wrn, sems.at[11]),
               pltpu.make_async_copy(wi_hbm.at[pl.ds(512, 1), :], win, sems.at[12]))
        cg.start()
        xcp[0].start()
        ch.start()
        cm.start()
        xcp[1].start()
        for c in wny:
            c.start()
        cg.wait()
        cm.wait()
        ch.wait()

        def getM(a):
            hc = HH[a, 0:128, :]
            hs = HH[a, 128:256, :]
            return jnp.concatenate(
                [jnp.concatenate([hc, -hs], axis=1), jnp.concatenate([hs, hc], axis=1)], axis=0)

        def phF(m, _):
            @pl.when(m < 6)
            def _():
                pltpu.make_async_copy(xb32.at[:, m + 2, :], xs.at[m + 2], sems.at[m + 2]).start()

            for k in (2 * m, 2 * m + 1):
                for c in wblk(k):
                    c.start()
            pltpu.make_async_copy(xb32.at[:, 0, :], xs.at[m], sems.at[m]).wait()
            def d1(half):
                for ch_ in range(8):
                    w = xs[m, 16 * ch_:16 * ch_ + 16, :]
                    xv = _bc(w << 16, f32) if half == 0 else _bc(w & jnp.uint32(HI), f32)
                    xc = [xv[:, 128 * c:128 * (c + 1)] for c in range(8)]
                    a0, a1 = xc[0] + xc[4], xc[0] - xc[4]
                    b0, b1 = xc[2] + xc[6], xc[2] - xc[6]
                    c0, c1 = xc[1] + xc[5], xc[1] - xc[5]
                    d0, d1_ = xc[3] + xc[7], xc[3] - xc[7]
                    p, q = a0 + b0, c0 + d0
                    y0, y4 = p + q, p - q
                    y2r, y2i = a0 - b0, d0 - c0
                    cm_, cp_ = RS * (c1 - d1_), RS * (c1 + d1_)
                    y1r, y1i = a1 + cm_, -b1 - cp_
                    y3r, y3i = a1 - cm_, b1 - cp_
                    for t, (yr, yi) in enumerate([(y1r, y1i), (y2r, y2i), (y3r, y3i), (y0, y4)]):
                        Y[half, t, 16 * ch_:16 * ch_ + 16, :] = jnp.concatenate([yr, yi], axis=1).astype(bf16)

            Ms = {}
            zs = {}

            def stage_a(u):
                half, t = divmod(u, 5)
                if t < 4:
                    o = lax.dot_general(G[t], Y[half, t], NT, preferred_element_type=f32)
                    zs[u] = jnp.concatenate([o[:128], o[128:]], axis=1).astype(bf16)
                else:
                    zs[u] = lax.dot_general(misc[2, 0:16, :], Y[half, 3, :, 0:128], NT,
                                            preferred_element_type=f32).astype(bf16)

            def stage_b(u):
                half, t = divmod(u, 5)
                a = 2 * m + half
                if half not in Ms:
                    Ms[half] = getM(a)
                Mx = Ms[half]
                if t < 4:
                    X = jnp.dot(zs.pop(u), Mx, preferred_element_type=f32)
                    Zr[a, 128 * t:128 * t + 128, :] = X[:, 0:128]
                    Zi[a, 128 * t:128 * t + 128, :] = X[:, 128:256]
                else:
                    Xn = jnp.dot(zs.pop(u), Mx[0:128, :], preferred_element_type=f32)
                    Zr[a, 512:528, :] = Xn[:, 0:128]
                    Zi[a, 512:528, :] = Xn[:, 128:256]

            d1(0)
            stage_a(0)
            stage_a(1)
            d1(1)
            for u in range(10):
                if u + 2 < 10:
                    stage_b(u)
                    stage_a(u + 2)
                else:
                    stage_b(u)
            return 0

        lax.fori_loop(0, 8, phF, 0)

        for k in range(16):
            for c in wblk(k):
                c.wait()
        for c in wny:
            c.wait()
        wr32 = wr.bitcast(u32)
        wi32 = wi.bitcast(u32)
        hi = jnp.uint32(HI)
        dcr = jnp.concatenate([_bc(wr32[k, 0:1, :] << 16, f32) for k in range(16)], axis=0)
        dci = jnp.concatenate([_bc(wi32[k, 0:1, :] << 16, f32) for k in range(16)], axis=0)
        nyr = jnp.concatenate([wrn[:, 128 * k:128 * (k + 1)].astype(f32) for k in range(16)], axis=0)
        nyi = jnp.concatenate([win[:, 128 * k:128 * (k + 1)].astype(f32) for k in range(16)], axis=0)
        st = jnp.concatenate([dcr, dci, nyr, nyi], axis=0)
        stb = st.astype(bf16)
        r1 = jnp.dot(stb, misc[0], preferred_element_type=f32)
        r2 = jnp.dot(stb, misc[1], preferred_element_type=f32)
        rr = jnp.concatenate([r1, r2], axis=0).astype(bf16)
        rp = jnp.dot(misc[2, 64:128, :], rr, preferred_element_type=f32)
        rid = lax.broadcasted_iota(jnp.int32, (64, 128), 0)
        sgn = jnp.where((rid & 16) == 0, 0.5, -0.5)
        WS[...] = 0.5 * st + sgn * rp

        POS = {1: 0, 7: 64, 2: 128, 6: 192, 3: 256, 5: 320, 0: 384, 4: 448}
        row8 = lax.broadcasted_iota(jnp.int32, (8, 128), 0)

        def mid(r, g, special):
            r0 = POS[r] + 8 * g
            if not special:
                r0 = pl.multiple_of(r0, 8)
            xs_ = [(Zr[a, pl.ds(r0, 8), :], Zi[a, pl.ds(r0, 8), :]) for a in range(16)]
            o = _fft16(xs_, False)
            if special:
                xn = [(Zr[a, 512:520, :], Zi[a, 512:520, :]) for a in range(16)]
                on = _fft16(xn, False)
                wsr, wsi = wr32, wi32
            else:
                g32 = pl.multiple_of(32 * g, 32)
                wsr = wr32.at[:, pl.ds(g32, 32), :]
                wsi = wi32.at[:, pl.ds(g32, 32), :]
            ys = []
            for k in range(16):
                a_ = wsr[k, pl.ds(r // 2, 8, stride=4), :]
                b_ = wsi[k, pl.ds(r // 2, 8, stride=4), :]
                if r % 2 == 0:
                    wre, wim = _bc(a_ << 16, f32), _bc(b_ << 16, f32)
                else:
                    wre, wim = _bc(a_ & hi, f32), _bc(b_ & hi, f32)
                if special:
                    wre = jnp.where(row8 == 0, jnp.broadcast_to(WS[k:k + 1, :], (8, 128)), wre)
                    wim = jnp.where(row8 == 0, jnp.broadcast_to(WS[16 + k:17 + k, :], (8, 128)), wim)
                xr, xi = o[k]
                yr = xr * wre - xi * wim
                yi = xr * wim + xi * wre
                if special:
                    nr = jnp.broadcast_to(WS[32 + k:33 + k, :], (8, 128))
                    ni = jnp.broadcast_to(WS[48 + k:49 + k, :], (8, 128))
                    zr_, zi_ = on[k]
                    yr = yr - (zr_ * ni + zi_ * nr)
                    yi = yi + (zr_ * nr - zi_ * ni)
                ys.append((yr, yi))
            u = _fft16(ys, True)
            for a in range(16):
                Zr[a, pl.ds(r0, 8), :] = u[a][0]
                Zi[a, pl.ds(r0, 8), :] = u[a][1]

        mid(0, 0, True)

        def phM(g, _):
            start_m(g)
            for r in range(1, 8):
                mid(r, g, False)

            @pl.when(g > 0)
            def _():
                mid(0, g, False)

            return 0

        lax.fori_loop(0, 8, phM, 0)

        def phI(m, _):
            start_i(m)
            Ms = {}
            vs = {}

            def stage_a(u):
                half, t = divmod(u, 4)
                a = 2 * m + half
                if half not in Ms:
                    Ms[half] = getM(a)
                yy = jnp.concatenate(
                    [Zr[a, 128 * t:128 * t + 128, :], Zi[a, 128 * t:128 * t + 128, :]], axis=1).astype(bf16)
                o = lax.dot_general(Ms[half], yy, NT, preferred_element_type=f32)
                vs[u] = jnp.concatenate([o[:128], o[128:]], axis=1).astype(bf16)

            def stage_b(u):
                half, t = divmod(u, 4)
                PQ[half, t] = jnp.dot(vs.pop(u), G[t if t < 3 else 4], preferred_element_type=f32)

            def d1inv(half):
                for ch_ in range(8):
                    rs = slice(16 * ch_, 16 * ch_ + 16)
                    P1, Q1 = PQ[half, 0, rs, 0:128], PQ[half, 0, rs, 128:256]
                    P2, Q2 = PQ[half, 1, rs, 0:128], PQ[half, 1, rs, 128:256]
                    P3, Q3 = PQ[half, 2, rs, 0:128], PQ[half, 2, rs, 128:256]
                    h0, h4 = PQ[half, 3, rs, 0:128], PQ[half, 3, rs, 128:256]
                    e, o_ = h0 + h4, h0 - h4
                    A, B = P1 + P3, Q1 - Q3
                    u_, v = P1 - P3, Q1 + Q3
                    T1_, T2_ = RS * (u_ - v), RS * (-u_ - v)
                    e1, e2 = e + P2, e - P2
                    o1, o2 = o_ - Q2, o_ + Q2
                    cols = jnp.concatenate(
                        [e1 + A, o1 + T1_, e2 - B, o2 + T2_, e1 - A, o1 - T1_, e2 + B, o2 - T2_], axis=1)
                    bits = _bc(cols.astype(bf16).astype(f32), u32)
                    if half == 0:
                        bs[m, rs, :] = bits >> 16
                    else:
                        bs[m, rs, :] = bs[m, rs, :] | bits

            stage_a(0)
            stage_a(1)
            for u in range(8):
                stage_b(u)
                if u + 2 < 8:
                    stage_a(u + 2)
                if u == 4:
                    d1inv(0)
            d1inv(1)
            return 0

        lax.fori_loop(0, 8, phI, 0)

    pl.run_scoped(
        scoped,
        pltpu.VMEM((8, 128, D), u32), pltpu.VMEM((16, 512, 128), bf16), pltpu.VMEM((16, 512, 128), bf16),
        pltpu.VMEM((1, S), bf16), pltpu.VMEM((1, S), bf16),
        pltpu.VMEM((5, 256, 256), bf16), pltpu.VMEM((16, 256, 128), bf16), pltpu.VMEM((3, 128, 128), bf16),
        pltpu.VMEM((2, 4, 128, 256), bf16), pltpu.VMEM((16, 528, 128), f32), pltpu.VMEM((16, 528, 128), f32),
        pltpu.VMEM((64, 128), f32), pltpu.VMEM((2, 4, 128, 256), f32))


def _kernel(x_hbm, mem0_hbm, wq_hbm, wk_hbm, wv_hbm, wo_hbm, xb_hbm, wr_hbm, wi_hbm, gw_hbm,
            g_hbm, h_hbm, misc_hbm, out_hbm,
            xv, xpre, mem0v, gwv, raw, wo, bs, bnat, gbuf, outb, bsems, wsems, msems, osem):
    cp_x = pltpu.make_async_copy(x_hbm.bitcast(u32), xv, msems.at[0])
    cp_mem = pltpu.make_async_copy(mem0_hbm, mem0v, msems.at[2])
    cp_gw = pltpu.make_async_copy(gw_hbm, gwv, msems.at[3])
    wsrc = [w.bitcast(u32) for w in (wq_hbm, wk_hbm, wv_hbm)]
    wo32 = wo_hbm.bitcast(u32)

    def cp_w(p):
        return [pltpu.make_async_copy(wsrc[i].at[:, p, :], raw.at[p, i], wsems.at[p]) for i in range(3)]

    def cp_wo(j):
        off = 128 * j if isinstance(j, int) else pl.multiple_of(128 * j, 128)
        return pltpu.make_async_copy(wo32.at[:, :, pl.ds(off, 128)], wo.at[j], msems.at[4])

    def start_m(g):
        @pl.when(g == 0)
        def _():
            cp_gw.start()
            cp_mem.start()
            cp_x.start()

        for c in cp_w(g):
            c.start()

    def start_i(m):
        for c in cp_w(m + 8):
            c.start()

    _b_phase(xb_hbm, wr_hbm, wi_hbm, g_hbm, h_hbm, misc_hbm, bs, bsems, start_m, start_i)
    bn32 = bnat.bitcast(u32)

    def a_phase(w3, pre, oc, ocr, acc, lhs):
        cp_x.wait()
        cp_gw.wait()
        gwf = gwv[...].astype(f32)
        for i in range(32):
            xpre[8 * i:8 * i + 8, :] = jnp.concatenate(
                [xv[32 * i + 12:32 * i + 16, :], xv[32 * i + 28:32 * i + 32, :]], axis=0)

        def prebulk(p, _):
            @pl.when(p < 8)
            def _():
                cp_wo(p).start()

            for i in range(3):
                pltpu.make_async_copy(wsrc[i].at[:, 0, :], raw.at[p, i], wsems.at[p]).wait()
            for i in range(3):
                e = raw[p, i, pl.ds(0, 512, stride=2), :]
                o = raw[p, i, pl.ds(1, 512, stride=2), :]
                w3[p, 0, i] = (e & jnp.uint32(0xFFFF)) | (o << 16)
                w3[p, 1, i] = (e >> 16) | (o & jnp.uint32(HI))
            for r in range(2):
                for i in range(3):
                    for c in range(2):
                        xl = _w2b(xpre[128 * c:128 * c + 128, :])
                        pre[p, r, i, 256 * c:256 * c + 256, :] = jnp.dot(
                            xl, _w2b(w3[p, r, i]), preferred_element_type=f32)
            for c in range(8):
                xw = xv[pl.ds(pl.multiple_of(64 * p + 8 * c, 8), 8), :]
                xx = _w2b(xw).astype(f32) * gwf
                part = xx[:, 0:128]
                for jj in range(1, 8):
                    part = part + xx[:, 128 * jj:128 * jj + 128]
                lg = jnp.sum(part, axis=1, keepdims=True)
                gbuf[pl.ds(pl.multiple_of(128 * p + 16 * c, 16), 16), :] = jnp.broadcast_to(
                    jax.nn.sigmoid(lg), (16, 128))
            for jj in range(8):
                dst = bn32.at[jj, pl.ds(pl.multiple_of(64 * p, 64), 64), :]
                for m in range(8):
                    dst[pl.ds(m, 8, stride=8), :] = bs[m, pl.ds(pl.multiple_of(8 * p, 8), 8), 128 * jj:128 * jj + 128]
            return 0

        lax.fori_loop(0, 16, prebulk, 0)
        cp_mem.wait()
        for j in range(8):
            cp_wo(j).wait()
        oc[...] = jnp.zeros(oc.shape, bf16)
        oc32 = oc.bitcast(u32)

        row = lax.broadcasted_iota(jnp.int32, (40, 128), 0)
        col = lax.broadcasted_iota(jnp.int32, (40, 128), 1)
        mask = ((col < 40) & (row >= 32)) | ((row < 32) & ((col <= row) | ((col >= 32) & (col < 40))))
        scale = DH ** -0.5
        bscale = 2.0 ** -20

        def wo_t(j, h):
            return _w2b(wo[j, h])

        def mix(a, b, g):
            return g * a + (1.0 - g) * (b.astype(f32) * bscale)

        def fill_piece(gr, gw_, src, j, half, accs):
            hs = range(16 * half, 16 * half + 16)
            l = jnp.concatenate([_w2b(src[h]) for h in hs], axis=1)
            w = _w2b(wo[j, 16 * half:16 * half + 16].reshape(16 * 64, 128))
            c = jnp.dot(l, w, preferred_element_type=f32)
            if half == 0:
                return c
            c = c + accs
            for q in range(4):
                sg = 4 * gr + q
                b = bnat[j, pl.ds(pl.multiple_of(32 * sg + 24, 8), 8), :]
                g = gbuf[pl.ds(pl.multiple_of(32 * sg + 24, 8), 8), :]
                outb[pl.ds(pl.multiple_of(128 * gw_ + 32 * q + 24, 8), 8),
                     pl.ds(pl.multiple_of(128 * j, 128), 128)] = mix(c[8 * q:8 * q + 8], b, g).astype(bf16)
            return None

        def out_copy(gi):
            return pltpu.make_async_copy(
                outb.at[pl.ds(pl.multiple_of(128 * gi, 128), 128), :],
                out_hbm.at[pl.ds(pl.multiple_of(128 * gi, 128), 128), :], osem)

        def step(s, mem):
            @pl.when((s % 4 == 0) & (s >= 8))
            def _():
                out_copy(s // 4 - 2).start()

            @pl.when(s % 4 == 0)
            def _():
                ocr[...] = oc32[...]

            r0 = pl.multiple_of(s * 16, 16)
            xs0 = _w2b(xv[pl.ds(r0, 8), :])
            xs1 = _w2b(xv[pl.ds(r0 + 8, 8), :])
            l1 = jnp.concatenate([xs1[0:8].astype(f32), mem], axis=0).astype(bf16)
            lhs[0:8, :] = pltpu.bitcast(xs0, u32)
            lhs[8:16, :] = pltpu.bitcast(l1, u32)
            grp = s // 4 - 1
            gr = jnp.maximum(grp, 0)
            gw_ = jnp.where(grp < 0, 16, grp)
            q4 = s % 4
            st = {}
            z8 = jnp.zeros((8, 128), f32)
            s8 = pl.multiple_of(s * 8, 8)

            def proj(h, i):
                r = jnp.dot(_w2b(lhs[...]), _w2b(w3[h // 2, h % 2, i]), preferred_element_type=f32)
                p_ = pre[h // 2, h % 2, i, pl.ds(s8, 8), :]
                if i == 0:
                    st[("qkv", h, i)] = jnp.concatenate([r[0:24], p_, r[24:32]], axis=0)
                else:
                    st[("qkv", h, i)] = jnp.concatenate([r[0:24], p_, r[24:32], z8], axis=0).astype(bf16)

            def qk(h):
                q = st.pop(("qkv", h, 0))
                k = st.pop(("qkv", h, 1))
                sc = lax.dot_general(q, k, NT, preferred_element_type=f32) * scale
                sc = jnp.concatenate([sc, jnp.zeros((40, 80), f32)], axis=1)
                sc = jnp.where(mask, sc, -1e9)
                m = jnp.max(sc, axis=1, keepdims=True)
                e = jnp.exp(sc - m)
                p = e * (1.0 / jnp.sum(e, axis=1, keepdims=True))
                st[("p", h)] = p[:, :48]

            def pv(h):
                o = lax.dot_general(st.pop(("p", h)), st.pop(("qkv", h, 2)), NN, preferred_element_type=f32)
                st[("o", h)] = jnp.concatenate([o[0:24], o[32:40]], axis=0).astype(bf16)
                oc[h, pl.ds(pl.multiple_of(8 * q4, 8), 8), :] = o[24:32].astype(bf16)

            def oproj(h):
                w = jnp.concatenate([wo_t(j, h) for j in range(8)], axis=1)
                c = jnp.dot(st.pop(("o", h)), w, preferred_element_type=f32)
                if h == 0:
                    acc[...] = c
                else:
                    acc[...] += c

            ok = lambda h: 0 <= h < H
            for t in range(H + 4):
                if ok(t):
                    proj(t, 0)
                    proj(t, 1)
                if ok(t - 1):
                    qk(t - 1)
                if ok(t):
                    proj(t, 2)
                else:
                    jj, half = (t - H) // 2, (t - H) % 2
                    st["fill"] = fill_piece(gr, gw_, ocr, 2 * q4 + jj, half, st.get("fill"))
                if ok(t - 3):
                    pv(t - 3)
                if ok(t - 4):
                    oproj(t - 4)
            a = acc[...]
            rs = pl.multiple_of(32 * s, 32)
            b0 = jnp.concatenate([bnat[j, pl.ds(rs, 16), :] for j in range(8)], axis=1)
            b1 = jnp.concatenate([bnat[j, pl.ds(rs + 16, 8), :] for j in range(8)], axis=1)
            g0 = gbuf[pl.ds(rs, 16), :]
            g1 = gbuf[pl.ds(rs + 16, 8), :]
            outb[pl.ds(rs, 16), :] = mix(a[0:16], b0, jnp.tile(g0, (1, 8))).astype(bf16)
            outb[pl.ds(rs + 16, 8), :] = mix(a[16:24], b1, jnp.tile(g1, (1, 8))).astype(bf16)
            return a[24:32]

        lax.fori_loop(0, NSEG, step, mem0v[...].astype(f32))

        for j in range(8):
            c = fill_piece(15, 15, oc32, j, 0, None)
            fill_piece(15, 15, oc32, j, 1, c)
        out_copy(14).start()
        out_copy(15).start()
        for gi in range(16):
            out_copy(gi).wait()

    pl.run_scoped(
        a_phase,
        pltpu.VMEM((16, 2, 3, 512, 128), u32), pltpu.VMEM((16, 2, 3, 512, 128), f32),
        pltpu.VMEM((H, 32, 128), bf16), pltpu.VMEM((H, 16, 128), u32), pltpu.VMEM((32, D), f32), pltpu.VMEM((16, D), u32))


@jax.jit
def pallas_gated_mix__memory_aug_recurrent_mem_tr__spectral_gfnet__prompt_kernel(
    A_x, A_mem0, A_Wq, A_Wk, A_Wv, A_Wo, A_seg_len, B_x, B_w_r, B_w_i, gate_w,
):
    del A_seg_len
    del B_x
    HB = pl.BlockSpec(memory_space=pltpu.HBM)
    out = pl.pallas_call(
        _kernel,
        out_shape=jax.ShapeDtypeStruct((S, D), bf16),
        in_specs=[HB] * 13,
        out_specs=HB,
        scratch_shapes=[
            pltpu.VMEM((S // 2, D), u32),
            pltpu.VMEM((NSEG * 4, D), u32),
            pltpu.VMEM((M_MEM, D), bf16),
            pltpu.VMEM((1, D), bf16),
            pltpu.VMEM((16, 3, D, DH), u32),
            pltpu.VMEM((8, H, DH // 2, 128), u32),
            pltpu.VMEM((8, 128, D), u32),
            pltpu.VMEM((8, S, 128), bf16),
            pltpu.VMEM((S, 128), f32),
            pltpu.VMEM((S + 128, D), bf16),
            pltpu.SemaphoreType.DMA((13,)),
            pltpu.SemaphoreType.DMA((16,)),
            pltpu.SemaphoreType.DMA((6,)),
            pltpu.SemaphoreType.DMA(()),
        ],
        compiler_params=pltpu.CompilerParams(vmem_limit_bytes=124 * 2 ** 20),
    )(
        A_x.reshape(S, D), A_mem0.reshape(M_MEM, D), A_Wq, A_Wk, A_Wv, A_Wo,
        A_x.reshape(128, 16, D), B_w_r.T, B_w_i.T, gate_w.reshape(1, D), _TAB_G, _TAB_H, _TAB_MISC,
    )
    return out.reshape(1, S, D)
```

```python
import numpy as np
import ml_dtypes
import jax
import jax.numpy as jnp
from jax import lax
import jax.experimental.pallas as pl
import jax.experimental.pallas.tpu as pltpu

f32, bf16, u32 = jnp.float32, jnp.bfloat16, jnp.uint32
S, D, H, DH, M_MEM, SEG = 2048, 1024, 32, 128, 8, 32
NSEG = S // SEG
RS = float(1 / np.sqrt(2))
NT = (((1,), (1,)), ((), ()))
NN = (((1,), (0,)), ((), ()))
HI = 0xFFFF0000


def _np_tables():
    bf = ml_dtypes.bfloat16
    dp = np.arange(128)
    j = np.arange(64)

    def cs(f):
        ang = 2 * np.pi * ((f[:, None] * dp[None, :]) % 1024) / 1024
        return np.cos(ang), np.sin(ang)

    G = np.zeros((5, 256, 256))
    for t in range(3):
        r = t + 1
        C, Sn = cs(r + 8 * j)
        C2, S2 = cs(8 - r + 8 * j)
        G[t, 0:64, 0:128] = C
        G[t, 0:64, 128:] = Sn
        G[t, 64:128, 0:128] = C2
        G[t, 64:128, 128:] = -S2
        G[t, 128:192, 0:128] = -Sn
        G[t, 128:192, 128:] = C
        G[t, 192:256, 0:128] = -S2
        G[t, 192:256, 128:] = -C2
    C0, S0 = cs(8 * j)
    C4, S4 = cs(4 + 8 * j)
    G[3, 0:64, 0:128] = C0
    G[3, 128:192, 0:128] = -S0
    G[3, 64:128, 128:] = C4
    G[3, 192:256, 128:] = -S4
    G[4] = G[3]
    G[4, 0, 0:128] = 0.5
    G[4, 128, 0:128] = 0.5 * (-1.0) ** dp
    HH = np.zeros((16, 256, 128))
    for a in range(16):
        ang = 2 * np.pi * (((a + 16 * dp)[:, None] * dp[None, :]) % 2048) / 2048
        HH[a, :128] = np.cos(ang)
        HH[a, 128:] = np.sin(ang)
    misc = np.zeros((3, 128, 128))
    misc[0, 128 - dp[1:], dp[1:]] = 1
    misc[1, 0, 0] = 1
    misc[2, 0, :] = (-1.0) ** dp
    for blk in range(4):
        for k1 in range(16):
            misc[2, 64 + 16 * blk + k1, 16 * blk + 15 - k1] = 1
            misc[2, 64 + 16 * blk + k1, 64 + 16 * blk + (16 - k1) % 16] = 1
    return G.astype(bf), HH.astype(bf), misc.astype(bf)


_TAB_G, _TAB_H, _TAB_MISC = _np_tables()


def _bc(x, dt):
    return lax.bitcast_convert_type(x, dt)


def _w2b(w):
    return pltpu.bitcast(w, bf16)


def _fft16(xs, inverse):
    sg = 1.0 if inverse else -1.0

    def dft4(a, b, c, d):
        t0 = (a[0] + c[0], a[1] + c[1])
        t1 = (a[0] - c[0], a[1] - c[1])
        t2 = (b[0] + d[0], b[1] + d[1])
        t3 = (b[0] - d[0], b[1] - d[1])
        o0 = (t0[0] + t2[0], t0[1] + t2[1])
        o2 = (t0[0] - t2[0], t0[1] - t2[1])
        m = (t1[0] + t3[1], t1[1] - t3[0])
        p = (t1[0] - t3[1], t1[1] + t3[0])
        return [o0, p, o2, m] if inverse else [o0, m, o2, p]

    t = [dft4(xs[a0], xs[4 + a0], xs[8 + a0], xs[12 + a0]) for a0 in range(4)]

    def tw(v, e):
        e = e % 16
        if e == 0:
            return v
        if e == 4:
            return (-v[1], v[0]) if inverse else (v[1], -v[0])
        if e == 2:
            if inverse:
                return ((v[0] - v[1]) * RS, (v[0] + v[1]) * RS)
            return ((v[0] + v[1]) * RS, (v[1] - v[0]) * RS)
        if e == 6:
            if inverse:
                return ((-v[0] - v[1]) * RS, (v[0] - v[1]) * RS)
            return ((v[1] - v[0]) * RS, (-v[0] - v[1]) * RS)
        c = float(np.cos(2 * np.pi * e / 16))
        s = float(sg * np.sin(2 * np.pi * e / 16))
        return (v[0] * c - v[1] * s, v[0] * s + v[1] * c)

    out = [None] * 16
    for k in range(4):
        u = [tw(t[a0][k], a0 * k) for a0 in range(4)]
        r = dft4(*u)
        for m in range(4):
            out[k + 4 * m] = r[m]
    return out


def _b_phase(xb_hbm, wr_hbm, wi_hbm, g_hbm, h_hbm, misc_hbm, bs, sems, start_m, start_i):
    def scoped(xs, wr, wi, wrn, win, G, HH, misc, Y, Zr, Zi, WS, PQ):
        xb32 = xb_hbm.bitcast(u32)
        xcp = [pltpu.make_async_copy(xb32.at[:, m, :], xs.at[m], sems.at[m]) for m in range(2)]
        cg = pltpu.make_async_copy(g_hbm, G, sems.at[8])

        def chh(m):
            return pltpu.make_async_copy(h_hbm.at[pl.ds(2 * m, 2)], HH.at[pl.ds(2 * m, 2)], sems.at[13 + m])

        cm = pltpu.make_async_copy(misc_hbm, misc, sems.at[10])
        def wblk(k):
            off = 128 * k if isinstance(k, int) else pl.multiple_of(128 * k, 128)
            return (pltpu.make_async_copy(wr_hbm.at[pl.ds(0, 512), pl.ds(off, 128)], wr.at[k], sems.at[11]),
                    pltpu.make_async_copy(wi_hbm.at[pl.ds(0, 512), pl.ds(off, 128)], wi.at[k], sems.at[12]))

        wny = (pltpu.make_async_copy(wr_hbm.at[pl.ds(512, 1), :], wrn, sems.at[11]),
               pltpu.make_async_copy(wi_hbm.at[pl.ds(512, 1), :], win, sems.at[12]))
        xcp[0].start()
        cg.start()
        chh(0).start()
        cm.start()
        xcp[1].start()
        chh(1).start()
        for c in wny:
            c.start()
        cg.wait()
        cm.wait()

        def getM(a):
            hc = HH[a, 0:128, :]
            hs = HH[a, 128:256, :]
            return jnp.concatenate(
                [jnp.concatenate([hc, -hs], axis=1), jnp.concatenate([hs, hc], axis=1)], axis=0)

        def phF(m, _):
            @pl.when(m < 6)
            def _():
                pltpu.make_async_copy(xb32.at[:, m + 2, :], xs.at[m + 2], sems.at[m + 2]).start()
                chh(m + 2).start()

            for k in (2 * m, 2 * m + 1):
                for c in wblk(k):
                    c.start()
            pltpu.make_async_copy(xb32.at[:, 0, :], xs.at[m], sems.at[m]).wait()
            chh(m).wait()
            def d1(half):
                for ch_ in range(8):
                    w = xs[m, 16 * ch_:16 * ch_ + 16, :]
                    xv = _bc(w << 16, f32) if half == 0 else _bc(w & jnp.uint32(HI), f32)
                    xc = [xv[:, 128 * c:128 * (c + 1)] for c in range(8)]
                    a0, a1 = xc[0] + xc[4], xc[0] - xc[4]
                    b0, b1 = xc[2] + xc[6], xc[2] - xc[6]
                    c0, c1 = xc[1] + xc[5], xc[1] - xc[5]
                    d0, d1_ = xc[3] + xc[7], xc[3] - xc[7]
                    p, q = a0 + b0, c0 + d0
                    y0, y4 = p + q, p - q
                    y2r, y2i = a0 - b0, d0 - c0
                    cm_, cp_ = RS * (c1 - d1_), RS * (c1 + d1_)
                    y1r, y1i = a1 + cm_, -b1 - cp_
                    y3r, y3i = a1 - cm_, b1 - cp_
                    for t, (yr, yi) in enumerate([(y1r, y1i), (y2r, y2i), (y3r, y3i), (y0, y4)]):
                        Y[half, t, 16 * ch_:16 * ch_ + 16, :] = jnp.concatenate([yr, yi], axis=1).astype(bf16)

            Ms = {}
            zs = {}

            def stage_a(u):
                half, t = divmod(u, 5)
                if t < 4:
                    o = lax.dot_general(G[t], Y[half, t], NT, preferred_element_type=f32)
                    zs[u] = jnp.concatenate([o[:128], o[128:]], axis=1).astype(bf16)
                else:
                    zs[u] = lax.dot_general(misc[2, 0:16, :], Y[half, 3, :, 0:128], NT,
                                            preferred_element_type=f32).astype(bf16)

            def stage_b(u):
                half, t = divmod(u, 5)
                a = 2 * m + half
                if half not in Ms:
                    Ms[half] = getM(a)
                Mx = Ms[half]
                if t < 4:
                    X = jnp.dot(zs.pop(u), Mx, preferred_element_type=f32)
                    Zr[a, 128 * t:128 * t + 128, :] = X[:, 0:128]
                    Zi[a, 128 * t:128 * t + 128, :] = X[:, 128:256]
                else:
                    Xn = jnp.dot(zs.pop(u), Mx[0:128, :], preferred_element_type=f32)
                    Zr[a, 512:528, :] = Xn[:, 0:128]
                    Zi[a, 512:528, :] = Xn[:, 128:256]

            d1(0)
            stage_a(0)
            stage_a(1)
            d1(1)
            for u in range(10):
                if u + 2 < 10:
                    stage_b(u)
                    stage_a(u + 2)
                else:
                    stage_b(u)
            return 0

        lax.fori_loop(0, 8, phF, 0)

        for k in range(16):
            for c in wblk(k):
                c.wait()
        for c in wny:
            c.wait()
        wr32 = wr.bitcast(u32)
        wi32 = wi.bitcast(u32)
        hi = jnp.uint32(HI)
        dcr = jnp.concatenate([_bc(wr32[k, 0:1, :] << 16, f32) for k in range(16)], axis=0)
        dci = jnp.concatenate([_bc(wi32[k, 0:1, :] << 16, f32) for k in range(16)], axis=0)
        nyr = jnp.concatenate([wrn[:, 128 * k:128 * (k + 1)].astype(f32) for k in range(16)], axis=0)
        nyi = jnp.concatenate([win[:, 128 * k:128 * (k + 1)].astype(f32) for k in range(16)], axis=0)
        st = jnp.concatenate([dcr, dci, nyr, nyi], axis=0)
        stb = st.astype(bf16)
        r1 = jnp.dot(stb, misc[0], preferred_element_type=f32)
        r2 = jnp.dot(stb, misc[1], preferred_element_type=f32)
        rr = jnp.concatenate([r1, r2], axis=0).astype(bf16)
        rp = jnp.dot(misc[2, 64:128, :], rr, preferred_element_type=f32)
        rid = lax.broadcasted_iota(jnp.int32, (64, 128), 0)
        sgn = jnp.where((rid & 16) == 0, 0.5, -0.5)
        WS[...] = 0.5 * st + sgn * rp

        POS = {1: 0, 7: 64, 2: 128, 6: 192, 3: 256, 5: 320, 0: 384, 4: 448}
        row8 = lax.broadcasted_iota(jnp.int32, (8, 128), 0)

        def mid(r, g, special):
            r0 = POS[r] + 8 * g
            if not special:
                r0 = pl.multiple_of(r0, 8)
            xs_ = [(Zr[a, pl.ds(r0, 8), :], Zi[a, pl.ds(r0, 8), :]) for a in range(16)]
            o = _fft16(xs_, False)
            if special:
                xn = [(Zr[a, 512:520, :], Zi[a, 512:520, :]) for a in range(16)]
                on = _fft16(xn, False)
                wsr, wsi = wr32, wi32
            else:
                g32 = pl.multiple_of(32 * g, 32)
                wsr = wr32.at[:, pl.ds(g32, 32), :]
                wsi = wi32.at[:, pl.ds(g32, 32), :]
            ys = []
            for k in range(16):
                a_ = wsr[k, pl.ds(r // 2, 8, stride=4), :]
                b_ = wsi[k, pl.ds(r // 2, 8, stride=4), :]
                if r % 2 == 0:
                    wre, wim = _bc(a_ << 16, f32), _bc(b_ << 16, f32)
                else:
                    wre, wim = _bc(a_ & hi, f32), _bc(b_ & hi, f32)
                if special:
                    wre = jnp.where(row8 == 0, jnp.broadcast_to(WS[k:k + 1, :], (8, 128)), wre)
                    wim = jnp.where(row8 == 0, jnp.broadcast_to(WS[16 + k:17 + k, :], (8, 128)), wim)
                xr, xi = o[k]
                yr = xr * wre - xi * wim
                yi = xr * wim + xi * wre
                if special:
                    nr = jnp.broadcast_to(WS[32 + k:33 + k, :], (8, 128))
                    ni = jnp.broadcast_to(WS[48 + k:49 + k, :], (8, 128))
                    zr_, zi_ = on[k]
                    yr = yr - (zr_ * ni + zi_ * nr)
                    yi = yi + (zr_ * nr - zi_ * ni)
                ys.append((yr, yi))
            u = _fft16(ys, True)
            for a in range(16):
                Zr[a, pl.ds(r0, 8), :] = u[a][0]
                Zi[a, pl.ds(r0, 8), :] = u[a][1]

        mid(0, 0, True)

        def phM(g, _):
            start_m(g)
            for r in range(1, 8):
                mid(r, g, False)

            @pl.when(g > 0)
            def _():
                mid(0, g, False)

            return 0

        lax.fori_loop(0, 8, phM, 0)

        def phI(m, _):
            start_i(m)
            Ms = {}
            vs = {}

            def stage_a(u):
                half, t = divmod(u, 4)
                a = 2 * m + half
                if half not in Ms:
                    Ms[half] = getM(a)
                yy = jnp.concatenate(
                    [Zr[a, 128 * t:128 * t + 128, :], Zi[a, 128 * t:128 * t + 128, :]], axis=1).astype(bf16)
                o = lax.dot_general(Ms[half], yy, NT, preferred_element_type=f32)
                vs[u] = jnp.concatenate([o[:128], o[128:]], axis=1).astype(bf16)

            def stage_b(u):
                half, t = divmod(u, 4)
                PQ[half, t] = jnp.dot(vs.pop(u), G[t if t < 3 else 4], preferred_element_type=f32)

            def d1inv(half):
                for ch_ in range(8):
                    rs = slice(16 * ch_, 16 * ch_ + 16)
                    P1, Q1 = PQ[half, 0, rs, 0:128], PQ[half, 0, rs, 128:256]
                    P2, Q2 = PQ[half, 1, rs, 0:128], PQ[half, 1, rs, 128:256]
                    P3, Q3 = PQ[half, 2, rs, 0:128], PQ[half, 2, rs, 128:256]
                    h0, h4 = PQ[half, 3, rs, 0:128], PQ[half, 3, rs, 128:256]
                    e, o_ = h0 + h4, h0 - h4
                    A, B = P1 + P3, Q1 - Q3
                    u_, v = P1 - P3, Q1 + Q3
                    T1_, T2_ = RS * (u_ - v), RS * (-u_ - v)
                    e1, e2 = e + P2, e - P2
                    o1, o2 = o_ - Q2, o_ + Q2
                    cols = jnp.concatenate(
                        [e1 + A, o1 + T1_, e2 - B, o2 + T2_, e1 - A, o1 - T1_, e2 + B, o2 - T2_], axis=1)
                    bits = _bc(cols.astype(bf16).astype(f32), u32)
                    if half == 0:
                        bs[m, rs, :] = bits >> 16
                    else:
                        bs[m, rs, :] = bs[m, rs, :] | bits

            stage_a(0)
            stage_a(1)
            for u in range(8):
                stage_b(u)
                if u + 2 < 8:
                    stage_a(u + 2)
                if u == 4:
                    d1inv(0)
            d1inv(1)
            return 0

        lax.fori_loop(0, 8, phI, 0)

    pl.run_scoped(
        scoped,
        pltpu.VMEM((8, 128, D), u32), pltpu.VMEM((16, 512, 128), bf16), pltpu.VMEM((16, 512, 128), bf16),
        pltpu.VMEM((1, S), bf16), pltpu.VMEM((1, S), bf16),
        pltpu.VMEM((5, 256, 256), bf16), pltpu.VMEM((16, 256, 128), bf16), pltpu.VMEM((3, 128, 128), bf16),
        pltpu.VMEM((2, 4, 128, 256), bf16), pltpu.VMEM((16, 528, 128), f32), pltpu.VMEM((16, 528, 128), f32),
        pltpu.VMEM((64, 128), f32), pltpu.VMEM((2, 4, 128, 256), f32))


def _kernel(x_hbm, mem0_hbm, wq_hbm, wk_hbm, wv_hbm, wo_hbm, xb_hbm, wr_hbm, wi_hbm, gw_hbm,
            g_hbm, h_hbm, misc_hbm, out_hbm,
            xv, xpre, mem0v, gwv, raw, wo, bs, bnat, gbuf, outb, bsems, wsems, msems, osem):
    cp_x = pltpu.make_async_copy(x_hbm.bitcast(u32), xv, msems.at[0])
    cp_mem = pltpu.make_async_copy(mem0_hbm, mem0v, msems.at[2])
    cp_gw = pltpu.make_async_copy(gw_hbm, gwv, msems.at[3])
    wsrc = [w.bitcast(u32) for w in (wq_hbm, wk_hbm, wv_hbm)]
    wo32 = wo_hbm.bitcast(u32)

    def cp_w(p):
        return [pltpu.make_async_copy(wsrc[i].at[:, p, :], raw.at[p, i], wsems.at[p]) for i in range(3)]

    def cp_wo(j):
        off = 128 * j if isinstance(j, int) else pl.multiple_of(128 * j, 128)
        return pltpu.make_async_copy(wo32.at[:, :, pl.ds(off, 128)], wo.at[j], msems.at[4])

    def start_m(g):
        @pl.when(g == 0)
        def _():
            cp_gw.start()
            cp_mem.start()
            cp_x.start()

        for c in cp_w(g):
            c.start()

    def start_i(m):
        for c in cp_w(m + 8):
            c.start()

    _b_phase(xb_hbm, wr_hbm, wi_hbm, g_hbm, h_hbm, misc_hbm, bs, bsems, start_m, start_i)
    bn32 = bnat.bitcast(u32)

    def a_phase(w3, pre, oc, ocr, acc, lhs):
        cp_x.wait()
        cp_gw.wait()
        gwf = gwv[...].astype(f32).reshape(1, D)
        for i in range(32):
            xpre[8 * i:8 * i + 8, :] = jnp.concatenate(
                [xv[32 * i + 12:32 * i + 16, :], xv[32 * i + 28:32 * i + 32, :]], axis=0)

        def prebulk(p, _):
            @pl.when(p < 8)
            def _():
                cp_wo(p).start()

            for i in range(3):
                pltpu.make_async_copy(wsrc[i].at[:, 0, :], raw.at[p, i], wsems.at[p]).wait()
            for i in range(3):
                e = raw[p, i, pl.ds(0, 512, stride=2), :]
                o = raw[p, i, pl.ds(1, 512, stride=2), :]
                w3[p, 0, i] = (e & jnp.uint32(0xFFFF)) | (o << 16)
                w3[p, 1, i] = (e >> 16) | (o & jnp.uint32(HI))
            for r in range(2):
                for i in range(3):
                    for c in range(2):
                        xl = _w2b(xpre[128 * c:128 * c + 128, :])
                        pre[p, r, i, 256 * c:256 * c + 256, :] = jnp.dot(
                            xl, _w2b(w3[p, r, i]), preferred_element_type=f32)
            for c in range(8):
                xw = xv[pl.ds(pl.multiple_of(64 * p + 8 * c, 8), 8), :]
                xx = _w2b(xw).astype(f32) * gwf
                part = xx[:, 0:128]
                for jj in range(1, 8):
                    part = part + xx[:, 128 * jj:128 * jj + 128]
                lg = jnp.sum(part, axis=1, keepdims=True)
                gbuf[pl.ds(pl.multiple_of(128 * p + 16 * c, 16), 16), :] = jnp.broadcast_to(
                    jax.nn.sigmoid(lg), (16, 128))
            for jj in range(8):
                dst = bn32.at[jj, pl.ds(pl.multiple_of(64 * p, 64), 64), :]
                for m in range(8):
                    dst[pl.ds(m, 8, stride=8), :] = bs[m, pl.ds(pl.multiple_of(8 * p, 8), 8), 128 * jj:128 * jj + 128]
            return 0

        lax.fori_loop(0, 16, prebulk, 0)
        cp_mem.wait()
        for j in range(8):
            cp_wo(j).wait()
        oc[...] = jnp.zeros(oc.shape, bf16)
        oc32 = oc.bitcast(u32)

        row = lax.broadcasted_iota(jnp.int32, (40, 128), 0)
        col = lax.broadcasted_iota(jnp.int32, (40, 128), 1)
        mask = ((col < 40) & (row >= 32)) | ((row < 32) & ((col <= row) | ((col >= 32) & (col < 40))))
        scale = DH ** -0.5
        bscale = 2.0 ** -20

        def wo_t(j, h):
            return _w2b(wo[j, h])

        def mix(a, b, g):
            return g * a + (1.0 - g) * (b.astype(f32) * bscale)

        def fill_piece(gr, gw_, src, j, half, accs):
            hs = range(16 * half, 16 * half + 16)
            l = jnp.concatenate([_w2b(src[h]) for h in hs], axis=1)
            w = _w2b(wo[j, 16 * half:16 * half + 16].reshape(16 * 64, 128))
            c = jnp.dot(l, w, preferred_element_type=f32)
            if half == 0:
                return c
            c = c + accs
            for q in range(4):
                sg = 4 * gr + q
                b = bnat[j, pl.ds(pl.multiple_of(32 * sg + 24, 8), 8), :]
                g = gbuf[pl.ds(pl.multiple_of(32 * sg + 24, 8), 8), :]
                outb[pl.ds(pl.multiple_of(128 * gw_ + 32 * q + 24, 8), 8),
                     pl.ds(pl.multiple_of(128 * j, 128), 128)] = mix(c[8 * q:8 * q + 8], b, g).astype(bf16)
            return None

        def out_copy(gi):
            return pltpu.make_async_copy(
                outb.at[pl.ds(pl.multiple_of(128 * gi, 128), 128), :],
                out_hbm.at[pl.ds(pl.multiple_of(128 * gi, 128), 128), :], osem)

        def step(q4, mem, grp4):
            s = 4 * grp4 + q4
            r0 = pl.multiple_of(s * 16, 16)
            xs0 = _w2b(xv[pl.ds(r0, 8), :])
            xs1 = _w2b(xv[pl.ds(r0 + 8, 8), :])
            l1 = jnp.concatenate([xs1[0:8].astype(f32), mem], axis=0).astype(bf16)
            lhs[0:8, :] = pltpu.bitcast(xs0, u32)
            lhs[8:16, :] = pltpu.bitcast(l1, u32)
            grp = grp4 - 1
            gr = jnp.maximum(grp, 0)
            gw_ = jnp.where(grp < 0, 16, grp)
            st = {}
            z8 = jnp.zeros((8, 128), f32)
            s8 = pl.multiple_of(s * 8, 8)

            def proj(h, i):
                r = jnp.dot(_w2b(lhs[...]), _w2b(w3[h // 2, h % 2, i]), preferred_element_type=f32)
                p_ = pre[h // 2, h % 2, i, pl.ds(s8, 8), :]
                if i == 0:
                    st[("qkv", h, i)] = jnp.concatenate([r[0:24], p_, r[24:32]], axis=0)
                else:
                    st[("qkv", h, i)] = jnp.concatenate([r[0:24], p_, r[24:32], z8], axis=0).astype(bf16)

            def qk(h):
                q = st.pop(("qkv", h, 0))
                k = st.pop(("qkv", h, 1))
                sc = lax.dot_general(q, k, NT, preferred_element_type=f32) * scale
                sc = jnp.concatenate([sc, jnp.zeros((40, 80), f32)], axis=1)
                sc = jnp.where(mask, sc, -1e9)
                m = jnp.max(sc, axis=1, keepdims=True)
                e = jnp.exp(sc - m)
                p = e * (1.0 / jnp.sum(e, axis=1, keepdims=True))
                st[("p", h)] = p[:, :48]

            def pv(h):
                o = lax.dot_general(st.pop(("p", h)), st.pop(("qkv", h, 2)), NN, preferred_element_type=f32)
                st[("o", h)] = jnp.concatenate([o[0:24], o[32:40]], axis=0).astype(bf16)
                oc[h, pl.ds(pl.multiple_of(8 * q4, 8), 8), :] = o[24:32].astype(bf16)

            def oproj(h):
                w = jnp.concatenate([wo_t(j, h) for j in range(8)], axis=1)
                c = jnp.dot(st.pop(("o", h)), w, preferred_element_type=f32)
                if h == 0:
                    acc[...] = c
                else:
                    acc[...] += c

            ok = lambda h: 0 <= h < H
            for t in range(H + 4):
                if ok(t):
                    proj(t, 0)
                    proj(t, 1)
                if ok(t - 1):
                    qk(t - 1)
                if ok(t):
                    proj(t, 2)
                else:
                    jj, half = (t - H) // 2, (t - H) % 2
                    st["fill"] = fill_piece(gr, gw_, ocr, 2 * q4 + jj, half, st.get("fill"))
                if ok(t - 3):
                    pv(t - 3)
                if ok(t - 4):
                    oproj(t - 4)
            a = acc[...]
            rs = pl.multiple_of(32 * s, 32)
            b0 = jnp.concatenate([bnat[j, pl.ds(rs, 16), :] for j in range(8)], axis=1)
            b1 = jnp.concatenate([bnat[j, pl.ds(rs + 16, 8), :] for j in range(8)], axis=1)
            g0 = gbuf[pl.ds(rs, 16), :]
            g1 = gbuf[pl.ds(rs + 16, 8), :]
            outb[pl.ds(rs, 16), :] = mix(a[0:16], b0, jnp.tile(g0, (1, 8))).astype(bf16)
            outb[pl.ds(rs + 16, 8), :] = mix(a[16:24], b1, jnp.tile(g1, (1, 8))).astype(bf16)
            return a[24:32]

        def group(grp4, mem):
            @pl.when(grp4 >= 2)
            def _():
                out_copy(grp4 - 2).start()

            ocr[...] = oc32[...]
            for q4 in range(4):
                mem = step(q4, mem, grp4)
            return mem

        lax.fori_loop(0, NSEG // 4, group, mem0v[...].astype(f32))

        out_copy(14).start()

        def tail_copy(j):
            return pltpu.make_async_copy(outb.at[pl.ds(S - 128, 128), pl.ds(128 * j, 128)],
                                         out_hbm.at[pl.ds(S - 128, 128), pl.ds(128 * j, 128)], osem)

        for j in range(8):
            c = fill_piece(15, 15, oc32, j, 0, None)
            fill_piece(15, 15, oc32, j, 1, c)
            tail_copy(j).start()
        for gi in range(15):
            out_copy(gi).wait()
        for j in range(8):
            tail_copy(j).wait()

    pl.run_scoped(
        a_phase,
        pltpu.VMEM((16, 2, 3, 512, 128), u32), pltpu.VMEM((16, 2, 3, 512, 128), f32),
        pltpu.VMEM((H, 32, 128), bf16), pltpu.VMEM((H, 16, 128), u32), pltpu.VMEM((32, D), f32), pltpu.VMEM((16, D), u32))


@jax.jit
def pallas_gated_mix__memory_aug_recurrent_mem_tr__spectral_gfnet__prompt_kernel(
    A_x, A_mem0, A_Wq, A_Wk, A_Wv, A_Wo, A_seg_len, B_x, B_w_r, B_w_i, gate_w,
):
    del A_seg_len
    del B_x
    HB = pl.BlockSpec(memory_space=pltpu.HBM)
    out = pl.pallas_call(
        _kernel,
        out_shape=jax.ShapeDtypeStruct((S, D), bf16),
        in_specs=[HB] * 13,
        out_specs=HB,
        scratch_shapes=[
            pltpu.VMEM((S // 2, D), u32),
            pltpu.VMEM((NSEG * 4, D), u32),
            pltpu.VMEM((M_MEM, D), bf16),
            pltpu.VMEM((D,), bf16),
            pltpu.VMEM((16, 3, D, DH), u32),
            pltpu.VMEM((8, H, DH // 2, 128), u32),
            pltpu.VMEM((8, 128, D), u32),
            pltpu.VMEM((8, S, 128), bf16),
            pltpu.VMEM((S, 128), f32),
            pltpu.VMEM((S + 128, D), bf16),
            pltpu.SemaphoreType.DMA((21,)),
            pltpu.SemaphoreType.DMA((16,)),
            pltpu.SemaphoreType.DMA((6,)),
            pltpu.SemaphoreType.DMA(()),
        ],
        compiler_params=pltpu.CompilerParams(vmem_limit_bytes=124 * 2 ** 20),
    )(
        A_x.reshape(S, D), A_mem0.reshape(M_MEM, D), A_Wq, A_Wk, A_Wv, A_Wo,
        A_x.reshape(128, 16, D), B_w_r.T, B_w_i.T, gate_w, _TAB_G, _TAB_H, _TAB_MISC,
    )
    return out.reshape(1, S, D)
```

```python
import numpy as np
import ml_dtypes
import jax
import jax.numpy as jnp
from jax import lax
import jax.experimental.pallas as pl
import jax.experimental.pallas.tpu as pltpu

f32, bf16, u32 = jnp.float32, jnp.bfloat16, jnp.uint32
S, D, H, DH, M_MEM, SEG = 2048, 1024, 32, 128, 8, 32
NSEG = S // SEG
RS = float(1 / np.sqrt(2))
NT = (((1,), (1,)), ((), ()))
NN = (((1,), (0,)), ((), ()))
HI = 0xFFFF0000


def _np_tables():
    bf = ml_dtypes.bfloat16
    dp = np.arange(128)
    j = np.arange(64)

    def cs(f):
        ang = 2 * np.pi * ((f[:, None] * dp[None, :]) % 1024) / 1024
        return np.cos(ang), np.sin(ang)

    G = np.zeros((5, 256, 256))
    for t in range(3):
        r = t + 1
        C, Sn = cs(r + 8 * j)
        C2, S2 = cs(8 - r + 8 * j)
        G[t, 0:64, 0:128] = C
        G[t, 0:64, 128:] = Sn
        G[t, 64:128, 0:128] = C2
        G[t, 64:128, 128:] = -S2
        G[t, 128:192, 0:128] = -Sn
        G[t, 128:192, 128:] = C
        G[t, 192:256, 0:128] = -S2
        G[t, 192:256, 128:] = -C2
    C0, S0 = cs(8 * j)
    C4, S4 = cs(4 + 8 * j)
    G[3, 0:64, 0:128] = C0
    G[3, 128:192, 0:128] = -S0
    G[3, 64:128, 128:] = C4
    G[3, 192:256, 128:] = -S4
    G[4] = G[3]
    G[4, 0, 0:128] = 0.5
    G[4, 128, 0:128] = 0.5 * (-1.0) ** dp
    HH = np.zeros((16, 256, 128))
    for a in range(16):
        ang = 2 * np.pi * (((a + 16 * dp)[:, None] * dp[None, :]) % 2048) / 2048
        HH[a, :128] = np.cos(ang)
        HH[a, 128:] = np.sin(ang)
    misc = np.zeros((3, 128, 128))
    misc[0, 128 - dp[1:], dp[1:]] = 1
    misc[1, 0, 0] = 1
    misc[2, 0, :] = (-1.0) ** dp
    for blk in range(4):
        for k1 in range(16):
            misc[2, 64 + 16 * blk + k1, 16 * blk + 15 - k1] = 1
            misc[2, 64 + 16 * blk + k1, 64 + 16 * blk + (16 - k1) % 16] = 1
    return G.astype(bf), HH.astype(bf), misc.astype(bf)


_TAB_G, _TAB_H, _TAB_MISC = _np_tables()


def _bc(x, dt):
    return lax.bitcast_convert_type(x, dt)


def _w2b(w):
    return pltpu.bitcast(w, bf16)


def _fft16(xs, inverse):
    sg = 1.0 if inverse else -1.0

    def dft4(a, b, c, d):
        t0 = (a[0] + c[0], a[1] + c[1])
        t1 = (a[0] - c[0], a[1] - c[1])
        t2 = (b[0] + d[0], b[1] + d[1])
        t3 = (b[0] - d[0], b[1] - d[1])
        o0 = (t0[0] + t2[0], t0[1] + t2[1])
        o2 = (t0[0] - t2[0], t0[1] - t2[1])
        m = (t1[0] + t3[1], t1[1] - t3[0])
        p = (t1[0] - t3[1], t1[1] + t3[0])
        return [o0, p, o2, m] if inverse else [o0, m, o2, p]

    t = [dft4(xs[a0], xs[4 + a0], xs[8 + a0], xs[12 + a0]) for a0 in range(4)]

    def tw(v, e):
        e = e % 16
        if e == 0:
            return v
        if e == 4:
            return (-v[1], v[0]) if inverse else (v[1], -v[0])
        if e == 2:
            if inverse:
                return ((v[0] - v[1]) * RS, (v[0] + v[1]) * RS)
            return ((v[0] + v[1]) * RS, (v[1] - v[0]) * RS)
        if e == 6:
            if inverse:
                return ((-v[0] - v[1]) * RS, (v[0] - v[1]) * RS)
            return ((v[1] - v[0]) * RS, (-v[0] - v[1]) * RS)
        c = float(np.cos(2 * np.pi * e / 16))
        s = float(sg * np.sin(2 * np.pi * e / 16))
        return (v[0] * c - v[1] * s, v[0] * s + v[1] * c)

    out = [None] * 16
    for k in range(4):
        u = [tw(t[a0][k], a0 * k) for a0 in range(4)]
        r = dft4(*u)
        for m in range(4):
            out[k + 4 * m] = r[m]
    return out


def _b_phase(xb_hbm, wr_hbm, wi_hbm, g_hbm, h_hbm, misc_hbm, bs, sems, start_m, start_i):
    def scoped(xs, wr, wi, wrn, win, G, HH, misc, Y, Zr, Zi, WS, PQ):
        xb32 = xb_hbm.bitcast(u32)
        xcp = [pltpu.make_async_copy(xb32.at[:, m, :], xs.at[m], sems.at[m]) for m in range(8)]
        cg = pltpu.make_async_copy(g_hbm, G, sems.at[8])

        def chh(m):
            return pltpu.make_async_copy(h_hbm.at[pl.ds(2 * m, 2)], HH.at[pl.ds(2 * m, 2)], sems.at[13 + m])

        cm = pltpu.make_async_copy(misc_hbm, misc, sems.at[10])
        def wblk(k):
            off = 128 * k if isinstance(k, int) else pl.multiple_of(128 * k, 128)
            return (pltpu.make_async_copy(wr_hbm.at[pl.ds(0, 512), pl.ds(off, 128)], wr.at[k], sems.at[11]),
                    pltpu.make_async_copy(wi_hbm.at[pl.ds(0, 512), pl.ds(off, 128)], wi.at[k], sems.at[12]))

        wny = (pltpu.make_async_copy(wr_hbm.at[pl.ds(512, 1), :], wrn, sems.at[11]),
               pltpu.make_async_copy(wi_hbm.at[pl.ds(512, 1), :], win, sems.at[12]))
        xcp[0].start()
        cg.start()
        chh(0).start()
        cm.start()
        for m in range(1, 8):
            xcp[m].start()
            chh(m).start()
        for c in wny:
            c.start()
        cg.wait()
        cm.wait()

        def getM(a):
            hc = HH[a, 0:128, :]
            hs = HH[a, 128:256, :]
            return jnp.concatenate(
                [jnp.concatenate([hc, -hs], axis=1), jnp.concatenate([hs, hc], axis=1)], axis=0)

        def phF(m, _):
            for k in (2 * m, 2 * m + 1):
                for c in wblk(k):
                    c.start()
            pltpu.make_async_copy(xb32.at[:, 0, :], xs.at[m], sems.at[m]).wait()
            chh(m).wait()
            def d1(half):
                for ch_ in range(8):
                    w = xs[m, 16 * ch_:16 * ch_ + 16, :]
                    xv = _bc(w << 16, f32) if half == 0 else _bc(w & jnp.uint32(HI), f32)
                    xc = [xv[:, 128 * c:128 * (c + 1)] for c in range(8)]
                    a0, a1 = xc[0] + xc[4], xc[0] - xc[4]
                    b0, b1 = xc[2] + xc[6], xc[2] - xc[6]
                    c0, c1 = xc[1] + xc[5], xc[1] - xc[5]
                    d0, d1_ = xc[3] + xc[7], xc[3] - xc[7]
                    p, q = a0 + b0, c0 + d0
                    y0, y4 = p + q, p - q
                    y2r, y2i = a0 - b0, d0 - c0
                    cm_, cp_ = RS * (c1 - d1_), RS * (c1 + d1_)
                    y1r, y1i = a1 + cm_, -b1 - cp_
                    y3r, y3i = a1 - cm_, b1 - cp_
                    for t, (yr, yi) in enumerate([(y1r, y1i), (y2r, y2i), (y3r, y3i), (y0, y4)]):
                        Y[half, t, 16 * ch_:16 * ch_ + 16, :] = jnp.concatenate([yr, yi], axis=1).astype(bf16)

            Ms = {}
            zs = {}

            def stage_a(u):
                half, t = divmod(u, 5)
                if t < 4:
                    o = lax.dot_general(G[t], Y[half, t], NT, preferred_element_type=f32)
                    zs[u] = jnp.concatenate([o[:128], o[128:]], axis=1).astype(bf16)
                else:
                    zs[u] = lax.dot_general(misc[2, 0:16, :], Y[half, 3, :, 0:128], NT,
                                            preferred_element_type=f32).astype(bf16)

            def stage_b(u):
                half, t = divmod(u, 5)
                a = 2 * m + half
                if half not in Ms:
                    Ms[half] = getM(a)
                Mx = Ms[half]
                if t < 4:
                    X = jnp.dot(zs.pop(u), Mx, preferred_element_type=f32)
                    Zr[a, 128 * t:128 * t + 128, :] = X[:, 0:128]
                    Zi[a, 128 * t:128 * t + 128, :] = X[:, 128:256]
                else:
                    Xn = jnp.dot(zs.pop(u), Mx[0:128, :], preferred_element_type=f32)
                    Zr[a, 512:528, :] = Xn[:, 0:128]
                    Zi[a, 512:528, :] = Xn[:, 128:256]

            d1(0)
            stage_a(0)
            stage_a(1)
            d1(1)
            for u in range(10):
                if u + 2 < 10:
                    stage_b(u)
                    stage_a(u + 2)
                else:
                    stage_b(u)
            return 0

        lax.fori_loop(0, 8, phF, 0)

        for k in range(16):
            for c in wblk(k):
                c.wait()
        for c in wny:
            c.wait()
        wr32 = wr.bitcast(u32)
        wi32 = wi.bitcast(u32)
        hi = jnp.uint32(HI)
        dcr = jnp.concatenate([_bc(wr32[k, 0:1, :] << 16, f32) for k in range(16)], axis=0)
        dci = jnp.concatenate([_bc(wi32[k, 0:1, :] << 16, f32) for k in range(16)], axis=0)
        nyr = jnp.concatenate([wrn[:, 128 * k:128 * (k + 1)].astype(f32) for k in range(16)], axis=0)
        nyi = jnp.concatenate([win[:, 128 * k:128 * (k + 1)].astype(f32) for k in range(16)], axis=0)
        st = jnp.concatenate([dcr, dci, nyr, nyi], axis=0)
        stb = st.astype(bf16)
        r1 = jnp.dot(stb, misc[0], preferred_element_type=f32)
        r2 = jnp.dot(stb, misc[1], preferred_element_type=f32)
        rr = jnp.concatenate([r1, r2], axis=0).astype(bf16)
        rp = jnp.dot(misc[2, 64:128, :], rr, preferred_element_type=f32)
        rid = lax.broadcasted_iota(jnp.int32, (64, 128), 0)
        sgn = jnp.where((rid & 16) == 0, 0.5, -0.5)
        WS[...] = 0.5 * st + sgn * rp

        POS = {1: 0, 7: 64, 2: 128, 6: 192, 3: 256, 5: 320, 0: 384, 4: 448}
        row8 = lax.broadcasted_iota(jnp.int32, (8, 128), 0)

        def mid(r, g, special):
            r0 = POS[r] + 8 * g
            if not special:
                r0 = pl.multiple_of(r0, 8)
            xs_ = [(Zr[a, pl.ds(r0, 8), :], Zi[a, pl.ds(r0, 8), :]) for a in range(16)]
            o = _fft16(xs_, False)
            if special:
                xn = [(Zr[a, 512:520, :], Zi[a, 512:520, :]) for a in range(16)]
                on = _fft16(xn, False)
                wsr, wsi = wr32, wi32
            else:
                g32 = pl.multiple_of(32 * g, 32)
                wsr = wr32.at[:, pl.ds(g32, 32), :]
                wsi = wi32.at[:, pl.ds(g32, 32), :]
            ys = []
            for k in range(16):
                a_ = wsr[k, pl.ds(r // 2, 8, stride=4), :]
                b_ = wsi[k, pl.ds(r // 2, 8, stride=4), :]
                if r % 2 == 0:
                    wre, wim = _bc(a_ << 16, f32), _bc(b_ << 16, f32)
                else:
                    wre, wim = _bc(a_ & hi, f32), _bc(b_ & hi, f32)
                if special:
                    wre = jnp.where(row8 == 0, jnp.broadcast_to(WS[k:k + 1, :], (8, 128)), wre)
                    wim = jnp.where(row8 == 0, jnp.broadcast_to(WS[16 + k:17 + k, :], (8, 128)), wim)
                xr, xi = o[k]
                yr = xr * wre - xi * wim
                yi = xr * wim + xi * wre
                if special:
                    nr = jnp.broadcast_to(WS[32 + k:33 + k, :], (8, 128))
                    ni = jnp.broadcast_to(WS[48 + k:49 + k, :], (8, 128))
                    zr_, zi_ = on[k]
                    yr = yr - (zr_ * ni + zi_ * nr)
                    yi = yi + (zr_ * nr - zi_ * ni)
                ys.append((yr, yi))
            u = _fft16(ys, True)
            for a in range(16):
                Zr[a, pl.ds(r0, 8), :] = u[a][0]
                Zi[a, pl.ds(r0, 8), :] = u[a][1]

        mid(0, 0, True)

        def phM(g, _):
            start_m(g)
            for r in range(1, 8):
                mid(r, g, False)

            @pl.when(g > 0)
            def _():
                mid(0, g, False)

            return 0

        lax.fori_loop(0, 8, phM, 0)

        def phI(m, _):
            start_i(m)
            Ms = {}
            vs = {}

            def stage_a(u):
                half, t = divmod(u, 4)
                a = 2 * m + half
                if half not in Ms:
                    Ms[half] = getM(a)
                yy = jnp.concatenate(
                    [Zr[a, 128 * t:128 * t + 128, :], Zi[a, 128 * t:128 * t + 128, :]], axis=1).astype(bf16)
                o = lax.dot_general(Ms[half], yy, NT, preferred_element_type=f32)
                vs[u] = jnp.concatenate([o[:128], o[128:]], axis=1).astype(bf16)

            def stage_b(u):
                half, t = divmod(u, 4)
                PQ[half, t] = jnp.dot(vs.pop(u), G[t if t < 3 else 4], preferred_element_type=f32)

            def d1inv(half):
                for ch_ in range(8):
                    rs = slice(16 * ch_, 16 * ch_ + 16)
                    P1, Q1 = PQ[half, 0, rs, 0:128], PQ[half, 0, rs, 128:256]
                    P2, Q2 = PQ[half, 1, rs, 0:128], PQ[half, 1, rs, 128:256]
                    P3, Q3 = PQ[half, 2, rs, 0:128], PQ[half, 2, rs, 128:256]
                    h0, h4 = PQ[half, 3, rs, 0:128], PQ[half, 3, rs, 128:256]
                    e, o_ = h0 + h4, h0 - h4
                    A, B = P1 + P3, Q1 - Q3
                    u_, v = P1 - P3, Q1 + Q3
                    T1_, T2_ = RS * (u_ - v), RS * (-u_ - v)
                    e1, e2 = e + P2, e - P2
                    o1, o2 = o_ - Q2, o_ + Q2
                    cols = jnp.concatenate(
                        [e1 + A, o1 + T1_, e2 - B, o2 + T2_, e1 - A, o1 - T1_, e2 + B, o2 - T2_], axis=1)
                    bits = _bc(cols.astype(bf16).astype(f32), u32)
                    if half == 0:
                        bs[m, rs, :] = bits >> 16
                    else:
                        bs[m, rs, :] = bs[m, rs, :] | bits

            stage_a(0)
            stage_a(1)
            for u in range(8):
                stage_b(u)
                if u + 2 < 8:
                    stage_a(u + 2)
                if u == 4:
                    d1inv(0)
            d1inv(1)
            return 0

        lax.fori_loop(0, 8, phI, 0)

    pl.run_scoped(
        scoped,
        pltpu.VMEM((8, 128, D), u32), pltpu.VMEM((16, 512, 128), bf16), pltpu.VMEM((16, 512, 128), bf16),
        pltpu.VMEM((1, S), bf16), pltpu.VMEM((1, S), bf16),
        pltpu.VMEM((5, 256, 256), bf16), pltpu.VMEM((16, 256, 128), bf16), pltpu.VMEM((3, 128, 128), bf16),
        pltpu.VMEM((2, 4, 128, 256), bf16), pltpu.VMEM((16, 528, 128), f32), pltpu.VMEM((16, 528, 128), f32),
        pltpu.VMEM((64, 128), f32), pltpu.VMEM((2, 4, 128, 256), f32))


def _kernel(x_hbm, mem0_hbm, wq_hbm, wk_hbm, wv_hbm, wo_hbm, xb_hbm, wr_hbm, wi_hbm, gw_hbm,
            g_hbm, h_hbm, misc_hbm, out_hbm,
            xv, xpre, mem0v, gwv, raw, wo, bs, bnat, gbuf, outb, bsems, wsems, msems, osem):
    cp_x = pltpu.make_async_copy(x_hbm.bitcast(u32), xv, msems.at[0])
    cp_mem = pltpu.make_async_copy(mem0_hbm, mem0v, msems.at[2])
    cp_gw = pltpu.make_async_copy(gw_hbm, gwv, msems.at[3])
    wsrc = [w.bitcast(u32) for w in (wq_hbm, wk_hbm, wv_hbm)]
    wo32 = wo_hbm.bitcast(u32)

    def cp_w(p):
        return [pltpu.make_async_copy(wsrc[i].at[:, p, :], raw.at[p, i], wsems.at[p]) for i in range(3)]

    def cp_wo(j):
        off = 128 * j if isinstance(j, int) else pl.multiple_of(128 * j, 128)
        return pltpu.make_async_copy(wo32.at[:, :, pl.ds(off, 128)], wo.at[j], msems.at[4])

    def start_m(g):
        @pl.when(g == 0)
        def _():
            cp_gw.start()
            cp_mem.start()
            cp_x.start()

        for c in cp_w(g):
            c.start()

    def start_i(m):
        for c in cp_w(m + 8):
            c.start()

    _b_phase(xb_hbm, wr_hbm, wi_hbm, g_hbm, h_hbm, misc_hbm, bs, bsems, start_m, start_i)
    bn32 = bnat.bitcast(u32)

    def a_phase(w3, pre, oc, ocr, acc, lhs):
        cp_x.wait()
        cp_gw.wait()
        gwf = gwv[...].astype(f32).reshape(1, D)
        for i in range(32):
            xpre[8 * i:8 * i + 8, :] = jnp.concatenate(
                [xv[32 * i + 12:32 * i + 16, :], xv[32 * i + 28:32 * i + 32, :]], axis=0)

        def prebulk(p, _):
            @pl.when(p < 8)
            def _():
                cp_wo(p).start()

            for i in range(3):
                pltpu.make_async_copy(wsrc[i].at[:, 0, :], raw.at[p, i], wsems.at[p]).wait()
            for i in range(3):
                e = raw[p, i, pl.ds(0, 512, stride=2), :]
                o = raw[p, i, pl.ds(1, 512, stride=2), :]
                w3[p, 0, i] = (e & jnp.uint32(0xFFFF)) | (o << 16)
                w3[p, 1, i] = (e >> 16) | (o & jnp.uint32(HI))
            for r in range(2):
                for i in range(3):
                    for c in range(2):
                        xl = _w2b(xpre[128 * c:128 * c + 128, :])
                        pre[p, r, i, 256 * c:256 * c + 256, :] = jnp.dot(
                            xl, _w2b(w3[p, r, i]), preferred_element_type=f32)
            for c in range(8):
                xw = xv[pl.ds(pl.multiple_of(64 * p + 8 * c, 8), 8), :]
                xx = _w2b(xw).astype(f32) * gwf
                part = xx[:, 0:128]
                for jj in range(1, 8):
                    part = part + xx[:, 128 * jj:128 * jj + 128]
                lg = jnp.sum(part, axis=1, keepdims=True)
                gbuf[pl.ds(pl.multiple_of(128 * p + 16 * c, 16), 16), :] = jnp.broadcast_to(
                    jax.nn.sigmoid(lg), (16, 128))
            for jj in range(8):
                dst = bn32.at[jj, pl.ds(pl.multiple_of(64 * p, 64), 64), :]
                for m in range(8):
                    dst[pl.ds(m, 8, stride=8), :] = bs[m, pl.ds(pl.multiple_of(8 * p, 8), 8), 128 * jj:128 * jj + 128]
            return 0

        lax.fori_loop(0, 16, prebulk, 0)
        cp_mem.wait()
        for j in range(8):
            cp_wo(j).wait()
        oc[...] = jnp.zeros(oc.shape, bf16)
        oc32 = oc.bitcast(u32)

        row = lax.broadcasted_iota(jnp.int32, (40, 128), 0)
        col = lax.broadcasted_iota(jnp.int32, (40, 128), 1)
        mask = ((col < 40) & (row >= 32)) | ((row < 32) & ((col <= row) | ((col >= 32) & (col < 40))))
        scale = DH ** -0.5
        bscale = 2.0 ** -20

        def wo_t(j, h):
            return _w2b(wo[j, h])

        def mix(a, b, g):
            return g * a + (1.0 - g) * (b.astype(f32) * bscale)

        def fill_piece(gr, gw_, src, j, half, accs):
            hs = range(16 * half, 16 * half + 16)
            l = jnp.concatenate([_w2b(src[h]) for h in hs], axis=1)
            w = _w2b(wo[j, 16 * half:16 * half + 16].reshape(16 * 64, 128))
            c = jnp.dot(l, w, preferred_element_type=f32)
            if half == 0:
                return c
            c = c + accs
            for q in range(4):
                sg = 4 * gr + q
                b = bnat[j, pl.ds(pl.multiple_of(32 * sg + 24, 8), 8), :]
                g = gbuf[pl.ds(pl.multiple_of(32 * sg + 24, 8), 8), :]
                outb[pl.ds(pl.multiple_of(128 * gw_ + 32 * q + 24, 8), 8),
                     pl.ds(pl.multiple_of(128 * j, 128), 128)] = mix(c[8 * q:8 * q + 8], b, g).astype(bf16)
            return None

        def out_copy(gi):
            return pltpu.make_async_copy(
                outb.at[pl.ds(pl.multiple_of(128 * gi, 128), 128), :],
                out_hbm.at[pl.ds(pl.multiple_of(128 * gi, 128), 128), :], osem)

        def step(q4, mem, grp4):
            s = 4 * grp4 + q4
            r0 = pl.multiple_of(s * 16, 16)
            xs0 = _w2b(xv[pl.ds(r0, 8), :])
            xs1 = _w2b(xv[pl.ds(r0 + 8, 8), :])
            l1 = jnp.concatenate([xs1[0:8].astype(f32), mem], axis=0).astype(bf16)
            lhs[0:8, :] = pltpu.bitcast(xs0, u32)
            lhs[8:16, :] = pltpu.bitcast(l1, u32)
            grp = grp4 - 1
            gr = jnp.maximum(grp, 0)
            gw_ = jnp.where(grp < 0, 16, grp)
            st = {}
            z8 = jnp.zeros((8, 128), f32)
            s8 = pl.multiple_of(s * 8, 8)

            def proj(h, i):
                r = jnp.dot(_w2b(lhs[...]), _w2b(w3[h // 2, h % 2, i]), preferred_element_type=f32)
                p_ = pre[h // 2, h % 2, i, pl.ds(s8, 8), :]
                if i == 0:
                    st[("qkv", h, i)] = jnp.concatenate([r[0:24], p_, r[24:32]], axis=0)
                else:
                    st[("qkv", h, i)] = jnp.concatenate([r[0:24], p_, r[24:32], z8], axis=0).astype(bf16)

            def qk(h):
                q = st.pop(("qkv", h, 0))
                k = st.pop(("qkv", h, 1))
                sc = lax.dot_general(q, k, NT, preferred_element_type=f32) * scale
                sc = jnp.concatenate([sc, jnp.zeros((40, 80), f32)], axis=1)
                sc = jnp.where(mask, sc, -1e9)
                m = jnp.max(sc, axis=1, keepdims=True)
                e = jnp.exp(sc - m)
                p = e * (1.0 / jnp.sum(e, axis=1, keepdims=True))
                st[("p", h)] = p[:, :48]

            def pv(h):
                o = lax.dot_general(st.pop(("p", h)), st.pop(("qkv", h, 2)), NN, preferred_element_type=f32)
                st[("o", h)] = jnp.concatenate([o[0:24], o[32:40]], axis=0).astype(bf16)
                oc[h, pl.ds(pl.multiple_of(8 * q4, 8), 8), :] = o[24:32].astype(bf16)

            def oproj(h):
                w = jnp.concatenate([wo_t(j, h) for j in range(8)], axis=1)
                c = jnp.dot(st.pop(("o", h)), w, preferred_element_type=f32)
                if h == 0:
                    acc[...] = c
                else:
                    acc[...] += c

            ok = lambda h: 0 <= h < H
            for t in range(H + 4):
                if ok(t):
                    proj(t, 0)
                    proj(t, 1)
                if ok(t - 1):
                    qk(t - 1)
                if ok(t):
                    proj(t, 2)
                else:
                    jj, half = (t - H) // 2, (t - H) % 2
                    st["fill"] = fill_piece(gr, gw_, ocr, 2 * q4 + jj, half, st.get("fill"))
                if ok(t - 3):
                    pv(t - 3)
                if ok(t - 4):
                    oproj(t - 4)
            a = acc[...]
            rs = pl.multiple_of(32 * s, 32)
            b0 = jnp.concatenate([bnat[j, pl.ds(rs, 16), :] for j in range(8)], axis=1)
            b1 = jnp.concatenate([bnat[j, pl.ds(rs + 16, 8), :] for j in range(8)], axis=1)
            g0 = gbuf[pl.ds(rs, 16), :]
            g1 = gbuf[pl.ds(rs + 16, 8), :]
            outb[pl.ds(rs, 16), :] = mix(a[0:16], b0, jnp.tile(g0, (1, 8))).astype(bf16)
            outb[pl.ds(rs + 16, 8), :] = mix(a[16:24], b1, jnp.tile(g1, (1, 8))).astype(bf16)
            return a[24:32]

        def group(grp4, mem):
            @pl.when(grp4 >= 2)
            def _():
                out_copy(grp4 - 2).start()

            ocr[...] = oc32[...]
            for q4 in range(4):
                mem = step(q4, mem, grp4)
            return mem

        lax.fori_loop(0, NSEG // 4, group, mem0v[...].astype(f32))

        out_copy(14).start()

        def tail_copy(j):
            return pltpu.make_async_copy(outb.at[pl.ds(S - 128, 128), pl.ds(128 * j, 128)],
                                         out_hbm.at[pl.ds(S - 128, 128), pl.ds(128 * j, 128)], osem)

        for j in range(8):
            c = fill_piece(15, 15, oc32, j, 0, None)
            fill_piece(15, 15, oc32, j, 1, c)
            tail_copy(j).start()
        for gi in range(15):
            out_copy(gi).wait()
        for j in range(8):
            tail_copy(j).wait()

    pl.run_scoped(
        a_phase,
        pltpu.VMEM((16, 2, 3, 512, 128), u32), pltpu.VMEM((16, 2, 3, 512, 128), f32),
        pltpu.VMEM((H, 32, 128), bf16), pltpu.VMEM((H, 16, 128), u32), pltpu.VMEM((32, D), f32), pltpu.VMEM((16, D), u32))


@jax.jit
def pallas_gated_mix__memory_aug_recurrent_mem_tr__spectral_gfnet__prompt_kernel(
    A_x, A_mem0, A_Wq, A_Wk, A_Wv, A_Wo, A_seg_len, B_x, B_w_r, B_w_i, gate_w,
):
    del A_seg_len
    del B_x
    HB = pl.BlockSpec(memory_space=pltpu.HBM)
    out = pl.pallas_call(
        _kernel,
        out_shape=jax.ShapeDtypeStruct((S, D), bf16),
        in_specs=[HB] * 13,
        out_specs=HB,
        scratch_shapes=[
            pltpu.VMEM((S // 2, D), u32),
            pltpu.VMEM((NSEG * 4, D), u32),
            pltpu.VMEM((M_MEM, D), bf16),
            pltpu.VMEM((D,), bf16),
            pltpu.VMEM((16, 3, D, DH), u32),
            pltpu.VMEM((8, H, DH // 2, 128), u32),
            pltpu.VMEM((8, 128, D), u32),
            pltpu.VMEM((8, S, 128), bf16),
            pltpu.VMEM((S, 128), f32),
            pltpu.VMEM((S + 128, D), bf16),
            pltpu.SemaphoreType.DMA((21,)),
            pltpu.SemaphoreType.DMA((16,)),
            pltpu.SemaphoreType.DMA((6,)),
            pltpu.SemaphoreType.DMA(()),
        ],
        compiler_params=pltpu.CompilerParams(
            vmem_limit_bytes=124 * 2 ** 20, flags={"XLA_TPU_EVENLY_DISTRIBUTE_CRITICAL_NODES": True}),
    )(
        A_x.reshape(S, D), A_mem0.reshape(M_MEM, D), A_Wq, A_Wk, A_Wv, A_Wo,
        A_x.reshape(128, 16, D), B_w_r.T, B_w_i.T, gate_w, _TAB_G, _TAB_H, _TAB_MISC,
    )
    return out.reshape(1, S, D)
```

```python
import numpy as np
import ml_dtypes
import jax
import jax.numpy as jnp
from jax import lax
import jax.experimental.pallas as pl
import jax.experimental.pallas.tpu as pltpu

f32, bf16, u32 = jnp.float32, jnp.bfloat16, jnp.uint32
S, D, H, DH, M_MEM, SEG = 2048, 1024, 32, 128, 8, 32
NSEG = S // SEG
RS = float(1 / np.sqrt(2))
NT = (((1,), (1,)), ((), ()))
NN = (((1,), (0,)), ((), ()))
HI = 0xFFFF0000


def _np_tables():
    bf = ml_dtypes.bfloat16
    dp = np.arange(128)
    j = np.arange(64)

    def cs(f):
        ang = 2 * np.pi * ((f[:, None] * dp[None, :]) % 1024) / 1024
        return np.cos(ang), np.sin(ang)

    G = np.zeros((5, 256, 256))
    for t in range(3):
        r = t + 1
        C, Sn = cs(r + 8 * j)
        C2, S2 = cs(8 - r + 8 * j)
        G[t, 0:64, 0:128] = C
        G[t, 0:64, 128:] = Sn
        G[t, 64:128, 0:128] = C2
        G[t, 64:128, 128:] = -S2
        G[t, 128:192, 0:128] = -Sn
        G[t, 128:192, 128:] = C
        G[t, 192:256, 0:128] = -S2
        G[t, 192:256, 128:] = -C2
    C0, S0 = cs(8 * j)
    C4, S4 = cs(4 + 8 * j)
    G[3, 0:64, 0:128] = C0
    G[3, 128:192, 0:128] = -S0
    G[3, 64:128, 128:] = C4
    G[3, 192:256, 128:] = -S4
    G[4] = G[3]
    G[4, 0, 0:128] = 0.5
    G[4, 128, 0:128] = 0.5 * (-1.0) ** dp
    HH = np.zeros((16, 256, 128))
    for a in range(16):
        ang = 2 * np.pi * (((a + 16 * dp)[:, None] * dp[None, :]) % 2048) / 2048
        HH[a, :128] = np.cos(ang)
        HH[a, 128:] = np.sin(ang)
    misc = np.zeros((3, 128, 128))
    misc[0, 128 - dp[1:], dp[1:]] = 1
    misc[1, 0, 0] = 1
    misc[2, 0, :] = (-1.0) ** dp
    for blk in range(4):
        for k1 in range(16):
            misc[2, 64 + 16 * blk + k1, 16 * blk + 15 - k1] = 1
            misc[2, 64 + 16 * blk + k1, 64 + 16 * blk + (16 - k1) % 16] = 1
    return G.astype(bf), HH.astype(bf), misc.astype(bf)


_TAB_G, _TAB_H, _TAB_MISC = _np_tables()


def _bc(x, dt):
    return lax.bitcast_convert_type(x, dt)


def _w2b(w):
    return pltpu.bitcast(w, bf16)


def _fft16(xs, inverse):
    sg = 1.0 if inverse else -1.0

    def dft4(a, b, c, d):
        t0 = (a[0] + c[0], a[1] + c[1])
        t1 = (a[0] - c[0], a[1] - c[1])
        t2 = (b[0] + d[0], b[1] + d[1])
        t3 = (b[0] - d[0], b[1] - d[1])
        o0 = (t0[0] + t2[0], t0[1] + t2[1])
        o2 = (t0[0] - t2[0], t0[1] - t2[1])
        m = (t1[0] + t3[1], t1[1] - t3[0])
        p = (t1[0] - t3[1], t1[1] + t3[0])
        return [o0, p, o2, m] if inverse else [o0, m, o2, p]

    t = [dft4(xs[a0], xs[4 + a0], xs[8 + a0], xs[12 + a0]) for a0 in range(4)]

    def tw(v, e):
        e = e % 16
        if e == 0:
            return v
        if e == 4:
            return (-v[1], v[0]) if inverse else (v[1], -v[0])
        if e == 2:
            if inverse:
                return ((v[0] - v[1]) * RS, (v[0] + v[1]) * RS)
            return ((v[0] + v[1]) * RS, (v[1] - v[0]) * RS)
        if e == 6:
            if inverse:
                return ((-v[0] - v[1]) * RS, (v[0] - v[1]) * RS)
            return ((v[1] - v[0]) * RS, (-v[0] - v[1]) * RS)
        c = float(np.cos(2 * np.pi * e / 16))
        s = float(sg * np.sin(2 * np.pi * e / 16))
        return (v[0] * c - v[1] * s, v[0] * s + v[1] * c)

    out = [None] * 16
    for k in range(4):
        u = [tw(t[a0][k], a0 * k) for a0 in range(4)]
        r = dft4(*u)
        for m in range(4):
            out[k + 4 * m] = r[m]
    return out


def _b_phase(xb_hbm, wr_hbm, wi_hbm, g_hbm, h_hbm, misc_hbm, bs, sems, start_m, start_i):
    def scoped(xs, wr, wi, wrn, win, G, HH, misc, Y, Zr, Zi, WS, PQ):
        xb32 = xb_hbm.bitcast(u32)
        xcp = [pltpu.make_async_copy(xb32.at[:, m, :], xs.at[m], sems.at[m]) for m in range(8)]
        cg = pltpu.make_async_copy(g_hbm, G, sems.at[8])

        def chh(m):
            return pltpu.make_async_copy(h_hbm.at[pl.ds(2 * m, 2)], HH.at[pl.ds(2 * m, 2)], sems.at[13 + m])

        cm = pltpu.make_async_copy(misc_hbm, misc, sems.at[10])
        def wblk(k):
            off = 128 * k if isinstance(k, int) else pl.multiple_of(128 * k, 128)
            return (pltpu.make_async_copy(wr_hbm.at[pl.ds(0, 512), pl.ds(off, 128)], wr.at[k], sems.at[11]),
                    pltpu.make_async_copy(wi_hbm.at[pl.ds(0, 512), pl.ds(off, 128)], wi.at[k], sems.at[12]))

        wny = (pltpu.make_async_copy(wr_hbm.at[pl.ds(512, 1), :], wrn, sems.at[11]),
               pltpu.make_async_copy(wi_hbm.at[pl.ds(512, 1), :], win, sems.at[12]))
        xcp[0].start()
        cg.start()
        chh(0).start()
        cm.start()
        for m in range(1, 8):
            xcp[m].start()
            chh(m).start()
        for c in wny:
            c.start()
        cg.wait()
        cm.wait()

        def getM(a):
            hc = HH[a, 0:128, :]
            hs = HH[a, 128:256, :]
            return jnp.concatenate(
                [jnp.concatenate([hc, -hs], axis=1), jnp.concatenate([hs, hc], axis=1)], axis=0)

        def phF(m, _):
            for k in (2 * m, 2 * m + 1):
                for c in wblk(k):
                    c.start()
            pltpu.make_async_copy(xb32.at[:, 0, :], xs.at[m], sems.at[m]).wait()
            chh(m).wait()
            def d1(half):
                for ch_ in range(8):
                    w = xs[m, 16 * ch_:16 * ch_ + 16, :]
                    xv = _bc(w << 16, f32) if half == 0 else _bc(w & jnp.uint32(HI), f32)
                    xc = [xv[:, 128 * c:128 * (c + 1)] for c in range(8)]
                    a0, a1 = xc[0] + xc[4], xc[0] - xc[4]
                    b0, b1 = xc[2] + xc[6], xc[2] - xc[6]
                    c0, c1 = xc[1] + xc[5], xc[1] - xc[5]
                    d0, d1_ = xc[3] + xc[7], xc[3] - xc[7]
                    p, q = a0 + b0, c0 + d0
                    y0, y4 = p + q, p - q
                    y2r, y2i = a0 - b0, d0 - c0
                    cm_, cp_ = RS * (c1 - d1_), RS * (c1 + d1_)
                    y1r, y1i = a1 + cm_, -b1 - cp_
                    y3r, y3i = a1 - cm_, b1 - cp_
                    for t, (yr, yi) in enumerate([(y1r, y1i), (y2r, y2i), (y3r, y3i), (y0, y4)]):
                        Y[half, t, 16 * ch_:16 * ch_ + 16, :] = jnp.concatenate([yr, yi], axis=1).astype(bf16)

            Ms = {}
            zs = {}

            def stage_a(u):
                half, t = divmod(u, 5)
                if t < 4:
                    o = lax.dot_general(G[t], Y[half, t], NT, preferred_element_type=f32)
                    zs[u] = jnp.concatenate([o[:128], o[128:]], axis=1).astype(bf16)
                else:
                    zs[u] = lax.dot_general(misc[2, 0:16, :], Y[half, 3, :, 0:128], NT,
                                            preferred_element_type=f32).astype(bf16)

            def stage_b(u):
                half, t = divmod(u, 5)
                a = 2 * m + half
                if half not in Ms:
                    Ms[half] = getM(a)
                Mx = Ms[half]
                if t < 4:
                    X = jnp.dot(zs.pop(u), Mx, preferred_element_type=f32)
                    Zr[a, 128 * t:128 * t + 128, :] = X[:, 0:128]
                    Zi[a, 128 * t:128 * t + 128, :] = X[:, 128:256]
                else:
                    Xn = jnp.dot(zs.pop(u), Mx[0:128, :], preferred_element_type=f32)
                    Zr[a, 512:528, :] = Xn[:, 0:128]
                    Zi[a, 512:528, :] = Xn[:, 128:256]

            d1(0)
            stage_a(0)
            stage_a(1)
            d1(1)
            for u in range(10):
                if u + 2 < 10:
                    stage_b(u)
                    stage_a(u + 2)
                else:
                    stage_b(u)
            return 0

        lax.fori_loop(0, 8, phF, 0)

        for k in range(16):
            for c in wblk(k):
                c.wait()
        for c in wny:
            c.wait()
        wr32 = wr.bitcast(u32)
        wi32 = wi.bitcast(u32)
        hi = jnp.uint32(HI)
        dcr = jnp.concatenate([_bc(wr32[k, 0:1, :] << 16, f32) for k in range(16)], axis=0)
        dci = jnp.concatenate([_bc(wi32[k, 0:1, :] << 16, f32) for k in range(16)], axis=0)
        nyr = jnp.concatenate([wrn[:, 128 * k:128 * (k + 1)].astype(f32) for k in range(16)], axis=0)
        nyi = jnp.concatenate([win[:, 128 * k:128 * (k + 1)].astype(f32) for k in range(16)], axis=0)
        st = jnp.concatenate([dcr, dci, nyr, nyi], axis=0)
        stb = st.astype(bf16)
        r1 = jnp.dot(stb, misc[0], preferred_element_type=f32)
        r2 = jnp.dot(stb, misc[1], preferred_element_type=f32)
        rr = jnp.concatenate([r1, r2], axis=0).astype(bf16)
        rp = jnp.dot(misc[2, 64:128, :], rr, preferred_element_type=f32)
        rid = lax.broadcasted_iota(jnp.int32, (64, 128), 0)
        sgn = jnp.where((rid & 16) == 0, 0.5, -0.5)
        WS[...] = 0.5 * st + sgn * rp

        POS = {1: 0, 7: 64, 2: 128, 6: 192, 3: 256, 5: 320, 0: 384, 4: 448}
        row8 = lax.broadcasted_iota(jnp.int32, (8, 128), 0)

        def mid(r, g, special):
            r0 = POS[r] + 8 * g
            if not special:
                r0 = pl.multiple_of(r0, 8)
            xs_ = [(Zr[a, pl.ds(r0, 8), :], Zi[a, pl.ds(r0, 8), :]) for a in range(16)]
            o = _fft16(xs_, False)
            if special:
                xn = [(Zr[a, 512:520, :], Zi[a, 512:520, :]) for a in range(16)]
                on = _fft16(xn, False)
                wsr, wsi = wr32, wi32
            else:
                g32 = pl.multiple_of(32 * g, 32)
                wsr = wr32.at[:, pl.ds(g32, 32), :]
                wsi = wi32.at[:, pl.ds(g32, 32), :]
            ys = []
            for k in range(16):
                a_ = wsr[k, pl.ds(r // 2, 8, stride=4), :]
                b_ = wsi[k, pl.ds(r // 2, 8, stride=4), :]
                if r % 2 == 0:
                    wre, wim = _bc(a_ << 16, f32), _bc(b_ << 16, f32)
                else:
                    wre, wim = _bc(a_ & hi, f32), _bc(b_ & hi, f32)
                if special:
                    wre = jnp.where(row8 == 0, jnp.broadcast_to(WS[k:k + 1, :], (8, 128)), wre)
                    wim = jnp.where(row8 == 0, jnp.broadcast_to(WS[16 + k:17 + k, :], (8, 128)), wim)
                xr, xi = o[k]
                yr = xr * wre - xi * wim
                yi = xr * wim + xi * wre
                if special:
                    nr = jnp.broadcast_to(WS[32 + k:33 + k, :], (8, 128))
                    ni = jnp.broadcast_to(WS[48 + k:49 + k, :], (8, 128))
                    zr_, zi_ = on[k]
                    yr = yr - (zr_ * ni + zi_ * nr)
                    yi = yi + (zr_ * nr - zi_ * ni)
                ys.append((yr, yi))
            u = _fft16(ys, True)
            for a in range(16):
                Zr[a, pl.ds(r0, 8), :] = u[a][0]
                Zi[a, pl.ds(r0, 8), :] = u[a][1]

        mid(0, 0, True)

        def phM(g, _):
            start_m(g)
            for r in range(1, 8):
                mid(r, g, False)

            @pl.when(g > 0)
            def _():
                mid(0, g, False)

            return 0

        lax.fori_loop(0, 8, phM, 0)

        def phI(m, _):
            start_i(m)
            Ms = {}
            vs = {}

            def stage_a(u):
                half, t = divmod(u, 4)
                a = 2 * m + half
                if half not in Ms:
                    Ms[half] = getM(a)
                yy = jnp.concatenate(
                    [Zr[a, 128 * t:128 * t + 128, :], Zi[a, 128 * t:128 * t + 128, :]], axis=1).astype(bf16)
                o = lax.dot_general(Ms[half], yy, NT, preferred_element_type=f32)
                vs[u] = jnp.concatenate([o[:128], o[128:]], axis=1).astype(bf16)

            def stage_b(u):
                half, t = divmod(u, 4)
                PQ[half, t] = jnp.dot(vs.pop(u), G[t if t < 3 else 4], preferred_element_type=f32)

            def d1inv(half):
                for ch_ in range(8):
                    rs = slice(16 * ch_, 16 * ch_ + 16)
                    P1, Q1 = PQ[half, 0, rs, 0:128], PQ[half, 0, rs, 128:256]
                    P2, Q2 = PQ[half, 1, rs, 0:128], PQ[half, 1, rs, 128:256]
                    P3, Q3 = PQ[half, 2, rs, 0:128], PQ[half, 2, rs, 128:256]
                    h0, h4 = PQ[half, 3, rs, 0:128], PQ[half, 3, rs, 128:256]
                    e, o_ = h0 + h4, h0 - h4
                    A, B = P1 + P3, Q1 - Q3
                    u_, v = P1 - P3, Q1 + Q3
                    T1_, T2_ = RS * (u_ - v), RS * (-u_ - v)
                    e1, e2 = e + P2, e - P2
                    o1, o2 = o_ - Q2, o_ + Q2
                    cols = jnp.concatenate(
                        [e1 + A, o1 + T1_, e2 - B, o2 + T2_, e1 - A, o1 - T1_, e2 + B, o2 - T2_], axis=1)
                    bits = _bc(cols.astype(bf16).astype(f32), u32)
                    if half == 0:
                        bs[m, rs, :] = bits >> 16
                    else:
                        bs[m, rs, :] = bs[m, rs, :] | bits

            stage_a(0)
            stage_a(1)
            for u in range(8):
                stage_b(u)
                if u + 2 < 8:
                    stage_a(u + 2)
                if u == 4:
                    d1inv(0)
            d1inv(1)
            return 0

        lax.fori_loop(0, 8, phI, 0)

    pl.run_scoped(
        scoped,
        pltpu.VMEM((8, 128, D), u32), pltpu.VMEM((16, 512, 128), bf16), pltpu.VMEM((16, 512, 128), bf16),
        pltpu.VMEM((1, S), bf16), pltpu.VMEM((1, S), bf16),
        pltpu.VMEM((5, 256, 256), bf16), pltpu.VMEM((16, 256, 128), bf16), pltpu.VMEM((3, 128, 128), bf16),
        pltpu.VMEM((2, 4, 128, 256), bf16), pltpu.VMEM((16, 528, 128), f32), pltpu.VMEM((16, 528, 128), f32),
        pltpu.VMEM((64, 128), f32), pltpu.VMEM((2, 4, 128, 256), f32))


def _kernel(x_hbm, mem0_hbm, wq_hbm, wk_hbm, wv_hbm, wo_hbm, xb_hbm, wr_hbm, wi_hbm, gw_hbm,
            g_hbm, h_hbm, misc_hbm, out_hbm,
            xv, xpre, mem0v, gwv, raw, wo, bs, bnat, gbuf, outb, bsems, wsems, msems, osem):
    cp_x = pltpu.make_async_copy(x_hbm.bitcast(u32), xv, msems.at[0])
    cp_mem = pltpu.make_async_copy(mem0_hbm, mem0v, msems.at[2])
    cp_gw = pltpu.make_async_copy(gw_hbm, gwv, msems.at[3])
    wsrc = [w.bitcast(u32) for w in (wq_hbm, wk_hbm, wv_hbm)]
    wo32 = wo_hbm.bitcast(u32)

    def cp_w(p):
        return [pltpu.make_async_copy(wsrc[i].at[:, p, :], raw.at[p, i], wsems.at[p]) for i in range(3)]

    def cp_wo(j):
        off = 128 * j if isinstance(j, int) else pl.multiple_of(128 * j, 128)
        return pltpu.make_async_copy(wo32.at[:, :, pl.ds(off, 128)], wo.at[j], msems.at[4])

    def start_m(g):
        @pl.when(g == 0)
        def _():
            cp_gw.start()
            cp_mem.start()
            cp_x.start()

        for c in cp_w(g):
            c.start()

    def start_i(m):
        for c in cp_w(m + 8):
            c.start()

    _b_phase(xb_hbm, wr_hbm, wi_hbm, g_hbm, h_hbm, misc_hbm, bs, bsems, start_m, start_i)
    bn32 = bnat.bitcast(u32)

    def a_phase(w3, pre, oc, ocr, acc, lhs):
        cp_x.wait()
        cp_gw.wait()
        gwf = gwv[...].astype(f32).reshape(1, D)
        for i in range(32):
            xpre[8 * i:8 * i + 8, :] = jnp.concatenate(
                [xv[32 * i + 12:32 * i + 16, :], xv[32 * i + 28:32 * i + 32, :]], axis=0)

        def prebulk_pair(p):
            for i in range(3):
                e = raw[p, i, pl.ds(0, 512, stride=2), :]
                o = raw[p, i, pl.ds(1, 512, stride=2), :]
                w3[p, 0, i] = (e & jnp.uint32(0xFFFF)) | (o << 16)
                w3[p, 1, i] = (e >> 16) | (o & jnp.uint32(HI))
            for r in range(2):
                for i in range(3):
                    for c in range(2):
                        xl = _w2b(xpre[128 * c:128 * c + 128, :])
                        pre[p, r, i, 256 * c:256 * c + 256, :] = jnp.dot(
                            xl, _w2b(w3[p, r, i]), preferred_element_type=f32)
            for c in range(8):
                xw = xv[pl.ds(pl.multiple_of(64 * p + 8 * c, 8), 8), :]
                xx = _w2b(xw).astype(f32) * gwf
                part = xx[:, 0:128]
                for jj in range(1, 8):
                    part = part + xx[:, 128 * jj:128 * jj + 128]
                lg = jnp.sum(part, axis=1, keepdims=True)
                gbuf[pl.ds(pl.multiple_of(128 * p + 16 * c, 16), 16), :] = jnp.broadcast_to(
                    jax.nn.sigmoid(lg), (16, 128))
            for jj in range(8):
                dst = bn32.at[jj, pl.ds(pl.multiple_of(64 * p, 64), 64), :]
                for m in range(8):
                    dst[pl.ds(m, 8, stride=8), :] = bs[m, pl.ds(pl.multiple_of(8 * p, 8), 8), 128 * jj:128 * jj + 128]

        def prebulk(pp, _):
            @pl.when(pp < 4)
            def _():
                cp_wo(2 * pp).start()
                cp_wo(2 * pp + 1).start()

            for p in (2 * pp, 2 * pp + 1):
                for i in range(3):
                    pltpu.make_async_copy(wsrc[i].at[:, 0, :], raw.at[p, i], wsems.at[p]).wait()
            prebulk_pair(2 * pp)
            prebulk_pair(2 * pp + 1)
            return 0

        lax.fori_loop(0, 8, prebulk, 0)
        cp_mem.wait()
        for j in range(8):
            cp_wo(j).wait()
        oc[...] = jnp.zeros(oc.shape, bf16)
        oc32 = oc.bitcast(u32)

        row = lax.broadcasted_iota(jnp.int32, (40, 128), 0)
        col = lax.broadcasted_iota(jnp.int32, (40, 128), 1)
        mask = ((col < 40) & (row >= 32)) | ((row < 32) & ((col <= row) | ((col >= 32) & (col < 40))))
        scale = DH ** -0.5
        bscale = 2.0 ** -20

        def wo_t(j, h):
            return _w2b(wo[j, h])

        def mix(a, b, g):
            return g * a + (1.0 - g) * (b.astype(f32) * bscale)

        def fill_piece(gr, gw_, src, j, half, accs):
            hs = range(16 * half, 16 * half + 16)
            l = jnp.concatenate([_w2b(src[h]) for h in hs], axis=1)
            w = _w2b(wo[j, 16 * half:16 * half + 16].reshape(16 * 64, 128))
            c = jnp.dot(l, w, preferred_element_type=f32)
            if half == 0:
                return c
            c = c + accs
            for q in range(4):
                sg = 4 * gr + q
                b = bnat[j, pl.ds(pl.multiple_of(32 * sg + 24, 8), 8), :]
                g = gbuf[pl.ds(pl.multiple_of(32 * sg + 24, 8), 8), :]
                outb[pl.ds(pl.multiple_of(128 * gw_ + 32 * q + 24, 8), 8),
                     pl.ds(pl.multiple_of(128 * j, 128), 128)] = mix(c[8 * q:8 * q + 8], b, g).astype(bf16)
            return None

        def out_copy(gi):
            return pltpu.make_async_copy(
                outb.at[pl.ds(pl.multiple_of(128 * gi, 128), 128), :],
                out_hbm.at[pl.ds(pl.multiple_of(128 * gi, 128), 128), :], osem)

        def step(q4, mem, grp4):
            s = 4 * grp4 + q4
            r0 = pl.multiple_of(s * 16, 16)
            xs0 = _w2b(xv[pl.ds(r0, 8), :])
            xs1 = _w2b(xv[pl.ds(r0 + 8, 8), :])
            l1 = jnp.concatenate([xs1[0:8].astype(f32), mem], axis=0).astype(bf16)
            lhs[0:8, :] = pltpu.bitcast(xs0, u32)
            lhs[8:16, :] = pltpu.bitcast(l1, u32)
            grp = grp4 - 1
            gr = jnp.maximum(grp, 0)
            gw_ = jnp.where(grp < 0, 16, grp)
            st = {}
            z8 = jnp.zeros((8, 128), f32)
            s8 = pl.multiple_of(s * 8, 8)

            def proj(h, i):
                r = jnp.dot(_w2b(lhs[...]), _w2b(w3[h // 2, h % 2, i]), preferred_element_type=f32)
                p_ = pre[h // 2, h % 2, i, pl.ds(s8, 8), :]
                if i == 0:
                    st[("qkv", h, i)] = jnp.concatenate([r[0:24], p_, r[24:32]], axis=0)
                else:
                    st[("qkv", h, i)] = jnp.concatenate([r[0:24], p_, r[24:32], z8], axis=0).astype(bf16)

            def qk(h):
                q = st.pop(("qkv", h, 0))
                k = st.pop(("qkv", h, 1))
                sc = lax.dot_general(q, k, NT, preferred_element_type=f32) * scale
                sc = jnp.concatenate([sc, jnp.zeros((40, 80), f32)], axis=1)
                sc = jnp.where(mask, sc, -1e9)
                m = jnp.max(sc, axis=1, keepdims=True)
                e = jnp.exp(sc - m)
                p = e * (1.0 / jnp.sum(e, axis=1, keepdims=True))
                st[("p", h)] = p[:, :48]

            def pv(h):
                o = lax.dot_general(st.pop(("p", h)), st.pop(("qkv", h, 2)), NN, preferred_element_type=f32)
                st[("o", h)] = jnp.concatenate([o[0:24], o[32:40]], axis=0).astype(bf16)
                oc[h, pl.ds(pl.multiple_of(8 * q4, 8), 8), :] = o[24:32].astype(bf16)

            def oproj(h):
                w = jnp.concatenate([wo_t(j, h) for j in range(8)], axis=1)
                c = jnp.dot(st.pop(("o", h)), w, preferred_element_type=f32)
                if h == 0:
                    acc[...] = c
                else:
                    acc[...] += c

            ok = lambda h: 0 <= h < H
            for t in range(H + 4):
                if ok(t):
                    proj(t, 0)
                    proj(t, 1)
                if ok(t - 1):
                    qk(t - 1)
                if ok(t):
                    proj(t, 2)
                else:
                    jj, half = (t - H) // 2, (t - H) % 2
                    st["fill"] = fill_piece(gr, gw_, ocr, 2 * q4 + jj, half, st.get("fill"))
                if ok(t - 3):
                    pv(t - 3)
                if ok(t - 4):
                    oproj(t - 4)
            a = acc[...]
            rs = pl.multiple_of(32 * s, 32)
            b0 = jnp.concatenate([bnat[j, pl.ds(rs, 16), :] for j in range(8)], axis=1)
            b1 = jnp.concatenate([bnat[j, pl.ds(rs + 16, 8), :] for j in range(8)], axis=1)
            g0 = gbuf[pl.ds(rs, 16), :]
            g1 = gbuf[pl.ds(rs + 16, 8), :]
            outb[pl.ds(rs, 16), :] = mix(a[0:16], b0, jnp.tile(g0, (1, 8))).astype(bf16)
            outb[pl.ds(rs + 16, 8), :] = mix(a[16:24], b1, jnp.tile(g1, (1, 8))).astype(bf16)
            return a[24:32]

        def group(grp4, mem):
            @pl.when(grp4 >= 2)
            def _():
                out_copy(grp4 - 2).start()

            ocr[...] = oc32[...]
            for q4 in range(4):
                mem = step(q4, mem, grp4)
            return mem

        lax.fori_loop(0, NSEG // 4, group, mem0v[...].astype(f32))

        out_copy(14).start()

        def tail_copy(j):
            return pltpu.make_async_copy(outb.at[pl.ds(S - 128, 128), pl.ds(128 * j, 128)],
                                         out_hbm.at[pl.ds(S - 128, 128), pl.ds(128 * j, 128)], osem)

        for j in range(8):
            c = fill_piece(15, 15, oc32, j, 0, None)
            fill_piece(15, 15, oc32, j, 1, c)
            tail_copy(j).start()
        for gi in range(15):
            out_copy(gi).wait()
        for j in range(8):
            tail_copy(j).wait()

    pl.run_scoped(
        a_phase,
        pltpu.VMEM((16, 2, 3, 512, 128), u32), pltpu.VMEM((16, 2, 3, 512, 128), f32),
        pltpu.VMEM((H, 32, 128), bf16), pltpu.VMEM((H, 16, 128), u32), pltpu.VMEM((32, D), f32), pltpu.VMEM((16, D), u32))


@jax.jit
def pallas_gated_mix__memory_aug_recurrent_mem_tr__spectral_gfnet__prompt_kernel(
    A_x, A_mem0, A_Wq, A_Wk, A_Wv, A_Wo, A_seg_len, B_x, B_w_r, B_w_i, gate_w,
):
    del A_seg_len
    del B_x
    HB = pl.BlockSpec(memory_space=pltpu.HBM)
    out = pl.pallas_call(
        _kernel,
        out_shape=jax.ShapeDtypeStruct((S, D), bf16),
        in_specs=[HB] * 13,
        out_specs=HB,
        scratch_shapes=[
            pltpu.VMEM((S // 2, D), u32),
            pltpu.VMEM((NSEG * 4, D), u32),
            pltpu.VMEM((M_MEM, D), bf16),
            pltpu.VMEM((D,), bf16),
            pltpu.VMEM((16, 3, D, DH), u32),
            pltpu.VMEM((8, H, DH // 2, 128), u32),
            pltpu.VMEM((8, 128, D), u32),
            pltpu.VMEM((8, S, 128), bf16),
            pltpu.VMEM((S, 128), f32),
            pltpu.VMEM((S + 128, D), bf16),
            pltpu.SemaphoreType.DMA((21,)),
            pltpu.SemaphoreType.DMA((16,)),
            pltpu.SemaphoreType.DMA((6,)),
            pltpu.SemaphoreType.DMA(()),
        ],
        compiler_params=pltpu.CompilerParams(
            vmem_limit_bytes=124 * 2 ** 20, flags={"XLA_TPU_EVENLY_DISTRIBUTE_CRITICAL_NODES": True}),
    )(
        A_x.reshape(S, D), A_mem0.reshape(M_MEM, D), A_Wq, A_Wk, A_Wv, A_Wo,
        A_x.reshape(128, 16, D), B_w_r.T, B_w_i.T, gate_w, _TAB_G, _TAB_H, _TAB_MISC,
    )
    return out.reshape(1, S, D)
```

```python
import numpy as np
import ml_dtypes
import jax
import jax.numpy as jnp
from jax import lax
import jax.experimental.pallas as pl
import jax.experimental.pallas.tpu as pltpu

f32, bf16, u32 = jnp.float32, jnp.bfloat16, jnp.uint32
S, D, H, DH, M_MEM, SEG = 2048, 1024, 32, 128, 8, 32
NSEG = S // SEG
RS = float(1 / np.sqrt(2))
NT = (((1,), (1,)), ((), ()))
NN = (((1,), (0,)), ((), ()))
HI = 0xFFFF0000


def _np_tables():
    bf = ml_dtypes.bfloat16
    dp = np.arange(128)
    j = np.arange(64)

    def cs(f):
        ang = 2 * np.pi * ((f[:, None] * dp[None, :]) % 1024) / 1024
        return np.cos(ang), np.sin(ang)

    G = np.zeros((5, 256, 256))
    for t in range(3):
        r = t + 1
        C, Sn = cs(r + 8 * j)
        C2, S2 = cs(8 - r + 8 * j)
        G[t, 0:64, 0:128] = C
        G[t, 0:64, 128:] = Sn
        G[t, 64:128, 0:128] = C2
        G[t, 64:128, 128:] = -S2
        G[t, 128:192, 0:128] = -Sn
        G[t, 128:192, 128:] = C
        G[t, 192:256, 0:128] = -S2
        G[t, 192:256, 128:] = -C2
    C0, S0 = cs(8 * j)
    C4, S4 = cs(4 + 8 * j)
    G[3, 0:64, 0:128] = C0
    G[3, 128:192, 0:128] = -S0
    G[3, 64:128, 128:] = C4
    G[3, 192:256, 128:] = -S4
    G[4] = G[3]
    G[4, 0, 0:128] = 0.5
    G[4, 128, 0:128] = 0.5 * (-1.0) ** dp
    HH = np.zeros((16, 256, 128))
    for a in range(16):
        ang = 2 * np.pi * (((a + 16 * dp)[:, None] * dp[None, :]) % 2048) / 2048
        HH[a, :128] = np.cos(ang)
        HH[a, 128:] = np.sin(ang)
    misc = np.zeros((3, 128, 128))
    misc[0, 128 - dp[1:], dp[1:]] = 1
    misc[1, 0, 0] = 1
    misc[2, 0, :] = (-1.0) ** dp
    for blk in range(4):
        for k1 in range(16):
            misc[2, 64 + 16 * blk + k1, 16 * blk + 15 - k1] = 1
            misc[2, 64 + 16 * blk + k1, 64 + 16 * blk + (16 - k1) % 16] = 1
    return G.astype(bf), HH.astype(bf), misc.astype(bf)


_TAB_G, _TAB_H, _TAB_MISC = _np_tables()


def _bc(x, dt):
    return lax.bitcast_convert_type(x, dt)


def _w2b(w):
    return pltpu.bitcast(w, bf16)


def _fft16(xs, inverse):
    sg = 1.0 if inverse else -1.0

    def dft4(a, b, c, d):
        t0 = (a[0] + c[0], a[1] + c[1])
        t1 = (a[0] - c[0], a[1] - c[1])
        t2 = (b[0] + d[0], b[1] + d[1])
        t3 = (b[0] - d[0], b[1] - d[1])
        o0 = (t0[0] + t2[0], t0[1] + t2[1])
        o2 = (t0[0] - t2[0], t0[1] - t2[1])
        m = (t1[0] + t3[1], t1[1] - t3[0])
        p = (t1[0] - t3[1], t1[1] + t3[0])
        return [o0, p, o2, m] if inverse else [o0, m, o2, p]

    t = [dft4(xs[a0], xs[4 + a0], xs[8 + a0], xs[12 + a0]) for a0 in range(4)]

    def tw(v, e):
        e = e % 16
        if e == 0:
            return v
        if e == 4:
            return (-v[1], v[0]) if inverse else (v[1], -v[0])
        if e == 2:
            if inverse:
                return ((v[0] - v[1]) * RS, (v[0] + v[1]) * RS)
            return ((v[0] + v[1]) * RS, (v[1] - v[0]) * RS)
        if e == 6:
            if inverse:
                return ((-v[0] - v[1]) * RS, (v[0] - v[1]) * RS)
            return ((v[1] - v[0]) * RS, (-v[0] - v[1]) * RS)
        c = float(np.cos(2 * np.pi * e / 16))
        s = float(sg * np.sin(2 * np.pi * e / 16))
        return (v[0] * c - v[1] * s, v[0] * s + v[1] * c)

    out = [None] * 16
    for k in range(4):
        u = [tw(t[a0][k], a0 * k) for a0 in range(4)]
        r = dft4(*u)
        for m in range(4):
            out[k + 4 * m] = r[m]
    return out


def _b_phase(xb_hbm, wr_hbm, wi_hbm, g_hbm, h_hbm, misc_hbm, bs, sems, start_m, start_i):
    def scoped(xs, wr, wi, wrn, win, G, HH, misc, Y, Zr, Zi, WS, PQ):
        xb32 = xb_hbm.bitcast(u32)
        xcp = [pltpu.make_async_copy(xb32.at[:, m, :], xs.at[m], sems.at[m]) for m in range(8)]
        cg = pltpu.make_async_copy(g_hbm, G, sems.at[8])

        def chh(m):
            return pltpu.make_async_copy(h_hbm.at[pl.ds(2 * m, 2)], HH.at[pl.ds(2 * m, 2)], sems.at[13 + m])

        cm = pltpu.make_async_copy(misc_hbm, misc, sems.at[10])
        def wblk(k):
            off = 128 * k if isinstance(k, int) else pl.multiple_of(128 * k, 128)
            return (pltpu.make_async_copy(wr_hbm.at[pl.ds(0, 512), pl.ds(off, 128)], wr.at[k], sems.at[11]),
                    pltpu.make_async_copy(wi_hbm.at[pl.ds(0, 512), pl.ds(off, 128)], wi.at[k], sems.at[12]))

        wny = (pltpu.make_async_copy(wr_hbm.at[pl.ds(512, 1), :], wrn, sems.at[11]),
               pltpu.make_async_copy(wi_hbm.at[pl.ds(512, 1), :], win, sems.at[12]))
        xcp[0].start()
        cg.start()
        chh(0).start()
        cm.start()
        for m in range(1, 8):
            xcp[m].start()
            chh(m).start()
        for c in wny:
            c.start()
        cg.wait()
        cm.wait()

        def getM(a):
            hc = HH[a, 0:128, :]
            hs = HH[a, 128:256, :]
            return jnp.concatenate(
                [jnp.concatenate([hc, -hs], axis=1), jnp.concatenate([hs, hc], axis=1)], axis=0)

        def phF(m, _):
            for k in (2 * m, 2 * m + 1):
                for c in wblk(k):
                    c.start()
            pltpu.make_async_copy(xb32.at[:, 0, :], xs.at[m], sems.at[m]).wait()
            chh(m).wait()
            def d1(half):
                for ch_ in range(8):
                    w = xs[m, 16 * ch_:16 * ch_ + 16, :]
                    xv = _bc(w << 16, f32) if half == 0 else _bc(w & jnp.uint32(HI), f32)
                    xc = [xv[:, 128 * c:128 * (c + 1)] for c in range(8)]
                    a0, a1 = xc[0] + xc[4], xc[0] - xc[4]
                    b0, b1 = xc[2] + xc[6], xc[2] - xc[6]
                    c0, c1 = xc[1] + xc[5], xc[1] - xc[5]
                    d0, d1_ = xc[3] + xc[7], xc[3] - xc[7]
                    p, q = a0 + b0, c0 + d0
                    y0, y4 = p + q, p - q
                    y2r, y2i = a0 - b0, d0 - c0
                    cm_, cp_ = RS * (c1 - d1_), RS * (c1 + d1_)
                    y1r, y1i = a1 + cm_, -b1 - cp_
                    y3r, y3i = a1 - cm_, b1 - cp_
                    for t, (yr, yi) in enumerate([(y1r, y1i), (y2r, y2i), (y3r, y3i), (y0, y4)]):
                        Y[half, t, 16 * ch_:16 * ch_ + 16, :] = jnp.concatenate([yr, yi], axis=1).astype(bf16)

            Ms = {}
            zs = {}

            def stage_a(u):
                half, t = divmod(u, 5)
                if t < 4:
                    o = lax.dot_general(G[t], Y[half, t], NT, preferred_element_type=f32)
                    zs[u] = jnp.concatenate([o[:128], o[128:]], axis=1).astype(bf16)
                else:
                    zs[u] = lax.dot_general(misc[2, 0:16, :], Y[half, 3, :, 0:128], NT,
                                            preferred_element_type=f32).astype(bf16)

            def stage_b(u):
                half, t = divmod(u, 5)
                a = 2 * m + half
                if half not in Ms:
                    Ms[half] = getM(a)
                Mx = Ms[half]
                if t < 4:
                    X = jnp.dot(zs.pop(u), Mx, preferred_element_type=f32)
                    Zr[a, 128 * t:128 * t + 128, :] = X[:, 0:128]
                    Zi[a, 128 * t:128 * t + 128, :] = X[:, 128:256]
                else:
                    Xn = jnp.dot(zs.pop(u), Mx[0:128, :], preferred_element_type=f32)
                    Zr[a, 512:528, :] = Xn[:, 0:128]
                    Zi[a, 512:528, :] = Xn[:, 128:256]

            d1(0)
            stage_a(0)
            stage_a(1)
            d1(1)
            for u in range(10):
                if u + 2 < 10:
                    stage_b(u)
                    stage_a(u + 2)
                else:
                    stage_b(u)
            return 0

        lax.fori_loop(0, 8, phF, 0)

        for k in range(16):
            for c in wblk(k):
                c.wait()
        for c in wny:
            c.wait()
        wr32 = wr.bitcast(u32)
        wi32 = wi.bitcast(u32)
        hi = jnp.uint32(HI)
        dcr = jnp.concatenate([_bc(wr32[k, 0:1, :] << 16, f32) for k in range(16)], axis=0)
        dci = jnp.concatenate([_bc(wi32[k, 0:1, :] << 16, f32) for k in range(16)], axis=0)
        nyr = jnp.concatenate([wrn[:, 128 * k:128 * (k + 1)].astype(f32) for k in range(16)], axis=0)
        nyi = jnp.concatenate([win[:, 128 * k:128 * (k + 1)].astype(f32) for k in range(16)], axis=0)
        st = jnp.concatenate([dcr, dci, nyr, nyi], axis=0)
        stb = st.astype(bf16)
        r1 = jnp.dot(stb, misc[0], preferred_element_type=f32)
        r2 = jnp.dot(stb, misc[1], preferred_element_type=f32)
        rr = jnp.concatenate([r1, r2], axis=0).astype(bf16)
        rp = jnp.dot(misc[2, 64:128, :], rr, preferred_element_type=f32)
        rid = lax.broadcasted_iota(jnp.int32, (64, 128), 0)
        sgn = jnp.where((rid & 16) == 0, 0.5, -0.5)
        WS[...] = 0.5 * st + sgn * rp

        POS = {1: 0, 7: 64, 2: 128, 6: 192, 3: 256, 5: 320, 0: 384, 4: 448}
        row8 = lax.broadcasted_iota(jnp.int32, (8, 128), 0)

        def mid(r, g, special):
            r0 = POS[r] + 8 * g
            if not special:
                r0 = pl.multiple_of(r0, 8)
            xs_ = [(Zr[a, pl.ds(r0, 8), :], Zi[a, pl.ds(r0, 8), :]) for a in range(16)]
            o = _fft16(xs_, False)
            if special:
                xn = [(Zr[a, 512:520, :], Zi[a, 512:520, :]) for a in range(16)]
                on = _fft16(xn, False)
                wsr, wsi = wr32, wi32
            else:
                g32 = pl.multiple_of(32 * g, 32)
                wsr = wr32.at[:, pl.ds(g32, 32), :]
                wsi = wi32.at[:, pl.ds(g32, 32), :]
            ys = []
            for k in range(16):
                a_ = wsr[k, pl.ds(r // 2, 8, stride=4), :]
                b_ = wsi[k, pl.ds(r // 2, 8, stride=4), :]
                if r % 2 == 0:
                    wre, wim = _bc(a_ << 16, f32), _bc(b_ << 16, f32)
                else:
                    wre, wim = _bc(a_ & hi, f32), _bc(b_ & hi, f32)
                if special:
                    wre = jnp.where(row8 == 0, jnp.broadcast_to(WS[k:k + 1, :], (8, 128)), wre)
                    wim = jnp.where(row8 == 0, jnp.broadcast_to(WS[16 + k:17 + k, :], (8, 128)), wim)
                xr, xi = o[k]
                yr = xr * wre - xi * wim
                yi = xr * wim + xi * wre
                if special:
                    nr = jnp.broadcast_to(WS[32 + k:33 + k, :], (8, 128))
                    ni = jnp.broadcast_to(WS[48 + k:49 + k, :], (8, 128))
                    zr_, zi_ = on[k]
                    yr = yr - (zr_ * ni + zi_ * nr)
                    yi = yi + (zr_ * nr - zi_ * ni)
                ys.append((yr, yi))
            u = _fft16(ys, True)
            for a in range(16):
                Zr[a, pl.ds(r0, 8), :] = u[a][0]
                Zi[a, pl.ds(r0, 8), :] = u[a][1]

        mid(0, 0, True)

        def phM(g, _):
            start_m(g)
            for r in range(1, 8):
                mid(r, g, False)

            @pl.when(g > 0)
            def _():
                mid(0, g, False)

            return 0

        lax.fori_loop(0, 8, phM, 0)

        def phI2(mm, _):
            start_i(2 * mm)
            start_i(2 * mm + 1)
            phI(2 * mm, 0)
            phI(2 * mm + 1, 2)
            return 0

        def phI(m, pb):
            Ms = {}
            vs = {}

            def stage_a(u):
                half, t = divmod(u, 4)
                a = 2 * m + half
                if half not in Ms:
                    Ms[half] = getM(a)
                yy = jnp.concatenate(
                    [Zr[a, 128 * t:128 * t + 128, :], Zi[a, 128 * t:128 * t + 128, :]], axis=1).astype(bf16)
                o = lax.dot_general(Ms[half], yy, NT, preferred_element_type=f32)
                vs[u] = jnp.concatenate([o[:128], o[128:]], axis=1).astype(bf16)

            def stage_b(u):
                half, t = divmod(u, 4)
                PQ[pb + half, t] = jnp.dot(vs.pop(u), G[t if t < 3 else 4], preferred_element_type=f32)

            def d1inv(half):
                for ch_ in range(8):
                    rs = slice(16 * ch_, 16 * ch_ + 16)
                    P1, Q1 = PQ[pb + half, 0, rs, 0:128], PQ[pb + half, 0, rs, 128:256]
                    P2, Q2 = PQ[pb + half, 1, rs, 0:128], PQ[pb + half, 1, rs, 128:256]
                    P3, Q3 = PQ[pb + half, 2, rs, 0:128], PQ[pb + half, 2, rs, 128:256]
                    h0, h4 = PQ[pb + half, 3, rs, 0:128], PQ[pb + half, 3, rs, 128:256]
                    e, o_ = h0 + h4, h0 - h4
                    A, B = P1 + P3, Q1 - Q3
                    u_, v = P1 - P3, Q1 + Q3
                    T1_, T2_ = RS * (u_ - v), RS * (-u_ - v)
                    e1, e2 = e + P2, e - P2
                    o1, o2 = o_ - Q2, o_ + Q2
                    cols = jnp.concatenate(
                        [e1 + A, o1 + T1_, e2 - B, o2 + T2_, e1 - A, o1 - T1_, e2 + B, o2 - T2_], axis=1)
                    bits = _bc(cols.astype(bf16).astype(f32), u32)
                    if half == 0:
                        bs[m, rs, :] = bits >> 16
                    else:
                        bs[m, rs, :] = bs[m, rs, :] | bits

            stage_a(0)
            stage_a(1)
            for u in range(8):
                stage_b(u)
                if u + 2 < 8:
                    stage_a(u + 2)
                if u == 4:
                    d1inv(0)
            d1inv(1)

        lax.fori_loop(0, 4, phI2, 0)

    pl.run_scoped(
        scoped,
        pltpu.VMEM((8, 128, D), u32), pltpu.VMEM((16, 512, 128), bf16), pltpu.VMEM((16, 512, 128), bf16),
        pltpu.VMEM((1, S), bf16), pltpu.VMEM((1, S), bf16),
        pltpu.VMEM((5, 256, 256), bf16), pltpu.VMEM((16, 256, 128), bf16), pltpu.VMEM((3, 128, 128), bf16),
        pltpu.VMEM((2, 4, 128, 256), bf16), pltpu.VMEM((16, 528, 128), f32), pltpu.VMEM((16, 528, 128), f32),
        pltpu.VMEM((64, 128), f32), pltpu.VMEM((4, 4, 128, 256), f32))


def _kernel(x_hbm, mem0_hbm, wq_hbm, wk_hbm, wv_hbm, wo_hbm, xb_hbm, wr_hbm, wi_hbm, gw_hbm,
            g_hbm, h_hbm, misc_hbm, out_hbm,
            xv, xpre, mem0v, gwv, raw, wo, bs, bnat, gbuf, outb, bsems, wsems, msems, osem):
    cp_x = pltpu.make_async_copy(x_hbm.bitcast(u32), xv, msems.at[0])
    cp_mem = pltpu.make_async_copy(mem0_hbm, mem0v, msems.at[2])
    cp_gw = pltpu.make_async_copy(gw_hbm, gwv, msems.at[3])
    wsrc = [w.bitcast(u32) for w in (wq_hbm, wk_hbm, wv_hbm)]
    wo32 = wo_hbm.bitcast(u32)

    def cp_w(p):
        return [pltpu.make_async_copy(wsrc[i].at[:, p, :], raw.at[p, i], wsems.at[p]) for i in range(3)]

    def cp_wo(j):
        off = 128 * j if isinstance(j, int) else pl.multiple_of(128 * j, 128)
        return pltpu.make_async_copy(wo32.at[:, :, pl.ds(off, 128)], wo.at[j], msems.at[4])

    def start_m(g):
        @pl.when(g == 0)
        def _():
            cp_gw.start()
            cp_mem.start()
            cp_x.start()

        for c in cp_w(g):
            c.start()

    def start_i(m):
        for c in cp_w(m + 8):
            c.start()

    _b_phase(xb_hbm, wr_hbm, wi_hbm, g_hbm, h_hbm, misc_hbm, bs, bsems, start_m, start_i)
    bn32 = bnat.bitcast(u32)

    def a_phase(w3, pre, oc, ocr, acc, lhs):
        cp_x.wait()
        cp_gw.wait()
        gwf = gwv[...].astype(f32).reshape(1, D)
        for i in range(32):
            xpre[8 * i:8 * i + 8, :] = jnp.concatenate(
                [xv[32 * i + 12:32 * i + 16, :], xv[32 * i + 28:32 * i + 32, :]], axis=0)

        def prebulk_pair(p):
            for i in range(3):
                e = raw[p, i, pl.ds(0, 512, stride=2), :]
                o = raw[p, i, pl.ds(1, 512, stride=2), :]
                w3[p, 0, i] = (e & jnp.uint32(0xFFFF)) | (o << 16)
                w3[p, 1, i] = (e >> 16) | (o & jnp.uint32(HI))
            for r in range(2):
                for i in range(3):
                    for c in range(2):
                        xl = _w2b(xpre[128 * c:128 * c + 128, :])
                        pre[p, r, i, 256 * c:256 * c + 256, :] = jnp.dot(
                            xl, _w2b(w3[p, r, i]), preferred_element_type=f32)
            for c in range(8):
                xw = xv[pl.ds(pl.multiple_of(64 * p + 8 * c, 8), 8), :]
                xx = _w2b(xw).astype(f32) * gwf
                part = xx[:, 0:128]
                for jj in range(1, 8):
                    part = part + xx[:, 128 * jj:128 * jj + 128]
                lg = jnp.sum(part, axis=1, keepdims=True)
                gbuf[pl.ds(pl.multiple_of(128 * p + 16 * c, 16), 16), :] = jnp.broadcast_to(
                    jax.nn.sigmoid(lg), (16, 128))
            for jj in range(8):
                dst = bn32.at[jj, pl.ds(pl.multiple_of(64 * p, 64), 64), :]
                for m in range(8):
                    dst[pl.ds(m, 8, stride=8), :] = bs[m, pl.ds(pl.multiple_of(8 * p, 8), 8), 128 * jj:128 * jj + 128]

        def prebulk(pp, _):
            @pl.when(pp < 4)
            def _():
                cp_wo(2 * pp).start()
                cp_wo(2 * pp + 1).start()

            for p in (2 * pp, 2 * pp + 1):
                for i in range(3):
                    pltpu.make_async_copy(wsrc[i].at[:, 0, :], raw.at[p, i], wsems.at[p]).wait()
            prebulk_pair(2 * pp)
            prebulk_pair(2 * pp + 1)
            return 0

        lax.fori_loop(0, 8, prebulk, 0)
        cp_mem.wait()
        for j in range(8):
            cp_wo(j).wait()
        oc[...] = jnp.zeros(oc.shape, bf16)
        oc32 = oc.bitcast(u32)

        row = lax.broadcasted_iota(jnp.int32, (40, 128), 0)
        col = lax.broadcasted_iota(jnp.int32, (40, 128), 1)
        mask = ((col < 40) & (row >= 32)) | ((row < 32) & ((col <= row) | ((col >= 32) & (col < 40))))
        scale = DH ** -0.5
        bscale = 2.0 ** -20

        def wo_t(j, h):
            return _w2b(wo[j, h])

        def mix(a, b, g):
            return g * a + (1.0 - g) * (b.astype(f32) * bscale)

        def fill_piece(gr, gw_, src, j, half, accs):
            hs = range(16 * half, 16 * half + 16)
            l = jnp.concatenate([_w2b(src[h]) for h in hs], axis=1)
            w = _w2b(wo[j, 16 * half:16 * half + 16].reshape(16 * 64, 128))
            c = jnp.dot(l, w, preferred_element_type=f32)
            if half == 0:
                return c
            c = c + accs
            for q in range(4):
                sg = 4 * gr + q
                b = bnat[j, pl.ds(pl.multiple_of(32 * sg + 24, 8), 8), :]
                g = gbuf[pl.ds(pl.multiple_of(32 * sg + 24, 8), 8), :]
                outb[pl.ds(pl.multiple_of(128 * gw_ + 32 * q + 24, 8), 8),
                     pl.ds(pl.multiple_of(128 * j, 128), 128)] = mix(c[8 * q:8 * q + 8], b, g).astype(bf16)
            return None

        def out_copy(gi):
            return pltpu.make_async_copy(
                outb.at[pl.ds(pl.multiple_of(128 * gi, 128), 128), :],
                out_hbm.at[pl.ds(pl.multiple_of(128 * gi, 128), 128), :], osem)

        def step(q4, mem, grp4):
            s = 4 * grp4 + q4
            r0 = pl.multiple_of(s * 16, 16)
            xs0 = _w2b(xv[pl.ds(r0, 8), :])
            xs1 = _w2b(xv[pl.ds(r0 + 8, 8), :])
            l1 = jnp.concatenate([xs1[0:8].astype(f32), mem], axis=0).astype(bf16)
            lhs[0:8, :] = pltpu.bitcast(xs0, u32)
            lhs[8:16, :] = pltpu.bitcast(l1, u32)
            grp = grp4 - 1
            gr = jnp.maximum(grp, 0)
            gw_ = jnp.where(grp < 0, 16, grp)
            st = {}
            z8 = jnp.zeros((8, 128), f32)
            s8 = pl.multiple_of(s * 8, 8)

            def proj(h, i):
                r = jnp.dot(_w2b(lhs[...]), _w2b(w3[h // 2, h % 2, i]), preferred_element_type=f32)
                p_ = pre[h // 2, h % 2, i, pl.ds(s8, 8), :]
                if i == 0:
                    st[("qkv", h, i)] = jnp.concatenate([r[0:24], p_, r[24:32]], axis=0)
                else:
                    st[("qkv", h, i)] = jnp.concatenate([r[0:24], p_, r[24:32], z8], axis=0).astype(bf16)

            def qk(h):
                q = st.pop(("qkv", h, 0))
                k = st.pop(("qkv", h, 1))
                sc = lax.dot_general(q, k, NT, preferred_element_type=f32) * scale
                sc = jnp.concatenate([sc, jnp.zeros((40, 80), f32)], axis=1)
                sc = jnp.where(mask, sc, -1e9)
                m = jnp.max(sc, axis=1, keepdims=True)
                e = jnp.exp(sc - m)
                p = e * (1.0 / jnp.sum(e, axis=1, keepdims=True))
                st[("p", h)] = p[:, :48]

            def pv(h):
                o = lax.dot_general(st.pop(("p", h)), st.pop(("qkv", h, 2)), NN, preferred_element_type=f32)
                st[("o", h)] = jnp.concatenate([o[0:24], o[32:40]], axis=0).astype(bf16)
                oc[h, pl.ds(pl.multiple_of(8 * q4, 8), 8), :] = o[24:32].astype(bf16)

            def oproj(h):
                w = jnp.concatenate([wo_t(j, h) for j in range(8)], axis=1)
                c = jnp.dot(st.pop(("o", h)), w, preferred_element_type=f32)
                if h == 0:
                    acc[...] = c
                else:
                    acc[...] += c

            ok = lambda h: 0 <= h < H
            for t in range(H + 4):
                if ok(t):
                    proj(t, 0)
                    proj(t, 1)
                if ok(t - 1):
                    qk(t - 1)
                if ok(t):
                    proj(t, 2)
                else:
                    jj, half = (t - H) // 2, (t - H) % 2
                    st["fill"] = fill_piece(gr, gw_, ocr, 2 * q4 + jj, half, st.get("fill"))
                if ok(t - 3):
                    pv(t - 3)
                if ok(t - 4):
                    oproj(t - 4)
            a = acc[...]
            rs = pl.multiple_of(32 * s, 32)
            b0 = jnp.concatenate([bnat[j, pl.ds(rs, 16), :] for j in range(8)], axis=1)
            b1 = jnp.concatenate([bnat[j, pl.ds(rs + 16, 8), :] for j in range(8)], axis=1)
            g0 = gbuf[pl.ds(rs, 16), :]
            g1 = gbuf[pl.ds(rs + 16, 8), :]
            outb[pl.ds(rs, 16), :] = mix(a[0:16], b0, jnp.tile(g0, (1, 8))).astype(bf16)
            outb[pl.ds(rs + 16, 8), :] = mix(a[16:24], b1, jnp.tile(g1, (1, 8))).astype(bf16)
            return a[24:32]

        def group(grp4, mem):
            @pl.when(grp4 >= 2)
            def _():
                out_copy(grp4 - 2).start()

            ocr[...] = oc32[...]
            for q4 in range(4):
                mem = step(q4, mem, grp4)
            return mem

        lax.fori_loop(0, NSEG // 4, group, mem0v[...].astype(f32))

        out_copy(14).start()

        def tail_copy(j):
            return pltpu.make_async_copy(outb.at[pl.ds(S - 128, 128), pl.ds(128 * j, 128)],
                                         out_hbm.at[pl.ds(S - 128, 128), pl.ds(128 * j, 128)], osem)

        for j in range(8):
            c = fill_piece(15, 15, oc32, j, 0, None)
            fill_piece(15, 15, oc32, j, 1, c)
            tail_copy(j).start()
        for gi in range(15):
            out_copy(gi).wait()
        for j in range(8):
            tail_copy(j).wait()

    pl.run_scoped(
        a_phase,
        pltpu.VMEM((16, 2, 3, 512, 128), u32), pltpu.VMEM((16, 2, 3, 512, 128), f32),
        pltpu.VMEM((H, 32, 128), bf16), pltpu.VMEM((H, 16, 128), u32), pltpu.VMEM((32, D), f32), pltpu.VMEM((16, D), u32))


@jax.jit
def pallas_gated_mix__memory_aug_recurrent_mem_tr__spectral_gfnet__prompt_kernel(
    A_x, A_mem0, A_Wq, A_Wk, A_Wv, A_Wo, A_seg_len, B_x, B_w_r, B_w_i, gate_w,
):
    del A_seg_len
    del B_x
    HB = pl.BlockSpec(memory_space=pltpu.HBM)
    out = pl.pallas_call(
        _kernel,
        out_shape=jax.ShapeDtypeStruct((S, D), bf16),
        in_specs=[HB] * 13,
        out_specs=HB,
        scratch_shapes=[
            pltpu.VMEM((S // 2, D), u32),
            pltpu.VMEM((NSEG * 4, D), u32),
            pltpu.VMEM((M_MEM, D), bf16),
            pltpu.VMEM((D,), bf16),
            pltpu.VMEM((16, 3, D, DH), u32),
            pltpu.VMEM((8, H, DH // 2, 128), u32),
            pltpu.VMEM((8, 128, D), u32),
            pltpu.VMEM((8, S, 128), bf16),
            pltpu.VMEM((S, 128), f32),
            pltpu.VMEM((S + 128, D), bf16),
            pltpu.SemaphoreType.DMA((21,)),
            pltpu.SemaphoreType.DMA((16,)),
            pltpu.SemaphoreType.DMA((6,)),
            pltpu.SemaphoreType.DMA(()),
        ],
        compiler_params=pltpu.CompilerParams(
            vmem_limit_bytes=124 * 2 ** 20, flags={"XLA_TPU_EVENLY_DISTRIBUTE_CRITICAL_NODES": True}),
    )(
        A_x.reshape(S, D), A_mem0.reshape(M_MEM, D), A_Wq, A_Wk, A_Wv, A_Wo,
        A_x.reshape(128, 16, D), B_w_r.T, B_w_i.T, gate_w, _TAB_G, _TAB_H, _TAB_MISC,
    )
    return out.reshape(1, S, D)
```

```python
import numpy as np
import ml_dtypes
import jax
import jax.numpy as jnp
from jax import lax
import jax.experimental.pallas as pl
import jax.experimental.pallas.tpu as pltpu

f32, bf16, u32 = jnp.float32, jnp.bfloat16, jnp.uint32
S, D, H, DH, M_MEM, SEG = 2048, 1024, 32, 128, 8, 32
NSEG = S // SEG
RS = float(1 / np.sqrt(2))
NT = (((1,), (1,)), ((), ()))
NN = (((1,), (0,)), ((), ()))
HI = 0xFFFF0000


def _np_tables():
    bf = ml_dtypes.bfloat16
    dp = np.arange(128)
    j = np.arange(64)

    def cs(f):
        ang = 2 * np.pi * ((f[:, None] * dp[None, :]) % 1024) / 1024
        return np.cos(ang), np.sin(ang)

    G = np.zeros((5, 256, 256))
    for t in range(3):
        r = t + 1
        C, Sn = cs(r + 8 * j)
        C2, S2 = cs(8 - r + 8 * j)
        G[t, 0:64, 0:128] = C
        G[t, 0:64, 128:] = Sn
        G[t, 64:128, 0:128] = C2
        G[t, 64:128, 128:] = -S2
        G[t, 128:192, 0:128] = -Sn
        G[t, 128:192, 128:] = C
        G[t, 192:256, 0:128] = -S2
        G[t, 192:256, 128:] = -C2
    C0, S0 = cs(8 * j)
    C4, S4 = cs(4 + 8 * j)
    G[3, 0:64, 0:128] = C0
    G[3, 128:192, 0:128] = -S0
    G[3, 64:128, 128:] = C4
    G[3, 192:256, 128:] = -S4
    G[4] = G[3]
    G[4, 0, 0:128] = 0.5
    G[4, 128, 0:128] = 0.5 * (-1.0) ** dp
    HH = np.zeros((16, 256, 128))
    for a in range(16):
        ang = 2 * np.pi * (((a + 16 * dp)[:, None] * dp[None, :]) % 2048) / 2048
        HH[a, :128] = np.cos(ang)
        HH[a, 128:] = np.sin(ang)
    misc = np.zeros((3, 128, 128))
    misc[0, 128 - dp[1:], dp[1:]] = 1
    misc[1, 0, 0] = 1
    misc[2, 0, :] = (-1.0) ** dp
    for blk in range(4):
        for k1 in range(16):
            misc[2, 64 + 16 * blk + k1, 16 * blk + 15 - k1] = 1
            misc[2, 64 + 16 * blk + k1, 64 + 16 * blk + (16 - k1) % 16] = 1
    return G.astype(bf), HH.astype(bf), misc.astype(bf)


_TAB_G, _TAB_H, _TAB_MISC = _np_tables()


def _bc(x, dt):
    return lax.bitcast_convert_type(x, dt)


def _w2b(w):
    return pltpu.bitcast(w, bf16)


def _fft16(xs, inverse):
    sg = 1.0 if inverse else -1.0

    def dft4(a, b, c, d):
        t0 = (a[0] + c[0], a[1] + c[1])
        t1 = (a[0] - c[0], a[1] - c[1])
        t2 = (b[0] + d[0], b[1] + d[1])
        t3 = (b[0] - d[0], b[1] - d[1])
        o0 = (t0[0] + t2[0], t0[1] + t2[1])
        o2 = (t0[0] - t2[0], t0[1] - t2[1])
        m = (t1[0] + t3[1], t1[1] - t3[0])
        p = (t1[0] - t3[1], t1[1] + t3[0])
        return [o0, p, o2, m] if inverse else [o0, m, o2, p]

    t = [dft4(xs[a0], xs[4 + a0], xs[8 + a0], xs[12 + a0]) for a0 in range(4)]

    def tw(v, e):
        e = e % 16
        if e == 0:
            return v
        if e == 4:
            return (-v[1], v[0]) if inverse else (v[1], -v[0])
        if e == 2:
            if inverse:
                return ((v[0] - v[1]) * RS, (v[0] + v[1]) * RS)
            return ((v[0] + v[1]) * RS, (v[1] - v[0]) * RS)
        if e == 6:
            if inverse:
                return ((-v[0] - v[1]) * RS, (v[0] - v[1]) * RS)
            return ((v[1] - v[0]) * RS, (-v[0] - v[1]) * RS)
        c = float(np.cos(2 * np.pi * e / 16))
        s = float(sg * np.sin(2 * np.pi * e / 16))
        return (v[0] * c - v[1] * s, v[0] * s + v[1] * c)

    out = [None] * 16
    for k in range(4):
        u = [tw(t[a0][k], a0 * k) for a0 in range(4)]
        r = dft4(*u)
        for m in range(4):
            out[k + 4 * m] = r[m]
    return out


def _b_phase(xb_hbm, wr_hbm, wi_hbm, g_hbm, h_hbm, misc_hbm, bs, sems, start_m, start_i):
    def scoped(xs, wr, wi, wdc, wny_, G, HH, misc, Y, Zr, Zi, WS, PQ):
        xb32 = xb_hbm.bitcast(u32)
        xcp = [pltpu.make_async_copy(xb32.at[:, m, :], xs.at[m], sems.at[m]) for m in range(8)]
        cg = pltpu.make_async_copy(g_hbm, G, sems.at[8])

        def chh(m):
            return pltpu.make_async_copy(h_hbm.at[pl.ds(2 * m, 2)], HH.at[pl.ds(2 * m, 2)], sems.at[13 + m])

        cm = pltpu.make_async_copy(misc_hbm, misc, sems.at[10])
        def wblk(k):
            off = 128 * k if isinstance(k, int) else pl.multiple_of(128 * k, 128)
            return (pltpu.make_async_copy(wr_hbm.at[pl.ds(0, 512), pl.ds(off, 128)], wr.at[k], sems.at[11]),
                    pltpu.make_async_copy(wi_hbm.at[pl.ds(0, 512), pl.ds(off, 128)], wi.at[k], sems.at[12]))

        wny, wnq = [], []
        for i, src in enumerate((wr_hbm, wi_hbm)):
            wny.append(pltpu.make_async_copy(src.at[pl.ds(0, 8), :], wdc.at[i], sems.at[9]))
            wnq.append(pltpu.make_async_copy(src.at[pl.ds(512, 1), :], wny_.at[i], sems.at[12]))
        cm.start()
        for c in wny + wnq:
            c.start()
        xcp[0].start()
        cg.start()
        chh(0).start()
        for m in range(1, 8):
            xcp[m].start()
            chh(m).start()
        cm.wait()
        for c in wny + wnq:
            c.wait()

        st = jnp.concatenate([ref[i, 0:1, 128 * k:128 * (k + 1)].astype(f32)
                              for ref in (wdc, wny_) for i in range(2) for k in range(16)], axis=0)
        stb = st.astype(bf16)
        r1 = jnp.dot(stb, misc[0], preferred_element_type=f32)
        r2 = jnp.dot(stb, misc[1], preferred_element_type=f32)
        rr = jnp.concatenate([r1, r2], axis=0).astype(bf16)
        rp = jnp.dot(misc[2, 64:128, :], rr, preferred_element_type=f32)
        rid = lax.broadcasted_iota(jnp.int32, (64, 128), 0)
        sgn = jnp.where((rid & 16) == 0, 0.5, -0.5)
        WS[...] = 0.5 * st + sgn * rp
        cg.wait()

        def getM(a):
            hc = HH[a, 0:128, :]
            hs = HH[a, 128:256, :]
            return jnp.concatenate(
                [jnp.concatenate([hc, -hs], axis=1), jnp.concatenate([hs, hc], axis=1)], axis=0)

        def phF(m, _):
            for k in (2 * m, 2 * m + 1):
                for c in wblk(k):
                    c.start()
            pltpu.make_async_copy(xb32.at[:, 0, :], xs.at[m], sems.at[m]).wait()
            chh(m).wait()
            def d1(half):
                for ch_ in range(8):
                    w = xs[m, 16 * ch_:16 * ch_ + 16, :]
                    xv = _bc(w << 16, f32) if half == 0 else _bc(w & jnp.uint32(HI), f32)
                    xc = [xv[:, 128 * c:128 * (c + 1)] for c in range(8)]
                    a0, a1 = xc[0] + xc[4], xc[0] - xc[4]
                    b0, b1 = xc[2] + xc[6], xc[2] - xc[6]
                    c0, c1 = xc[1] + xc[5], xc[1] - xc[5]
                    d0, d1_ = xc[3] + xc[7], xc[3] - xc[7]
                    p, q = a0 + b0, c0 + d0
                    y0, y4 = p + q, p - q
                    y2r, y2i = a0 - b0, d0 - c0
                    cm_, cp_ = RS * (c1 - d1_), RS * (c1 + d1_)
                    y1r, y1i = a1 + cm_, -b1 - cp_
                    y3r, y3i = a1 - cm_, b1 - cp_
                    for t, (yr, yi) in enumerate([(y1r, y1i), (y2r, y2i), (y3r, y3i), (y0, y4)]):
                        Y[half, t, 16 * ch_:16 * ch_ + 16, :] = jnp.concatenate([yr, yi], axis=1).astype(bf16)

            Ms = {}
            zs = {}

            def stage_a(u):
                half, t = divmod(u, 5)
                if t < 4:
                    o = lax.dot_general(G[t], Y[half, t], NT, preferred_element_type=f32)
                    zs[u] = jnp.concatenate([o[:128], o[128:]], axis=1).astype(bf16)
                else:
                    zs[u] = lax.dot_general(misc[2, 0:16, :], Y[half, 3, :, 0:128], NT,
                                            preferred_element_type=f32).astype(bf16)

            def stage_b(u):
                half, t = divmod(u, 5)
                a = 2 * m + half
                if half not in Ms:
                    Ms[half] = getM(a)
                Mx = Ms[half]
                if t < 4:
                    X = jnp.dot(zs.pop(u), Mx, preferred_element_type=f32)
                    Zr[a, 128 * t:128 * t + 128, :] = X[:, 0:128]
                    Zi[a, 128 * t:128 * t + 128, :] = X[:, 128:256]
                else:
                    Xn = jnp.dot(zs.pop(u), Mx[0:128, :], preferred_element_type=f32)
                    Zr[a, 512:528, :] = Xn[:, 0:128]
                    Zi[a, 512:528, :] = Xn[:, 128:256]

            d1(0)
            stage_a(0)
            stage_a(1)
            d1(1)
            for u in range(10):
                if u + 2 < 10:
                    stage_b(u)
                    stage_a(u + 2)
                else:
                    stage_b(u)
            return 0

        lax.fori_loop(0, 8, phF, 0)

        for k in range(16):
            for c in wblk(k):
                c.wait()
        wr32 = wr.bitcast(u32)
        wi32 = wi.bitcast(u32)
        hi = jnp.uint32(HI)

        POS = {1: 0, 7: 64, 2: 128, 6: 192, 3: 256, 5: 320, 0: 384, 4: 448}
        row8 = lax.broadcasted_iota(jnp.int32, (8, 128), 0)

        def mid(r, g, special):
            r0 = POS[r] + 8 * g
            if not special:
                r0 = pl.multiple_of(r0, 8)
            xs_ = [(Zr[a, pl.ds(r0, 8), :], Zi[a, pl.ds(r0, 8), :]) for a in range(16)]
            o = _fft16(xs_, False)
            if special:
                xn = [(Zr[a, 512:520, :], Zi[a, 512:520, :]) for a in range(16)]
                on = _fft16(xn, False)
                wsr, wsi = wr32, wi32
            else:
                g32 = pl.multiple_of(32 * g, 32)
                wsr = wr32.at[:, pl.ds(g32, 32), :]
                wsi = wi32.at[:, pl.ds(g32, 32), :]
            ys = []
            for k in range(16):
                a_ = wsr[k, pl.ds(r // 2, 8, stride=4), :]
                b_ = wsi[k, pl.ds(r // 2, 8, stride=4), :]
                if r % 2 == 0:
                    wre, wim = _bc(a_ << 16, f32), _bc(b_ << 16, f32)
                else:
                    wre, wim = _bc(a_ & hi, f32), _bc(b_ & hi, f32)
                if special:
                    wre = jnp.where(row8 == 0, jnp.broadcast_to(WS[k:k + 1, :], (8, 128)), wre)
                    wim = jnp.where(row8 == 0, jnp.broadcast_to(WS[16 + k:17 + k, :], (8, 128)), wim)
                xr, xi = o[k]
                yr = xr * wre - xi * wim
                yi = xr * wim + xi * wre
                if special:
                    nr = jnp.broadcast_to(WS[32 + k:33 + k, :], (8, 128))
                    ni = jnp.broadcast_to(WS[48 + k:49 + k, :], (8, 128))
                    zr_, zi_ = on[k]
                    yr = yr - (zr_ * ni + zi_ * nr)
                    yi = yi + (zr_ * nr - zi_ * ni)
                ys.append((yr, yi))
            u = _fft16(ys, True)
            for a in range(16):
                Zr[a, pl.ds(r0, 8), :] = u[a][0]
                Zi[a, pl.ds(r0, 8), :] = u[a][1]

        mid(0, 0, True)

        def phM(g, _):
            start_m(g)
            for r in range(1, 8):
                mid(r, g, False)

            @pl.when(g > 0)
            def _():
                mid(0, g, False)

            return 0

        lax.fori_loop(0, 8, phM, 0)

        def phI2(mm, _):
            start_i(2 * mm)
            start_i(2 * mm + 1)
            phI(2 * mm, 0)
            phI(2 * mm + 1, 2)
            return 0

        def phI(m, pb):
            Ms = {}
            vs = {}

            def stage_a(u):
                half, t = divmod(u, 4)
                a = 2 * m + half
                if half not in Ms:
                    Ms[half] = getM(a)
                yy = jnp.concatenate(
                    [Zr[a, 128 * t:128 * t + 128, :], Zi[a, 128 * t:128 * t + 128, :]], axis=1).astype(bf16)
                o = lax.dot_general(Ms[half], yy, NT, preferred_element_type=f32)
                vs[u] = jnp.concatenate([o[:128], o[128:]], axis=1).astype(bf16)

            def stage_b(u):
                half, t = divmod(u, 4)
                PQ[pb + half, t] = jnp.dot(vs.pop(u), G[t if t < 3 else 4], preferred_element_type=f32)

            def d1inv(half):
                for ch_ in range(8):
                    rs = slice(16 * ch_, 16 * ch_ + 16)
                    P1, Q1 = PQ[pb + half, 0, rs, 0:128], PQ[pb + half, 0, rs, 128:256]
                    P2, Q2 = PQ[pb + half, 1, rs, 0:128], PQ[pb + half, 1, rs, 128:256]
                    P3, Q3 = PQ[pb + half, 2, rs, 0:128], PQ[pb + half, 2, rs, 128:256]
                    h0, h4 = PQ[pb + half, 3, rs, 0:128], PQ[pb + half, 3, rs, 128:256]
                    e, o_ = h0 + h4, h0 - h4
                    A, B = P1 + P3, Q1 - Q3
                    u_, v = P1 - P3, Q1 + Q3
                    T1_, T2_ = RS * (u_ - v), RS * (-u_ - v)
                    e1, e2 = e + P2, e - P2
                    o1, o2 = o_ - Q2, o_ + Q2
                    cols = jnp.concatenate(
                        [e1 + A, o1 + T1_, e2 - B, o2 + T2_, e1 - A, o1 - T1_, e2 + B, o2 - T2_], axis=1)
                    bits = _bc(cols.astype(bf16).astype(f32), u32)
                    if half == 0:
                        bs[m, rs, :] = bits >> 16
                    else:
                        bs[m, rs, :] = bs[m, rs, :] | bits

            stage_a(0)
            stage_a(1)
            for u in range(8):
                stage_b(u)
                if u + 2 < 8:
                    stage_a(u + 2)
                if u == 4:
                    d1inv(0)
            d1inv(1)

        lax.fori_loop(0, 4, phI2, 0)

    pl.run_scoped(
        scoped,
        pltpu.VMEM((8, 128, D), u32), pltpu.VMEM((16, 512, 128), bf16), pltpu.VMEM((16, 512, 128), bf16),
        pltpu.VMEM((2, 8, S), bf16), pltpu.VMEM((2, 1, S), bf16),
        pltpu.VMEM((5, 256, 256), bf16), pltpu.VMEM((16, 256, 128), bf16), pltpu.VMEM((3, 128, 128), bf16),
        pltpu.VMEM((2, 4, 128, 256), bf16), pltpu.VMEM((16, 528, 128), f32), pltpu.VMEM((16, 528, 128), f32),
        pltpu.VMEM((64, 128), f32), pltpu.VMEM((4, 4, 128, 256), f32))


def _kernel(x_hbm, mem0_hbm, wq_hbm, wk_hbm, wv_hbm, wo_hbm, xb_hbm, wr_hbm, wi_hbm, gw_hbm,
            g_hbm, h_hbm, misc_hbm, out_hbm,
            xv, xpre, mem0v, gwv, raw, wo, bs, bnat, gbuf, outb, bsems, wsems, msems, osem):
    cp_x = pltpu.make_async_copy(x_hbm.bitcast(u32), xv, msems.at[0])
    cp_mem = pltpu.make_async_copy(mem0_hbm, mem0v, msems.at[2])
    cp_gw = pltpu.make_async_copy(gw_hbm, gwv, msems.at[3])
    wsrc = [w.bitcast(u32) for w in (wq_hbm, wk_hbm, wv_hbm)]
    wo32 = wo_hbm.bitcast(u32)

    def cp_w(p):
        return [pltpu.make_async_copy(wsrc[i].at[:, p, :], raw.at[p, i], wsems.at[p]) for i in range(3)]

    def cp_wo(j):
        off = 128 * j if isinstance(j, int) else pl.multiple_of(128 * j, 128)
        return pltpu.make_async_copy(wo32.at[:, :, pl.ds(off, 128)], wo.at[j], msems.at[4])

    def start_m(g):
        @pl.when(g == 0)
        def _():
            cp_gw.start()
            cp_mem.start()
            cp_x.start()

        for c in cp_w(g):
            c.start()

    def start_i(m):
        for c in cp_w(m + 8):
            c.start()

    _b_phase(xb_hbm, wr_hbm, wi_hbm, g_hbm, h_hbm, misc_hbm, bs, bsems, start_m, start_i)
    bn32 = bnat.bitcast(u32)

    def a_phase(w3, pre, oc, ocr, acc, lhs):
        cp_x.wait()
        cp_gw.wait()
        gwf = gwv[...].astype(f32).reshape(1, D)
        for i in range(32):
            xpre[8 * i:8 * i + 8, :] = jnp.concatenate(
                [xv[32 * i + 12:32 * i + 16, :], xv[32 * i + 28:32 * i + 32, :]], axis=0)

        def prebulk_pair(p):
            for i in range(3):
                e = raw[p, i, pl.ds(0, 512, stride=2), :]
                o = raw[p, i, pl.ds(1, 512, stride=2), :]
                w3[p, 0, i] = (e & jnp.uint32(0xFFFF)) | (o << 16)
                w3[p, 1, i] = (e >> 16) | (o & jnp.uint32(HI))
            for r in range(2):
                for i in range(3):
                    for c in range(2):
                        xl = _w2b(xpre[128 * c:128 * c + 128, :])
                        pre[p, r, i, 256 * c:256 * c + 256, :] = jnp.dot(
                            xl, _w2b(w3[p, r, i]), preferred_element_type=f32)
            for c in range(8):
                xw = xv[pl.ds(pl.multiple_of(64 * p + 8 * c, 8), 8), :]
                xx = _w2b(xw).astype(f32) * gwf
                part = xx[:, 0:128]
                for jj in range(1, 8):
                    part = part + xx[:, 128 * jj:128 * jj + 128]
                lg = jnp.sum(part, axis=1, keepdims=True)
                gbuf[pl.ds(pl.multiple_of(128 * p + 16 * c, 16), 16), :] = jnp.broadcast_to(
                    jax.nn.sigmoid(lg), (16, 128))
            for jj in range(8):
                dst = bn32.at[jj, pl.ds(pl.multiple_of(64 * p, 64), 64), :]
                for m in range(8):
                    dst[pl.ds(m, 8, stride=8), :] = bs[m, pl.ds(pl.multiple_of(8 * p, 8), 8), 128 * jj:128 * jj + 128]

        def prebulk(pp, _):
            @pl.when(pp < 4)
            def _():
                cp_wo(2 * pp).start()
                cp_wo(2 * pp + 1).start()

            for p in (2 * pp, 2 * pp + 1):
                for i in range(3):
                    pltpu.make_async_copy(wsrc[i].at[:, 0, :], raw.at[p, i], wsems.at[p]).wait()
            prebulk_pair(2 * pp)
            prebulk_pair(2 * pp + 1)
            return 0

        lax.fori_loop(0, 8, prebulk, 0)
        cp_mem.wait()
        for j in range(8):
            cp_wo(j).wait()
        oc[...] = jnp.zeros(oc.shape, bf16)
        oc32 = oc.bitcast(u32)

        row = lax.broadcasted_iota(jnp.int32, (40, 128), 0)
        col = lax.broadcasted_iota(jnp.int32, (40, 128), 1)
        mask = ((col < 40) & (row >= 32)) | ((row < 32) & ((col <= row) | ((col >= 32) & (col < 40))))
        scale = DH ** -0.5
        bscale = 2.0 ** -20

        def wo_t(j, h):
            return _w2b(wo[j, h])

        def mix(a, b, g):
            return g * a + (1.0 - g) * (b.astype(f32) * bscale)

        def fill_piece(gr, gw_, src, j, half, accs):
            hs = range(16 * half, 16 * half + 16)
            l = jnp.concatenate([_w2b(src[h]) for h in hs], axis=1)
            w = _w2b(wo[j, 16 * half:16 * half + 16].reshape(16 * 64, 128))
            c = jnp.dot(l, w, preferred_element_type=f32)
            if half == 0:
                return c
            c = c + accs
            for q in range(4):
                sg = 4 * gr + q
                b = bnat[j, pl.ds(pl.multiple_of(32 * sg + 24, 8), 8), :]
                g = gbuf[pl.ds(pl.multiple_of(32 * sg + 24, 8), 8), :]
                outb[pl.ds(pl.multiple_of(128 * gw_ + 32 * q + 24, 8), 8),
                     pl.ds(pl.multiple_of(128 * j, 128), 128)] = mix(c[8 * q:8 * q + 8], b, g).astype(bf16)
            return None

        def out_copy(gi):
            return pltpu.make_async_copy(
                outb.at[pl.ds(pl.multiple_of(128 * gi, 128), 128), :],
                out_hbm.at[pl.ds(pl.multiple_of(128 * gi, 128), 128), :], osem)

        def step(q4, mem, grp4):
            s = 4 * grp4 + q4
            r0 = pl.multiple_of(s * 16, 16)
            xs0 = _w2b(xv[pl.ds(r0, 8), :])
            xs1 = _w2b(xv[pl.ds(r0 + 8, 8), :])
            l1 = jnp.concatenate([xs1[0:8].astype(f32), mem], axis=0).astype(bf16)
            lhs[0:8, :] = pltpu.bitcast(xs0, u32)
            lhs[8:16, :] = pltpu.bitcast(l1, u32)
            grp = grp4 - 1
            gr = jnp.maximum(grp, 0)
            gw_ = jnp.where(grp < 0, 16, grp)
            st = {}
            z8 = jnp.zeros((8, 128), f32)
            s8 = pl.multiple_of(s * 8, 8)

            def proj(h, i):
                r = jnp.dot(_w2b(lhs[...]), _w2b(w3[h // 2, h % 2, i]), preferred_element_type=f32)
                p_ = pre[h // 2, h % 2, i, pl.ds(s8, 8), :]
                if i == 0:
                    st[("qkv", h, i)] = jnp.concatenate([r[0:24], p_, r[24:32]], axis=0)
                else:
                    st[("qkv", h, i)] = jnp.concatenate([r[0:24], p_, r[24:32], z8], axis=0).astype(bf16)

            def qk(h):
                q = st.pop(("qkv", h, 0))
                k = st.pop(("qkv", h, 1))
                sc = lax.dot_general(q, k, NT, preferred_element_type=f32) * scale
                sc = jnp.concatenate([sc, jnp.zeros((40, 80), f32)], axis=1)
                sc = jnp.where(mask, sc, -1e9)
                m = jnp.max(sc, axis=1, keepdims=True)
                e = jnp.exp(sc - m)
                p = e * (1.0 / jnp.sum(e, axis=1, keepdims=True))
                st[("p", h)] = p[:, :48]

            def pv(h):
                o = lax.dot_general(st.pop(("p", h)), st.pop(("qkv", h, 2)), NN, preferred_element_type=f32)
                st[("o", h)] = jnp.concatenate([o[0:24], o[32:40]], axis=0).astype(bf16)
                oc[h, pl.ds(pl.multiple_of(8 * q4, 8), 8), :] = o[24:32].astype(bf16)

            def oproj(h):
                w = jnp.concatenate([wo_t(j, h) for j in range(8)], axis=1)
                c = jnp.dot(st.pop(("o", h)), w, preferred_element_type=f32)
                if h == 0:
                    acc[...] = c
                else:
                    acc[...] += c

            ok = lambda h: 0 <= h < H
            for t in range(H + 4):
                if ok(t):
                    proj(t, 0)
                    proj(t, 1)
                if ok(t - 1):
                    qk(t - 1)
                if ok(t):
                    proj(t, 2)
                else:
                    jj, half = (t - H) // 2, (t - H) % 2
                    st["fill"] = fill_piece(gr, gw_, ocr, 2 * q4 + jj, half, st.get("fill"))
                if ok(t - 3):
                    pv(t - 3)
                if ok(t - 4):
                    oproj(t - 4)
            a = acc[...]
            rs = pl.multiple_of(32 * s, 32)
            b0 = jnp.concatenate([bnat[j, pl.ds(rs, 16), :] for j in range(8)], axis=1)
            b1 = jnp.concatenate([bnat[j, pl.ds(rs + 16, 8), :] for j in range(8)], axis=1)
            g0 = gbuf[pl.ds(rs, 16), :]
            g1 = gbuf[pl.ds(rs + 16, 8), :]
            outb[pl.ds(rs, 16), :] = mix(a[0:16], b0, jnp.tile(g0, (1, 8))).astype(bf16)
            outb[pl.ds(rs + 16, 8), :] = mix(a[16:24], b1, jnp.tile(g1, (1, 8))).astype(bf16)
            return a[24:32]

        def group(grp4, mem):
            @pl.when(grp4 >= 2)
            def _():
                out_copy(grp4 - 2).start()

            ocr[...] = oc32[...]
            for q4 in range(4):
                mem = step(q4, mem, grp4)
            return mem

        lax.fori_loop(0, NSEG // 4, group, mem0v[...].astype(f32))

        out_copy(14).start()

        def tail_copy(j):
            return pltpu.make_async_copy(outb.at[pl.ds(S - 128, 128), pl.ds(128 * j, 128)],
                                         out_hbm.at[pl.ds(S - 128, 128), pl.ds(128 * j, 128)], osem)

        for j in range(8):
            c = fill_piece(15, 15, oc32, j, 0, None)
            fill_piece(15, 15, oc32, j, 1, c)
            tail_copy(j).start()
        for gi in range(15):
            out_copy(gi).wait()
        for j in range(8):
            tail_copy(j).wait()

    pl.run_scoped(
        a_phase,
        pltpu.VMEM((16, 2, 3, 512, 128), u32), pltpu.VMEM((16, 2, 3, 512, 128), f32),
        pltpu.VMEM((H, 32, 128), bf16), pltpu.VMEM((H, 16, 128), u32), pltpu.VMEM((32, D), f32), pltpu.VMEM((16, D), u32))


@jax.jit
def pallas_gated_mix__memory_aug_recurrent_mem_tr__spectral_gfnet__prompt_kernel(
    A_x, A_mem0, A_Wq, A_Wk, A_Wv, A_Wo, A_seg_len, B_x, B_w_r, B_w_i, gate_w,
):
    del A_seg_len
    del B_x
    HB = pl.BlockSpec(memory_space=pltpu.HBM)
    out = pl.pallas_call(
        _kernel,
        out_shape=jax.ShapeDtypeStruct((S, D), bf16),
        in_specs=[HB] * 13,
        out_specs=HB,
        scratch_shapes=[
            pltpu.VMEM((S // 2, D), u32),
            pltpu.VMEM((NSEG * 4, D), u32),
            pltpu.VMEM((M_MEM, D), bf16),
            pltpu.VMEM((D,), bf16),
            pltpu.VMEM((16, 3, D, DH), u32),
            pltpu.VMEM((8, H, DH // 2, 128), u32),
            pltpu.VMEM((8, 128, D), u32),
            pltpu.VMEM((8, S, 128), bf16),
            pltpu.VMEM((S, 128), f32),
            pltpu.VMEM((S + 128, D), bf16),
            pltpu.SemaphoreType.DMA((21,)),
            pltpu.SemaphoreType.DMA((16,)),
            pltpu.SemaphoreType.DMA((6,)),
            pltpu.SemaphoreType.DMA(()),
        ],
        compiler_params=pltpu.CompilerParams(
            vmem_limit_bytes=124 * 2 ** 20, flags={"XLA_TPU_EVENLY_DISTRIBUTE_CRITICAL_NODES": True}),
    )(
        A_x.reshape(S, D), A_mem0.reshape(M_MEM, D), A_Wq, A_Wk, A_Wv, A_Wo,
        A_x.reshape(128, 16, D), B_w_r.T, B_w_i.T, gate_w, _TAB_G, _TAB_H, _TAB_MISC,
    )
    return out.reshape(1, S, D)
```

```python
import numpy as np
import ml_dtypes
import jax
import jax.numpy as jnp
from jax import lax
import jax.experimental.pallas as pl
import jax.experimental.pallas.tpu as pltpu

f32, bf16, u32 = jnp.float32, jnp.bfloat16, jnp.uint32
S, D, H, DH, M_MEM, SEG = 2048, 1024, 32, 128, 8, 32
NSEG = S // SEG
RS = float(1 / np.sqrt(2))
NT = (((1,), (1,)), ((), ()))
NN = (((1,), (0,)), ((), ()))
HI = 0xFFFF0000


def _np_tables():
    bf = ml_dtypes.bfloat16
    dp = np.arange(128)
    j = np.arange(64)

    def cs(f):
        ang = 2 * np.pi * ((f[:, None] * dp[None, :]) % 1024) / 1024
        return np.cos(ang), np.sin(ang)

    G = np.zeros((5, 256, 256))
    for t in range(3):
        r = t + 1
        C, Sn = cs(r + 8 * j)
        C2, S2 = cs(8 - r + 8 * j)
        G[t, 0:64, 0:128] = C
        G[t, 0:64, 128:] = Sn
        G[t, 64:128, 0:128] = C2
        G[t, 64:128, 128:] = -S2
        G[t, 128:192, 0:128] = -Sn
        G[t, 128:192, 128:] = C
        G[t, 192:256, 0:128] = -S2
        G[t, 192:256, 128:] = -C2
    C0, S0 = cs(8 * j)
    C4, S4 = cs(4 + 8 * j)
    G[3, 0:64, 0:128] = C0
    G[3, 128:192, 0:128] = -S0
    G[3, 64:128, 128:] = C4
    G[3, 192:256, 128:] = -S4
    G[4] = G[3]
    G[4, 0, 0:128] = 0.5
    G[4, 128, 0:128] = 0.5 * (-1.0) ** dp
    HH = np.zeros((16, 256, 128))
    for a in range(16):
        ang = 2 * np.pi * (((a + 16 * dp)[:, None] * dp[None, :]) % 2048) / 2048
        HH[a, :128] = np.cos(ang)
        HH[a, 128:] = np.sin(ang)
    misc = np.zeros((3, 128, 128))
    misc[0, 128 - dp[1:], dp[1:]] = 1
    misc[1, 0, 0] = 1
    misc[2, 0, :] = (-1.0) ** dp
    for blk in range(4):
        for k1 in range(16):
            misc[2, 64 + 16 * blk + k1, 16 * blk + 15 - k1] = 1
            misc[2, 64 + 16 * blk + k1, 64 + 16 * blk + (16 - k1) % 16] = 1
    return G.astype(bf), HH.astype(bf), misc.astype(bf)


_TAB_G, _TAB_H, _TAB_MISC = _np_tables()


def _bc(x, dt):
    return lax.bitcast_convert_type(x, dt)


def _w2b(w):
    return pltpu.bitcast(w, bf16)


def _fft16(xs, inverse):
    sg = 1.0 if inverse else -1.0

    def dft4(a, b, c, d):
        t0 = (a[0] + c[0], a[1] + c[1])
        t1 = (a[0] - c[0], a[1] - c[1])
        t2 = (b[0] + d[0], b[1] + d[1])
        t3 = (b[0] - d[0], b[1] - d[1])
        o0 = (t0[0] + t2[0], t0[1] + t2[1])
        o2 = (t0[0] - t2[0], t0[1] - t2[1])
        m = (t1[0] + t3[1], t1[1] - t3[0])
        p = (t1[0] - t3[1], t1[1] + t3[0])
        return [o0, p, o2, m] if inverse else [o0, m, o2, p]

    t = [dft4(xs[a0], xs[4 + a0], xs[8 + a0], xs[12 + a0]) for a0 in range(4)]

    def tw(v, e):
        e = e % 16
        if e == 0:
            return v
        if e == 4:
            return (-v[1], v[0]) if inverse else (v[1], -v[0])
        if e == 2:
            if inverse:
                return ((v[0] - v[1]) * RS, (v[0] + v[1]) * RS)
            return ((v[0] + v[1]) * RS, (v[1] - v[0]) * RS)
        if e == 6:
            if inverse:
                return ((-v[0] - v[1]) * RS, (v[0] - v[1]) * RS)
            return ((v[1] - v[0]) * RS, (-v[0] - v[1]) * RS)
        c = float(np.cos(2 * np.pi * e / 16))
        s = float(sg * np.sin(2 * np.pi * e / 16))
        return (v[0] * c - v[1] * s, v[0] * s + v[1] * c)

    out = [None] * 16
    for k in range(4):
        u = [tw(t[a0][k], a0 * k) for a0 in range(4)]
        r = dft4(*u)
        for m in range(4):
            out[k + 4 * m] = r[m]
    return out


def _b_phase(xb_hbm, wr_hbm, wi_hbm, g_hbm, h_hbm, misc_hbm, bs, sems, start_f, start_i):
    def scoped(xs, wr, wi, wdc, wny_, G, HH, misc, Y, Zr, Zi, WS, PQ):
        xb32 = xb_hbm.bitcast(u32)
        xcp = [pltpu.make_async_copy(xb32.at[:, m, :], xs.at[m], sems.at[m]) for m in range(8)]
        cg = pltpu.make_async_copy(g_hbm, G, sems.at[8])

        def chh(m):
            return pltpu.make_async_copy(h_hbm.at[pl.ds(2 * m, 2)], HH.at[pl.ds(2 * m, 2)], sems.at[13 + m])

        cm = pltpu.make_async_copy(misc_hbm, misc, sems.at[10])
        def wblk(k):
            off = 128 * k if isinstance(k, int) else pl.multiple_of(128 * k, 128)
            return (pltpu.make_async_copy(wr_hbm.at[pl.ds(0, 512), pl.ds(off, 128)], wr.at[k], sems.at[11]),
                    pltpu.make_async_copy(wi_hbm.at[pl.ds(0, 512), pl.ds(off, 128)], wi.at[k], sems.at[12]))

        wny, wnq = [], []
        for i, src in enumerate((wr_hbm, wi_hbm)):
            wny.append(pltpu.make_async_copy(src.at[pl.ds(0, 8), :], wdc.at[i], sems.at[9]))
            wnq.append(pltpu.make_async_copy(src.at[pl.ds(512, 1), :], wny_.at[i], sems.at[12]))
        cm.start()
        for c in wny + wnq:
            c.start()
        xcp[0].start()
        cg.start()
        chh(0).start()
        for m in range(1, 8):
            xcp[m].start()
            chh(m).start()
        cm.wait()
        for c in wny + wnq:
            c.wait()

        st = jnp.concatenate([ref[i, 0:1, 128 * k:128 * (k + 1)].astype(f32)
                              for ref in (wdc, wny_) for i in range(2) for k in range(16)], axis=0)
        stb = st.astype(bf16)
        r1 = jnp.dot(stb, misc[0], preferred_element_type=f32)
        r2 = jnp.dot(stb, misc[1], preferred_element_type=f32)
        rr = jnp.concatenate([r1, r2], axis=0).astype(bf16)
        rp = jnp.dot(misc[2, 64:128, :], rr, preferred_element_type=f32)
        rid = lax.broadcasted_iota(jnp.int32, (64, 128), 0)
        sgn = jnp.where((rid & 16) == 0, 0.5, -0.5)
        WS[...] = 0.5 * st + sgn * rp
        cg.wait()

        def getM(a):
            hc = HH[a, 0:128, :]
            hs = HH[a, 128:256, :]
            return jnp.concatenate(
                [jnp.concatenate([hc, -hs], axis=1), jnp.concatenate([hs, hc], axis=1)], axis=0)

        def phF(m, _):
            for k in (2 * m, 2 * m + 1):
                for c in wblk(k):
                    c.start()
            pltpu.make_async_copy(xb32.at[:, 0, :], xs.at[m], sems.at[m]).wait()
            chh(m).wait()
            def d1(half):
                for ch_ in range(8):
                    w = xs[m, 16 * ch_:16 * ch_ + 16, :]
                    xv = _bc(w << 16, f32) if half == 0 else _bc(w & jnp.uint32(HI), f32)
                    xc = [xv[:, 128 * c:128 * (c + 1)] for c in range(8)]
                    a0, a1 = xc[0] + xc[4], xc[0] - xc[4]
                    b0, b1 = xc[2] + xc[6], xc[2] - xc[6]
                    c0, c1 = xc[1] + xc[5], xc[1] - xc[5]
                    d0, d1_ = xc[3] + xc[7], xc[3] - xc[7]
                    p, q = a0 + b0, c0 + d0
                    y0, y4 = p + q, p - q
                    y2r, y2i = a0 - b0, d0 - c0
                    cm_, cp_ = RS * (c1 - d1_), RS * (c1 + d1_)
                    y1r, y1i = a1 + cm_, -b1 - cp_
                    y3r, y3i = a1 - cm_, b1 - cp_
                    for t, (yr, yi) in enumerate([(y1r, y1i), (y2r, y2i), (y3r, y3i), (y0, y4)]):
                        Y[half, t, 16 * ch_:16 * ch_ + 16, :] = jnp.concatenate([yr, yi], axis=1).astype(bf16)

            Ms = {}
            zs = {}

            def stage_a(u):
                half, t = divmod(u, 5)
                if t < 4:
                    o = lax.dot_general(G[t], Y[half, t], NT, preferred_element_type=f32)
                    zs[u] = jnp.concatenate([o[:128], o[128:]], axis=1).astype(bf16)
                else:
                    zs[u] = lax.dot_general(misc[2, 0:16, :], Y[half, 3, :, 0:128], NT,
                                            preferred_element_type=f32).astype(bf16)

            def stage_b(u):
                half, t = divmod(u, 5)
                a = 2 * m + half
                if half not in Ms:
                    Ms[half] = getM(a)
                Mx = Ms[half]
                if t < 4:
                    X = jnp.dot(zs.pop(u), Mx, preferred_element_type=f32)
                    Zr[a, 128 * t:128 * t + 128, :] = X[:, 0:128]
                    Zi[a, 128 * t:128 * t + 128, :] = X[:, 128:256]
                else:
                    Xn = jnp.dot(zs.pop(u), Mx[0:128, :], preferred_element_type=f32)
                    Zr[a, 512:528, :] = Xn[:, 0:128]
                    Zi[a, 512:528, :] = Xn[:, 128:256]

            d1(0)
            stage_a(0)
            stage_a(1)
            d1(1)
            for u in range(10):
                if u + 2 < 10:
                    stage_b(u)
                    stage_a(u + 2)
                else:
                    stage_b(u)
            return 0

        lax.fori_loop(0, 8, phF, 0)
        start_f()

        for k in range(16):
            for c in wblk(k):
                c.wait()
        wr32 = wr.bitcast(u32)
        wi32 = wi.bitcast(u32)
        hi = jnp.uint32(HI)

        POS = {1: 0, 7: 64, 2: 128, 6: 192, 3: 256, 5: 320, 0: 384, 4: 448}
        row8 = lax.broadcasted_iota(jnp.int32, (8, 128), 0)

        def mid(r, g, special):
            r0 = POS[r] + 8 * g
            if not special:
                r0 = pl.multiple_of(r0, 8)
            xs_ = [(Zr[a, pl.ds(r0, 8), :], Zi[a, pl.ds(r0, 8), :]) for a in range(16)]
            o = _fft16(xs_, False)
            if special:
                xn = [(Zr[a, 512:520, :], Zi[a, 512:520, :]) for a in range(16)]
                on = _fft16(xn, False)
                wsr, wsi = wr32, wi32
            else:
                g32 = pl.multiple_of(32 * g, 32)
                wsr = wr32.at[:, pl.ds(g32, 32), :]
                wsi = wi32.at[:, pl.ds(g32, 32), :]
            ys = []
            for k in range(16):
                a_ = wsr[k, pl.ds(r // 2, 8, stride=4), :]
                b_ = wsi[k, pl.ds(r // 2, 8, stride=4), :]
                if r % 2 == 0:
                    wre, wim = _bc(a_ << 16, f32), _bc(b_ << 16, f32)
                else:
                    wre, wim = _bc(a_ & hi, f32), _bc(b_ & hi, f32)
                if special:
                    wre = jnp.where(row8 == 0, jnp.broadcast_to(WS[k:k + 1, :], (8, 128)), wre)
                    wim = jnp.where(row8 == 0, jnp.broadcast_to(WS[16 + k:17 + k, :], (8, 128)), wim)
                xr, xi = o[k]
                yr = xr * wre - xi * wim
                yi = xr * wim + xi * wre
                if special:
                    nr = jnp.broadcast_to(WS[32 + k:33 + k, :], (8, 128))
                    ni = jnp.broadcast_to(WS[48 + k:49 + k, :], (8, 128))
                    zr_, zi_ = on[k]
                    yr = yr - (zr_ * ni + zi_ * nr)
                    yi = yi + (zr_ * nr - zi_ * ni)
                ys.append((yr, yi))
            u = _fft16(ys, True)
            for a in range(16):
                Zr[a, pl.ds(r0, 8), :] = u[a][0]
                Zi[a, pl.ds(r0, 8), :] = u[a][1]

        mid(0, 0, True)

        def phM(g, _):
            for r in range(1, 8):
                mid(r, g, False)

            @pl.when(g > 0)
            def _():
                mid(0, g, False)

            return 0

        lax.fori_loop(0, 8, phM, 0)

        def phI2(mm, _):
            start_i(mm)
            phI(2 * mm, 0)
            phI(2 * mm + 1, 2)
            return 0

        def phI(m, pb):
            Ms = {}
            vs = {}

            def stage_a(u):
                half, t = divmod(u, 4)
                a = 2 * m + half
                if half not in Ms:
                    Ms[half] = getM(a)
                yy = jnp.concatenate(
                    [Zr[a, 128 * t:128 * t + 128, :], Zi[a, 128 * t:128 * t + 128, :]], axis=1).astype(bf16)
                o = lax.dot_general(Ms[half], yy, NT, preferred_element_type=f32)
                vs[u] = jnp.concatenate([o[:128], o[128:]], axis=1).astype(bf16)

            def stage_b(u):
                half, t = divmod(u, 4)
                PQ[pb + half, t] = jnp.dot(vs.pop(u), G[t if t < 3 else 4], preferred_element_type=f32)

            def d1inv(half):
                for ch_ in range(8):
                    rs = slice(16 * ch_, 16 * ch_ + 16)
                    P1, Q1 = PQ[pb + half, 0, rs, 0:128], PQ[pb + half, 0, rs, 128:256]
                    P2, Q2 = PQ[pb + half, 1, rs, 0:128], PQ[pb + half, 1, rs, 128:256]
                    P3, Q3 = PQ[pb + half, 2, rs, 0:128], PQ[pb + half, 2, rs, 128:256]
                    h0, h4 = PQ[pb + half, 3, rs, 0:128], PQ[pb + half, 3, rs, 128:256]
                    e, o_ = h0 + h4, h0 - h4
                    A, B = P1 + P3, Q1 - Q3
                    u_, v = P1 - P3, Q1 + Q3
                    T1_, T2_ = RS * (u_ - v), RS * (-u_ - v)
                    e1, e2 = e + P2, e - P2
                    o1, o2 = o_ - Q2, o_ + Q2
                    cols = jnp.concatenate(
                        [e1 + A, o1 + T1_, e2 - B, o2 + T2_, e1 - A, o1 - T1_, e2 + B, o2 - T2_], axis=1)
                    bits = _bc(cols.astype(bf16).astype(f32), u32)
                    if half == 0:
                        bs[m, rs, :] = bits >> 16
                    else:
                        bs[m, rs, :] = bs[m, rs, :] | bits

            stage_a(0)
            stage_a(1)
            for u in range(8):
                stage_b(u)
                if u + 2 < 8:
                    stage_a(u + 2)
                if u == 4:
                    d1inv(0)
            d1inv(1)

        lax.fori_loop(0, 4, phI2, 0)

    pl.run_scoped(
        scoped,
        pltpu.VMEM((8, 128, D), u32), pltpu.VMEM((16, 512, 128), bf16), pltpu.VMEM((16, 512, 128), bf16),
        pltpu.VMEM((2, 8, S), bf16), pltpu.VMEM((2, 1, S), bf16),
        pltpu.VMEM((5, 256, 256), bf16), pltpu.VMEM((16, 256, 128), bf16), pltpu.VMEM((3, 128, 128), bf16),
        pltpu.VMEM((2, 4, 128, 256), bf16), pltpu.VMEM((16, 528, 128), f32), pltpu.VMEM((16, 528, 128), f32),
        pltpu.VMEM((64, 128), f32), pltpu.VMEM((4, 4, 128, 256), f32))


def _kernel(x_hbm, mem0_hbm, wq_hbm, wk_hbm, wv_hbm, wo_hbm, xb_hbm, wr_hbm, wi_hbm, gw_hbm,
            g_hbm, h_hbm, misc_hbm, out_hbm,
            xv, xpre, mem0v, gwv, raw, wo, bs, bnat, gbuf, outb, bsems, wsems, msems, osem):
    cp_x = pltpu.make_async_copy(x_hbm.bitcast(u32), xv, msems.at[0])
    cp_mem = pltpu.make_async_copy(mem0_hbm, mem0v, msems.at[2])
    cp_gw = pltpu.make_async_copy(gw_hbm, gwv, msems.at[3])
    wsrc = [w.bitcast(u32) for w in (wq_hbm, wk_hbm, wv_hbm)]
    wo32 = wo_hbm.bitcast(u32)

    def cp_w(p):
        return [pltpu.make_async_copy(wsrc[i].at[:, p, :], raw.at[p, i], wsems.at[p]) for i in range(3)]

    def cp_wo(j):
        off = 128 * j if isinstance(j, int) else pl.multiple_of(128 * j, 128)
        return pltpu.make_async_copy(wo32.at[:, :, pl.ds(off, 128)], wo.at[j], msems.at[4])

    def start_f():
        cp_gw.start()
        cp_mem.start()
        cp_x.start()
        for p in range(4):
            for c in cp_w(p):
                c.start()

    def start_i(mm):
        for q in range(3):
            for c in cp_w(4 + 3 * mm + q):
                c.start()

    _b_phase(xb_hbm, wr_hbm, wi_hbm, g_hbm, h_hbm, misc_hbm, bs, bsems, start_f, start_i)
    bn32 = bnat.bitcast(u32)

    def a_phase(w3, pre, oc, ocr, acc, lhs):
        cp_x.wait()
        cp_gw.wait()
        gwf = gwv[...].astype(f32).reshape(1, D)
        for i in range(32):
            xpre[8 * i:8 * i + 8, :] = jnp.concatenate(
                [xv[32 * i + 12:32 * i + 16, :], xv[32 * i + 28:32 * i + 32, :]], axis=0)

        def prebulk_pair(p):
            for i in range(3):
                e = raw[p, i, pl.ds(0, 512, stride=2), :]
                o = raw[p, i, pl.ds(1, 512, stride=2), :]
                w3[p, 0, i] = (e & jnp.uint32(0xFFFF)) | (o << 16)
                w3[p, 1, i] = (e >> 16) | (o & jnp.uint32(HI))
            for r in range(2):
                for i in range(3):
                    for c in range(2):
                        xl = _w2b(xpre[128 * c:128 * c + 128, :])
                        pre[p, r, i, 256 * c:256 * c + 256, :] = jnp.dot(
                            xl, _w2b(w3[p, r, i]), preferred_element_type=f32)
            for c in range(8):
                xw = xv[pl.ds(pl.multiple_of(64 * p + 8 * c, 8), 8), :]
                xx = _w2b(xw).astype(f32) * gwf
                part = xx[:, 0:128]
                for jj in range(1, 8):
                    part = part + xx[:, 128 * jj:128 * jj + 128]
                lg = jnp.sum(part, axis=1, keepdims=True)
                gbuf[pl.ds(pl.multiple_of(128 * p + 16 * c, 16), 16), :] = jnp.broadcast_to(
                    jax.nn.sigmoid(lg), (16, 128))
            for jj in range(8):
                dst = bn32.at[jj, pl.ds(pl.multiple_of(64 * p, 64), 64), :]
                for m in range(8):
                    dst[pl.ds(m, 8, stride=8), :] = bs[m, pl.ds(pl.multiple_of(8 * p, 8), 8), 128 * jj:128 * jj + 128]

        def prebulk(pp, _):
            @pl.when(pp < 4)
            def _():
                cp_wo(2 * pp).start()
                cp_wo(2 * pp + 1).start()

            for p in (2 * pp, 2 * pp + 1):
                for i in range(3):
                    pltpu.make_async_copy(wsrc[i].at[:, 0, :], raw.at[p, i], wsems.at[p]).wait()
            prebulk_pair(2 * pp)
            prebulk_pair(2 * pp + 1)
            return 0

        lax.fori_loop(0, 8, prebulk, 0)
        cp_mem.wait()
        for j in range(8):
            cp_wo(j).wait()
        oc[...] = jnp.zeros(oc.shape, bf16)
        oc32 = oc.bitcast(u32)

        row = lax.broadcasted_iota(jnp.int32, (40, 128), 0)
        col = lax.broadcasted_iota(jnp.int32, (40, 128), 1)
        mask = ((col < 40) & (row >= 32)) | ((row < 32) & ((col <= row) | ((col >= 32) & (col < 40))))
        scale = DH ** -0.5
        bscale = 2.0 ** -20

        def wo_t(j, h):
            return _w2b(wo[j, h])

        def mix(a, b, g):
            return g * a + (1.0 - g) * (b.astype(f32) * bscale)

        def fill_piece(gr, gw_, src, j, half, accs):
            hs = range(16 * half, 16 * half + 16)
            l = jnp.concatenate([_w2b(src[h]) for h in hs], axis=1)
            w = _w2b(wo[j, 16 * half:16 * half + 16].reshape(16 * 64, 128))
            c = jnp.dot(l, w, preferred_element_type=f32)
            if half == 0:
                return c
            c = c + accs
            for q in range(4):
                sg = 4 * gr + q
                b = bnat[j, pl.ds(pl.multiple_of(32 * sg + 24, 8), 8), :]
                g = gbuf[pl.ds(pl.multiple_of(32 * sg + 24, 8), 8), :]
                outb[pl.ds(pl.multiple_of(128 * gw_ + 32 * q + 24, 8), 8),
                     pl.ds(pl.multiple_of(128 * j, 128), 128)] = mix(c[8 * q:8 * q + 8], b, g).astype(bf16)
            return None

        def out_copy(gi):
            return pltpu.make_async_copy(
                outb.at[pl.ds(pl.multiple_of(128 * gi, 128), 128), :],
                out_hbm.at[pl.ds(pl.multiple_of(128 * gi, 128), 128), :], osem)

        def step(q4, mem, grp4):
            s = 4 * grp4 + q4
            r0 = pl.multiple_of(s * 16, 16)
            xs0 = _w2b(xv[pl.ds(r0, 8), :])
            xs1 = _w2b(xv[pl.ds(r0 + 8, 8), :])
            l1 = jnp.concatenate([xs1[0:8].astype(f32), mem], axis=0).astype(bf16)
            lhs[0:8, :] = pltpu.bitcast(xs0, u32)
            lhs[8:16, :] = pltpu.bitcast(l1, u32)
            grp = grp4 - 1
            gr = jnp.maximum(grp, 0)
            gw_ = jnp.where(grp < 0, 16, grp)
            st = {}
            z8 = jnp.zeros((8, 128), f32)
            s8 = pl.multiple_of(s * 8, 8)

            def proj(h, i):
                r = jnp.dot(_w2b(lhs[...]), _w2b(w3[h // 2, h % 2, i]), preferred_element_type=f32)
                p_ = pre[h // 2, h % 2, i, pl.ds(s8, 8), :]
                if i == 0:
                    st[("qkv", h, i)] = jnp.concatenate([r[0:24], p_, r[24:32]], axis=0)
                else:
                    st[("qkv", h, i)] = jnp.concatenate([r[0:24], p_, r[24:32], z8], axis=0).astype(bf16)

            def qk(h):
                q = st.pop(("qkv", h, 0))
                k = st.pop(("qkv", h, 1))
                sc = lax.dot_general(q, k, NT, preferred_element_type=f32) * scale
                sc = jnp.concatenate([sc, jnp.zeros((40, 80), f32)], axis=1)
                sc = jnp.where(mask, sc, -1e9)
                m = jnp.max(sc, axis=1, keepdims=True)
                e = jnp.exp(sc - m)
                p = e * (1.0 / jnp.sum(e, axis=1, keepdims=True))
                st[("p", h)] = p[:, :48]

            def pv(h):
                o = lax.dot_general(st.pop(("p", h)), st.pop(("qkv", h, 2)), NN, preferred_element_type=f32)
                st[("o", h)] = jnp.concatenate([o[0:24], o[32:40]], axis=0).astype(bf16)
                oc[h, pl.ds(pl.multiple_of(8 * q4, 8), 8), :] = o[24:32].astype(bf16)

            def oproj(h):
                w = jnp.concatenate([wo_t(j, h) for j in range(8)], axis=1)
                c = jnp.dot(st.pop(("o", h)), w, preferred_element_type=f32)
                if h == 0:
                    acc[...] = c
                else:
                    acc[...] += c

            ok = lambda h: 0 <= h < H
            for t in range(H + 4):
                if ok(t):
                    proj(t, 0)
                    proj(t, 1)
                if ok(t - 1):
                    qk(t - 1)
                if ok(t):
                    proj(t, 2)
                else:
                    jj, half = (t - H) // 2, (t - H) % 2
                    st["fill"] = fill_piece(gr, gw_, ocr, 2 * q4 + jj, half, st.get("fill"))
                if ok(t - 3):
                    pv(t - 3)
                if ok(t - 4):
                    oproj(t - 4)
            a = acc[...]
            rs = pl.multiple_of(32 * s, 32)
            b0 = jnp.concatenate([bnat[j, pl.ds(rs, 16), :] for j in range(8)], axis=1)
            b1 = jnp.concatenate([bnat[j, pl.ds(rs + 16, 8), :] for j in range(8)], axis=1)
            g0 = gbuf[pl.ds(rs, 16), :]
            g1 = gbuf[pl.ds(rs + 16, 8), :]
            outb[pl.ds(rs, 16), :] = mix(a[0:16], b0, jnp.tile(g0, (1, 8))).astype(bf16)
            outb[pl.ds(rs + 16, 8), :] = mix(a[16:24], b1, jnp.tile(g1, (1, 8))).astype(bf16)
            return a[24:32]

        def group(grp4, mem):
            @pl.when(grp4 >= 2)
            def _():
                out_copy(grp4 - 2).start()

            ocr[...] = oc32[...]
            for q4 in range(4):
                mem = step(q4, mem, grp4)
            return mem

        lax.fori_loop(0, NSEG // 4, group, mem0v[...].astype(f32))

        out_copy(14).start()

        def tail_copy(j):
            return pltpu.make_async_copy(outb.at[pl.ds(S - 128, 128), pl.ds(128 * j, 128)],
                                         out_hbm.at[pl.ds(S - 128, 128), pl.ds(128 * j, 128)], osem)

        for j in range(8):
            c = fill_piece(15, 15, oc32, j, 0, None)
            fill_piece(15, 15, oc32, j, 1, c)
            tail_copy(j).start()
        for gi in range(15):
            out_copy(gi).wait()
        for j in range(8):
            tail_copy(j).wait()

    pl.run_scoped(
        a_phase,
        pltpu.VMEM((16, 2, 3, 512, 128), u32), pltpu.VMEM((16, 2, 3, 512, 128), f32),
        pltpu.VMEM((H, 32, 128), bf16), pltpu.VMEM((H, 16, 128), u32), pltpu.VMEM((32, D), f32), pltpu.VMEM((16, D), u32))


@jax.jit
def pallas_gated_mix__memory_aug_recurrent_mem_tr__spectral_gfnet__prompt_kernel(
    A_x, A_mem0, A_Wq, A_Wk, A_Wv, A_Wo, A_seg_len, B_x, B_w_r, B_w_i, gate_w,
):
    del A_seg_len
    del B_x
    HB = pl.BlockSpec(memory_space=pltpu.HBM)
    out = pl.pallas_call(
        _kernel,
        out_shape=jax.ShapeDtypeStruct((S, D), bf16),
        in_specs=[HB] * 13,
        out_specs=HB,
        scratch_shapes=[
            pltpu.VMEM((S // 2, D), u32),
            pltpu.VMEM((NSEG * 4, D), u32),
            pltpu.VMEM((M_MEM, D), bf16),
            pltpu.VMEM((D,), bf16),
            pltpu.VMEM((16, 3, D, DH), u32),
            pltpu.VMEM((8, H, DH // 2, 128), u32),
            pltpu.VMEM((8, 128, D), u32),
            pltpu.VMEM((8, S, 128), bf16),
            pltpu.VMEM((S, 128), f32),
            pltpu.VMEM((S + 128, D), bf16),
            pltpu.SemaphoreType.DMA((21,)),
            pltpu.SemaphoreType.DMA((16,)),
            pltpu.SemaphoreType.DMA((6,)),
            pltpu.SemaphoreType.DMA(()),
        ],
        compiler_params=pltpu.CompilerParams(
            vmem_limit_bytes=124 * 2 ** 20, flags={"XLA_TPU_EVENLY_DISTRIBUTE_CRITICAL_NODES": True}),
    )(
        A_x.reshape(S, D), A_mem0.reshape(M_MEM, D), A_Wq, A_Wk, A_Wv, A_Wo,
        A_x.reshape(128, 16, D), B_w_r.T, B_w_i.T, gate_w, _TAB_G, _TAB_H, _TAB_MISC,
    )
    return out.reshape(1, S, D)
```

```python
import numpy as np
import ml_dtypes
import jax
import jax.numpy as jnp
from jax import lax
import jax.experimental.pallas as pl
import jax.experimental.pallas.tpu as pltpu

f32, bf16, u32 = jnp.float32, jnp.bfloat16, jnp.uint32
S, D, H, DH, M_MEM, SEG = 2048, 1024, 32, 128, 8, 32
NSEG = S // SEG
RS = float(1 / np.sqrt(2))
NT = (((1,), (1,)), ((), ()))
NN = (((1,), (0,)), ((), ()))
HI = 0xFFFF0000
OLAG = 6
TAIL_ORDER = "q31 p29 o26 f0 o27 p30 o28 f1 p31 o29 o30 f2 o31 f3"


def _np_tables():
    bf = ml_dtypes.bfloat16
    dp = np.arange(128)
    j = np.arange(64)

    def cs(f):
        ang = 2 * np.pi * ((f[:, None] * dp[None, :]) % 1024) / 1024
        return np.cos(ang), np.sin(ang)

    G = np.zeros((5, 256, 256))
    for t in range(3):
        r = t + 1
        C, Sn = cs(r + 8 * j)
        C2, S2 = cs(8 - r + 8 * j)
        G[t, 0:64, 0:128] = C
        G[t, 0:64, 128:] = Sn
        G[t, 64:128, 0:128] = C2
        G[t, 64:128, 128:] = -S2
        G[t, 128:192, 0:128] = -Sn
        G[t, 128:192, 128:] = C
        G[t, 192:256, 0:128] = -S2
        G[t, 192:256, 128:] = -C2
    C0, S0 = cs(8 * j)
    C4, S4 = cs(4 + 8 * j)
    G[3, 0:64, 0:128] = C0
    G[3, 128:192, 0:128] = -S0
    G[3, 64:128, 128:] = C4
    G[3, 192:256, 128:] = -S4
    G[4] = G[3]
    G[4, 0, 0:128] = 0.5
    G[4, 128, 0:128] = 0.5 * (-1.0) ** dp
    HH = np.zeros((16, 256, 128))
    for a in range(16):
        ang = 2 * np.pi * (((a + 16 * dp)[:, None] * dp[None, :]) % 2048) / 2048
        HH[a, :128] = np.cos(ang)
        HH[a, 128:] = np.sin(ang)
    misc = np.zeros((3, 128, 128))
    misc[0, 128 - dp[1:], dp[1:]] = 1
    misc[1, 0, 0] = 1
    misc[2, 0, :] = (-1.0) ** dp
    for blk in range(4):
        for k1 in range(16):
            misc[2, 64 + 16 * blk + k1, 16 * blk + 15 - k1] = 1
            misc[2, 64 + 16 * blk + k1, 64 + 16 * blk + (16 - k1) % 16] = 1
    return G.astype(bf), HH.astype(bf), misc.astype(bf)


_TAB_G, _TAB_H, _TAB_MISC = _np_tables()


def _bc(x, dt):
    return lax.bitcast_convert_type(x, dt)


def _w2b(w):
    return pltpu.bitcast(w, bf16)


def _fft16(xs, inverse):
    sg = 1.0 if inverse else -1.0

    def dft4(a, b, c, d):
        t0 = (a[0] + c[0], a[1] + c[1])
        t1 = (a[0] - c[0], a[1] - c[1])
        t2 = (b[0] + d[0], b[1] + d[1])
        t3 = (b[0] - d[0], b[1] - d[1])
        o0 = (t0[0] + t2[0], t0[1] + t2[1])
        o2 = (t0[0] - t2[0], t0[1] - t2[1])
        m = (t1[0] + t3[1], t1[1] - t3[0])
        p = (t1[0] - t3[1], t1[1] + t3[0])
        return [o0, p, o2, m] if inverse else [o0, m, o2, p]

    t = [dft4(xs[a0], xs[4 + a0], xs[8 + a0], xs[12 + a0]) for a0 in range(4)]

    def tw(v, e):
        e = e % 16
        if e == 0:
            return v
        if e == 4:
            return (-v[1], v[0]) if inverse else (v[1], -v[0])
        if e == 2:
            if inverse:
                return ((v[0] - v[1]) * RS, (v[0] + v[1]) * RS)
            return ((v[0] + v[1]) * RS, (v[1] - v[0]) * RS)
        if e == 6:
            if inverse:
                return ((-v[0] - v[1]) * RS, (v[0] - v[1]) * RS)
            return ((v[1] - v[0]) * RS, (-v[0] - v[1]) * RS)
        c = float(np.cos(2 * np.pi * e / 16))
        s = float(sg * np.sin(2 * np.pi * e / 16))
        return (v[0] * c - v[1] * s, v[0] * s + v[1] * c)

    out = [None] * 16
    for k in range(4):
        u = [tw(t[a0][k], a0 * k) for a0 in range(4)]
        r = dft4(*u)
        for m in range(4):
            out[k + 4 * m] = r[m]
    return out


def _b_phase(xb_hbm, wr_hbm, wi_hbm, g_hbm, h_hbm, misc_hbm, bs, sems, start_f, start_i):
    def scoped(xs, wr, wi, wdc, wny_, G, HH, misc, Y, Zr, Zi, WS, PQ):
        xb32 = xb_hbm.bitcast(u32)
        xcp = [pltpu.make_async_copy(xb32.at[:, m, :], xs.at[m], sems.at[m]) for m in range(8)]
        cg = pltpu.make_async_copy(g_hbm, G, sems.at[8])

        def chh(m):
            return pltpu.make_async_copy(h_hbm.at[pl.ds(2 * m, 2)], HH.at[pl.ds(2 * m, 2)], sems.at[13 + m])

        cm = pltpu.make_async_copy(misc_hbm, misc, sems.at[10])
        def wblk(k):
            off = 128 * k if isinstance(k, int) else pl.multiple_of(128 * k, 128)
            return (pltpu.make_async_copy(wr_hbm.at[pl.ds(0, 512), pl.ds(off, 128)], wr.at[k], sems.at[11]),
                    pltpu.make_async_copy(wi_hbm.at[pl.ds(0, 512), pl.ds(off, 128)], wi.at[k], sems.at[12]))

        wny, wnq = [], []
        for i, src in enumerate((wr_hbm, wi_hbm)):
            wny.append(pltpu.make_async_copy(src.at[pl.ds(0, 8), :], wdc.at[i], sems.at[9]))
            wnq.append(pltpu.make_async_copy(src.at[pl.ds(512, 1), :], wny_.at[i], sems.at[12]))
        cm.start()
        for c in wny + wnq:
            c.start()
        xcp[0].start()
        cg.start()
        chh(0).start()
        for m in range(1, 8):
            xcp[m].start()
            chh(m).start()
        cm.wait()
        for c in wny + wnq:
            c.wait()

        st = jnp.concatenate([ref[i, 0:1, 128 * k:128 * (k + 1)].astype(f32)
                              for ref in (wdc, wny_) for i in range(2) for k in range(16)], axis=0)
        stb = st.astype(bf16)
        r1 = jnp.dot(stb, misc[0], preferred_element_type=f32)
        r2 = jnp.dot(stb, misc[1], preferred_element_type=f32)
        rr = jnp.concatenate([r1, r2], axis=0).astype(bf16)
        rp = jnp.dot(misc[2, 64:128, :], rr, preferred_element_type=f32)
        rid = lax.broadcasted_iota(jnp.int32, (64, 128), 0)
        sgn = jnp.where((rid & 16) == 0, 0.5, -0.5)
        WS[...] = 0.5 * st + sgn * rp
        cg.wait()

        def getM(a):
            hc = HH[a, 0:128, :]
            hs = HH[a, 128:256, :]
            return jnp.concatenate(
                [jnp.concatenate([hc, -hs], axis=1), jnp.concatenate([hs, hc], axis=1)], axis=0)

        def phF(m, _):
            for k in (2 * m, 2 * m + 1):
                for c in wblk(k):
                    c.start()
            pltpu.make_async_copy(xb32.at[:, 0, :], xs.at[m], sems.at[m]).wait()
            chh(m).wait()
            def d1(half):
                for ch_ in range(8):
                    w = xs[m, 16 * ch_:16 * ch_ + 16, :]
                    xv = _bc(w << 16, f32) if half == 0 else _bc(w & jnp.uint32(HI), f32)
                    xc = [xv[:, 128 * c:128 * (c + 1)] for c in range(8)]
                    a0, a1 = xc[0] + xc[4], xc[0] - xc[4]
                    b0, b1 = xc[2] + xc[6], xc[2] - xc[6]
                    c0, c1 = xc[1] + xc[5], xc[1] - xc[5]
                    d0, d1_ = xc[3] + xc[7], xc[3] - xc[7]
                    p, q = a0 + b0, c0 + d0
                    y0, y4 = p + q, p - q
                    y2r, y2i = a0 - b0, d0 - c0
                    cm_, cp_ = RS * (c1 - d1_), RS * (c1 + d1_)
                    y1r, y1i = a1 + cm_, -b1 - cp_
                    y3r, y3i = a1 - cm_, b1 - cp_
                    for t, (yr, yi) in enumerate([(y1r, y1i), (y2r, y2i), (y3r, y3i), (y0, y4)]):
                        Y[half, t, 16 * ch_:16 * ch_ + 16, :] = jnp.concatenate([yr, yi], axis=1).astype(bf16)

            Ms = {}
            zs = {}

            def stage_a(u):
                half, t = divmod(u, 5)
                if t < 4:
                    o = lax.dot_general(G[t], Y[half, t], NT, preferred_element_type=f32)
                    zs[u] = jnp.concatenate([o[:128], o[128:]], axis=1).astype(bf16)
                else:
                    zs[u] = lax.dot_general(misc[2, 0:16, :], Y[half, 3, :, 0:128], NT,
                                            preferred_element_type=f32).astype(bf16)

            def stage_b(u):
                half, t = divmod(u, 5)
                a = 2 * m + half
                if half not in Ms:
                    Ms[half] = getM(a)
                Mx = Ms[half]
                if t < 4:
                    X = jnp.dot(zs.pop(u), Mx, preferred_element_type=f32)
                    Zr[a, 128 * t:128 * t + 128, :] = X[:, 0:128]
                    Zi[a, 128 * t:128 * t + 128, :] = X[:, 128:256]
                else:
                    Xn = jnp.dot(zs.pop(u), Mx[0:128, :], preferred_element_type=f32)
                    Zr[a, 512:528, :] = Xn[:, 0:128]
                    Zi[a, 512:528, :] = Xn[:, 128:256]

            d1(0)
            stage_a(0)
            stage_a(1)
            d1(1)
            for u in range(10):
                if u + 2 < 10:
                    stage_b(u)
                    stage_a(u + 2)
                else:
                    stage_b(u)
            return 0

        lax.fori_loop(0, 8, phF, 0)
        start_f()

        for k in range(16):
            for c in wblk(k):
                c.wait()
        wr32 = wr.bitcast(u32)
        wi32 = wi.bitcast(u32)
        hi = jnp.uint32(HI)

        POS = {1: 0, 7: 64, 2: 128, 6: 192, 3: 256, 5: 320, 0: 384, 4: 448}
        row8 = lax.broadcasted_iota(jnp.int32, (8, 128), 0)

        def mid(r, g, special):
            r0 = POS[r] + 8 * g
            if not special:
                r0 = pl.multiple_of(r0, 8)
            xs_ = [(Zr[a, pl.ds(r0, 8), :], Zi[a, pl.ds(r0, 8), :]) for a in range(16)]
            o = _fft16(xs_, False)
            if special:
                xn = [(Zr[a, 512:520, :], Zi[a, 512:520, :]) for a in range(16)]
                on = _fft16(xn, False)
                wsr, wsi = wr32, wi32
            else:
                g32 = pl.multiple_of(32 * g, 32)
                wsr = wr32.at[:, pl.ds(g32, 32), :]
                wsi = wi32.at[:, pl.ds(g32, 32), :]
            ys = []
            for k in range(16):
                a_ = wsr[k, pl.ds(r // 2, 8, stride=4), :]
                b_ = wsi[k, pl.ds(r // 2, 8, stride=4), :]
                if r % 2 == 0:
                    wre, wim = _bc(a_ << 16, f32), _bc(b_ << 16, f32)
                else:
                    wre, wim = _bc(a_ & hi, f32), _bc(b_ & hi, f32)
                if special:
                    wre = jnp.where(row8 == 0, jnp.broadcast_to(WS[k:k + 1, :], (8, 128)), wre)
                    wim = jnp.where(row8 == 0, jnp.broadcast_to(WS[16 + k:17 + k, :], (8, 128)), wim)
                xr, xi = o[k]
                yr = xr * wre - xi * wim
                yi = xr * wim + xi * wre
                if special:
                    nr = jnp.broadcast_to(WS[32 + k:33 + k, :], (8, 128))
                    ni = jnp.broadcast_to(WS[48 + k:49 + k, :], (8, 128))
                    zr_, zi_ = on[k]
                    yr = yr - (zr_ * ni + zi_ * nr)
                    yi = yi + (zr_ * nr - zi_ * ni)
                ys.append((yr, yi))
            u = _fft16(ys, True)
            for a in range(16):
                Zr[a, pl.ds(r0, 8), :] = u[a][0]
                Zi[a, pl.ds(r0, 8), :] = u[a][1]

        mid(0, 0, True)

        def phM(g, _):
            for r in range(1, 8):
                mid(r, g, False)

            @pl.when(g > 0)
            def _():
                mid(0, g, False)

            return 0

        lax.fori_loop(0, 8, phM, 0)

        def phI2(mm, _):
            start_i(mm)
            phI(2 * mm, 0)
            phI(2 * mm + 1, 2)
            return 0

        def phI(m, pb):
            Ms = {}
            vs = {}

            def stage_a(u):
                half, t = divmod(u, 4)
                a = 2 * m + half
                if half not in Ms:
                    Ms[half] = getM(a)
                yy = jnp.concatenate(
                    [Zr[a, 128 * t:128 * t + 128, :], Zi[a, 128 * t:128 * t + 128, :]], axis=1).astype(bf16)
                o = lax.dot_general(Ms[half], yy, NT, preferred_element_type=f32)
                vs[u] = jnp.concatenate([o[:128], o[128:]], axis=1).astype(bf16)

            def stage_b(u):
                half, t = divmod(u, 4)
                PQ[pb + half, t] = jnp.dot(vs.pop(u), G[t if t < 3 else 4], preferred_element_type=f32)

            def d1inv(half):
                for ch_ in range(8):
                    rs = slice(16 * ch_, 16 * ch_ + 16)
                    P1, Q1 = PQ[pb + half, 0, rs, 0:128], PQ[pb + half, 0, rs, 128:256]
                    P2, Q2 = PQ[pb + half, 1, rs, 0:128], PQ[pb + half, 1, rs, 128:256]
                    P3, Q3 = PQ[pb + half, 2, rs, 0:128], PQ[pb + half, 2, rs, 128:256]
                    h0, h4 = PQ[pb + half, 3, rs, 0:128], PQ[pb + half, 3, rs, 128:256]
                    e, o_ = h0 + h4, h0 - h4
                    A, B = P1 + P3, Q1 - Q3
                    u_, v = P1 - P3, Q1 + Q3
                    T1_, T2_ = RS * (u_ - v), RS * (-u_ - v)
                    e1, e2 = e + P2, e - P2
                    o1, o2 = o_ - Q2, o_ + Q2
                    cols = jnp.concatenate(
                        [e1 + A, o1 + T1_, e2 - B, o2 + T2_, e1 - A, o1 - T1_, e2 + B, o2 - T2_], axis=1)
                    bits = _bc(cols.astype(bf16).astype(f32), u32)
                    if half == 0:
                        bs[m, rs, :] = bits >> 16
                    else:
                        bs[m, rs, :] = bs[m, rs, :] | bits

            stage_a(0)
            stage_a(1)
            for u in range(8):
                stage_b(u)
                if u + 2 < 8:
                    stage_a(u + 2)
                if u == 4:
                    d1inv(0)
            d1inv(1)

        lax.fori_loop(0, 4, phI2, 0)

    pl.run_scoped(
        scoped,
        pltpu.VMEM((8, 128, D), u32), pltpu.VMEM((16, 512, 128), bf16), pltpu.VMEM((16, 512, 128), bf16),
        pltpu.VMEM((2, 8, S), bf16), pltpu.VMEM((2, 1, S), bf16),
        pltpu.VMEM((5, 256, 256), bf16), pltpu.VMEM((16, 256, 128), bf16), pltpu.VMEM((3, 128, 128), bf16),
        pltpu.VMEM((2, 4, 128, 256), bf16), pltpu.VMEM((16, 528, 128), f32), pltpu.VMEM((16, 528, 128), f32),
        pltpu.VMEM((64, 128), f32), pltpu.VMEM((4, 4, 128, 256), f32))


def _kernel(x_hbm, mem0_hbm, wq_hbm, wk_hbm, wv_hbm, wo_hbm, xb_hbm, wr_hbm, wi_hbm, gw_hbm,
            g_hbm, h_hbm, misc_hbm, out_hbm,
            xv, xpre, mem0v, gwv, raw, wo, bs, bnat, gbuf, outb, bsems, wsems, msems, osem):
    cp_x = pltpu.make_async_copy(x_hbm.bitcast(u32), xv, msems.at[0])
    cp_mem = pltpu.make_async_copy(mem0_hbm, mem0v, msems.at[2])
    cp_gw = pltpu.make_async_copy(gw_hbm, gwv, msems.at[3])
    wsrc = [w.bitcast(u32) for w in (wq_hbm, wk_hbm, wv_hbm)]
    wo32 = wo_hbm.bitcast(u32)

    def cp_w(p):
        return [pltpu.make_async_copy(wsrc[i].at[:, p, :], raw.at[p, i], wsems.at[p]) for i in range(3)]

    def cp_wo(j):
        off = 128 * j if isinstance(j, int) else pl.multiple_of(128 * j, 128)
        return pltpu.make_async_copy(wo32.at[:, :, pl.ds(off, 128)], wo.at[j], msems.at[4])

    def start_f():
        cp_gw.start()
        cp_mem.start()
        cp_x.start()
        for p in range(4):
            for c in cp_w(p):
                c.start()

    def start_i(mm):
        for q in range(3):
            for c in cp_w(4 + 3 * mm + q):
                c.start()

    _b_phase(xb_hbm, wr_hbm, wi_hbm, g_hbm, h_hbm, misc_hbm, bs, bsems, start_f, start_i)
    bn32 = bnat.bitcast(u32)

    def a_phase(w3, pre, oc, ocr, acc, lhs):
        cp_x.wait()
        cp_gw.wait()
        gwf = gwv[...].astype(f32).reshape(1, D)
        for i in range(32):
            xpre[8 * i:8 * i + 8, :] = jnp.concatenate(
                [xv[32 * i + 12:32 * i + 16, :], xv[32 * i + 28:32 * i + 32, :]], axis=0)

        def prebulk_pair(p):
            for i in range(3):
                e = raw[p, i, pl.ds(0, 512, stride=2), :]
                o = raw[p, i, pl.ds(1, 512, stride=2), :]
                w3[p, 0, i] = (e & jnp.uint32(0xFFFF)) | (o << 16)
                w3[p, 1, i] = (e >> 16) | (o & jnp.uint32(HI))
            for r in range(2):
                for i in range(3):
                    for c in range(2):
                        xl = _w2b(xpre[128 * c:128 * c + 128, :])
                        pre[p, r, i, 256 * c:256 * c + 256, :] = jnp.dot(
                            xl, _w2b(w3[p, r, i]), preferred_element_type=f32)
            for c in range(8):
                xw = xv[pl.ds(pl.multiple_of(64 * p + 8 * c, 8), 8), :]
                xx = _w2b(xw).astype(f32) * gwf
                part = xx[:, 0:128]
                for jj in range(1, 8):
                    part = part + xx[:, 128 * jj:128 * jj + 128]
                lg = jnp.sum(part, axis=1, keepdims=True)
                gbuf[pl.ds(pl.multiple_of(128 * p + 16 * c, 16), 16), :] = jnp.broadcast_to(
                    jax.nn.sigmoid(lg), (16, 128))
            for jj in range(8):
                dst = bn32.at[jj, pl.ds(pl.multiple_of(64 * p, 64), 64), :]
                for m in range(8):
                    dst[pl.ds(m, 8, stride=8), :] = bs[m, pl.ds(pl.multiple_of(8 * p, 8), 8), 128 * jj:128 * jj + 128]

        def prebulk(pp, _):
            @pl.when(pp < 4)
            def _():
                cp_wo(2 * pp).start()
                cp_wo(2 * pp + 1).start()

            for p in (2 * pp, 2 * pp + 1):
                for i in range(3):
                    pltpu.make_async_copy(wsrc[i].at[:, 0, :], raw.at[p, i], wsems.at[p]).wait()
            prebulk_pair(2 * pp)
            prebulk_pair(2 * pp + 1)
            return 0

        lax.fori_loop(0, 8, prebulk, 0)
        cp_mem.wait()
        for j in range(8):
            cp_wo(j).wait()
        oc[...] = jnp.zeros(oc.shape, bf16)
        oc32 = oc.bitcast(u32)

        row = lax.broadcasted_iota(jnp.int32, (40, 128), 0)
        col = lax.broadcasted_iota(jnp.int32, (40, 128), 1)
        mask = ((col < 40) & (row >= 32)) | ((row < 32) & ((col <= row) | ((col >= 32) & (col < 40))))
        scale = DH ** -0.5
        bscale = 2.0 ** -20

        def wo_t(j, h):
            return _w2b(wo[j, h])

        def mix(a, b, g):
            return g * a + (1.0 - g) * (b.astype(f32) * bscale)

        def fill_piece(gr, gw_, src, j, half, accs):
            hs = range(16 * half, 16 * half + 16)
            l = jnp.concatenate([_w2b(src[h]) for h in hs], axis=1)
            w = _w2b(wo[j, 16 * half:16 * half + 16].reshape(16 * 64, 128))
            c = jnp.dot(l, w, preferred_element_type=f32)
            if half == 0:
                return c
            c = c + accs
            for q in range(4):
                sg = 4 * gr + q
                b = bnat[j, pl.ds(pl.multiple_of(32 * sg + 24, 8), 8), :]
                g = gbuf[pl.ds(pl.multiple_of(32 * sg + 24, 8), 8), :]
                outb[pl.ds(pl.multiple_of(128 * gw_ + 32 * q + 24, 8), 8),
                     pl.ds(pl.multiple_of(128 * j, 128), 128)] = mix(c[8 * q:8 * q + 8], b, g).astype(bf16)
            return None

        def out_copy(gi):
            return pltpu.make_async_copy(
                outb.at[pl.ds(pl.multiple_of(128 * gi, 128), 128), :],
                out_hbm.at[pl.ds(pl.multiple_of(128 * gi, 128), 128), :], osem)

        def step(q4, mem, grp4):
            s = 4 * grp4 + q4
            r0 = pl.multiple_of(s * 16, 16)
            xs0 = _w2b(xv[pl.ds(r0, 8), :])
            xs1 = _w2b(xv[pl.ds(r0 + 8, 8), :])
            l1 = jnp.concatenate([xs1[0:8].astype(f32), mem], axis=0).astype(bf16)
            lhs[0:8, :] = pltpu.bitcast(xs0, u32)
            lhs[8:16, :] = pltpu.bitcast(l1, u32)
            grp = grp4 - 1
            gr = jnp.maximum(grp, 0)
            gw_ = jnp.where(grp < 0, 16, grp)
            st = {}
            z8 = jnp.zeros((8, 128), f32)
            s8 = pl.multiple_of(s * 8, 8)

            def proj(h, i):
                r = jnp.dot(_w2b(lhs[...]), _w2b(w3[h // 2, h % 2, i]), preferred_element_type=f32)
                p_ = pre[h // 2, h % 2, i, pl.ds(s8, 8), :]
                if i == 0:
                    st[("qkv", h, i)] = jnp.concatenate([r[0:24], p_, r[24:32]], axis=0)
                else:
                    st[("qkv", h, i)] = jnp.concatenate([r[0:24], p_, r[24:32], z8], axis=0).astype(bf16)

            def qk(h):
                q = st.pop(("qkv", h, 0))
                k = st.pop(("qkv", h, 1))
                sc = lax.dot_general(q, k, NT, preferred_element_type=f32) * scale
                sc = jnp.concatenate([sc, jnp.zeros((40, 80), f32)], axis=1)
                sc = jnp.where(mask, sc, -1e9)
                m = jnp.max(sc, axis=1, keepdims=True)
                e = jnp.exp(sc - m)
                p = e * (1.0 / jnp.sum(e, axis=1, keepdims=True))
                st[("p", h)] = p[:, :48]

            def pv(h):
                o = lax.dot_general(st.pop(("p", h)), st.pop(("qkv", h, 2)), NN, preferred_element_type=f32)
                st[("o", h)] = jnp.concatenate([o[0:24], o[32:40]], axis=0).astype(bf16)
                oc[h, pl.ds(pl.multiple_of(8 * q4, 8), 8), :] = o[24:32].astype(bf16)

            def oproj(h):
                w = jnp.concatenate([wo_t(j, h) for j in range(8)], axis=1)
                c = jnp.dot(st.pop(("o", h)), w, preferred_element_type=f32)
                if h == 0:
                    acc[...] = c
                else:
                    acc[...] += c

            ok = lambda h: 0 <= h < H
            for t in range(H):
                proj(t, 0)
                proj(t, 1)
                if ok(t - 1):
                    qk(t - 1)
                proj(t, 2)
                if ok(t - 3):
                    pv(t - 3)
                if ok(t - OLAG):
                    oproj(t - OLAG)

            def fill(n):
                st["fill"] = fill_piece(gr, gw_, ocr, 2 * q4 + n // 2, n % 2, st.get("fill"))

            for tok in TAIL_ORDER.split():
                {"q": qk, "p": pv, "o": oproj, "f": fill}[tok[0]](int(tok[1:]))
            a = acc[...]
            rs = pl.multiple_of(32 * s, 32)
            b0 = jnp.concatenate([bnat[j, pl.ds(rs, 16), :] for j in range(8)], axis=1)
            b1 = jnp.concatenate([bnat[j, pl.ds(rs + 16, 8), :] for j in range(8)], axis=1)
            g0 = gbuf[pl.ds(rs, 16), :]
            g1 = gbuf[pl.ds(rs + 16, 8), :]
            outb[pl.ds(rs, 16), :] = mix(a[0:16], b0, jnp.tile(g0, (1, 8))).astype(bf16)
            outb[pl.ds(rs + 16, 8), :] = mix(a[16:24], b1, jnp.tile(g1, (1, 8))).astype(bf16)
            return a[24:32]

        def group(grp4, mem):
            @pl.when(grp4 >= 2)
            def _():
                out_copy(grp4 - 2).start()

            ocr[...] = oc32[...]
            for q4 in range(4):
                mem = step(q4, mem, grp4)
            return mem

        lax.fori_loop(0, NSEG // 4, group, mem0v[...].astype(f32))

        out_copy(14).start()

        def tail_copy(j):
            return pltpu.make_async_copy(outb.at[pl.ds(S - 128, 128), pl.ds(128 * j, 128)],
                                         out_hbm.at[pl.ds(S - 128, 128), pl.ds(128 * j, 128)], osem)

        for j in range(8):
            c = fill_piece(15, 15, oc32, j, 0, None)
            fill_piece(15, 15, oc32, j, 1, c)
            tail_copy(j).start()
        for gi in range(15):
            out_copy(gi).wait()
        for j in range(8):
            tail_copy(j).wait()

    pl.run_scoped(
        a_phase,
        pltpu.VMEM((16, 2, 3, 512, 128), u32), pltpu.VMEM((16, 2, 3, 512, 128), f32),
        pltpu.VMEM((H, 32, 128), bf16), pltpu.VMEM((H, 16, 128), u32), pltpu.VMEM((32, D), f32), pltpu.VMEM((16, D), u32))


@jax.jit
def pallas_gated_mix__memory_aug_recurrent_mem_tr__spectral_gfnet__prompt_kernel(
    A_x, A_mem0, A_Wq, A_Wk, A_Wv, A_Wo, A_seg_len, B_x, B_w_r, B_w_i, gate_w,
):
    del A_seg_len
    del B_x
    HB = pl.BlockSpec(memory_space=pltpu.HBM)
    out = pl.pallas_call(
        _kernel,
        out_shape=jax.ShapeDtypeStruct((S, D), bf16),
        in_specs=[HB] * 13,
        out_specs=HB,
        scratch_shapes=[
            pltpu.VMEM((S // 2, D), u32),
            pltpu.VMEM((NSEG * 4, D), u32),
            pltpu.VMEM((M_MEM, D), bf16),
            pltpu.VMEM((D,), bf16),
            pltpu.VMEM((16, 3, D, DH), u32),
            pltpu.VMEM((8, H, DH // 2, 128), u32),
            pltpu.VMEM((8, 128, D), u32),
            pltpu.VMEM((8, S, 128), bf16),
            pltpu.VMEM((S, 128), f32),
            pltpu.VMEM((S + 128, D), bf16),
            pltpu.SemaphoreType.DMA((21,)),
            pltpu.SemaphoreType.DMA((16,)),
            pltpu.SemaphoreType.DMA((6,)),
            pltpu.SemaphoreType.DMA(()),
        ],
        compiler_params=pltpu.CompilerParams(
            vmem_limit_bytes=124 * 2 ** 20, flags={"XLA_TPU_EVENLY_DISTRIBUTE_CRITICAL_NODES": True}),
    )(
        A_x.reshape(S, D), A_mem0.reshape(M_MEM, D), A_Wq, A_Wk, A_Wv, A_Wo,
        A_x.reshape(128, 16, D), B_w_r.T, B_w_i.T, gate_w, _TAB_G, _TAB_H, _TAB_MISC,
    )
    return out.reshape(1, S, D)
```

```python
import numpy as np
import ml_dtypes
import jax
import jax.numpy as jnp
from jax import lax
import jax.experimental.pallas as pl
import jax.experimental.pallas.tpu as pltpu

f32, bf16, u32 = jnp.float32, jnp.bfloat16, jnp.uint32
S, D, H, DH, M_MEM, SEG = 2048, 1024, 32, 128, 8, 32
NSEG = S // SEG
RS = float(1 / np.sqrt(2))
NT = (((1,), (1,)), ((), ()))
NN = (((1,), (0,)), ((), ()))
HI = 0xFFFF0000
SLOT_ORDER = "a0 a1 a2 q1 p3 o6"
TAIL_ORDER = "q31 f0 p29 o26 o27 p30 o28 f1 p31 o29 o30 f2 o31 f3"


def _np_tables():
    bf = ml_dtypes.bfloat16
    dp = np.arange(128)
    j = np.arange(64)

    def cs(f):
        ang = 2 * np.pi * ((f[:, None] * dp[None, :]) % 1024) / 1024
        return np.cos(ang), np.sin(ang)

    G = np.zeros((5, 256, 256))
    for t in range(3):
        r = t + 1
        C, Sn = cs(r + 8 * j)
        C2, S2 = cs(8 - r + 8 * j)
        G[t, 0:64, 0:128] = C
        G[t, 0:64, 128:] = Sn
        G[t, 64:128, 0:128] = C2
        G[t, 64:128, 128:] = -S2
        G[t, 128:192, 0:128] = -Sn
        G[t, 128:192, 128:] = C
        G[t, 192:256, 0:128] = -S2
        G[t, 192:256, 128:] = -C2
    C0, S0 = cs(8 * j)
    C4, S4 = cs(4 + 8 * j)
    G[3, 0:64, 0:128] = C0
    G[3, 128:192, 0:128] = -S0
    G[3, 64:128, 128:] = C4
    G[3, 192:256, 128:] = -S4
    G[4] = G[3]
    G[4, 0, 0:128] = 0.5
    G[4, 128, 0:128] = 0.5 * (-1.0) ** dp
    HH = np.zeros((16, 256, 128))
    for a in range(16):
        ang = 2 * np.pi * (((a + 16 * dp)[:, None] * dp[None, :]) % 2048) / 2048
        HH[a, :128] = np.cos(ang)
        HH[a, 128:] = np.sin(ang)
    misc = np.zeros((3, 128, 128))
    misc[0, 128 - dp[1:], dp[1:]] = 1
    misc[1, 0, 0] = 1
    misc[2, 0, :] = (-1.0) ** dp
    for blk in range(4):
        for k1 in range(16):
            misc[2, 64 + 16 * blk + k1, 16 * blk + 15 - k1] = 1
            misc[2, 64 + 16 * blk + k1, 64 + 16 * blk + (16 - k1) % 16] = 1
    return G.astype(bf), HH.astype(bf), misc.astype(bf)


_TAB_G, _TAB_H, _TAB_MISC = _np_tables()


def _bc(x, dt):
    return lax.bitcast_convert_type(x, dt)


def _w2b(w):
    return pltpu.bitcast(w, bf16)


def _fft16(xs, inverse):
    sg = 1.0 if inverse else -1.0

    def dft4(a, b, c, d):
        t0 = (a[0] + c[0], a[1] + c[1])
        t1 = (a[0] - c[0], a[1] - c[1])
        t2 = (b[0] + d[0], b[1] + d[1])
        t3 = (b[0] - d[0], b[1] - d[1])
        o0 = (t0[0] + t2[0], t0[1] + t2[1])
        o2 = (t0[0] - t2[0], t0[1] - t2[1])
        m = (t1[0] + t3[1], t1[1] - t3[0])
        p = (t1[0] - t3[1], t1[1] + t3[0])
        return [o0, p, o2, m] if inverse else [o0, m, o2, p]

    t = [dft4(xs[a0], xs[4 + a0], xs[8 + a0], xs[12 + a0]) for a0 in range(4)]

    def tw(v, e):
        e = e % 16
        if e == 0:
            return v
        if e == 4:
            return (-v[1], v[0]) if inverse else (v[1], -v[0])
        if e == 2:
            if inverse:
                return ((v[0] - v[1]) * RS, (v[0] + v[1]) * RS)
            return ((v[0] + v[1]) * RS, (v[1] - v[0]) * RS)
        if e == 6:
            if inverse:
                return ((-v[0] - v[1]) * RS, (v[0] - v[1]) * RS)
            return ((v[1] - v[0]) * RS, (-v[0] - v[1]) * RS)
        c = float(np.cos(2 * np.pi * e / 16))
        s = float(sg * np.sin(2 * np.pi * e / 16))
        return (v[0] * c - v[1] * s, v[0] * s + v[1] * c)

    out = [None] * 16
    for k in range(4):
        u = [tw(t[a0][k], a0 * k) for a0 in range(4)]
        r = dft4(*u)
        for m in range(4):
            out[k + 4 * m] = r[m]
    return out


def _b_phase(xb_hbm, wr_hbm, wi_hbm, g_hbm, h_hbm, misc_hbm, bs, sems, start_f, start_i):
    def scoped(xs, wr, wi, wdc, wny_, G, HH, misc, Y, Zr, Zi, WS, PQ):
        xb32 = xb_hbm.bitcast(u32)
        xcp = [pltpu.make_async_copy(xb32.at[:, m, :], xs.at[m], sems.at[m]) for m in range(8)]
        cg = pltpu.make_async_copy(g_hbm, G, sems.at[8])

        def chh(m):
            return pltpu.make_async_copy(h_hbm.at[pl.ds(2 * m, 2)], HH.at[pl.ds(2 * m, 2)], sems.at[13 + m])

        cm = pltpu.make_async_copy(misc_hbm, misc, sems.at[10])
        def wblk(k):
            off = 128 * k if isinstance(k, int) else pl.multiple_of(128 * k, 128)
            return (pltpu.make_async_copy(wr_hbm.at[pl.ds(0, 512), pl.ds(off, 128)], wr.at[k], sems.at[11]),
                    pltpu.make_async_copy(wi_hbm.at[pl.ds(0, 512), pl.ds(off, 128)], wi.at[k], sems.at[12]))

        wny, wnq = [], []
        for i, src in enumerate((wr_hbm, wi_hbm)):
            wny.append(pltpu.make_async_copy(src.at[pl.ds(0, 8), :], wdc.at[i], sems.at[9]))
            wnq.append(pltpu.make_async_copy(src.at[pl.ds(512, 1), :], wny_.at[i], sems.at[12]))
        cm.start()
        for c in wny + wnq:
            c.start()
        xcp[0].start()
        cg.start()
        chh(0).start()
        for m in range(1, 8):
            xcp[m].start()
            chh(m).start()
        cm.wait()
        for c in wny + wnq:
            c.wait()

        st = jnp.concatenate([ref[i, 0:1, 128 * k:128 * (k + 1)].astype(f32)
                              for ref in (wdc, wny_) for i in range(2) for k in range(16)], axis=0)
        stb = st.astype(bf16)
        r1 = jnp.dot(stb, misc[0], preferred_element_type=f32)
        r2 = jnp.dot(stb, misc[1], preferred_element_type=f32)
        rr = jnp.concatenate([r1, r2], axis=0).astype(bf16)
        rp = jnp.dot(misc[2, 64:128, :], rr, preferred_element_type=f32)
        rid = lax.broadcasted_iota(jnp.int32, (64, 128), 0)
        sgn = jnp.where((rid & 16) == 0, 0.5, -0.5)
        WS[...] = 0.5 * st + sgn * rp
        cg.wait()

        def getM(a):
            hc = HH[a, 0:128, :]
            hs = HH[a, 128:256, :]
            return jnp.concatenate(
                [jnp.concatenate([hc, -hs], axis=1), jnp.concatenate([hs, hc], axis=1)], axis=0)

        def phF(m, _):
            for k in (2 * m, 2 * m + 1):
                for c in wblk(k):
                    c.start()
            pltpu.make_async_copy(xb32.at[:, 0, :], xs.at[m], sems.at[m]).wait()
            chh(m).wait()
            def d1(half):
                for ch_ in range(8):
                    w = xs[m, 16 * ch_:16 * ch_ + 16, :]
                    xv = _bc(w << 16, f32) if half == 0 else _bc(w & jnp.uint32(HI), f32)
                    xc = [xv[:, 128 * c:128 * (c + 1)] for c in range(8)]
                    a0, a1 = xc[0] + xc[4], xc[0] - xc[4]
                    b0, b1 = xc[2] + xc[6], xc[2] - xc[6]
                    c0, c1 = xc[1] + xc[5], xc[1] - xc[5]
                    d0, d1_ = xc[3] + xc[7], xc[3] - xc[7]
                    p, q = a0 + b0, c0 + d0
                    y0, y4 = p + q, p - q
                    y2r, y2i = a0 - b0, d0 - c0
                    cm_, cp_ = RS * (c1 - d1_), RS * (c1 + d1_)
                    y1r, y1i = a1 + cm_, -b1 - cp_
                    y3r, y3i = a1 - cm_, b1 - cp_
                    for t, (yr, yi) in enumerate([(y1r, y1i), (y2r, y2i), (y3r, y3i), (y0, y4)]):
                        Y[half, t, 16 * ch_:16 * ch_ + 16, :] = jnp.concatenate([yr, yi], axis=1).astype(bf16)

            Ms = {}
            zs = {}

            def stage_a(u):
                half, t = divmod(u, 5)
                if t < 4:
                    o = lax.dot_general(G[t], Y[half, t], NT, preferred_element_type=f32)
                    zs[u] = jnp.concatenate([o[:128], o[128:]], axis=1).astype(bf16)
                else:
                    zs[u] = lax.dot_general(misc[2, 0:16, :], Y[half, 3, :, 0:128], NT,
                                            preferred_element_type=f32).astype(bf16)

            def stage_b(u):
                half, t = divmod(u, 5)
                a = 2 * m + half
                if half not in Ms:
                    Ms[half] = getM(a)
                Mx = Ms[half]
                if t < 4:
                    X = jnp.dot(zs.pop(u), Mx, preferred_element_type=f32)
                    Zr[a, 128 * t:128 * t + 128, :] = X[:, 0:128]
                    Zi[a, 128 * t:128 * t + 128, :] = X[:, 128:256]
                else:
                    Xn = jnp.dot(zs.pop(u), Mx[0:128, :], preferred_element_type=f32)
                    Zr[a, 512:528, :] = Xn[:, 0:128]
                    Zi[a, 512:528, :] = Xn[:, 128:256]

            d1(0)
            stage_a(0)
            stage_a(1)
            d1(1)
            for u in range(10):
                if u + 2 < 10:
                    stage_b(u)
                    stage_a(u + 2)
                else:
                    stage_b(u)
            return 0

        lax.fori_loop(0, 8, phF, 0)
        start_f()

        for k in range(16):
            for c in wblk(k):
                c.wait()
        wr32 = wr.bitcast(u32)
        wi32 = wi.bitcast(u32)
        hi = jnp.uint32(HI)

        POS = {1: 0, 7: 64, 2: 128, 6: 192, 3: 256, 5: 320, 0: 384, 4: 448}
        row8 = lax.broadcasted_iota(jnp.int32, (8, 128), 0)

        def mid(r, g, special):
            r0 = POS[r] + 8 * g
            if not special:
                r0 = pl.multiple_of(r0, 8)
            xs_ = [(Zr[a, pl.ds(r0, 8), :], Zi[a, pl.ds(r0, 8), :]) for a in range(16)]
            o = _fft16(xs_, False)
            if special:
                xn = [(Zr[a, 512:520, :], Zi[a, 512:520, :]) for a in range(16)]
                on = _fft16(xn, False)
                wsr, wsi = wr32, wi32
            else:
                g32 = pl.multiple_of(32 * g, 32)
                wsr = wr32.at[:, pl.ds(g32, 32), :]
                wsi = wi32.at[:, pl.ds(g32, 32), :]
            ys = []
            for k in range(16):
                a_ = wsr[k, pl.ds(r // 2, 8, stride=4), :]
                b_ = wsi[k, pl.ds(r // 2, 8, stride=4), :]
                if r % 2 == 0:
                    wre, wim = _bc(a_ << 16, f32), _bc(b_ << 16, f32)
                else:
                    wre, wim = _bc(a_ & hi, f32), _bc(b_ & hi, f32)
                if special:
                    wre = jnp.where(row8 == 0, jnp.broadcast_to(WS[k:k + 1, :], (8, 128)), wre)
                    wim = jnp.where(row8 == 0, jnp.broadcast_to(WS[16 + k:17 + k, :], (8, 128)), wim)
                xr, xi = o[k]
                yr = xr * wre - xi * wim
                yi = xr * wim + xi * wre
                if special:
                    nr = jnp.broadcast_to(WS[32 + k:33 + k, :], (8, 128))
                    ni = jnp.broadcast_to(WS[48 + k:49 + k, :], (8, 128))
                    zr_, zi_ = on[k]
                    yr = yr - (zr_ * ni + zi_ * nr)
                    yi = yi + (zr_ * nr - zi_ * ni)
                ys.append((yr, yi))
            u = _fft16(ys, True)
            for a in range(16):
                Zr[a, pl.ds(r0, 8), :] = u[a][0]
                Zi[a, pl.ds(r0, 8), :] = u[a][1]

        mid(0, 0, True)

        def phM(g, _):
            for r in range(1, 8):
                mid(r, g, False)

            @pl.when(g > 0)
            def _():
                mid(0, g, False)

            return 0

        lax.fori_loop(0, 8, phM, 0)

        def phI2(mm, _):
            start_i(mm)
            phI(2 * mm, 0)
            phI(2 * mm + 1, 2)
            return 0

        def phI(m, pb):
            Ms = {}
            vs = {}

            def stage_a(u):
                half, t = divmod(u, 4)
                a = 2 * m + half
                if half not in Ms:
                    Ms[half] = getM(a)
                yy = jnp.concatenate(
                    [Zr[a, 128 * t:128 * t + 128, :], Zi[a, 128 * t:128 * t + 128, :]], axis=1).astype(bf16)
                o = lax.dot_general(Ms[half], yy, NT, preferred_element_type=f32)
                vs[u] = jnp.concatenate([o[:128], o[128:]], axis=1).astype(bf16)

            def stage_b(u):
                half, t = divmod(u, 4)
                PQ[pb + half, t] = jnp.dot(vs.pop(u), G[t if t < 3 else 4], preferred_element_type=f32)

            def d1inv(half):
                for ch_ in range(8):
                    rs = slice(16 * ch_, 16 * ch_ + 16)
                    P1, Q1 = PQ[pb + half, 0, rs, 0:128], PQ[pb + half, 0, rs, 128:256]
                    P2, Q2 = PQ[pb + half, 1, rs, 0:128], PQ[pb + half, 1, rs, 128:256]
                    P3, Q3 = PQ[pb + half, 2, rs, 0:128], PQ[pb + half, 2, rs, 128:256]
                    h0, h4 = PQ[pb + half, 3, rs, 0:128], PQ[pb + half, 3, rs, 128:256]
                    e, o_ = h0 + h4, h0 - h4
                    A, B = P1 + P3, Q1 - Q3
                    u_, v = P1 - P3, Q1 + Q3
                    T1_, T2_ = RS * (u_ - v), RS * (-u_ - v)
                    e1, e2 = e + P2, e - P2
                    o1, o2 = o_ - Q2, o_ + Q2
                    cols = jnp.concatenate(
                        [e1 + A, o1 + T1_, e2 - B, o2 + T2_, e1 - A, o1 - T1_, e2 + B, o2 - T2_], axis=1)
                    bits = _bc(cols.astype(bf16).astype(f32), u32)
                    if half == 0:
                        bs[m, rs, :] = bits >> 16
                    else:
                        bs[m, rs, :] = bs[m, rs, :] | bits

            stage_a(0)
            stage_a(1)
            for u in range(8):
                stage_b(u)
                if u + 2 < 8:
                    stage_a(u + 2)
                if u == 4:
                    d1inv(0)
            d1inv(1)

        lax.fori_loop(0, 4, phI2, 0)

    pl.run_scoped(
        scoped,
        pltpu.VMEM((8, 128, D), u32), pltpu.VMEM((16, 512, 128), bf16), pltpu.VMEM((16, 512, 128), bf16),
        pltpu.VMEM((2, 8, S), bf16), pltpu.VMEM((2, 1, S), bf16),
        pltpu.VMEM((5, 256, 256), bf16), pltpu.VMEM((16, 256, 128), bf16), pltpu.VMEM((3, 128, 128), bf16),
        pltpu.VMEM((2, 4, 128, 256), bf16), pltpu.VMEM((16, 528, 128), f32), pltpu.VMEM((16, 528, 128), f32),
        pltpu.VMEM((64, 128), f32), pltpu.VMEM((4, 4, 128, 256), f32))


def _kernel(x_hbm, mem0_hbm, wq_hbm, wk_hbm, wv_hbm, wo_hbm, xb_hbm, wr_hbm, wi_hbm, gw_hbm,
            g_hbm, h_hbm, misc_hbm, out_hbm,
            xv, xpre, mem0v, gwv, raw, wo, bs, bnat, gbuf, outb, bsems, wsems, msems, osem):
    cp_x = pltpu.make_async_copy(x_hbm.bitcast(u32), xv, msems.at[0])
    cp_mem = pltpu.make_async_copy(mem0_hbm, mem0v, msems.at[2])
    cp_gw = pltpu.make_async_copy(gw_hbm, gwv, msems.at[3])
    wsrc = [w.bitcast(u32) for w in (wq_hbm, wk_hbm, wv_hbm)]
    wo32 = wo_hbm.bitcast(u32)

    def cp_w(p):
        return [pltpu.make_async_copy(wsrc[i].at[:, p, :], raw.at[p, i], wsems.at[p]) for i in range(3)]

    def cp_wo(j):
        off = 128 * j if isinstance(j, int) else pl.multiple_of(128 * j, 128)
        return pltpu.make_async_copy(wo32.at[:, :, pl.ds(off, 128)], wo.at[j], msems.at[4])

    def start_f():
        cp_gw.start()
        cp_mem.start()
        cp_x.start()
        for p in range(4):
            for c in cp_w(p):
                c.start()

    def start_i(mm):
        for q in range(3):
            for c in cp_w(4 + 3 * mm + q):
                c.start()

    _b_phase(xb_hbm, wr_hbm, wi_hbm, g_hbm, h_hbm, misc_hbm, bs, bsems, start_f, start_i)
    bn32 = bnat.bitcast(u32)

    def a_phase(w3, pre, oc, ocr, acc, lhs):
        cp_x.wait()
        cp_gw.wait()
        gwf = gwv[...].astype(f32).reshape(1, D)
        for i in range(32):
            xpre[8 * i:8 * i + 8, :] = jnp.concatenate(
                [xv[32 * i + 12:32 * i + 16, :], xv[32 * i + 28:32 * i + 32, :]], axis=0)

        def prebulk_pair(p):
            for i in range(3):
                e = raw[p, i, pl.ds(0, 512, stride=2), :]
                o = raw[p, i, pl.ds(1, 512, stride=2), :]
                w3[p, 0, i] = (e & jnp.uint32(0xFFFF)) | (o << 16)
                w3[p, 1, i] = (e >> 16) | (o & jnp.uint32(HI))
            for r in range(2):
                for i in range(3):
                    for c in range(2):
                        xl = _w2b(xpre[128 * c:128 * c + 128, :])
                        pre[p, r, i, 256 * c:256 * c + 256, :] = jnp.dot(
                            xl, _w2b(w3[p, r, i]), preferred_element_type=f32)
            for c in range(8):
                xw = xv[pl.ds(pl.multiple_of(64 * p + 8 * c, 8), 8), :]
                xx = _w2b(xw).astype(f32) * gwf
                part = xx[:, 0:128]
                for jj in range(1, 8):
                    part = part + xx[:, 128 * jj:128 * jj + 128]
                lg = jnp.sum(part, axis=1, keepdims=True)
                gbuf[pl.ds(pl.multiple_of(128 * p + 16 * c, 16), 16), :] = jnp.broadcast_to(
                    jax.nn.sigmoid(lg), (16, 128))
            for jj in range(8):
                dst = bn32.at[jj, pl.ds(pl.multiple_of(64 * p, 64), 64), :]
                for m in range(8):
                    dst[pl.ds(m, 8, stride=8), :] = bs[m, pl.ds(pl.multiple_of(8 * p, 8), 8), 128 * jj:128 * jj + 128]

        def prebulk(pp, _):
            @pl.when(pp < 4)
            def _():
                cp_wo(2 * pp).start()
                cp_wo(2 * pp + 1).start()

            for p in (2 * pp, 2 * pp + 1):
                for i in range(3):
                    pltpu.make_async_copy(wsrc[i].at[:, 0, :], raw.at[p, i], wsems.at[p]).wait()
            prebulk_pair(2 * pp)
            prebulk_pair(2 * pp + 1)
            return 0

        lax.fori_loop(0, 8, prebulk, 0)
        cp_mem.wait()
        for j in range(8):
            cp_wo(j).wait()
        oc[...] = jnp.zeros(oc.shape, bf16)
        oc32 = oc.bitcast(u32)

        row = lax.broadcasted_iota(jnp.int32, (40, 128), 0)
        col = lax.broadcasted_iota(jnp.int32, (40, 128), 1)
        mask = ((col < 40) & (row >= 32)) | ((row < 32) & ((col <= row) | ((col >= 32) & (col < 40))))
        scale = DH ** -0.5
        bscale = 2.0 ** -20

        def wo_t(j, h):
            return _w2b(wo[j, h])

        def mix(a, b, g):
            return g * a + (1.0 - g) * (b.astype(f32) * bscale)

        def fill_piece(gr, gw_, src, j, half, accs):
            hs = range(16 * half, 16 * half + 16)
            l = jnp.concatenate([_w2b(src[h]) for h in hs], axis=1)
            w = _w2b(wo[j, 16 * half:16 * half + 16].reshape(16 * 64, 128))
            c = jnp.dot(l, w, preferred_element_type=f32)
            if half == 0:
                return c
            c = c + accs
            for q in range(4):
                sg = 4 * gr + q
                b = bnat[j, pl.ds(pl.multiple_of(32 * sg + 24, 8), 8), :]
                g = gbuf[pl.ds(pl.multiple_of(32 * sg + 24, 8), 8), :]
                outb[pl.ds(pl.multiple_of(128 * gw_ + 32 * q + 24, 8), 8),
                     pl.ds(pl.multiple_of(128 * j, 128), 128)] = mix(c[8 * q:8 * q + 8], b, g).astype(bf16)
            return None

        def out_copy(gi):
            return pltpu.make_async_copy(
                outb.at[pl.ds(pl.multiple_of(128 * gi, 128), 128), :],
                out_hbm.at[pl.ds(pl.multiple_of(128 * gi, 128), 128), :], osem)

        def step(q4, mem, grp4):
            s = 4 * grp4 + q4
            r0 = pl.multiple_of(s * 16, 16)
            xs0 = _w2b(xv[pl.ds(r0, 8), :])
            xs1 = _w2b(xv[pl.ds(r0 + 8, 8), :])
            l1 = jnp.concatenate([xs1[0:8].astype(f32), mem], axis=0).astype(bf16)
            lhs[0:8, :] = pltpu.bitcast(xs0, u32)
            lhs[8:16, :] = pltpu.bitcast(l1, u32)
            grp = grp4 - 1
            gr = jnp.maximum(grp, 0)
            gw_ = jnp.where(grp < 0, 16, grp)
            st = {}
            z8 = jnp.zeros((8, 128), f32)
            s8 = pl.multiple_of(s * 8, 8)

            def proj(h, i):
                r = jnp.dot(_w2b(lhs[...]), _w2b(w3[h // 2, h % 2, i]), preferred_element_type=f32)
                p_ = pre[h // 2, h % 2, i, pl.ds(s8, 8), :]
                if i == 0:
                    st[("qkv", h, i)] = jnp.concatenate([r[0:24], p_, r[24:32]], axis=0)
                else:
                    st[("qkv", h, i)] = jnp.concatenate([r[0:24], p_, r[24:32], z8], axis=0).astype(bf16)

            def qk(h):
                q = st.pop(("qkv", h, 0))
                k = st.pop(("qkv", h, 1))
                sc = lax.dot_general(q, k, NT, preferred_element_type=f32) * scale
                sc = jnp.concatenate([sc, jnp.zeros((40, 80), f32)], axis=1)
                sc = jnp.where(mask, sc, -1e9)
                m = jnp.max(sc, axis=1, keepdims=True)
                e = jnp.exp(sc - m)
                p = e * (1.0 / jnp.sum(e, axis=1, keepdims=True))
                st[("p", h)] = p[:, :48]

            def pv(h):
                o = lax.dot_general(st.pop(("p", h)), st.pop(("qkv", h, 2)), NN, preferred_element_type=f32)
                st[("o", h)] = jnp.concatenate([o[0:24], o[32:40]], axis=0).astype(bf16)
                oc[h, pl.ds(pl.multiple_of(8 * q4, 8), 8), :] = o[24:32].astype(bf16)

            def oproj(h):
                w = jnp.concatenate([wo_t(j, h) for j in range(8)], axis=1)
                c = jnp.dot(st.pop(("o", h)), w, preferred_element_type=f32)
                if h == 0:
                    acc[...] = c
                else:
                    acc[...] += c

            ok = lambda h: 0 <= h < H
            for t in range(H):
                for tok in SLOT_ORDER.split():
                    n = int(tok[1:])
                    if tok[0] == "a":
                        proj(t, n)
                    elif ok(t - n):
                        {"q": qk, "p": pv, "o": oproj}[tok[0]](t - n)

            def fill(n):
                st["fill"] = fill_piece(gr, gw_, ocr, 2 * q4 + n // 2, n % 2, st.get("fill"))

            for tok in TAIL_ORDER.split():
                {"q": qk, "p": pv, "o": oproj, "f": fill}[tok[0]](int(tok[1:]))
            a = acc[...]
            rs = pl.multiple_of(32 * s, 32)
            b0 = jnp.concatenate([bnat[j, pl.ds(rs, 16), :] for j in range(8)], axis=1)
            b1 = jnp.concatenate([bnat[j, pl.ds(rs + 16, 8), :] for j in range(8)], axis=1)
            g0 = gbuf[pl.ds(rs, 16), :]
            g1 = gbuf[pl.ds(rs + 16, 8), :]
            outb[pl.ds(rs, 16), :] = mix(a[0:16], b0, jnp.tile(g0, (1, 8))).astype(bf16)
            outb[pl.ds(rs + 16, 8), :] = mix(a[16:24], b1, jnp.tile(g1, (1, 8))).astype(bf16)
            return a[24:32]

        def group(grp4, mem):
            @pl.when(grp4 >= 2)
            def _():
                out_copy(grp4 - 2).start()

            ocr[...] = oc32[...]
            for q4 in range(4):
                mem = step(q4, mem, grp4)
            return mem

        lax.fori_loop(0, NSEG // 4, group, mem0v[...].astype(f32))

        out_copy(14).start()

        def tail_copy(j):
            return pltpu.make_async_copy(outb.at[pl.ds(S - 128, 128), pl.ds(128 * j, 128)],
                                         out_hbm.at[pl.ds(S - 128, 128), pl.ds(128 * j, 128)], osem)

        for j in range(8):
            c = fill_piece(15, 15, oc32, j, 0, None)
            fill_piece(15, 15, oc32, j, 1, c)
            tail_copy(j).start()
        for gi in range(15):
            out_copy(gi).wait()
        for j in range(8):
            tail_copy(j).wait()

    pl.run_scoped(
        a_phase,
        pltpu.VMEM((16, 2, 3, 512, 128), u32), pltpu.VMEM((16, 2, 3, 512, 128), f32),
        pltpu.VMEM((H, 32, 128), bf16), pltpu.VMEM((H, 16, 128), u32), pltpu.VMEM((32, D), f32), pltpu.VMEM((16, D), u32))


@jax.jit
def pallas_gated_mix__memory_aug_recurrent_mem_tr__spectral_gfnet__prompt_kernel(
    A_x, A_mem0, A_Wq, A_Wk, A_Wv, A_Wo, A_seg_len, B_x, B_w_r, B_w_i, gate_w,
):
    del A_seg_len
    del B_x
    HB = pl.BlockSpec(memory_space=pltpu.HBM)
    out = pl.pallas_call(
        _kernel,
        out_shape=jax.ShapeDtypeStruct((S, D), bf16),
        in_specs=[HB] * 13,
        out_specs=HB,
        scratch_shapes=[
            pltpu.VMEM((S // 2, D), u32),
            pltpu.VMEM((NSEG * 4, D), u32),
            pltpu.VMEM((M_MEM, D), bf16),
            pltpu.VMEM((D,), bf16),
            pltpu.VMEM((16, 3, D, DH), u32),
            pltpu.VMEM((8, H, DH // 2, 128), u32),
            pltpu.VMEM((8, 128, D), u32),
            pltpu.VMEM((8, S, 128), bf16),
            pltpu.VMEM((S, 128), f32),
            pltpu.VMEM((S + 128, D), bf16),
            pltpu.SemaphoreType.DMA((21,)),
            pltpu.SemaphoreType.DMA((16,)),
            pltpu.SemaphoreType.DMA((6,)),
            pltpu.SemaphoreType.DMA(()),
        ],
        compiler_params=pltpu.CompilerParams(
            vmem_limit_bytes=124 * 2 ** 20, flags={"XLA_TPU_EVENLY_DISTRIBUTE_CRITICAL_NODES": True}),
    )(
        A_x.reshape(S, D), A_mem0.reshape(M_MEM, D), A_Wq, A_Wk, A_Wv, A_Wo,
        A_x.reshape(128, 16, D), B_w_r.T, B_w_i.T, gate_w, _TAB_G, _TAB_H, _TAB_MISC,
    )
    return out.reshape(1, S, D)
```

```python
import numpy as np
import ml_dtypes
import jax
import jax.numpy as jnp
from jax import lax
import jax.experimental.pallas as pl
import jax.experimental.pallas.tpu as pltpu

f32, bf16, u32 = jnp.float32, jnp.bfloat16, jnp.uint32
S, D, H, DH, M_MEM, SEG = 2048, 1024, 32, 128, 8, 32
NSEG = S // SEG
RS = float(1 / np.sqrt(2))
NT = (((1,), (1,)), ((), ()))
NN = (((1,), (0,)), ((), ()))
HI = 0xFFFF0000
F_LOOK, F_D1, I_LOOK, I_D1 = 4, 1, 4, 4
SLOT_ORDER = "a0 a1 a2 q1 p3 o6"
TAIL_ORDER = "f0 q31 p29 o26 o27 o28 o29 f1 p30 p31 f2 o30 o31 f3"


def _np_tables():
    bf = ml_dtypes.bfloat16
    dp = np.arange(128)
    j = np.arange(64)

    def cs(f):
        ang = 2 * np.pi * ((f[:, None] * dp[None, :]) % 1024) / 1024
        return np.cos(ang), np.sin(ang)

    G = np.zeros((5, 256, 256))
    for t in range(3):
        r = t + 1
        C, Sn = cs(r + 8 * j)
        C2, S2 = cs(8 - r + 8 * j)
        G[t, 0:64, 0:128] = C
        G[t, 0:64, 128:] = Sn
        G[t, 64:128, 0:128] = C2
        G[t, 64:128, 128:] = -S2
        G[t, 128:192, 0:128] = -Sn
        G[t, 128:192, 128:] = C
        G[t, 192:256, 0:128] = -S2
        G[t, 192:256, 128:] = -C2
    C0, S0 = cs(8 * j)
    C4, S4 = cs(4 + 8 * j)
    G[3, 0:64, 0:128] = C0
    G[3, 128:192, 0:128] = -S0
    G[3, 64:128, 128:] = C4
    G[3, 192:256, 128:] = -S4
    G[4] = G[3]
    G[4, 0, 0:128] = 0.5
    G[4, 128, 0:128] = 0.5 * (-1.0) ** dp
    HH = np.zeros((16, 256, 128))
    for a in range(16):
        ang = 2 * np.pi * (((a + 16 * dp)[:, None] * dp[None, :]) % 2048) / 2048
        HH[a, :128] = np.cos(ang)
        HH[a, 128:] = np.sin(ang)
    misc = np.zeros((3, 128, 128))
    misc[0, 128 - dp[1:], dp[1:]] = 1
    misc[1, 0, 0] = 1
    misc[2, 0, :] = (-1.0) ** dp
    for blk in range(4):
        for k1 in range(16):
            misc[2, 64 + 16 * blk + k1, 16 * blk + 15 - k1] = 1
            misc[2, 64 + 16 * blk + k1, 64 + 16 * blk + (16 - k1) % 16] = 1
    return G.astype(bf), HH.astype(bf), misc.astype(bf)


_TAB_G, _TAB_H, _TAB_MISC = _np_tables()


def _bc(x, dt):
    return lax.bitcast_convert_type(x, dt)


def _w2b(w):
    return pltpu.bitcast(w, bf16)


def _fft16(xs, inverse):
    sg = 1.0 if inverse else -1.0

    def dft4(a, b, c, d):
        t0 = (a[0] + c[0], a[1] + c[1])
        t1 = (a[0] - c[0], a[1] - c[1])
        t2 = (b[0] + d[0], b[1] + d[1])
        t3 = (b[0] - d[0], b[1] - d[1])
        o0 = (t0[0] + t2[0], t0[1] + t2[1])
        o2 = (t0[0] - t2[0], t0[1] - t2[1])
        m = (t1[0] + t3[1], t1[1] - t3[0])
        p = (t1[0] - t3[1], t1[1] + t3[0])
        return [o0, p, o2, m] if inverse else [o0, m, o2, p]

    t = [dft4(xs[a0], xs[4 + a0], xs[8 + a0], xs[12 + a0]) for a0 in range(4)]

    def tw(v, e):
        e = e % 16
        if e == 0:
            return v
        if e == 4:
            return (-v[1], v[0]) if inverse else (v[1], -v[0])
        if e == 2:
            if inverse:
                return ((v[0] - v[1]) * RS, (v[0] + v[1]) * RS)
            return ((v[0] + v[1]) * RS, (v[1] - v[0]) * RS)
        if e == 6:
            if inverse:
                return ((-v[0] - v[1]) * RS, (v[0] - v[1]) * RS)
            return ((v[1] - v[0]) * RS, (-v[0] - v[1]) * RS)
        c = float(np.cos(2 * np.pi * e / 16))
        s = float(sg * np.sin(2 * np.pi * e / 16))
        return (v[0] * c - v[1] * s, v[0] * s + v[1] * c)

    out = [None] * 16
    for k in range(4):
        u = [tw(t[a0][k], a0 * k) for a0 in range(4)]
        r = dft4(*u)
        for m in range(4):
            out[k + 4 * m] = r[m]
    return out


def _b_phase(xb_hbm, wr_hbm, wi_hbm, g_hbm, h_hbm, misc_hbm, bs, sems, start_f, start_i):
    def scoped(xs, wr, wi, wdc, wny_, G, HH, misc, Y, Zr, Zi, WS, PQ):
        xb32 = xb_hbm.bitcast(u32)
        xcp = [pltpu.make_async_copy(xb32.at[:, m, :], xs.at[m], sems.at[m]) for m in range(8)]
        cg = pltpu.make_async_copy(g_hbm, G, sems.at[8])

        def chh(m):
            return pltpu.make_async_copy(h_hbm.at[pl.ds(2 * m, 2)], HH.at[pl.ds(2 * m, 2)], sems.at[13 + m])

        cm = pltpu.make_async_copy(misc_hbm, misc, sems.at[10])
        def wblk(k):
            off = 128 * k if isinstance(k, int) else pl.multiple_of(128 * k, 128)
            return (pltpu.make_async_copy(wr_hbm.at[pl.ds(0, 512), pl.ds(off, 128)], wr.at[k], sems.at[11]),
                    pltpu.make_async_copy(wi_hbm.at[pl.ds(0, 512), pl.ds(off, 128)], wi.at[k], sems.at[12]))

        wny, wnq = [], []
        for i, src in enumerate((wr_hbm, wi_hbm)):
            wny.append(pltpu.make_async_copy(src.at[pl.ds(0, 8), :], wdc.at[i], sems.at[9]))
            wnq.append(pltpu.make_async_copy(src.at[pl.ds(512, 1), :], wny_.at[i], sems.at[12]))
        cm.start()
        for c in wny + wnq:
            c.start()
        xcp[0].start()
        cg.start()
        chh(0).start()
        for m in range(1, 8):
            xcp[m].start()
            chh(m).start()
        cm.wait()
        for c in wny + wnq:
            c.wait()

        st = jnp.concatenate([ref[i, 0:1, 128 * k:128 * (k + 1)].astype(f32)
                              for ref in (wdc, wny_) for i in range(2) for k in range(16)], axis=0)
        stb = st.astype(bf16)
        r1 = jnp.dot(stb, misc[0], preferred_element_type=f32)
        r2 = jnp.dot(stb, misc[1], preferred_element_type=f32)
        rr = jnp.concatenate([r1, r2], axis=0).astype(bf16)
        rp = jnp.dot(misc[2, 64:128, :], rr, preferred_element_type=f32)
        rid = lax.broadcasted_iota(jnp.int32, (64, 128), 0)
        sgn = jnp.where((rid & 16) == 0, 0.5, -0.5)
        WS[...] = 0.5 * st + sgn * rp
        cg.wait()

        def getM(a):
            hc = HH[a, 0:128, :]
            hs = HH[a, 128:256, :]
            return jnp.concatenate(
                [jnp.concatenate([hc, -hs], axis=1), jnp.concatenate([hs, hc], axis=1)], axis=0)

        def phF(m, _):
            for k in (2 * m, 2 * m + 1):
                for c in wblk(k):
                    c.start()
            pltpu.make_async_copy(xb32.at[:, 0, :], xs.at[m], sems.at[m]).wait()
            chh(m).wait()
            def d1(half):
                for ch_ in range(8):
                    w = xs[m, 16 * ch_:16 * ch_ + 16, :]
                    xv = _bc(w << 16, f32) if half == 0 else _bc(w & jnp.uint32(HI), f32)
                    xc = [xv[:, 128 * c:128 * (c + 1)] for c in range(8)]
                    a0, a1 = xc[0] + xc[4], xc[0] - xc[4]
                    b0, b1 = xc[2] + xc[6], xc[2] - xc[6]
                    c0, c1 = xc[1] + xc[5], xc[1] - xc[5]
                    d0, d1_ = xc[3] + xc[7], xc[3] - xc[7]
                    p, q = a0 + b0, c0 + d0
                    y0, y4 = p + q, p - q
                    y2r, y2i = a0 - b0, d0 - c0
                    cm_, cp_ = RS * (c1 - d1_), RS * (c1 + d1_)
                    y1r, y1i = a1 + cm_, -b1 - cp_
                    y3r, y3i = a1 - cm_, b1 - cp_
                    for t, (yr, yi) in enumerate([(y1r, y1i), (y2r, y2i), (y3r, y3i), (y0, y4)]):
                        Y[half, t, 16 * ch_:16 * ch_ + 16, :] = jnp.concatenate([yr, yi], axis=1).astype(bf16)

            Ms = {}
            zs = {}

            def stage_a(u):
                half, t = divmod(u, 5)
                if t < 4:
                    o = lax.dot_general(G[t], Y[half, t], NT, preferred_element_type=f32)
                    zs[u] = jnp.concatenate([o[:128], o[128:]], axis=1).astype(bf16)
                else:
                    zs[u] = lax.dot_general(misc[2, 0:16, :], Y[half, 3, :, 0:128], NT,
                                            preferred_element_type=f32).astype(bf16)

            def stage_b(u):
                half, t = divmod(u, 5)
                a = 2 * m + half
                if half not in Ms:
                    Ms[half] = getM(a)
                Mx = Ms[half]
                if t < 4:
                    X = jnp.dot(zs.pop(u), Mx, preferred_element_type=f32)
                    Zr[a, 128 * t:128 * t + 128, :] = X[:, 0:128]
                    Zi[a, 128 * t:128 * t + 128, :] = X[:, 128:256]
                else:
                    Xn = jnp.dot(zs.pop(u), Mx[0:128, :], preferred_element_type=f32)
                    Zr[a, 512:528, :] = Xn[:, 0:128]
                    Zi[a, 512:528, :] = Xn[:, 128:256]

            d1(0)
            for u in range(F_LOOK):
                stage_a(u)
                if u == F_D1:
                    d1(1)
            for u in range(10):
                stage_b(u)
                if u + F_LOOK == F_D1:
                    d1(1)
                if u + F_LOOK < 10:
                    stage_a(u + F_LOOK)
            return 0

        lax.fori_loop(0, 8, phF, 0)
        start_f()

        for k in range(16):
            for c in wblk(k):
                c.wait()
        wr32 = wr.bitcast(u32)
        wi32 = wi.bitcast(u32)
        hi = jnp.uint32(HI)

        POS = {1: 0, 7: 64, 2: 128, 6: 192, 3: 256, 5: 320, 0: 384, 4: 448}
        row8 = lax.broadcasted_iota(jnp.int32, (8, 128), 0)

        def mid(r, g, special):
            r0 = POS[r] + 8 * g
            if not special:
                r0 = pl.multiple_of(r0, 8)
            xs_ = [(Zr[a, pl.ds(r0, 8), :], Zi[a, pl.ds(r0, 8), :]) for a in range(16)]
            o = _fft16(xs_, False)
            if special:
                xn = [(Zr[a, 512:520, :], Zi[a, 512:520, :]) for a in range(16)]
                on = _fft16(xn, False)
                wsr, wsi = wr32, wi32
            else:
                g32 = pl.multiple_of(32 * g, 32)
                wsr = wr32.at[:, pl.ds(g32, 32), :]
                wsi = wi32.at[:, pl.ds(g32, 32), :]
            ys = []
            for k in range(16):
                a_ = wsr[k, pl.ds(r // 2, 8, stride=4), :]
                b_ = wsi[k, pl.ds(r // 2, 8, stride=4), :]
                if r % 2 == 0:
                    wre, wim = _bc(a_ << 16, f32), _bc(b_ << 16, f32)
                else:
                    wre, wim = _bc(a_ & hi, f32), _bc(b_ & hi, f32)
                if special:
                    wre = jnp.where(row8 == 0, jnp.broadcast_to(WS[k:k + 1, :], (8, 128)), wre)
                    wim = jnp.where(row8 == 0, jnp.broadcast_to(WS[16 + k:17 + k, :], (8, 128)), wim)
                xr, xi = o[k]
                yr = xr * wre - xi * wim
                yi = xr * wim + xi * wre
                if special:
                    nr = jnp.broadcast_to(WS[32 + k:33 + k, :], (8, 128))
                    ni = jnp.broadcast_to(WS[48 + k:49 + k, :], (8, 128))
                    zr_, zi_ = on[k]
                    yr = yr - (zr_ * ni + zi_ * nr)
                    yi = yi + (zr_ * nr - zi_ * ni)
                ys.append((yr, yi))
            u = _fft16(ys, True)
            for a in range(16):
                Zr[a, pl.ds(r0, 8), :] = u[a][0]
                Zi[a, pl.ds(r0, 8), :] = u[a][1]

        mid(0, 0, True)

        def phM(g, _):
            for r in range(1, 8):
                mid(r, g, False)

            @pl.when(g > 0)
            def _():
                mid(0, g, False)

            return 0

        lax.fori_loop(0, 8, phM, 0)

        def phI2(mm, _):
            start_i(mm)
            phI(2 * mm, 0)
            phI(2 * mm + 1, 2)
            return 0

        def phI(m, pb):
            Ms = {}
            vs = {}

            def stage_a(u):
                half, t = divmod(u, 4)
                a = 2 * m + half
                if half not in Ms:
                    Ms[half] = getM(a)
                yy = jnp.concatenate(
                    [Zr[a, 128 * t:128 * t + 128, :], Zi[a, 128 * t:128 * t + 128, :]], axis=1).astype(bf16)
                o = lax.dot_general(Ms[half], yy, NT, preferred_element_type=f32)
                vs[u] = jnp.concatenate([o[:128], o[128:]], axis=1).astype(bf16)

            def stage_b(u):
                half, t = divmod(u, 4)
                PQ[pb + half, t] = jnp.dot(vs.pop(u), G[t if t < 3 else 4], preferred_element_type=f32)

            def d1inv(half):
                for ch_ in range(8):
                    rs = slice(16 * ch_, 16 * ch_ + 16)
                    P1, Q1 = PQ[pb + half, 0, rs, 0:128], PQ[pb + half, 0, rs, 128:256]
                    P2, Q2 = PQ[pb + half, 1, rs, 0:128], PQ[pb + half, 1, rs, 128:256]
                    P3, Q3 = PQ[pb + half, 2, rs, 0:128], PQ[pb + half, 2, rs, 128:256]
                    h0, h4 = PQ[pb + half, 3, rs, 0:128], PQ[pb + half, 3, rs, 128:256]
                    e, o_ = h0 + h4, h0 - h4
                    A, B = P1 + P3, Q1 - Q3
                    u_, v = P1 - P3, Q1 + Q3
                    T1_, T2_ = RS * (u_ - v), RS * (-u_ - v)
                    e1, e2 = e + P2, e - P2
                    o1, o2 = o_ - Q2, o_ + Q2
                    cols = jnp.concatenate(
                        [e1 + A, o1 + T1_, e2 - B, o2 + T2_, e1 - A, o1 - T1_, e2 + B, o2 - T2_], axis=1)
                    bits = _bc(cols.astype(bf16).astype(f32), u32)
                    if half == 0:
                        bs[m, rs, :] = bits >> 16
                    else:
                        bs[m, rs, :] = bs[m, rs, :] | bits

            for u in range(I_LOOK):
                stage_a(u)
            for u in range(8):
                stage_b(u)
                if u + I_LOOK < 8:
                    stage_a(u + I_LOOK)
                if u == I_D1:
                    d1inv(0)
            d1inv(1)

        lax.fori_loop(0, 4, phI2, 0)

    pl.run_scoped(
        scoped,
        pltpu.VMEM((8, 128, D), u32), pltpu.VMEM((16, 512, 128), bf16), pltpu.VMEM((16, 512, 128), bf16),
        pltpu.VMEM((2, 8, S), bf16), pltpu.VMEM((2, 1, S), bf16),
        pltpu.VMEM((5, 256, 256), bf16), pltpu.VMEM((16, 256, 128), bf16), pltpu.VMEM((3, 128, 128), bf16),
        pltpu.VMEM((2, 4, 128, 256), bf16), pltpu.VMEM((16, 528, 128), f32), pltpu.VMEM((16, 528, 128), f32),
        pltpu.VMEM((64, 128), f32), pltpu.VMEM((4, 4, 128, 256), f32))


def _kernel(x_hbm, mem0_hbm, wq_hbm, wk_hbm, wv_hbm, wo_hbm, xb_hbm, wr_hbm, wi_hbm, gw_hbm,
            g_hbm, h_hbm, misc_hbm, out_hbm,
            xv, xpre, mem0v, gwv, raw, wo, bs, bnat, gbuf, outb, bsems, wsems, msems, osem):
    cp_x = pltpu.make_async_copy(x_hbm.bitcast(u32), xv, msems.at[0])
    cp_mem = pltpu.make_async_copy(mem0_hbm, mem0v, msems.at[2])
    cp_gw = pltpu.make_async_copy(gw_hbm, gwv, msems.at[3])
    wsrc = [w.bitcast(u32) for w in (wq_hbm, wk_hbm, wv_hbm)]
    wo32 = wo_hbm.bitcast(u32)

    def cp_w(p):
        return [pltpu.make_async_copy(wsrc[i].at[:, p, :], raw.at[p, i], wsems.at[p]) for i in range(3)]

    def cp_wo(j):
        off = 128 * j if isinstance(j, int) else pl.multiple_of(128 * j, 128)
        return pltpu.make_async_copy(wo32.at[:, :, pl.ds(off, 128)], wo.at[j], msems.at[4])

    def start_f():
        cp_gw.start()
        cp_mem.start()
        cp_x.start()
        for p in range(4):
            for c in cp_w(p):
                c.start()

    def start_i(mm):
        for q in range(3):
            for c in cp_w(4 + 3 * mm + q):
                c.start()

    _b_phase(xb_hbm, wr_hbm, wi_hbm, g_hbm, h_hbm, misc_hbm, bs, bsems, start_f, start_i)
    bn32 = bnat.bitcast(u32)

    def a_phase(w3, pre, oc, ocr, acc, lhs):
        cp_x.wait()
        cp_gw.wait()
        gwf = gwv[...].astype(f32).reshape(1, D)
        for i in range(32):
            xpre[8 * i:8 * i + 8, :] = jnp.concatenate(
                [xv[32 * i + 12:32 * i + 16, :], xv[32 * i + 28:32 * i + 32, :]], axis=0)

        def prebulk_pair(p):
            for i in range(3):
                e = raw[p, i, pl.ds(0, 512, stride=2), :]
                o = raw[p, i, pl.ds(1, 512, stride=2), :]
                w3[p, 0, i] = (e & jnp.uint32(0xFFFF)) | (o << 16)
                w3[p, 1, i] = (e >> 16) | (o & jnp.uint32(HI))
            for r in range(2):
                for i in range(3):
                    for c in range(2):
                        xl = _w2b(xpre[128 * c:128 * c + 128, :])
                        pre[p, r, i, 256 * c:256 * c + 256, :] = jnp.dot(
                            xl, _w2b(w3[p, r, i]), preferred_element_type=f32)
            for c in range(8):
                xw = xv[pl.ds(pl.multiple_of(64 * p + 8 * c, 8), 8), :]
                xx = _w2b(xw).astype(f32) * gwf
                part = xx[:, 0:128]
                for jj in range(1, 8):
                    part = part + xx[:, 128 * jj:128 * jj + 128]
                lg = jnp.sum(part, axis=1, keepdims=True)
                gbuf[pl.ds(pl.multiple_of(128 * p + 16 * c, 16), 16), :] = jnp.broadcast_to(
                    jax.nn.sigmoid(lg), (16, 128))
            for jj in range(8):
                dst = bn32.at[jj, pl.ds(pl.multiple_of(64 * p, 64), 64), :]
                for m in range(8):
                    dst[pl.ds(m, 8, stride=8), :] = bs[m, pl.ds(pl.multiple_of(8 * p, 8), 8), 128 * jj:128 * jj + 128]

        def prebulk(pp, _):
            @pl.when(pp < 4)
            def _():
                cp_wo(2 * pp).start()
                cp_wo(2 * pp + 1).start()

            for p in (2 * pp, 2 * pp + 1):
                for i in range(3):
                    pltpu.make_async_copy(wsrc[i].at[:, 0, :], raw.at[p, i], wsems.at[p]).wait()
            prebulk_pair(2 * pp)
            prebulk_pair(2 * pp + 1)
            return 0

        lax.fori_loop(0, 8, prebulk, 0)
        cp_mem.wait()
        for j in range(8):
            cp_wo(j).wait()
        oc[...] = jnp.zeros(oc.shape, bf16)
        oc32 = oc.bitcast(u32)

        row = lax.broadcasted_iota(jnp.int32, (40, 128), 0)
        col = lax.broadcasted_iota(jnp.int32, (40, 128), 1)
        mask = ((col < 40) & (row >= 32)) | ((row < 32) & ((col <= row) | ((col >= 32) & (col < 40))))
        scale = DH ** -0.5
        bscale = 2.0 ** -20

        def wo_t(j, h):
            return _w2b(wo[j, h])

        def mix(a, b, g):
            return g * a + (1.0 - g) * (b.astype(f32) * bscale)

        def fill_piece(gr, gw_, src, j, half, accs):
            hs = range(16 * half, 16 * half + 16)
            l = jnp.concatenate([_w2b(src[h]) for h in hs], axis=1)
            w = _w2b(wo[j, 16 * half:16 * half + 16].reshape(16 * 64, 128))
            c = jnp.dot(l, w, preferred_element_type=f32)
            if half == 0:
                return c
            c = c + accs
            for q in range(4):
                sg = 4 * gr + q
                b = bnat[j, pl.ds(pl.multiple_of(32 * sg + 24, 8), 8), :]
                g = gbuf[pl.ds(pl.multiple_of(32 * sg + 24, 8), 8), :]
                outb[pl.ds(pl.multiple_of(128 * gw_ + 32 * q + 24, 8), 8),
                     128 * j:128 * j + 128] = mix(c[8 * q:8 * q + 8], b, g).astype(bf16)
            return None

        def out_copy(gi):
            return pltpu.make_async_copy(
                outb.at[pl.ds(pl.multiple_of(128 * gi, 128), 128), :],
                out_hbm.at[pl.ds(pl.multiple_of(128 * gi, 128), 128), :], osem)

        def step(q4, mem, grp4):
            s = 4 * grp4 + q4
            r0 = pl.multiple_of(s * 16, 16)
            xs0 = _w2b(xv[pl.ds(r0, 8), :])
            xs1 = _w2b(xv[pl.ds(r0 + 8, 8), :])
            l1 = jnp.concatenate([xs1[0:8].astype(f32), mem], axis=0).astype(bf16)
            lhs[0:8, :] = pltpu.bitcast(xs0, u32)
            lhs[8:16, :] = pltpu.bitcast(l1, u32)
            grp = grp4 - 1
            gr = jnp.maximum(grp, 0)
            gw_ = jnp.where(grp < 0, 16, grp)
            st = {}
            z8 = jnp.zeros((8, 128), f32)
            s8 = pl.multiple_of(s * 8, 8)

            def proj(h, i):
                r = jnp.dot(_w2b(lhs[...]), _w2b(w3[h // 2, h % 2, i]), preferred_element_type=f32)
                p_ = pre[h // 2, h % 2, i, pl.ds(s8, 8), :]
                if i == 0:
                    st[("qkv", h, i)] = jnp.concatenate([r[0:24], p_, r[24:32]], axis=0)
                else:
                    st[("qkv", h, i)] = jnp.concatenate([r[0:24], p_, r[24:32], z8], axis=0).astype(bf16)

            def qk(h):
                q = st.pop(("qkv", h, 0))
                k = st.pop(("qkv", h, 1))
                sc = lax.dot_general(q, k, NT, preferred_element_type=f32) * scale
                sc = jnp.concatenate([sc, jnp.zeros((40, 80), f32)], axis=1)
                sc = jnp.where(mask, sc, -1e9)
                m = jnp.max(sc, axis=1, keepdims=True)
                e = jnp.exp(sc - m)
                p = e * (1.0 / jnp.sum(e, axis=1, keepdims=True))
                st[("p", h)] = p[:, :48]

            def pv(h):
                o = lax.dot_general(st.pop(("p", h)), st.pop(("qkv", h, 2)), NN, preferred_element_type=f32)
                st[("o", h)] = jnp.concatenate([o[0:24], o[32:40]], axis=0).astype(bf16)
                oc[h, 8 * q4:8 * q4 + 8, :] = o[24:32].astype(bf16)

            def oproj(h):
                w = jnp.concatenate([wo_t(j, h) for j in range(8)], axis=1)
                c = jnp.dot(st.pop(("o", h)), w, preferred_element_type=f32)
                if h == 0:
                    acc[...] = c
                else:
                    acc[...] += c

            ok = lambda h: 0 <= h < H
            for t in range(H):
                for tok in SLOT_ORDER.split():
                    n = int(tok[1:])
                    if tok[0] == "a":
                        proj(t, n)
                    elif ok(t - n):
                        {"q": qk, "p": pv, "o": oproj}[tok[0]](t - n)

            def fill(n):
                st["fill"] = fill_piece(gr, gw_, ocr, 2 * q4 + n // 2, n % 2, st.get("fill"))

            for tok in TAIL_ORDER.split():
                {"q": qk, "p": pv, "o": oproj, "f": fill}[tok[0]](int(tok[1:]))
            a = acc[...]
            rs = pl.multiple_of(32 * s, 32)
            b0 = jnp.concatenate([bnat[j, pl.ds(rs, 16), :] for j in range(8)], axis=1)
            b1 = jnp.concatenate([bnat[j, pl.ds(rs + 16, 8), :] for j in range(8)], axis=1)
            g0 = gbuf[pl.ds(rs, 16), :]
            g1 = gbuf[pl.ds(rs + 16, 8), :]
            outb[pl.ds(rs, 16), :] = mix(a[0:16], b0, jnp.tile(g0, (1, 8))).astype(bf16)
            outb[pl.ds(rs + 16, 8), :] = mix(a[16:24], b1, jnp.tile(g1, (1, 8))).astype(bf16)
            return a[24:32]

        def group(grp4, mem):
            @pl.when(grp4 >= 2)
            def _():
                out_copy(grp4 - 2).start()

            ocr[...] = oc32[...]
            for q4 in range(4):
                mem = step(q4, mem, grp4)
            return mem

        lax.fori_loop(0, NSEG // 4, group, mem0v[...].astype(f32))

        out_copy(14).start()

        def tail_copy(j):
            return pltpu.make_async_copy(outb.at[pl.ds(S - 128, 128), pl.ds(128 * j, 128)],
                                         out_hbm.at[pl.ds(S - 128, 128), pl.ds(128 * j, 128)], osem)

        for j in range(8):
            c = fill_piece(15, 15, oc32, j, 0, None)
            fill_piece(15, 15, oc32, j, 1, c)
            tail_copy(j).start()
        for gi in range(15):
            out_copy(gi).wait()
        for j in range(8):
            tail_copy(j).wait()

    pl.run_scoped(
        a_phase,
        pltpu.VMEM((16, 2, 3, 512, 128), u32), pltpu.VMEM((16, 2, 3, 512, 128), f32),
        pltpu.VMEM((H, 32, 128), bf16), pltpu.VMEM((H, 16, 128), u32), pltpu.VMEM((32, D), f32), pltpu.VMEM((16, D), u32))


@jax.jit
def pallas_gated_mix__memory_aug_recurrent_mem_tr__spectral_gfnet__prompt_kernel(
    A_x, A_mem0, A_Wq, A_Wk, A_Wv, A_Wo, A_seg_len, B_x, B_w_r, B_w_i, gate_w,
):
    del A_seg_len
    del B_x
    HB = pl.BlockSpec(memory_space=pltpu.HBM)
    out = pl.pallas_call(
        _kernel,
        out_shape=jax.ShapeDtypeStruct((S, D), bf16),
        in_specs=[HB] * 13,
        out_specs=HB,
        scratch_shapes=[
            pltpu.VMEM((S // 2, D), u32),
            pltpu.VMEM((NSEG * 4, D), u32),
            pltpu.VMEM((M_MEM, D), bf16),
            pltpu.VMEM((D,), bf16),
            pltpu.VMEM((16, 3, D, DH), u32),
            pltpu.VMEM((8, H, DH // 2, 128), u32),
            pltpu.VMEM((8, 128, D), u32),
            pltpu.VMEM((8, S, 128), bf16),
            pltpu.VMEM((S, 128), f32),
            pltpu.VMEM((S + 128, D), bf16),
            pltpu.SemaphoreType.DMA((21,)),
            pltpu.SemaphoreType.DMA((16,)),
            pltpu.SemaphoreType.DMA((6,)),
            pltpu.SemaphoreType.DMA(()),
        ],
        compiler_params=pltpu.CompilerParams(
            vmem_limit_bytes=124 * 2 ** 20, flags={"XLA_TPU_EVENLY_DISTRIBUTE_CRITICAL_NODES": True}),
    )(
        A_x.reshape(S, D), A_mem0.reshape(M_MEM, D), A_Wq, A_Wk, A_Wv, A_Wo,
        A_x.reshape(128, 16, D), B_w_r.T, B_w_i.T, gate_w, _TAB_G, _TAB_H, _TAB_MISC,
    )
    return out.reshape(1, S, D)
```

```python
import numpy as np
import ml_dtypes
import jax
import jax.numpy as jnp
from jax import lax
import jax.experimental.pallas as pl
import jax.experimental.pallas.tpu as pltpu

f32, bf16, u32 = jnp.float32, jnp.bfloat16, jnp.uint32
S, D, H, DH, M_MEM, SEG = 2048, 1024, 32, 128, 8, 32
NSEG = S // SEG
RS = float(1 / np.sqrt(2))
NT = (((1,), (1,)), ((), ()))
NN = (((1,), (0,)), ((), ()))
HI = 0xFFFF0000
F_LOOK, F_D1, I_LOOK = 4, 1, 4
SLOT_ORDER = "a0 a1 a2 q1 p3 o6"
TAIL_ORDER = "f0 q31 p29 o26 o27 o28 o29 f1 p30 p31 f2 o30 o31 f3"


def _np_tables():
    bf = ml_dtypes.bfloat16
    dp = np.arange(128)
    j = np.arange(64)

    def cs(f):
        ang = 2 * np.pi * ((f[:, None] * dp[None, :]) % 1024) / 1024
        return np.cos(ang), np.sin(ang)

    G = np.zeros((5, 256, 256))
    for t in range(3):
        r = t + 1
        C, Sn = cs(r + 8 * j)
        C2, S2 = cs(8 - r + 8 * j)
        G[t, 0:64, 0:128] = C
        G[t, 0:64, 128:] = Sn
        G[t, 64:128, 0:128] = C2
        G[t, 64:128, 128:] = -S2
        G[t, 128:192, 0:128] = -Sn
        G[t, 128:192, 128:] = C
        G[t, 192:256, 0:128] = -S2
        G[t, 192:256, 128:] = -C2
    C0, S0 = cs(8 * j)
    C4, S4 = cs(4 + 8 * j)
    G[3, 0:64, 0:128] = C0
    G[3, 128:192, 0:128] = -S0
    G[3, 64:128, 128:] = C4
    G[3, 192:256, 128:] = -S4
    G[4] = G[3]
    G[4, 0, 0:128] = 0.5
    G[4, 128, 0:128] = 0.5 * (-1.0) ** dp
    HH = np.zeros((16, 256, 128))
    for a in range(16):
        ang = 2 * np.pi * (((a + 16 * dp)[:, None] * dp[None, :]) % 2048) / 2048
        HH[a, :128] = np.cos(ang)
        HH[a, 128:] = np.sin(ang)
    misc = np.zeros((3, 128, 128))
    misc[0, 128 - dp[1:], dp[1:]] = 1
    misc[1, 0, 0] = 1
    misc[2, 0, :] = (-1.0) ** dp
    for blk in range(4):
        for k1 in range(16):
            misc[2, 64 + 16 * blk + k1, 16 * blk + 15 - k1] = 1
            misc[2, 64 + 16 * blk + k1, 64 + 16 * blk + (16 - k1) % 16] = 1
    return G.astype(bf), HH.astype(bf), misc.astype(bf)


_TAB_G, _TAB_H, _TAB_MISC = _np_tables()


def _bc(x, dt):
    return lax.bitcast_convert_type(x, dt)


def _w2b(w):
    return pltpu.bitcast(w, bf16)


def _fft16(xs, inverse):
    sg = 1.0 if inverse else -1.0

    def dft4(a, b, c, d):
        t0 = (a[0] + c[0], a[1] + c[1])
        t1 = (a[0] - c[0], a[1] - c[1])
        t2 = (b[0] + d[0], b[1] + d[1])
        t3 = (b[0] - d[0], b[1] - d[1])
        o0 = (t0[0] + t2[0], t0[1] + t2[1])
        o2 = (t0[0] - t2[0], t0[1] - t2[1])
        m = (t1[0] + t3[1], t1[1] - t3[0])
        p = (t1[0] - t3[1], t1[1] + t3[0])
        return [o0, p, o2, m] if inverse else [o0, m, o2, p]

    t = [dft4(xs[a0], xs[4 + a0], xs[8 + a0], xs[12 + a0]) for a0 in range(4)]

    def tw(v, e):
        e = e % 16
        if e == 0:
            return v
        if e == 4:
            return (-v[1], v[0]) if inverse else (v[1], -v[0])
        if e == 2:
            if inverse:
                return ((v[0] - v[1]) * RS, (v[0] + v[1]) * RS)
            return ((v[0] + v[1]) * RS, (v[1] - v[0]) * RS)
        if e == 6:
            if inverse:
                return ((-v[0] - v[1]) * RS, (v[0] - v[1]) * RS)
            return ((v[1] - v[0]) * RS, (-v[0] - v[1]) * RS)
        c = float(np.cos(2 * np.pi * e / 16))
        s = float(sg * np.sin(2 * np.pi * e / 16))
        return (v[0] * c - v[1] * s, v[0] * s + v[1] * c)

    out = [None] * 16
    for k in range(4):
        u = [tw(t[a0][k], a0 * k) for a0 in range(4)]
        r = dft4(*u)
        for m in range(4):
            out[k + 4 * m] = r[m]
    return out


def _b_phase(xb_hbm, wr_hbm, wi_hbm, g_hbm, h_hbm, misc_hbm, bs, sems, start_f, start_i):
    def scoped(xs, wr, wi, wdc, wny_, G, HH, misc, Y, Zr, Zi, WS, PQ):
        xb32 = xb_hbm.bitcast(u32)
        xcp = [pltpu.make_async_copy(xb32.at[:, m, :], xs.at[m], sems.at[m]) for m in range(8)]
        cg = pltpu.make_async_copy(g_hbm, G, sems.at[8])

        def chh(m):
            return pltpu.make_async_copy(h_hbm.at[pl.ds(2 * m, 2)], HH.at[pl.ds(2 * m, 2)], sems.at[13 + m])

        cm = pltpu.make_async_copy(misc_hbm, misc, sems.at[10])
        def wblk(k):
            off = 128 * k if isinstance(k, int) else pl.multiple_of(128 * k, 128)
            return (pltpu.make_async_copy(wr_hbm.at[pl.ds(0, 512), pl.ds(off, 128)], wr.at[k], sems.at[11]),
                    pltpu.make_async_copy(wi_hbm.at[pl.ds(0, 512), pl.ds(off, 128)], wi.at[k], sems.at[12]))

        wny, wnq = [], []
        for i, src in enumerate((wr_hbm, wi_hbm)):
            wny.append(pltpu.make_async_copy(src.at[pl.ds(0, 8), :], wdc.at[i], sems.at[9]))
            wnq.append(pltpu.make_async_copy(src.at[pl.ds(512, 1), :], wny_.at[i], sems.at[12]))
        cm.start()
        for c in wny + wnq:
            c.start()
        xcp[0].start()
        cg.start()
        chh(0).start()
        for m in range(1, 8):
            xcp[m].start()
            chh(m).start()
        cm.wait()
        for c in wny + wnq:
            c.wait()

        st = jnp.concatenate([ref[i, 0:1, 128 * k:128 * (k + 1)].astype(f32)
                              for ref in (wdc, wny_) for i in range(2) for k in range(16)], axis=0)
        stb = st.astype(bf16)
        r1 = jnp.dot(stb, misc[0], preferred_element_type=f32)
        r2 = jnp.dot(stb, misc[1], preferred_element_type=f32)
        rr = jnp.concatenate([r1, r2], axis=0).astype(bf16)
        rp = jnp.dot(misc[2, 64:128, :], rr, preferred_element_type=f32)
        rid = lax.broadcasted_iota(jnp.int32, (64, 128), 0)
        sgn = jnp.where((rid & 16) == 0, 0.5, -0.5)
        WS[...] = 0.5 * st + sgn * rp
        cg.wait()

        def getM(a):
            hc = HH[a, 0:128, :]
            hs = HH[a, 128:256, :]
            return jnp.concatenate(
                [jnp.concatenate([hc, -hs], axis=1), jnp.concatenate([hs, hc], axis=1)], axis=0)

        def phF(m, _):
            for k in (2 * m, 2 * m + 1):
                for c in wblk(k):
                    c.start()
            pltpu.make_async_copy(xb32.at[:, 0, :], xs.at[m], sems.at[m]).wait()
            chh(m).wait()
            def d1(half):
                for ch_ in range(8):
                    w = xs[m, 16 * ch_:16 * ch_ + 16, :]
                    xv = _bc(w << 16, f32) if half == 0 else _bc(w & jnp.uint32(HI), f32)
                    xc = [xv[:, 128 * c:128 * (c + 1)] for c in range(8)]
                    a0, a1 = xc[0] + xc[4], xc[0] - xc[4]
                    b0, b1 = xc[2] + xc[6], xc[2] - xc[6]
                    c0, c1 = xc[1] + xc[5], xc[1] - xc[5]
                    d0, d1_ = xc[3] + xc[7], xc[3] - xc[7]
                    p, q = a0 + b0, c0 + d0
                    y0, y4 = p + q, p - q
                    y2r, y2i = a0 - b0, d0 - c0
                    cm_, cp_ = RS * (c1 - d1_), RS * (c1 + d1_)
                    y1r, y1i = a1 + cm_, -b1 - cp_
                    y3r, y3i = a1 - cm_, b1 - cp_
                    for t, (yr, yi) in enumerate([(y1r, y1i), (y2r, y2i), (y3r, y3i), (y0, y4)]):
                        Y[half, t, 16 * ch_:16 * ch_ + 16, :] = jnp.concatenate([yr, yi], axis=1).astype(bf16)

            Ms = {}
            zs = {}

            def stage_a(u):
                half, t = divmod(u, 5)
                if t < 4:
                    o = lax.dot_general(G[t], Y[half, t], NT, preferred_element_type=f32)
                    zs[u] = jnp.concatenate([o[:128], o[128:]], axis=1).astype(bf16)
                else:
                    zs[u] = lax.dot_general(misc[2, 0:16, :], Y[half, 3, :, 0:128], NT,
                                            preferred_element_type=f32).astype(bf16)

            def stage_b(u):
                half, t = divmod(u, 5)
                a = 2 * m + half
                if half not in Ms:
                    Ms[half] = getM(a)
                Mx = Ms[half]
                if t < 4:
                    X = jnp.dot(zs.pop(u), Mx, preferred_element_type=f32)
                    Zr[a, 128 * t:128 * t + 128, :] = X[:, 0:128]
                    Zi[a, 128 * t:128 * t + 128, :] = X[:, 128:256]
                else:
                    Xn = jnp.dot(zs.pop(u), Mx[0:128, :], preferred_element_type=f32)
                    Zr[a, 512:528, :] = Xn[:, 0:128]
                    Zi[a, 512:528, :] = Xn[:, 128:256]

            d1(0)
            for u in range(F_LOOK):
                stage_a(u)
                if u == F_D1:
                    d1(1)
            for u in range(10):
                stage_b(u)
                if u + F_LOOK == F_D1:
                    d1(1)
                if u + F_LOOK < 10:
                    stage_a(u + F_LOOK)
            return 0

        lax.fori_loop(0, 8, phF, 0)
        start_f()

        for k in range(16):
            for c in wblk(k):
                c.wait()
        wr32 = wr.bitcast(u32)
        wi32 = wi.bitcast(u32)
        hi = jnp.uint32(HI)

        POS = {1: 0, 7: 64, 2: 128, 6: 192, 3: 256, 5: 320, 0: 384, 4: 448}
        row8 = lax.broadcasted_iota(jnp.int32, (8, 128), 0)

        def mid(r, g, special):
            r0 = POS[r] + 8 * g
            if not special:
                r0 = pl.multiple_of(r0, 8)
            xs_ = [(Zr[a, pl.ds(r0, 8), :], Zi[a, pl.ds(r0, 8), :]) for a in range(16)]
            o = _fft16(xs_, False)
            if special:
                xn = [(Zr[a, 512:520, :], Zi[a, 512:520, :]) for a in range(16)]
                on = _fft16(xn, False)
                wsr, wsi = wr32, wi32
            else:
                g32 = pl.multiple_of(32 * g, 32)
                wsr = wr32.at[:, pl.ds(g32, 32), :]
                wsi = wi32.at[:, pl.ds(g32, 32), :]
            ys = []
            for k in range(16):
                a_ = wsr[k, pl.ds(r // 2, 8, stride=4), :]
                b_ = wsi[k, pl.ds(r // 2, 8, stride=4), :]
                if r % 2 == 0:
                    wre, wim = _bc(a_ << 16, f32), _bc(b_ << 16, f32)
                else:
                    wre, wim = _bc(a_ & hi, f32), _bc(b_ & hi, f32)
                if special:
                    wre = jnp.where(row8 == 0, jnp.broadcast_to(WS[k:k + 1, :], (8, 128)), wre)
                    wim = jnp.where(row8 == 0, jnp.broadcast_to(WS[16 + k:17 + k, :], (8, 128)), wim)
                xr, xi = o[k]
                yr = xr * wre - xi * wim
                yi = xr * wim + xi * wre
                if special:
                    nr = jnp.broadcast_to(WS[32 + k:33 + k, :], (8, 128))
                    ni = jnp.broadcast_to(WS[48 + k:49 + k, :], (8, 128))
                    zr_, zi_ = on[k]
                    yr = yr - (zr_ * ni + zi_ * nr)
                    yi = yi + (zr_ * nr - zi_ * ni)
                ys.append((yr, yi))
            u = _fft16(ys, True)
            for a in range(16):
                Zr[a, pl.ds(r0, 8), :] = u[a][0]
                Zi[a, pl.ds(r0, 8), :] = u[a][1]

        mid(0, 0, True)

        def phM(g, _):
            for r in range(1, 8):
                mid(r, g, False)

            @pl.when(g > 0)
            def _():
                mid(0, g, False)

            return 0

        lax.fori_loop(0, 8, phM, 0)

        def phI(mm, _):
            start_i(mm)
            Ms = {}
            vs = {}

            def stage_a(u):
                c, t = divmod(u, 4)
                a = 4 * mm + c
                if c not in Ms:
                    Ms[c] = getM(a)
                yy = jnp.concatenate(
                    [Zr[a, 128 * t:128 * t + 128, :], Zi[a, 128 * t:128 * t + 128, :]], axis=1).astype(bf16)
                o = lax.dot_general(Ms[c], yy, NT, preferred_element_type=f32)
                vs[u] = jnp.concatenate([o[:128], o[128:]], axis=1).astype(bf16)

            def stage_b(u):
                c, t = divmod(u, 4)
                PQ[c, t] = jnp.dot(vs.pop(u), G[t if t < 3 else 4], preferred_element_type=f32)

            def d1inv(c):
                for ch_ in range(8):
                    rs = slice(16 * ch_, 16 * ch_ + 16)
                    P1, Q1 = PQ[c, 0, rs, 0:128], PQ[c, 0, rs, 128:256]
                    P2, Q2 = PQ[c, 1, rs, 0:128], PQ[c, 1, rs, 128:256]
                    P3, Q3 = PQ[c, 2, rs, 0:128], PQ[c, 2, rs, 128:256]
                    h0, h4 = PQ[c, 3, rs, 0:128], PQ[c, 3, rs, 128:256]
                    e, o_ = h0 + h4, h0 - h4
                    A, B = P1 + P3, Q1 - Q3
                    u_, v = P1 - P3, Q1 + Q3
                    T1_, T2_ = RS * (u_ - v), RS * (-u_ - v)
                    e1, e2 = e + P2, e - P2
                    o1, o2 = o_ - Q2, o_ + Q2
                    cols = jnp.concatenate(
                        [e1 + A, o1 + T1_, e2 - B, o2 + T2_, e1 - A, o1 - T1_, e2 + B, o2 - T2_], axis=1)
                    bits = _bc(cols.astype(bf16).astype(f32), u32)
                    if c % 2 == 0:
                        bs[2 * mm + c // 2, rs, :] = bits >> 16
                    else:
                        bs[2 * mm + c // 2, rs, :] = bs[2 * mm + c // 2, rs, :] | bits

            for u in range(I_LOOK):
                stage_a(u)
            for u in range(16):
                stage_b(u)
                if u + I_LOOK < 16:
                    stage_a(u + I_LOOK)
                if u % 4 == 3:
                    d1inv(u // 4)
            return 0

        lax.fori_loop(0, 4, phI, 0)

    pl.run_scoped(
        scoped,
        pltpu.VMEM((8, 128, D), u32), pltpu.VMEM((16, 512, 128), bf16), pltpu.VMEM((16, 512, 128), bf16),
        pltpu.VMEM((2, 8, S), bf16), pltpu.VMEM((2, 1, S), bf16),
        pltpu.VMEM((5, 256, 256), bf16), pltpu.VMEM((16, 256, 128), bf16), pltpu.VMEM((3, 128, 128), bf16),
        pltpu.VMEM((2, 4, 128, 256), bf16), pltpu.VMEM((16, 528, 128), f32), pltpu.VMEM((16, 528, 128), f32),
        pltpu.VMEM((64, 128), f32), pltpu.VMEM((4, 4, 128, 256), f32))


def _kernel(x_hbm, mem0_hbm, wq_hbm, wk_hbm, wv_hbm, wo_hbm, xb_hbm, wr_hbm, wi_hbm, gw_hbm,
            g_hbm, h_hbm, misc_hbm, out_hbm,
            xv, xpre, mem0v, gwv, raw, wo, bs, bnat, gbuf, outb, bsems, wsems, msems, osem):
    cp_x = pltpu.make_async_copy(x_hbm.bitcast(u32), xv, msems.at[0])
    cp_mem = pltpu.make_async_copy(mem0_hbm, mem0v, msems.at[2])
    cp_gw = pltpu.make_async_copy(gw_hbm, gwv, msems.at[3])
    wsrc = [w.bitcast(u32) for w in (wq_hbm, wk_hbm, wv_hbm)]
    wo32 = wo_hbm.bitcast(u32)

    def cp_w(p):
        return [pltpu.make_async_copy(wsrc[i].at[:, p, :], raw.at[p, i], wsems.at[p]) for i in range(3)]

    def cp_wo(j):
        off = 128 * j if isinstance(j, int) else pl.multiple_of(128 * j, 128)
        return pltpu.make_async_copy(wo32.at[:, :, pl.ds(off, 128)], wo.at[j], msems.at[4])

    def start_f():
        cp_gw.start()
        cp_mem.start()
        cp_x.start()
        for p in range(4):
            for c in cp_w(p):
                c.start()

    def start_i(mm):
        for q in range(3):
            for c in cp_w(4 + 3 * mm + q):
                c.start()

    _b_phase(xb_hbm, wr_hbm, wi_hbm, g_hbm, h_hbm, misc_hbm, bs, bsems, start_f, start_i)
    bn32 = bnat.bitcast(u32)

    def a_phase(w3, pre, oc, ocr, acc, lhs):
        cp_x.wait()
        cp_gw.wait()
        gwf = gwv[...].astype(f32).reshape(1, D)
        for i in range(32):
            xpre[8 * i:8 * i + 8, :] = jnp.concatenate(
                [xv[32 * i + 12:32 * i + 16, :], xv[32 * i + 28:32 * i + 32, :]], axis=0)

        def prebulk_pair(p):
            for i in range(3):
                e = raw[p, i, pl.ds(0, 512, stride=2), :]
                o = raw[p, i, pl.ds(1, 512, stride=2), :]
                w3[p, 0, i] = (e & jnp.uint32(0xFFFF)) | (o << 16)
                w3[p, 1, i] = (e >> 16) | (o & jnp.uint32(HI))
            for r in range(2):
                for i in range(3):
                    for c in range(2):
                        xl = _w2b(xpre[128 * c:128 * c + 128, :])
                        pre[p, r, i, 256 * c:256 * c + 256, :] = jnp.dot(
                            xl, _w2b(w3[p, r, i]), preferred_element_type=f32)
            for c in range(8):
                xw = xv[pl.ds(pl.multiple_of(64 * p + 8 * c, 8), 8), :]
                xx = _w2b(xw).astype(f32) * gwf
                part = xx[:, 0:128]
                for jj in range(1, 8):
                    part = part + xx[:, 128 * jj:128 * jj + 128]
                lg = jnp.sum(part, axis=1, keepdims=True)
                gbuf[pl.ds(pl.multiple_of(128 * p + 16 * c, 16), 16), :] = jnp.broadcast_to(
                    jax.nn.sigmoid(lg), (16, 128))
            for jj in range(8):
                dst = bn32.at[jj, pl.ds(pl.multiple_of(64 * p, 64), 64), :]
                for m in range(8):
                    dst[pl.ds(m, 8, stride=8), :] = bs[m, pl.ds(pl.multiple_of(8 * p, 8), 8), 128 * jj:128 * jj + 128]

        def prebulk(pp, _):
            @pl.when(pp < 4)
            def _():
                cp_wo(2 * pp).start()
                cp_wo(2 * pp + 1).start()

            for p in (2 * pp, 2 * pp + 1):
                for i in range(3):
                    pltpu.make_async_copy(wsrc[i].at[:, 0, :], raw.at[p, i], wsems.at[p]).wait()
            prebulk_pair(2 * pp)
            prebulk_pair(2 * pp + 1)
            return 0

        lax.fori_loop(0, 8, prebulk, 0)
        cp_mem.wait()
        for j in range(8):
            cp_wo(j).wait()
        oc[...] = jnp.zeros(oc.shape, bf16)
        oc32 = oc.bitcast(u32)

        row = lax.broadcasted_iota(jnp.int32, (40, 128), 0)
        col = lax.broadcasted_iota(jnp.int32, (40, 128), 1)
        mask = ((col < 40) & (row >= 32)) | ((row < 32) & ((col <= row) | ((col >= 32) & (col < 40))))
        scale = DH ** -0.5
        bscale = 2.0 ** -20

        def wo_t(j, h):
            return _w2b(wo[j, h])

        def mix(a, b, g):
            return g * a + (1.0 - g) * (b.astype(f32) * bscale)

        def fill_piece(gr, gw_, src, j, half, accs):
            hs = range(16 * half, 16 * half + 16)
            l = jnp.concatenate([_w2b(src[h]) for h in hs], axis=1)
            w = _w2b(wo[j, 16 * half:16 * half + 16].reshape(16 * 64, 128))
            c = jnp.dot(l, w, preferred_element_type=f32)
            if half == 0:
                return c
            c = c + accs
            for q in range(4):
                sg = 4 * gr + q
                b = bnat[j, pl.ds(pl.multiple_of(32 * sg + 24, 8), 8), :]
                g = gbuf[pl.ds(pl.multiple_of(32 * sg + 24, 8), 8), :]
                outb[pl.ds(pl.multiple_of(128 * gw_ + 32 * q + 24, 8), 8),
                     128 * j:128 * j + 128] = mix(c[8 * q:8 * q + 8], b, g).astype(bf16)
            return None

        def out_copy(gi):
            return pltpu.make_async_copy(
                outb.at[pl.ds(pl.multiple_of(128 * gi, 128), 128), :],
                out_hbm.at[pl.ds(pl.multiple_of(128 * gi, 128), 128), :], osem)

        def step(q4, mem, grp4):
            s = 4 * grp4 + q4
            r0 = pl.multiple_of(s * 16, 16)
            xs0 = _w2b(xv[pl.ds(r0, 8), :])
            xs1 = _w2b(xv[pl.ds(r0 + 8, 8), :])
            l1 = jnp.concatenate([xs1[0:8].astype(f32), mem], axis=0).astype(bf16)
            lhs[0:8, :] = pltpu.bitcast(xs0, u32)
            lhs[8:16, :] = pltpu.bitcast(l1, u32)
            grp = grp4 - 1
            gr = jnp.maximum(grp, 0)
            gw_ = jnp.where(grp < 0, 16, grp)
            st = {}
            z8 = jnp.zeros((8, 128), f32)
            s8 = pl.multiple_of(s * 8, 8)

            def proj(h, i):
                r = jnp.dot(_w2b(lhs[...]), _w2b(w3[h // 2, h % 2, i]), preferred_element_type=f32)
                p_ = pre[h // 2, h % 2, i, pl.ds(s8, 8), :]
                if i == 0:
                    st[("qkv", h, i)] = jnp.concatenate([r[0:24], p_, r[24:32]], axis=0)
                else:
                    st[("qkv", h, i)] = jnp.concatenate([r[0:24], p_, r[24:32], z8], axis=0).astype(bf16)

            def qk(h):
                q = st.pop(("qkv", h, 0))
                k = st.pop(("qkv", h, 1))
                sc = lax.dot_general(q, k, NT, preferred_element_type=f32) * scale
                sc = jnp.concatenate([sc, jnp.zeros((40, 80), f32)], axis=1)
                sc = jnp.where(mask, sc, -1e9)
                m = jnp.max(sc, axis=1, keepdims=True)
                e = jnp.exp(sc - m)
                p = e * (1.0 / jnp.sum(e, axis=1, keepdims=True))
                st[("p", h)] = p[:, :48]

            def pv(h):
                o = lax.dot_general(st.pop(("p", h)), st.pop(("qkv", h, 2)), NN, preferred_element_type=f32)
                st[("o", h)] = jnp.concatenate([o[0:24], o[32:40]], axis=0).astype(bf16)
                oc[h, 8 * q4:8 * q4 + 8, :] = o[24:32].astype(bf16)

            def oproj(h):
                w = jnp.concatenate([wo_t(j, h) for j in range(8)], axis=1)
                c = jnp.dot(st.pop(("o", h)), w, preferred_element_type=f32)
                if h == 0:
                    acc[...] = c
                else:
                    acc[...] += c

            ok = lambda h: 0 <= h < H
            for t in range(H):
                for tok in SLOT_ORDER.split():
                    n = int(tok[1:])
                    if tok[0] == "a":
                        proj(t, n)
                    elif ok(t - n):
                        {"q": qk, "p": pv, "o": oproj}[tok[0]](t - n)

            def fill(n):
                st["fill"] = fill_piece(gr, gw_, ocr, 2 * q4 + n // 2, n % 2, st.get("fill"))

            for tok in TAIL_ORDER.split():
                {"q": qk, "p": pv, "o": oproj, "f": fill}[tok[0]](int(tok[1:]))
            a = acc[...]
            rs = pl.multiple_of(32 * s, 32)
            b0 = jnp.concatenate([bnat[j, pl.ds(rs, 16), :] for j in range(8)], axis=1)
            b1 = jnp.concatenate([bnat[j, pl.ds(rs + 16, 8), :] for j in range(8)], axis=1)
            g0 = gbuf[pl.ds(rs, 16), :]
            g1 = gbuf[pl.ds(rs + 16, 8), :]
            outb[pl.ds(rs, 16), :] = mix(a[0:16], b0, jnp.tile(g0, (1, 8))).astype(bf16)
            outb[pl.ds(rs + 16, 8), :] = mix(a[16:24], b1, jnp.tile(g1, (1, 8))).astype(bf16)
            return a[24:32]

        def group(grp4, mem):
            @pl.when(grp4 >= 2)
            def _():
                out_copy(grp4 - 2).start()

            ocr[...] = oc32[...]
            for q4 in range(4):
                mem = step(q4, mem, grp4)
            return mem

        lax.fori_loop(0, NSEG // 4, group, mem0v[...].astype(f32))

        out_copy(14).start()

        def tail_copy(j):
            return pltpu.make_async_copy(outb.at[pl.ds(S - 128, 128), pl.ds(128 * j, 128)],
                                         out_hbm.at[pl.ds(S - 128, 128), pl.ds(128 * j, 128)], osem)

        for j in range(8):
            c = fill_piece(15, 15, oc32, j, 0, None)
            fill_piece(15, 15, oc32, j, 1, c)
            tail_copy(j).start()
        for gi in range(15):
            out_copy(gi).wait()
        for j in range(8):
            tail_copy(j).wait()

    pl.run_scoped(
        a_phase,
        pltpu.VMEM((16, 2, 3, 512, 128), u32), pltpu.VMEM((16, 2, 3, 512, 128), f32),
        pltpu.VMEM((H, 32, 128), bf16), pltpu.VMEM((H, 16, 128), u32), pltpu.VMEM((32, D), f32), pltpu.VMEM((16, D), u32))


@jax.jit
def pallas_gated_mix__memory_aug_recurrent_mem_tr__spectral_gfnet__prompt_kernel(
    A_x, A_mem0, A_Wq, A_Wk, A_Wv, A_Wo, A_seg_len, B_x, B_w_r, B_w_i, gate_w,
):
    del A_seg_len
    del B_x
    HB = pl.BlockSpec(memory_space=pltpu.HBM)
    out = pl.pallas_call(
        _kernel,
        out_shape=jax.ShapeDtypeStruct((S, D), bf16),
        in_specs=[HB] * 13,
        out_specs=HB,
        scratch_shapes=[
            pltpu.VMEM((S // 2, D), u32),
            pltpu.VMEM((NSEG * 4, D), u32),
            pltpu.VMEM((M_MEM, D), bf16),
            pltpu.VMEM((D,), bf16),
            pltpu.VMEM((16, 3, D, DH), u32),
            pltpu.VMEM((8, H, DH // 2, 128), u32),
            pltpu.VMEM((8, 128, D), u32),
            pltpu.VMEM((8, S, 128), bf16),
            pltpu.VMEM((S, 128), f32),
            pltpu.VMEM((S + 128, D), bf16),
            pltpu.SemaphoreType.DMA((21,)),
            pltpu.SemaphoreType.DMA((16,)),
            pltpu.SemaphoreType.DMA((6,)),
            pltpu.SemaphoreType.DMA(()),
        ],
        compiler_params=pltpu.CompilerParams(
            vmem_limit_bytes=124 * 2 ** 20, flags={"XLA_TPU_EVENLY_DISTRIBUTE_CRITICAL_NODES": True}),
    )(
        A_x.reshape(S, D), A_mem0.reshape(M_MEM, D), A_Wq, A_Wk, A_Wv, A_Wo,
        A_x.reshape(128, 16, D), B_w_r.T, B_w_i.T, gate_w, _TAB_G, _TAB_H, _TAB_MISC,
    )
    return out.reshape(1, S, D)
```
